```python
import jax
import jax.numpy as jnp

def _softmax(x, axis=-1):
    return jax.nn.softmax(x, axis=axis)
def _gelu(x):
    return jax.nn.gelu(x, approximate=True)
def _silu(x):
    return jax.nn.silu(x)
def _sigmoid(x):
    return jax.nn.sigmoid(x)
def _layernorm(x, axis=-1, eps=1e-5):
    m = jnp.mean(x, axis=axis, keepdims=True)
    v = jnp.var(x, axis=axis, keepdims=True)
    return (x - m) / jnp.sqrt(v + eps)
def _scatter_add(tgt, idx, src, axis=0):
    return tgt.at[idx].add(src)
def _segment_sum(src, seg, n):
    return jax.ops.segment_sum(src, seg, n)
class _Rng:
    def __init__(self, key):
        self._k = key
    def _next(self):
        self._k, sub = jax.random.split(self._k)
        return sub
    def normal(self, shape):
        return jax.random.normal(self._next(), shape, dtype=jnp.bfloat16)
    def randint(self, lo, hi, shape):
        return jax.random.randint(self._next(), shape, lo, hi, dtype=jnp.int32)
    def uniform(self, shape, lo=0.0, hi=1.0):
        return jax.random.uniform(self._next(), shape, jnp.bfloat16, lo, hi)
    def permutation(self, n):
        return jax.random.permutation(self._next(), n)


kernel_name = 'gated_mix__compressed_kv_cla__ssm_conv_s5__prompt'

def setup_inputs():
    _rng = _Rng(jax.random.key(int.from_bytes(__import__("os").urandom(4), "little")))
    _w = (lambda a: (lambda t: t.astype(jnp.bfloat16) if jnp.issubdtype(t.dtype, jnp.floating) else t)(jnp.asarray(a)))
    def _A_setup():
        B, H, Sq, Sk, D, M = 1, 16, 2048, 2048, 256, 448
        Dc = 4 * D
        return {
            "x": _w((lambda *s: _rng.normal(s) * 0.05)(B, Sq, M)),
            "c_kv": _w((lambda *s: _rng.normal(s) * 0.05)(B, Sk, Dc)),
            "w_q": _w((lambda *s: _rng.normal(s) * 0.05)(M, H, D) * (M ** -0.5)),
            "w_uk": _w((lambda *s: _rng.normal(s) * 0.05)(Dc, H, D) * (Dc ** -0.5)),
            "w_uv": _w((lambda *s: _rng.normal(s) * 0.05)(Dc, H, D) * (Dc ** -0.5)),
            "w_o": _w((lambda *s: _rng.normal(s) * 0.05)(H, D, M) * ((H * D) ** -0.5)),
        }
    _A_in = _A_setup()

    def _B_setup():
        B, S, D = 1, 2048, 448
        P = D
        Lambda_re = -0.5 * jnp.exp((lambda *s: _rng.normal(s) * 0.05)(P))
        Lambda_im = (lambda *s: _rng.normal(s) * 0.05)(P) * 1.0
        B_re = (lambda *s: _rng.normal(s) * 0.05)(P, D) * (D ** -0.5)
        B_im = (lambda *s: _rng.normal(s) * 0.05)(P, D) * (D ** -0.5)
        C_re = (lambda *s: _rng.normal(s) * 0.05)(D, P) * (P ** -0.5)
        C_im = (lambda *s: _rng.normal(s) * 0.05)(D, P) * (P ** -0.5)
        log_dt = (lambda *s: _rng.normal(s) * 0.05)(P) * 0.3 - 2.0
        Dskip = (lambda *s: _rng.normal(s) * 0.05)(D)
        return {
            "x": _w((lambda *s: _rng.normal(s) * 0.05)(B, S, D)),
            "Lambda_re": _w(Lambda_re),
            "Lambda_im": _w(Lambda_im),
            "B_re": _w(B_re),
            "B_im": _w(B_im),
            "C_re": _w(C_re),
            "C_im": _w(C_im),
            "log_dt": _w(log_dt),
            "Dskip": _w(Dskip),
        }
    _B_in = _B_setup()

    return {
        "A_x": _A_in["x"],
        "A_c_kv": _A_in["c_kv"],
        "A_w_q": _A_in["w_q"],
        "A_w_uk": _A_in["w_uk"],
        "A_w_uv": _A_in["w_uv"],
        "A_w_o": _A_in["w_o"],
        "B_x": _B_in["x"],
        "B_Lambda_re": _B_in["Lambda_re"],
        "B_Lambda_im": _B_in["Lambda_im"],
        "B_B_re": _B_in["B_re"],
        "B_B_im": _B_in["B_im"],
        "B_C_re": _B_in["C_re"],
        "B_C_im": _B_in["C_im"],
        "B_log_dt": _B_in["log_dt"],
        "B_Dskip": _B_in["Dskip"],
        "gate_w": _w((lambda *s: _rng.normal(s) * 0.05)(448)),
    }

def reference(A_x, A_c_kv, A_w_q, A_w_uk, A_w_uv, A_w_o, B_x, B_Lambda_re, B_Lambda_im, B_B_re, B_B_im, B_C_re, B_C_im, B_log_dt, B_Dskip, gate_w):
    def _A_ref(x, c_kv, w_q, w_uk, w_uv, w_o):
        B, Sq, M = x.shape[0], x.shape[1], x.shape[2]
        Sk = c_kv.shape[1]
        H, D = w_q.shape[1], w_q.shape[2]
        q = jnp.einsum("bqm,mhd->bhqd", x, w_q)
        k = jnp.einsum("bkc,chd->bhkd", c_kv, w_uk)
        v = jnp.einsum("bkc,chd->bhkd", c_kv, w_uv)
        scores = jnp.einsum("bhqd,bhkd->bhqk", q, k) * (D ** -0.5)
        off = Sk - Sq
        qi = jnp.arange(Sq)[:, None]
        kj = jnp.arange(Sk)[None, :]
        cmask = kj <= (qi + off)
        scores = jnp.where(cmask[None, None], scores, -1e9)
        p = _softmax(scores, axis=-1)
        ctx = jnp.einsum("bhqk,bhkd->bhqd", p, v)
        return jnp.einsum("bhqd,hdm->bqm", ctx, w_o)

    def _B_ref(x, Lambda_re, Lambda_im, B_re, B_im, C_re, C_im, log_dt, Dskip):
        Bsz, L, H = x.shape
        Lam = Lambda_re + 1j * Lambda_im
        Bmat = B_re + 1j * B_im
        Cmat = C_re + 1j * C_im
        dt = jnp.exp(log_dt)
        Lam_bar = jnp.exp(dt * Lam)
        B_bar = ((Lam_bar - 1.0) / Lam)[:, None] * Bmat
        Bu = jnp.einsum("bld,pd->blp", x + 0j, B_bar)
        h = jnp.zeros_like(Bu[:, 0, :])
        hs = []
        for t in range(L):
            h = Lam_bar[None, :] * h + Bu[:, t, :]
            hs.append(h)
        hseq = jnp.stack(hs, 1)
        y = 2.0 * jnp.einsum("blp,dp->bld", hseq, Cmat).real + x * Dskip[None, None, :]
        return y

    x = A_x
    g = _sigmoid((x * gate_w).sum(-1, keepdims=True))
    a = _A_ref(x, A_c_kv, A_w_q, A_w_uk, A_w_uv, A_w_o)
    b = _B_ref(x, B_Lambda_re, B_Lambda_im, B_B_re, B_B_im, B_C_re, B_C_im, B_log_dt, B_Dskip)
    return g * a + (1 - g) * b
```

```python
import functools

import jax
import jax.numpy as jnp
import jax.experimental.pallas as pl
import jax.experimental.pallas.tpu as pltpu

F32 = jnp.float32
BF16 = jnp.bfloat16
U32 = jnp.uint32

NT_DIMS = (((1,), (1,)), ((), ()))
LOG2E = 1.4426950408889634

TQ = 128
TP = 256
TU = 512
TO = 256
LANE = 128


def _dot(a, b):
    return jnp.dot(a, b, preferred_element_type=F32)


def _dot_nt(a, b):
    return jax.lax.dot_general(a, b, NT_DIMS, preferred_element_type=F32)


def _unpack(w32, shift):
    v = (w32 << shift) & jnp.uint32(0xFFFF0000)
    return pltpu.bitcast(v, F32).astype(BF16)


def _cmul_add(ar, ai, xr, xi, yr, yi):
    return (ar * xr - ai * xi) + yr, (ar * xi + ai * xr) + yi


def _kernel(xt_hbm, c_hbm, wq_hbm, wuk_hbm, wuv_hbm, wot_hbm,
            bre_hbm, bim_hbm, cre_hbm, cim_hbm, vec_ref,
            o_hbm,
            xt_ref, x_ref, c_ref, wq_buf, wk_buf, wv_buf, wot_ref,
            b_ref, cre_ref, cim_ref, u_ref, hs_ref, st_ref, lam_ref,
            ctx_ref, o_buf, wsem, xsem, msem, osem,
            *, S, M, H, D):
    P = M
    PT = (P + LANE - 1) // LANE
    PP = PT * LANE
    TS = S // H

    def w_copies(pair, slot):
        return [
            pltpu.make_async_copy(src.bitcast(U32).at[:, pair, :],
                                  dst.at[slot], wsem.at[k, slot])
            for k, (src, dst) in enumerate(
                ((wq_hbm, wq_buf), (wuk_hbm, wk_buf), (wuv_hbm, wv_buf)))
        ]

    def x_copy(j):
        cols = pl.ds(j * TU, TU)
        return pltpu.make_async_copy(xt_hbm.at[:, cols], xt_ref.at[:, cols], xsem.at[j])

    bre_cp = pltpu.make_async_copy(bre_hbm, b_ref.at[pl.ds(0, P), :], msem.at[0])
    bim_cp = pltpu.make_async_copy(bim_hbm, b_ref.at[pl.ds(PP, P), :], msem.at[1])
    c_cp = pltpu.make_async_copy(c_hbm, c_ref, msem.at[2])
    cre_cp = pltpu.make_async_copy(cre_hbm, cre_ref, msem.at[3])
    cim_cp = pltpu.make_async_copy(cim_hbm, cim_ref, msem.at[4])
    wot_cp = pltpu.make_async_copy(wot_hbm, wot_ref, msem.at[5])

    x_copy(0).start()
    bre_cp.start()
    bim_cp.start()
    for j in range(1, S // TU):
        x_copy(j).start()
    for cp in w_copies(0, 0):
        cp.start()
    c_cp.start()
    cre_cp.start()
    cim_cp.start()
    wot_cp.start()

    vec = vec_ref[...].astype(F32)
    lre, lim, ldt = vec[0:1], vec[1:2], vec[2:3]
    dt = jnp.exp(ldt).astype(BF16).astype(F32)
    e = jnp.exp(dt * lre)
    ang = dt * lim
    ar = e * jnp.cos(ang)
    ai = e * jnp.sin(ang)
    zpad = jnp.zeros((1, PP - P), F32)
    pr = jnp.concatenate([ar, zpad], axis=1)
    pi = jnp.concatenate([ai, zpad], axis=1)
    for j in range(4):
        lam_ref[2 * j] = jnp.broadcast_to(pr, (8, PP))
        lam_ref[2 * j + 1] = jnp.broadcast_to(pi, (8, PP))
        pr, pi = pr * pr - pi * pi, 2.0 * pr * pi

    b_ref[pl.ds(P, PP - P), :] = jnp.zeros((PP - P, M), BF16)
    b_ref[pl.ds(PP + P, PP - P), :] = jnp.zeros((PP - P, M), BF16)
    u_ref[pl.ds(0, 8), :] = jnp.zeros((8, 2 * PP), F32)
    st_ref[...] = jnp.zeros(st_ref.shape, F32)
    bre_cp.wait()
    bim_cp.wait()

    def u_step(j, _):
        x_copy(j).wait()
        t0 = pl.multiple_of(j * TU, TU)
        xc = xt_ref[:, pl.ds(t0, TU)].T
        x_ref[pl.ds(t0, TU), :] = xc
        u_ref[pl.ds(t0 + 8, TU), :] = _dot_nt(xc, b_ref[...])
        return 0

    jax.lax.fori_loop(0, S // TU, u_step, 0)
    c_cp.wait()

    def head_step(h, _):
        pair = h // 2
        slot = pair % 2

        @pl.when(h % 2 == 0)
        def _wait_weights():
            for cp in w_copies(pair, slot):
                cp.wait()

            @pl.when(pair + 1 < H // 2)
            def _():
                for cp in w_copies(pair + 1, 1 - slot):
                    cp.start()

        t0 = pl.multiple_of(h * TS, TS)
        w = u_ref[pl.ds(t0, TS + 8), :]
        wr, wi = w[:, :PP], w[:, PP:]
        for j in range(3):
            lr = lam_ref[2 * j, 0:1, :]
            li = lam_ref[2 * j + 1, 0:1, :]
            wr, wi = _cmul_add(lr, li, pltpu.roll(wr, 1 << j, 0), pltpu.roll(wi, 1 << j, 0), wr, wi)
        l8r, l8i = lam_ref[6], lam_ref[7]
        sr, si = st_ref[0], st_ref[1]
        hrs, his = [], []
        for k in range(1, TS // 8 + 1):
            sr, si = _cmul_add(l8r, l8i, sr, si, wr[8 * k:8 * k + 8], wi[8 * k:8 * k + 8])
            hrs.append(sr)
            his.append(si)
        st_ref[0] = sr
        st_ref[1] = si
        hs_ref[pl.ds(t0, TS), :] = jnp.concatenate(
            [jnp.concatenate(hrs, axis=0), jnp.concatenate(his, axis=0)], axis=1).astype(BF16)

        shift = (16 * (1 - h % 2)).astype(U32)
        wkv = jnp.concatenate([_unpack(wk_buf[slot], shift), _unpack(wv_buf[slot], shift)], axis=1)
        wq = _unpack(wq_buf[slot], shift)
        qscale = (D ** -0.5) * LOG2E
        row = jax.lax.broadcasted_iota(jnp.int32, (TQ, TQ), 0)
        col = jax.lax.broadcasted_iota(jnp.int32, (TQ, TQ), 1)
        causal = col <= row

        ks, vs, qs, ss = [], [], [], {}

        def proj_kv(r):
            kv = _dot(c_ref[pl.ds(r * TP, TP), :], wkv).astype(BF16)
            ks.append(kv[:, :D])
            vs.append(kv[:, D:])

        def proj_q(r):
            qs.append((_dot(x_ref[pl.ds(r * TP, TP), :], wq) * qscale).astype(BF16))

        def qk(i):
            lo, hi = i * TQ, (i + 1) * TQ
            q = jnp.concatenate(qs, axis=0)[lo:hi]
            k = jnp.concatenate(ks, axis=0)[:hi]
            ss[i] = jax.lax.dot_general(q, k, NT_DIMS, preferred_element_type=F32)

        def pv(i):
            lo, hi = i * TQ, (i + 1) * TQ
            s = ss.pop(i)
            sd = jnp.where(causal, s[:, lo:], -1e9 * LOG2E)
            s = sd if i == 0 else jnp.concatenate([s[:, :lo], sd], axis=1)
            m = jnp.max(s, axis=-1, keepdims=True)
            p = jnp.exp2(s - m)
            l = jnp.sum(p, axis=-1, keepdims=True)
            v = jnp.concatenate(vs, axis=0)[:hi]
            ctx = jnp.dot(p.astype(BF16), v, preferred_element_type=F32)
            ctx_ref[h, lo:hi, :] = (ctx * (1.0 / l)).astype(BF16)

        nb = TP // TQ
        nr = S // TP
        for r in range(nr):
            proj_kv(r)
            if r >= 2:
                for i in range((r - 2) * nb, (r - 1) * nb):
                    pv(i)
            proj_q(r)
            if r >= 1:
                for i in range((r - 1) * nb, r * nb):
                    qk(i)
        for i in range((nr - 1) * nb, nr * nb):
            qk(i)
            pv(i - nb)
        for i in range((nr - 1) * nb, nr * nb):
            pv(i)
        return 0

    jax.lax.fori_loop(0, H, head_step, 0)

    cre_cp.wait()
    cim_cp.wait()
    wot_cp.wait()
    ar, ai = lam_ref[0, 0:1, :P], lam_ref[1, 0:1, :P]
    sc = jnp.maximum(jnp.abs(lre), jnp.abs(lim))
    nre, nim = lre / sc, lim / sc
    den = (nre * nre + nim * nim) * sc
    gr = ((ar - 1.0) * nre + ai * nim) / den
    gi = (ai * nre - (ar - 1.0) * nim) / den
    cre = cre_ref[...].astype(F32)
    cim = cim_ref[...].astype(F32)
    zcol = jnp.zeros((M, PP - P), BF16)
    ccat = jnp.concatenate([(2.0 * (cre * gr - cim * gi)).astype(BF16), zcol,
                            (-2.0 * (cre * gi + cim * gr)).astype(BF16), zcol], axis=1)
    vpad = jnp.concatenate([vec, jnp.zeros((8, PP - P), F32)], axis=1)
    dcol = jnp.broadcast_to(vpad[3:4], (LANE, PP)).T[:M]
    gcol = jnp.broadcast_to(vpad[4:5], (LANE, PP)).T[:M]
    dcol = jnp.concatenate([dcol] * (TO // LANE), axis=1)
    gcol = jnp.concatenate([gcol] * (TO // LANE), axis=1)

    def o_copy(j, slot):
        return pltpu.make_async_copy(o_buf.at[slot], o_hbm.at[:, pl.ds(j * TO, TO)], osem.at[slot])

    def o_step(j, _):
        slot = j % 2

        @pl.when(j >= 2)
        def _():
            o_copy(j - 2, slot).wait()

        t0 = pl.multiple_of(j * TO, TO)
        rows = pl.ds(t0, TO)
        wot = jnp.concatenate([wot_ref[k] for k in range(H)], axis=1)
        ctx = jnp.concatenate([ctx_ref[k, rows, :] for k in range(H)], axis=1)
        yt = _dot_nt(ccat, hs_ref[rows, :])
        at = _dot_nt(wot, ctx)
        xt = xt_ref[:, rows].astype(F32)
        z = jnp.sum((xt * gcol).astype(BF16).astype(F32), axis=0, keepdims=True)
        g = jax.nn.sigmoid(z.astype(BF16).astype(F32)).astype(BF16).astype(F32)
        omg = (1.0 - g).astype(BF16).astype(F32)
        o_buf[slot] = g * at + omg * (yt + (xt * dcol).astype(BF16).astype(F32))
        o_copy(j, slot).start()
        return 0

    no = S // TO
    jax.lax.fori_loop(0, no, o_step, 0)
    o_copy(no - 2, no % 2).wait()
    o_copy(no - 1, (no - 1) % 2).wait()


@jax.jit
def pallas_gated_mix__compressed_kv_cla__ssm_conv_s5__prompt_kernel(
    A_x: jax.Array,
    A_c_kv: jax.Array,
    A_w_q: jax.Array,
    A_w_uk: jax.Array,
    A_w_uv: jax.Array,
    A_w_o: jax.Array,
    B_x: jax.Array,
    B_Lambda_re: jax.Array,
    B_Lambda_im: jax.Array,
    B_B_re: jax.Array,
    B_B_im: jax.Array,
    B_C_re: jax.Array,
    B_C_im: jax.Array,
    B_log_dt: jax.Array,
    B_Dskip: jax.Array,
    gate_w: jax.Array,
):
    del B_x
    _, S, M = A_x.shape
    C = A_c_kv.shape[2]
    H, D = A_w_q.shape[1], A_w_q.shape[2]
    PP = (M + LANE - 1) // LANE * LANE

    hbm = pl.BlockSpec(memory_space=pl.ANY)
    vec = jnp.stack([B_Lambda_re, B_Lambda_im, B_log_dt, B_Dskip, gate_w,
                     gate_w, gate_w, gate_w])

    out_t = pl.pallas_call(
        functools.partial(_kernel, S=S, M=M, H=H, D=D),
        in_specs=[hbm] * 10 + [pl.BlockSpec(memory_space=pltpu.VMEM)],
        out_specs=hbm,
        out_shape=jax.ShapeDtypeStruct((M, S), F32),
        scratch_shapes=[
            pltpu.VMEM((M, S), BF16),
            pltpu.VMEM((S, M), BF16),
            pltpu.VMEM((S, C), BF16),
            pltpu.VMEM((2, M, D), U32),
            pltpu.VMEM((2, C, D), U32),
            pltpu.VMEM((2, C, D), U32),
            pltpu.VMEM((H, M, D), BF16),
            pltpu.VMEM((2 * PP, M), BF16),
            pltpu.VMEM((M, M), BF16),
            pltpu.VMEM((M, M), BF16),
            pltpu.VMEM((S + 8, 2 * PP), F32),
            pltpu.VMEM((S, 2 * PP), BF16),
            pltpu.VMEM((2, 8, PP), F32),
            pltpu.VMEM((8, 8, PP), F32),
            pltpu.VMEM((H, S, D), BF16),
            pltpu.VMEM((2, M, TO), F32),
            pltpu.SemaphoreType.DMA((3, 2)),
            pltpu.SemaphoreType.DMA((S // TU,)),
            pltpu.SemaphoreType.DMA((6,)),
            pltpu.SemaphoreType.DMA((2,)),
        ],
        compiler_params=pltpu.CompilerParams(
            vmem_limit_bytes=120 * 1024 * 1024,
        ),
    )(
        jnp.swapaxes(A_x, 1, 2).reshape(M, S), A_c_kv.reshape(S, C),
        A_w_q, A_w_uk, A_w_uv, jnp.swapaxes(A_w_o, 1, 2),
        B_B_re, B_B_im, B_C_re, B_C_im, vec,
    )
    return jnp.swapaxes(out_t.reshape(1, M, S), 1, 2)
```

```python
import functools

import jax
import jax.numpy as jnp
import jax.experimental.pallas as pl
import jax.experimental.pallas.tpu as pltpu

F32 = jnp.float32
BF16 = jnp.bfloat16
U32 = jnp.uint32

NT_DIMS = (((1,), (1,)), ((), ()))
LOG2E = 1.4426950408889634

TQ = 128
TP = 256
TU = 512
TO = 256
LANE = 128
SSM_AT = 1
PACE = True
POSTNORM = False
ANCHOR = 3
PACE_FROM = 6
PACE_ROWS = 8


def _dot(a, b):
    return jnp.dot(a, b, preferred_element_type=F32)


def _dot_nt(a, b):
    return jax.lax.dot_general(a, b, NT_DIMS, preferred_element_type=F32)


def _unpack(w32, shift):
    v = (w32 << shift) & jnp.uint32(0xFFFF0000)
    return pltpu.bitcast(v, F32)


def _as_bf16(w32):
    return pltpu.bitcast(w32, BF16)


def _as_u32(v):
    return pltpu.bitcast(v, U32)


def _cmul_add(ar, ai, xr, xi, yr, yi):
    return (ar * xr - ai * xi) + yr, (ar * xi + ai * xr) + yi


def _kernel(xt_hbm, c_hbm, wq_hbm, wuk_hbm, wuv_hbm, wot_hbm,
            bre_hbm, bim_hbm, cre_hbm, cim_hbm, vec_ref,
            o_hbm,
            xt_ref, x_ref, c_ref, wq_buf, wk_buf, wv_buf, wot_ref,
            b_ref, cre_ref, cim_ref, cc_ref, u_ref, ys_ref, st_ref, lam_ref,
            ctx_ref, o_buf, zero_ref, wsem, xsem, msem, osem,
            *, S, M, H, D):
    P = M
    PT = (P + LANE - 1) // LANE
    PP = PT * LANE
    TS = S // H

    def w_copies(pair, slot):
        return [
            pltpu.make_async_copy(src.bitcast(U32).at[:, pair, :],
                                  dst.at[slot], wsem.at[k, slot])
            for k, (src, dst) in enumerate(
                ((wq_hbm, wq_buf), (wuk_hbm, wk_buf), (wuv_hbm, wv_buf)))
        ]

    def x_copy(j):
        cols = pl.ds(j * TU, TU)
        return pltpu.make_async_copy(xt_hbm.at[:, cols], xt_ref.at[:, cols], xsem.at[j])

    bre_cp = pltpu.make_async_copy(bre_hbm, b_ref.at[pl.ds(0, P), :], msem.at[0])
    bim_cp = pltpu.make_async_copy(bim_hbm, b_ref.at[pl.ds(PP, P), :], msem.at[1])
    c_cp = pltpu.make_async_copy(c_hbm.bitcast(U32), c_ref, msem.at[2])
    cre_cp = pltpu.make_async_copy(cre_hbm, cre_ref, msem.at[3])
    cim_cp = pltpu.make_async_copy(cim_hbm, cim_ref, msem.at[4])
    wot_cp = pltpu.make_async_copy(wot_hbm.bitcast(U32), wot_ref, msem.at[5])

    x_copy(0).start()
    bre_cp.start()
    bim_cp.start()
    cre_cp.start()
    cim_cp.start()
    for j in range(1, S // TU):
        x_copy(j).start()
    for cp in w_copies(0, 0):
        cp.start()
    c_cp.start()
    wot_cp.start()

    zero_ref[0] = 0
    vec = vec_ref[...].astype(F32)
    lre, lim, ldt = vec[0:1], vec[1:2], vec[2:3]
    dt = jnp.exp(ldt).astype(BF16).astype(F32)
    e = jnp.exp(dt * lre)
    ang = dt * lim
    ar = e * jnp.cos(ang)
    ai = e * jnp.sin(ang)
    zpad = jnp.zeros((1, PP - P), F32)
    pr = jnp.concatenate([ar, zpad], axis=1)
    pi = jnp.concatenate([ai, zpad], axis=1)
    for j in range(4):
        lam_ref[2 * j] = jnp.broadcast_to(pr, (8, PP))
        lam_ref[2 * j + 1] = jnp.broadcast_to(pi, (8, PP))
        pr, pi = pr * pr - pi * pi, 2.0 * pr * pi

    sc = jnp.maximum(jnp.abs(lre), jnp.abs(lim))
    nre, nim = lre / sc, lim / sc
    den = (nre * nre + nim * nim) * sc
    gr = ((ar - 1.0) * nre + ai * nim) / den
    gi = (ai * nre - (ar - 1.0) * nim) / den
    b_ref[pl.ds(P, PP - P), :] = jnp.zeros((PP - P, M), BF16)
    b_ref[pl.ds(PP + P, PP - P), :] = jnp.zeros((PP - P, M), BF16)
    u_ref[pl.ds(0, 8), :] = jnp.zeros((8, 2 * PP), F32)
    st_ref[...] = jnp.zeros(st_ref.shape, F32)
    bre_cp.wait()
    bim_cp.wait()
    cre_cp.wait()
    cim_cp.wait()
    MC = M // (S // TU)

    def u_step(j, _):
        x_copy(j).wait()
        crows = pl.ds(pl.multiple_of(j * MC, 16), MC)
        cre = cre_ref[crows, :].astype(F32)
        cim = cim_ref[crows, :].astype(F32)
        zcol = jnp.zeros((MC, PP - P), F32)
        cc_ref[pl.ds(pl.multiple_of(j * (MC // 2), 8), MC // 2), :] = _as_u32(jnp.concatenate(
            [2.0 * (cre * gr - cim * gi), zcol, -2.0 * (cre * gi + cim * gr), zcol],
            axis=1).astype(BF16))
        t0 = pl.multiple_of(j * TU, TU)
        xc = xt_ref[:, pl.ds(t0, TU)].T
        x_ref[pl.ds(pl.multiple_of(j * (TU // 2), TU // 2), TU // 2), :] = _as_u32(xc)
        u_ref[pl.ds(t0 + 8, TU), :] = _dot_nt(xc, b_ref[...])
        return 0

    jax.lax.fori_loop(0, S // TU, u_step, 0)
    c_cp.wait()

    def head_step(h, _):
        pair = h // 2
        slot = pair % 2

        @pl.when(h % 2 == 0)
        def _wait_weights():
            for cp in w_copies(pair, slot):
                cp.wait()

            @pl.when(pair + 1 < H // 2)
            def _():
                for cp in w_copies(pair + 1, 1 - slot):
                    cp.start()

        ys = []

        def ssm_tile(t):
            t0 = pl.multiple_of(h * TS, TS)
            cr, ci = pl.ds(t * LANE, LANE), pl.ds(PP + t * LANE, LANE)
            wr = u_ref[pl.ds(t0, TS + 8), cr]
            wi = u_ref[pl.ds(t0, TS + 8), ci]
            for j in range(3):
                lr = lam_ref[2 * j, 0:1, cr]
                li = lam_ref[2 * j + 1, 0:1, cr]
                wr, wi = _cmul_add(lr, li, pltpu.roll(wr, 1 << j, 0), pltpu.roll(wi, 1 << j, 0), wr, wi)
            l8r, l8i = lam_ref[6, :, cr], lam_ref[7, :, cr]
            sr, si = st_ref[0, :, cr], st_ref[1, :, cr]
            hrs, his = [], []
            for k in range(1, TS // 8 + 1):
                sr, si = _cmul_add(l8r, l8i, sr, si, wr[8 * k:8 * k + 8], wi[8 * k:8 * k + 8])
                hrs.append(sr)
                his.append(si)
                if PACE:
                    sr = pltpu.roll(sr, zero_ref[0], 1)
            st_ref[0, :, cr] = sr
            st_ref[1, :, cr] = si
            hs = jnp.concatenate(
                [jnp.concatenate(hrs, axis=0), jnp.concatenate(his, axis=0)], axis=1).astype(BF16)
            cc = _as_bf16(jnp.concatenate([cc_ref[:, cr], cc_ref[:, ci]], axis=1))
            y = jax.lax.dot_general(cc, hs, NT_DIMS, preferred_element_type=F32)
            ys[:] = [y + ys[0] if ys else y]
            if t == PT - 1:
                ys_ref[h] = ys[0]

        shift = (16 * (1 - h % 2)).astype(U32)
        wkv = jnp.concatenate([_unpack(wk_buf[slot], shift), _unpack(wv_buf[slot], shift)], axis=1).astype(BF16)
        wq = _unpack(wq_buf[slot], shift).astype(BF16)
        qscale = (D ** -0.5) * LOG2E
        row = jax.lax.broadcasted_iota(jnp.int32, (TQ, TQ), 0)
        col = jax.lax.broadcasted_iota(jnp.int32, (TQ, TQ), 1)
        causal = col <= row

        ks, vs, qs, ss, pending = [], [], [], {}, []

        def proj_kv(r):
            c = _as_bf16(c_ref[pl.ds(r * TP // 2, TP // 2), :])
            kv = jnp.dot(c, wkv, preferred_element_type=F32)
            ks.append(kv[:, :D])
            vs.append(kv[:, D:])

        def proj_q(r):
            x = _as_bf16(x_ref[pl.ds(r * TP // 2, TP // 2), :])
            qs.append(_dot(x, wq) * qscale)

        def qk(i):
            lo, hi = i * TQ, (i + 1) * TQ
            q = jnp.concatenate(qs, axis=0)[lo:hi].astype(BF16)
            if POSTNORM:
                while pending and pending[0][0] <= i - ANCHOR:
                    q = _as_bf16(_as_u32(q) | (pending.pop(0)[1] & zero_ref[0].astype(U32)))
            k = jnp.concatenate(ks, axis=0)[:hi].astype(BF16)
            ss[i] = jax.lax.dot_general(q, k, NT_DIMS, preferred_element_type=F32)

        def pv(i):
            lo, hi = i * TQ, (i + 1) * TQ
            s = ss.pop(i)
            sd = jnp.where(causal, s[:, lo:], -1e9 * LOG2E)
            s = sd if i == 0 else jnp.concatenate([s[:, :lo], sd], axis=1)
            m = jnp.max(s, axis=-1, keepdims=True)
            if i >= PACE_FROM:
                mb = _as_u32(jnp.broadcast_to(m, (TQ, LANE)))
                ps, parts = [], []
                for g in range(0, TQ, PACE_ROWS):
                    mg = mb[g:g + PACE_ROWS]
                    if parts:
                        mg = mg | (_as_u32(parts[-1]) & zero_ref[0].astype(U32))
                    mg = pltpu.bitcast(mg, F32)
                    pg = [jnp.exp2(s[g:g + PACE_ROWS, t * LANE:(t + 1) * LANE] - mg) for t in range(hi // LANE)]
                    ps.append(jnp.concatenate(pg, axis=1))
                    parts.append(functools.reduce(lambda a, b: a + b, pg))
                p = jnp.concatenate(ps, axis=0)
                l = jnp.sum(jnp.concatenate(parts, axis=0), axis=-1, keepdims=True)
            else:
                p = jnp.exp2(s - m)
                l = jnp.sum(p, axis=-1, keepdims=True)
            rl = pl.reciprocal(l, approx=True)
            rl = rl * (2.0 - l * rl)
            v = jnp.concatenate(vs, axis=0)[:hi].astype(BF16)
            if POSTNORM:
                ctx = jnp.dot(p.astype(BF16), v, preferred_element_type=F32) * rl
            else:
                ctx = jnp.dot((p * rl).astype(BF16), v, preferred_element_type=F32)
            ctx = _as_u32(ctx.astype(BF16))
            pending.append((i, ctx))
            ctx_ref[h, lo // 2:hi // 2, :] = ctx

        nb = TP // TQ
        nr = S // TP
        for r in range(nr):
            proj_kv(r)
            if r >= 2:
                for i in range((r - 2) * nb, (r - 1) * nb):
                    pv(i)
            proj_q(r)
            if SSM_AT <= r < SSM_AT + PT:
                ssm_tile(r - SSM_AT)
            if r >= 1:
                for i in range((r - 1) * nb, r * nb):
                    qk(i)
        for i in range((nr - 1) * nb, nr * nb):
            qk(i)
            pv(i - nb)
        for i in range((nr - 1) * nb, nr * nb):
            pv(i)
        return 0

    jax.lax.fori_loop(0, H, head_step, 0)

    wot_cp.wait()
    vpad = jnp.concatenate([vec, jnp.zeros((8, PP - P), F32)], axis=1)
    dcol = jnp.broadcast_to(vpad[3:4], (LANE, PP)).T[:M]
    gcol = jnp.broadcast_to(vpad[4:5], (LANE, PP)).T[:M]
    dcol = jnp.concatenate([dcol] * (TO // LANE), axis=1)
    gcol = jnp.concatenate([gcol] * (TO // LANE), axis=1)

    def o_copy(j, slot):
        return pltpu.make_async_copy(o_buf.at[slot], o_hbm.at[:, pl.ds(j * TO, TO)], osem.at[slot])

    def o_step(j, _):
        slot = j % 2

        @pl.when(j >= 2)
        def _():
            o_copy(j - 2, slot).wait()

        t0 = pl.multiple_of(j * TO, TO)
        rows = pl.ds(t0, TO)
        rows2 = pl.ds(pl.multiple_of(j * (TO // 2), TO // 2), TO // 2)
        wot = _as_bf16(jnp.concatenate([wot_ref[k] for k in range(H)], axis=1))
        ctx = _as_bf16(jnp.concatenate([ctx_ref[k, rows2, :] for k in range(H)], axis=1))
        yt = jnp.concatenate([ys_ref[j * (TO // TS) + k] for k in range(TO // TS)], axis=1)
        at = _dot_nt(wot, ctx)
        xt = xt_ref[:, rows].astype(F32)
        z = jnp.sum((xt * gcol).astype(BF16).astype(F32), axis=0, keepdims=True)
        g = jax.nn.sigmoid(z.astype(BF16).astype(F32)).astype(BF16).astype(F32)
        omg = (1.0 - g).astype(BF16).astype(F32)
        o_buf[slot] = g * at + omg * (yt + (xt * dcol).astype(BF16).astype(F32))
        o_copy(j, slot).start()
        return 0

    no = S // TO
    jax.lax.fori_loop(0, no, o_step, 0)
    o_copy(no - 2, no % 2).wait()
    o_copy(no - 1, (no - 1) % 2).wait()


@jax.jit
def pallas_gated_mix__compressed_kv_cla__ssm_conv_s5__prompt_kernel(
    A_x: jax.Array,
    A_c_kv: jax.Array,
    A_w_q: jax.Array,
    A_w_uk: jax.Array,
    A_w_uv: jax.Array,
    A_w_o: jax.Array,
    B_x: jax.Array,
    B_Lambda_re: jax.Array,
    B_Lambda_im: jax.Array,
    B_B_re: jax.Array,
    B_B_im: jax.Array,
    B_C_re: jax.Array,
    B_C_im: jax.Array,
    B_log_dt: jax.Array,
    B_Dskip: jax.Array,
    gate_w: jax.Array,
):
    del B_x
    _, S, M = A_x.shape
    C = A_c_kv.shape[2]
    H, D = A_w_q.shape[1], A_w_q.shape[2]
    PP = (M + LANE - 1) // LANE * LANE

    hbm = pl.BlockSpec(memory_space=pl.ANY)
    vec = jnp.stack([B_Lambda_re, B_Lambda_im, B_log_dt, B_Dskip, gate_w,
                     gate_w, gate_w, gate_w])

    out_t = pl.pallas_call(
        functools.partial(_kernel, S=S, M=M, H=H, D=D),
        in_specs=[hbm] * 10 + [pl.BlockSpec(memory_space=pltpu.VMEM)],
        out_specs=hbm,
        out_shape=jax.ShapeDtypeStruct((M, S), F32),
        scratch_shapes=[
            pltpu.VMEM((M, S), BF16),
            pltpu.VMEM((S // 2, M), U32),
            pltpu.VMEM((S // 2, C), U32),
            pltpu.VMEM((2, M, D), U32),
            pltpu.VMEM((2, C, D), U32),
            pltpu.VMEM((2, C, D), U32),
            pltpu.VMEM((H, M // 2, D), U32),
            pltpu.VMEM((2 * PP, M), BF16),
            pltpu.VMEM((M, M), BF16),
            pltpu.VMEM((M, M), BF16),
            pltpu.VMEM((M // 2, 2 * PP), U32),
            pltpu.VMEM((S + 8, 2 * PP), F32),
            pltpu.VMEM((H, M, S // H), F32),
            pltpu.VMEM((2, 8, PP), F32),
            pltpu.VMEM((8, 8, PP), F32),
            pltpu.VMEM((H, S // 2, D), U32),
            pltpu.VMEM((2, M, TO), F32),
            pltpu.SMEM((1,), jnp.int32),
            pltpu.SemaphoreType.DMA((3, 2)),
            pltpu.SemaphoreType.DMA((S // TU,)),
            pltpu.SemaphoreType.DMA((6,)),
            pltpu.SemaphoreType.DMA((2,)),
        ],
        compiler_params=pltpu.CompilerParams(
            vmem_limit_bytes=120 * 1024 * 1024,
        ),
    )(
        jnp.swapaxes(A_x, 1, 2).reshape(M, S), A_c_kv.reshape(S, C),
        A_w_q, A_w_uk, A_w_uv, jnp.swapaxes(A_w_o, 1, 2),
        B_B_re, B_B_im, B_C_re, B_C_im, vec,
    )
    return jnp.swapaxes(out_t.reshape(1, M, S), 1, 2)
```

```python
import functools

import jax
import jax.numpy as jnp
import jax.experimental.pallas as pl
import jax.experimental.pallas.tpu as pltpu

F32 = jnp.float32
BF16 = jnp.bfloat16
U32 = jnp.uint32

NT_DIMS = (((1,), (1,)), ((), ()))
LOG2E = 1.4426950408889634

TQ = 128
TP = 256
TU = 512
TO = 256
LANE = 128
HALF = LANE // 2
SSM_AT = 1
PACE_FROM = 6
PACE_ROWS = 8


def _dot_nt(a, b):
    return jax.lax.dot_general(a, b, NT_DIMS, preferred_element_type=F32)


def _unpack(w32, shift):
    v = (w32 << shift) & jnp.uint32(0xFFFF0000)
    return pltpu.bitcast(v, F32)


def _as_bf16(w32):
    return pltpu.bitcast(w32, BF16)


def _as_u32(v):
    return pltpu.bitcast(v, U32)


def _kernel(xt_hbm, c_hbm, wq_hbm, wuk_hbm, wuv_hbm, wot_hbm,
            bre_hbm, bim_hbm, cre_hbm, cim_hbm,
            lre_hbm, lim_hbm, ldt_hbm, dsk_hbm, gw_hbm,
            o_hbm,
            xt_ref, x_ref, c_ref, wq_buf, wk_buf, wv_buf, wot_ref,
            b_ref, cre_ref, cim_ref, cmid_ref, u_ref, ys_ref, st_ref, co_ref, col_ref,
            lre_ref, lim_ref, ldt_ref, dsk_ref, gw_ref,
            ctx_ref, o_buf, zero_ref, wsem, xsem, msem, vsem, osem,
            *, S, M, H, D):
    P = M
    FT = P // LANE
    PF = FT * LANE
    assert P - PF == HALF
    PP = PF + LANE
    TS = S // H

    def w_copies(pair, slot):
        return [
            pltpu.make_async_copy(src.bitcast(U32).at[:, pair, :],
                                  dst.at[slot], wsem.at[k, slot])
            for k, (src, dst) in enumerate(
                ((wuk_hbm, wk_buf), (wuv_hbm, wv_buf), (wq_hbm, wq_buf)))
        ]

    def x_copy(j):
        cols = pl.ds(j * TU, TU)
        return pltpu.make_async_copy(xt_hbm.at[:, cols], xt_ref.at[:, cols], xsem.at[j])

    bre32, bim32 = bre_hbm.bitcast(U32), bim_hbm.bitcast(U32)
    b_cps = [
        pltpu.make_async_copy(bre32, b_ref.at[pl.ds(0, P // 2), :], msem.at[0]),
        pltpu.make_async_copy(bim32.at[pl.ds(PF // 2, HALF // 2), :],
                              b_ref.at[pl.ds(P // 2, HALF // 2), :], msem.at[1]),
        pltpu.make_async_copy(bim32.at[pl.ds(0, PF // 2), :],
                              b_ref.at[pl.ds(PP // 2, PF // 2), :], msem.at[2]),
    ]
    c_cp = pltpu.make_async_copy(c_hbm.bitcast(U32), c_ref, msem.at[3])
    cre_cp = pltpu.make_async_copy(cre_hbm.bitcast(U32), cre_ref, msem.at[4])
    cim_cp = pltpu.make_async_copy(cim_hbm.bitcast(U32), cim_ref, msem.at[5])
    wot_cp = pltpu.make_async_copy(wot_hbm.bitcast(U32), wot_ref, msem.at[6])
    v_cps = [pltpu.make_async_copy(src, dst, vsem.at[k]) for k, (src, dst) in enumerate(
        ((lre_hbm, lre_ref), (lim_hbm, lim_ref), (ldt_hbm, ldt_ref),
         (dsk_hbm, dsk_ref), (gw_hbm, gw_ref)))]

    for cp in v_cps:
        cp.start()
    x_copy(0).start()
    for cp in b_cps:
        cp.start()
    for j in range(1, S // TU):
        x_copy(j).start()
    for cp in w_copies(0, 0):
        cp.start()
    c_cp.start()
    cre_cp.start()
    cim_cp.start()

    zero_ref[0] = 0
    u_ref[pl.ds(0, 8), :] = jnp.zeros((8, u_ref.shape[1]), F32)
    st_ref[...] = jnp.zeros(st_ref.shape, F32)
    for cp in v_cps:
        cp.wait()

    row = lambda r: r[...].astype(F32).reshape(1, P)
    lre, lim = row(lre_ref), row(lim_ref)
    dt = jnp.exp(row(ldt_ref)).astype(BF16).astype(F32)
    e = jnp.exp(dt * lre)
    ang = dt * lim
    ar = e * jnp.cos(ang)
    ai = e * jnp.sin(ang)
    sc = jnp.maximum(jnp.abs(lre), jnp.abs(lim))
    nre, nim = lre / sc, lim / sc
    den = (nre * nre + nim * nim) * sc
    gr = 2.0 * ((ar - 1.0) * nre + ai * nim) / den
    gi = 2.0 * (ai * nre - (ar - 1.0) * nim) / den

    def put(k, full, lo, hi):
        v = jnp.concatenate([full[:, :PF], lo[:, PF:], hi[:, PF:]], axis=1)
        co_ref[k] = jnp.broadcast_to(v, (8, PP))

    put(0, gr, gr, -gr)
    put(1, gi, -gi, -gi)
    pr, pi = ar, -ai
    for j in range(1, 5):
        put(2 * j, pr, pr, pr)
        put(2 * j + 1, pi, -pi, pi)
        pr, pi = pr * pr - pi * pi, 2.0 * pr * pi

    zpad = jnp.zeros((1, PP - P), F32)
    for k, r in enumerate((dsk_ref, gw_ref)):
        v = jnp.concatenate([row(r), zpad], axis=1)
        col_ref[k] = jnp.broadcast_to(v, (LANE, PP)).T[:M]

    for cp in b_cps:
        cp.wait()

    def u_step(j, _):
        x_copy(j).wait()
        t0 = pl.multiple_of(j * TU, TU)
        xc = xt_ref[:, pl.ds(t0, TU)].T
        x_ref[pl.ds(pl.multiple_of(j * (TU // 2), TU // 2), TU // 2), :] = _as_u32(xc)
        u_ref[pl.ds(t0 + 8, TU), :] = _dot_nt(xc, _as_bf16(b_ref[...]))
        return 0

    jax.lax.fori_loop(0, S // TU, u_step, 0)
    wot_cp.start()
    cre_cp.wait()
    cim_cp.wait()
    cmid_ref[...] = jnp.concatenate([cre_ref[:, PF:], cim_ref[:, PF:]], axis=1)
    c_cp.wait()

    def head_step(h, _):
        pair = h // 2
        slot = pair % 2

        @pl.when(h % 2 == 0)
        def _wait_weights():
            for cp in w_copies(pair, slot):
                cp.wait()

            @pl.when(pair + 1 < H // 2)
            def _():
                for cp in w_copies(pair + 1, 1 - slot):
                    cp.start()

        zero = zero_ref[0]

        ys = []

        def ssm_tile(t):
            rows = pl.ds(pl.multiple_of(h * TS, TS), TS + 8)
            cr, ci = pl.ds(t * LANE, LANE), pl.ds(PP + t * LANE, LANE)
            co = lambda k, n=8: co_ref[k, 0:n, cr]
            if t < FT:
                mul = lambda a, b, x: (a * x[0] - b * x[1], a * x[1] + b * x[0])
                ur, ui = u_ref[rows, cr], u_ref[rows, ci]
                w = (co(0, 1) * ur - co(1, 1) * ui, -(co(0, 1) * ui + co(1, 1) * ur))
                s = (st_ref[:, cr], st_ref[:, ci])
            else:
                mul = lambda a, b, x: (a * x[0] + b * pltpu.roll(x[0], HALF, 1),)
                w = mul(co(0, 1), co(1, 1), (u_ref[rows, cr],))
                s = (st_ref[:, cr],)
            for j in range(3):
                d = mul(co(2 * j + 2, 1), co(2 * j + 3, 1), [pltpu.roll(v, 1 << j, 0) for v in w])
                w = [a + b for a, b in zip(d, w)]
            gs = []
            for k in range(1, TS // 8 + 1):
                s = [a + b[8 * k:8 * k + 8] for a, b in zip(mul(co(8), co(9), s), w)]
                gs.append(jnp.concatenate(s, axis=1))
                if t < FT:
                    s = [pltpu.roll(s[0], zero, 1), s[1]]
            st_ref[:, cr] = s[0]
            if t < FT:
                st_ref[:, ci] = s[1]
                cc = jnp.concatenate([cre_ref[:, cr], cim_ref[:, cr]], axis=1)
            else:
                cc = cmid_ref[...]
            g = jnp.concatenate(gs, axis=0).astype(BF16)
            y = jax.lax.dot_general(_as_bf16(cc), g, NT_DIMS, preferred_element_type=F32)
            ys[:] = [y + ys[0] if ys else y]
            if t == FT:
                ys_ref[h] = ys[0]

        shift = (16 * (1 - h % 2)).astype(U32)
        wkv = jnp.concatenate([_unpack(wk_buf[slot], shift), _unpack(wv_buf[slot], shift)],
                              axis=1).astype(BF16)
        wq = _unpack(wq_buf[slot], shift).astype(BF16)
        qscale = (D ** -0.5) * LOG2E
        causal = (jax.lax.broadcasted_iota(jnp.int32, (TQ, TQ), 1)
                  <= jax.lax.broadcasted_iota(jnp.int32, (TQ, TQ), 0))

        ks, vs, qs, ss = [], [], [], {}

        def proj_kv(r):
            c = _as_bf16(c_ref[pl.ds(r * TP // 2, TP // 2), :])
            kv = jnp.dot(c, wkv, preferred_element_type=F32)
            ks.append(kv[:, :D])
            vs.append(kv[:, D:])

        def proj_q(r):
            x = _as_bf16(x_ref[pl.ds(r * TP // 2, TP // 2), :])
            qs.append(jnp.dot(x, wq, preferred_element_type=F32) * qscale)

        def qk(i):
            lo, hi = i * TQ, (i + 1) * TQ
            q = jnp.concatenate(qs, axis=0)[lo:hi].astype(BF16)
            k = jnp.concatenate(ks, axis=0)[:hi].astype(BF16)
            ss[i] = jax.lax.dot_general(q, k, NT_DIMS, preferred_element_type=F32)

        def pv(i):
            lo, hi = i * TQ, (i + 1) * TQ
            s = ss.pop(i)
            sd = jnp.where(causal, s[:, lo:], -1e9 * LOG2E)
            s = sd if i == 0 else jnp.concatenate([s[:, :lo], sd], axis=1)
            m = jnp.max(s, axis=-1, keepdims=True)
            if i >= PACE_FROM:
                mb = _as_u32(jnp.broadcast_to(m, (TQ, LANE)))
                ps, parts = [], []
                for g in range(0, TQ, PACE_ROWS):
                    mg = mb[g:g + PACE_ROWS]
                    if parts:
                        mg = mg | (_as_u32(parts[-1]) & zero.astype(U32))
                    mg = pltpu.bitcast(mg, F32)
                    pg = [jnp.exp2(s[g:g + PACE_ROWS, t * LANE:(t + 1) * LANE] - mg)
                          for t in range(hi // LANE)]
                    ps.append(jnp.concatenate(pg, axis=1))
                    parts.append(functools.reduce(lambda a, b: a + b, pg))
                p = jnp.concatenate(ps, axis=0)
                l = jnp.sum(jnp.concatenate(parts, axis=0), axis=-1, keepdims=True)
            else:
                p = jnp.exp2(s - m)
                l = jnp.sum(p, axis=-1, keepdims=True)
            rl = pl.reciprocal(l, approx=True)
            rl = rl * (2.0 - l * rl)
            v = jnp.concatenate(vs, axis=0)[:hi].astype(BF16)
            ctx = jnp.dot((p * rl).astype(BF16), v, preferred_element_type=F32)
            ctx_ref[h, lo // 2:hi // 2, :] = _as_u32(ctx.astype(BF16))

        nb = TP // TQ
        nr = S // TP
        for r in range(nr):
            proj_kv(r)
            if r >= 2:
                for i in range((r - 2) * nb, (r - 1) * nb):
                    pv(i)
            proj_q(r)
            if SSM_AT <= r <= SSM_AT + FT:
                ssm_tile(r - SSM_AT)
            if r >= 1:
                for i in range((r - 1) * nb, r * nb):
                    qk(i)
        for i in range((nr - 1) * nb, nr * nb):
            qk(i)
            pv(i - nb)
        for i in range((nr - 1) * nb, nr * nb):
            pv(i)
        return 0

    jax.lax.fori_loop(0, H, head_step, 0)

    wot_cp.wait()

    def o_copy(j, slot):
        return pltpu.make_async_copy(o_buf.at[slot], o_hbm.at[:, pl.ds(j * TO, TO)], osem.at[slot])

    def o_step(j, _):
        slot = j % 2

        @pl.when(j >= 2)
        def _():
            o_copy(j - 2, slot).wait()

        rows2 = pl.ds(pl.multiple_of(j * (TO // 2), TO // 2), TO // 2)
        wot = _as_bf16(jnp.concatenate([wot_ref[k] for k in range(H)], axis=1))
        ctx = _as_bf16(jnp.concatenate([ctx_ref[k, rows2, :] for k in range(H)], axis=1))
        yt = jnp.concatenate([ys_ref[j * (TO // TS) + k] for k in range(TO // TS)], axis=1)
        at = _dot_nt(wot, ctx)
        xt = xt_ref[:, pl.ds(pl.multiple_of(j * TO, TO), TO)].astype(F32)
        dcol = jnp.concatenate([col_ref[0]] * (TO // LANE), axis=1)
        gcol = jnp.concatenate([col_ref[1]] * (TO // LANE), axis=1)
        z = jnp.sum((xt * gcol).astype(BF16).astype(F32), axis=0, keepdims=True)
        g = jax.nn.sigmoid(z.astype(BF16).astype(F32)).astype(BF16).astype(F32)
        omg = (1.0 - g).astype(BF16).astype(F32)
        o_buf[slot] = g * at + omg * (yt + (xt * dcol).astype(BF16).astype(F32))
        o_copy(j, slot).start()
        return 0

    no = S // TO
    jax.lax.fori_loop(0, no, o_step, 0)
    o_copy(no - 2, no % 2).wait()
    o_copy(no - 1, (no - 1) % 2).wait()


@jax.jit
def pallas_gated_mix__compressed_kv_cla__ssm_conv_s5__prompt_kernel(
    A_x: jax.Array,
    A_c_kv: jax.Array,
    A_w_q: jax.Array,
    A_w_uk: jax.Array,
    A_w_uv: jax.Array,
    A_w_o: jax.Array,
    B_x: jax.Array,
    B_Lambda_re: jax.Array,
    B_Lambda_im: jax.Array,
    B_B_re: jax.Array,
    B_B_im: jax.Array,
    B_C_re: jax.Array,
    B_C_im: jax.Array,
    B_log_dt: jax.Array,
    B_Dskip: jax.Array,
    gate_w: jax.Array,
):
    del B_x
    _, S, M = A_x.shape
    C = A_c_kv.shape[2]
    H, D = A_w_q.shape[1], A_w_q.shape[2]
    PP = (M + LANE - 1) // LANE * LANE

    hbm = pl.BlockSpec(memory_space=pl.ANY)
    out_t = pl.pallas_call(
        functools.partial(_kernel, S=S, M=M, H=H, D=D),
        in_specs=[hbm] * 15,
        out_specs=hbm,
        out_shape=jax.ShapeDtypeStruct((M, S), F32),
        scratch_shapes=[
            pltpu.VMEM((M, S), BF16),
            pltpu.VMEM((S // 2, M), U32),
            pltpu.VMEM((S // 2, C), U32),
            pltpu.VMEM((2, M, D), U32),
            pltpu.VMEM((2, C, D), U32),
            pltpu.VMEM((2, C, D), U32),
            pltpu.VMEM((H, M // 2, D), U32),
            pltpu.VMEM((M, M), U32),
            pltpu.VMEM((M // 2, M), U32),
            pltpu.VMEM((M // 2, M), U32),
            pltpu.VMEM((M // 2, LANE), U32),
            pltpu.VMEM((S + 8, 2 * M), F32),
            pltpu.VMEM((H, M, S // H), F32),
            pltpu.VMEM((8, 2 * M), F32),
            pltpu.VMEM((10, 8, PP), F32),
            pltpu.VMEM((2, M, LANE), F32),
        ] + [pltpu.VMEM((M,), BF16)] * 5 + [
            pltpu.VMEM((H, S // 2, D), U32),
            pltpu.VMEM((2, M, TO), F32),
            pltpu.SMEM((1,), jnp.int32),
            pltpu.SemaphoreType.DMA((3, 2)),
            pltpu.SemaphoreType.DMA((S // TU,)),
            pltpu.SemaphoreType.DMA((7,)),
            pltpu.SemaphoreType.DMA((5,)),
            pltpu.SemaphoreType.DMA((2,)),
        ],
        compiler_params=pltpu.CompilerParams(
            vmem_limit_bytes=120 * 1024 * 1024,
        ),
    )(
        jnp.swapaxes(A_x, 1, 2).reshape(M, S), A_c_kv.reshape(S, C),
        A_w_q, A_w_uk, A_w_uv, jnp.swapaxes(A_w_o, 1, 2),
        B_B_re, B_B_im, B_C_re, B_C_im,
        B_Lambda_re, B_Lambda_im, B_log_dt, B_Dskip, gate_w,
    )
    return jnp.swapaxes(out_t.reshape(1, M, S), 1, 2)
```

```python
import functools

import jax
import jax.numpy as jnp
import jax.experimental.pallas as pl
import jax.experimental.pallas.tpu as pltpu

F32 = jnp.float32
BF16 = jnp.bfloat16
U32 = jnp.uint32

NT_DIMS = (((1,), (1,)), ((), ()))
LOG2E = 1.4426950408889634

TQ = 128
TP = 256
TU = 512
TO = 256
LANE = 128
HALF = LANE // 2
SSM_AT = 1
PACE_FROM = 6
PACE_ROWS = 8


def _dot_nt(a, b):
    return jax.lax.dot_general(a, b, NT_DIMS, preferred_element_type=F32)


def _unpack(w32, shift):
    v = (w32 << shift) & jnp.uint32(0xFFFF0000)
    return pltpu.bitcast(v, F32)


def _as_bf16(w32):
    return pltpu.bitcast(w32, BF16)


def _as_u32(v):
    return pltpu.bitcast(v, U32)


def _strassen_lhs(a11, a12, a21, a22):
    return [a11 + a22, a21 + a22, a11, a22, a11 + a12, a21 - a11, a12 - a22]


def _strassen_rhs(b11, b12, b21, b22):
    return [b11 + b22, b11, b12 - b22, b21 - b11, b22, b11 + b12, b21 + b22]


def _strassen_out(m):
    return ((m[0] + m[3]) + (m[6] - m[4]), m[2] + m[4],
            m[1] + m[3], (m[0] - m[1]) + (m[2] + m[5]))


SUMS = (0, 1, 4, 5, 6)
ORDER = (1, 4, 2, 3, 0, 5, 6)


def _kernel(xt_hbm, c_hbm, wq_hbm, wuk_hbm, wuv_hbm, wot_hbm,
            bre_hbm, bim_hbm, cre_hbm, cim_hbm,
            lre_hbm, lim_hbm, ldt_hbm, dsk_hbm, gw_hbm,
            o_hbm,
            xt_ref, x_ref, c_ref, l_ref, wq_buf, wk_buf, wv_buf, wot_ref,
            b_ref, cre_ref, cim_ref, cmid_ref, u_ref, ys_ref, st_ref, co_ref, col_ref,
            lre_ref, lim_ref, ldt_ref, dsk_ref, gw_ref,
            ctx_ref, o_buf, zero_ref, wsem, xsem, msem, vsem, osem,
            *, S, M, H, D):
    P = M
    FT = P // LANE
    PF = FT * LANE
    assert P - PF == HALF
    PP = PF + LANE
    TS = S // H

    def w_copies(pair, slot):
        return [
            pltpu.make_async_copy(src.bitcast(U32).at[:, pair, :],
                                  dst.at[slot], wsem.at[k, slot])
            for k, (src, dst) in enumerate(
                ((wuk_hbm, wk_buf), (wuv_hbm, wv_buf), (wq_hbm, wq_buf)))
        ]

    def x_copy(j):
        cols = pl.ds(j * TU, TU)
        return pltpu.make_async_copy(xt_hbm.at[:, cols], xt_ref.at[:, cols], xsem.at[j])

    bre32, bim32 = bre_hbm.bitcast(U32), bim_hbm.bitcast(U32)
    b_cps = [
        pltpu.make_async_copy(bre32, b_ref.at[pl.ds(0, P // 2), :], msem.at[0]),
        pltpu.make_async_copy(bim32.at[pl.ds(PF // 2, HALF // 2), :],
                              b_ref.at[pl.ds(P // 2, HALF // 2), :], msem.at[1]),
        pltpu.make_async_copy(bim32.at[pl.ds(0, PF // 2), :],
                              b_ref.at[pl.ds(PP // 2, PF // 2), :], msem.at[2]),
    ]
    c_cp = pltpu.make_async_copy(c_hbm.bitcast(U32), c_ref, msem.at[3])
    cre_cp = pltpu.make_async_copy(cre_hbm.bitcast(U32), cre_ref, msem.at[4])
    cim_cp = pltpu.make_async_copy(cim_hbm.bitcast(U32), cim_ref, msem.at[5])
    wot_cp = pltpu.make_async_copy(wot_hbm.bitcast(U32), wot_ref, msem.at[6])
    v_cps = [pltpu.make_async_copy(src, dst, vsem.at[k]) for k, (src, dst) in enumerate(
        ((lre_hbm, lre_ref), (lim_hbm, lim_ref), (ldt_hbm, ldt_ref),
         (dsk_hbm, dsk_ref), (gw_hbm, gw_ref)))]

    for cp in v_cps:
        cp.start()
    x_copy(0).start()
    for cp in b_cps:
        cp.start()
    for j in range(1, S // TU):
        x_copy(j).start()
    c_cp.start()
    for cp in w_copies(0, 0):
        cp.start()
    cre_cp.start()
    cim_cp.start()

    zero_ref[0] = 0
    u_ref[pl.ds(0, 8), :] = jnp.zeros((8, u_ref.shape[1]), F32)
    st_ref[...] = jnp.zeros(st_ref.shape, F32)
    for cp in v_cps:
        cp.wait()

    row = lambda r: r[...].astype(F32).reshape(1, P)
    lre, lim = row(lre_ref), row(lim_ref)
    dt = jnp.exp(row(ldt_ref)).astype(BF16).astype(F32)
    e = jnp.exp(dt * lre)
    ang = dt * lim
    ar = e * jnp.cos(ang)
    ai = e * jnp.sin(ang)
    sc = jnp.maximum(jnp.abs(lre), jnp.abs(lim))
    nre, nim = lre / sc, lim / sc
    den = (nre * nre + nim * nim) * sc
    gr = 2.0 * ((ar - 1.0) * nre + ai * nim) / den
    gi = 2.0 * (ai * nre - (ar - 1.0) * nim) / den

    def put(k, full, lo, hi):
        v = jnp.concatenate([full[:, :PF], lo[:, PF:], hi[:, PF:]], axis=1)
        co_ref[k] = jnp.broadcast_to(v, (8, PP))

    put(0, gr, gr, -gr)
    put(1, gi, -gi, -gi)
    pr, pi = ar, -ai
    for j in range(1, 5):
        put(2 * j, pr, pr, pr)
        put(2 * j + 1, pi, -pi, pi)
        pr, pi = pr * pr - pi * pi, 2.0 * pr * pi

    zpad = jnp.zeros((1, PP - P), F32)
    for k, r in enumerate((dsk_ref, gw_ref)):
        v = jnp.concatenate([row(r), zpad], axis=1)
        col_ref[k] = jnp.broadcast_to(v, (LANE, PP)).T[:M]

    for cp in b_cps:
        cp.wait()

    def u_step(j, _):
        x_copy(j).wait()
        t0 = pl.multiple_of(j * TU, TU)
        xc = xt_ref[:, pl.ds(t0, TU)].T
        x_ref[pl.ds(pl.multiple_of(j * (TU // 2), TU // 2), TU // 2), :] = _as_u32(xc)
        u_ref[pl.ds(t0 + 8, TU), :] = _dot_nt(xc, _as_bf16(b_ref[...]))
        return 0

    jax.lax.fori_loop(0, S // TU, u_step, 0)
    wot_cp.start()
    c_cp.wait()
    CH = c_ref.shape[1] // 2
    TH = TP // 2

    def l_step(r, _):
        c = _as_bf16(c_ref[pl.ds(pl.multiple_of(r * TH, TH), TH), :]).astype(F32)
        ls = _strassen_lhs(c[:TH, :CH], c[:TH, CH:], c[TH:, :CH], c[TH:, CH:])
        for n, k in enumerate(SUMS):
            l_ref[n, pl.ds(pl.multiple_of(r * (TH // 2), TH // 2), TH // 2), :] = (
                _as_u32(ls[k].astype(BF16)))
        return 0

    jax.lax.fori_loop(0, S // TP, l_step, 0)
    cre_cp.wait()
    cim_cp.wait()
    cmid_ref[...] = jnp.concatenate([cre_ref[:, PF:], cim_ref[:, PF:]], axis=1)

    def head_step(h, _):
        pair = h // 2
        slot = pair % 2

        @pl.when(h % 2 == 0)
        def _wait_weights():
            for cp in w_copies(pair, slot):
                cp.wait()

            @pl.when(pair + 1 < H // 2)
            def _():
                for cp in w_copies(pair + 1, 1 - slot):
                    cp.start()

        zero = zero_ref[0]

        ys = []

        def ssm_tile(t):
            rows = pl.ds(pl.multiple_of(h * TS, TS), TS + 8)
            cr, ci = pl.ds(t * LANE, LANE), pl.ds(PP + t * LANE, LANE)
            co = lambda k, n=8: co_ref[k, 0:n, cr]
            if t < FT:
                mul = lambda a, b, x: (a * x[0] - b * x[1], a * x[1] + b * x[0])
                ur, ui = u_ref[rows, cr], u_ref[rows, ci]
                w = (co(0, 1) * ur - co(1, 1) * ui, -(co(0, 1) * ui + co(1, 1) * ur))
                s = (st_ref[:, cr], st_ref[:, ci])
            else:
                mul = lambda a, b, x: (a * x[0] + b * pltpu.roll(x[0], HALF, 1),)
                w = mul(co(0, 1), co(1, 1), (u_ref[rows, cr],))
                s = (st_ref[:, cr],)
            for j in range(3):
                d = mul(co(2 * j + 2, 1), co(2 * j + 3, 1), [pltpu.roll(v, 1 << j, 0) for v in w])
                w = [a + b for a, b in zip(d, w)]
            gs = []
            for k in range(1, TS // 8 + 1):
                s = [a + b[8 * k:8 * k + 8] for a, b in zip(mul(co(8), co(9), s), w)]
                gs.append(jnp.concatenate(s, axis=1))
                if t < FT:
                    s = [pltpu.roll(s[0], zero, 1), s[1]]
            st_ref[:, cr] = s[0]
            if t < FT:
                st_ref[:, ci] = s[1]
                cc = jnp.concatenate([cre_ref[:, cr], cim_ref[:, cr]], axis=1)
            else:
                cc = cmid_ref[...]
            g = jnp.concatenate(gs, axis=0).astype(BF16)
            y = jax.lax.dot_general(_as_bf16(cc), g, NT_DIMS, preferred_element_type=F32)
            ys[:] = [y + ys[0] if ys else y]
            if t == FT:
                ys_ref[h] = ys[0]

        shift = (16 * (1 - h % 2)).astype(U32)
        DH = D // 2
        wk, wv = _unpack(wk_buf[slot], shift), _unpack(wv_buf[slot], shift)
        wl = jnp.concatenate([wk[:, :DH], wv[:, :DH]], axis=1)
        wr = jnp.concatenate([wk[:, DH:], wv[:, DH:]], axis=1)
        rw = [v.astype(BF16) for v in _strassen_rhs(wl[:CH], wr[:CH], wl[CH:], wr[CH:])]
        wq = _unpack(wq_buf[slot], shift).astype(BF16)
        qscale = (D ** -0.5) * LOG2E
        causal = (jax.lax.broadcasted_iota(jnp.int32, (TQ, TQ), 1)
                  <= jax.lax.broadcasted_iota(jnp.int32, (TQ, TQ), 0))

        ks, vs, qs, ss = [], [], [], {}

        def proj_kv(r):
            ms = [None] * 7
            for k in ORDER:
                if k in SUMS:
                    a = l_ref[SUMS.index(k), pl.ds(r * TH // 2, TH // 2), :]
                elif k == 2:
                    a = c_ref[pl.ds(r * TH, TH // 2), pl.ds(0, CH)]
                else:
                    a = c_ref[pl.ds(r * TH + TH // 2, TH // 2), pl.ds(CH, CH)]
                ms[k] = jnp.dot(_as_bf16(a), rw[k], preferred_element_type=F32)
            c11, c12, c21, c22 = _strassen_out(ms)
            for lft, rgt in ((c11, c12), (c21, c22)):
                ks.append(jnp.concatenate([lft[:, :DH], rgt[:, :DH]], axis=1))
                vs.append(jnp.concatenate([lft[:, DH:], rgt[:, DH:]], axis=1))

        def proj_q(r):
            x = _as_bf16(x_ref[pl.ds(r * TP // 2, TP // 2), :])
            qs.append(jnp.dot(x, wq, preferred_element_type=F32) * qscale)

        def qk(i):
            lo, hi = i * TQ, (i + 1) * TQ
            q = jnp.concatenate(qs, axis=0)[lo:hi].astype(BF16)
            k = jnp.concatenate(ks, axis=0)[:hi].astype(BF16)
            ss[i] = jax.lax.dot_general(q, k, NT_DIMS, preferred_element_type=F32)

        def pv(i):
            lo, hi = i * TQ, (i + 1) * TQ
            s = ss.pop(i)
            sd = jnp.where(causal, s[:, lo:], -1e9 * LOG2E)
            s = sd if i == 0 else jnp.concatenate([s[:, :lo], sd], axis=1)
            m = jnp.max(s, axis=-1, keepdims=True)
            if i >= PACE_FROM:
                mb = _as_u32(jnp.broadcast_to(m, (TQ, LANE)))
                ps, parts = [], []
                for g in range(0, TQ, PACE_ROWS):
                    mg = mb[g:g + PACE_ROWS]
                    if parts:
                        mg = mg | (_as_u32(parts[-1]) & zero.astype(U32))
                    mg = pltpu.bitcast(mg, F32)
                    pg = [jnp.exp2(s[g:g + PACE_ROWS, t * LANE:(t + 1) * LANE] - mg)
                          for t in range(hi // LANE)]
                    ps.append(jnp.concatenate(pg, axis=1))
                    parts.append(functools.reduce(lambda a, b: a + b, pg))
                p = jnp.concatenate(ps, axis=0)
                l = jnp.sum(jnp.concatenate(parts, axis=0), axis=-1, keepdims=True)
            else:
                p = jnp.exp2(s - m)
                l = jnp.sum(p, axis=-1, keepdims=True)
            rl = pl.reciprocal(l, approx=True)
            rl = rl * (2.0 - l * rl)
            v = jnp.concatenate(vs, axis=0)[:hi].astype(BF16)
            ctx = jnp.dot((p * rl).astype(BF16), v, preferred_element_type=F32)
            ctx_ref[h, lo // 2:hi // 2, :] = _as_u32(ctx.astype(BF16))

        nb = TP // TQ
        nr = S // TP
        for r in range(nr):
            proj_kv(r)
            if r >= 2:
                for i in range((r - 2) * nb, (r - 1) * nb):
                    pv(i)
            proj_q(r)
            if SSM_AT <= r <= SSM_AT + FT:
                ssm_tile(r - SSM_AT)
            if r >= 1:
                for i in range((r - 1) * nb, r * nb):
                    qk(i)
        for i in range((nr - 1) * nb, nr * nb):
            qk(i)
            pv(i - nb)
        for i in range((nr - 1) * nb, nr * nb):
            pv(i)
        return 0

    jax.lax.fori_loop(0, H, head_step, 0)

    wot_cp.wait()

    def o_copy(j, slot):
        return pltpu.make_async_copy(o_buf.at[slot], o_hbm.at[:, pl.ds(j * TO, TO)], osem.at[slot])

    def o_step(j, _):
        slot = j % 2

        @pl.when(j >= 2)
        def _():
            o_copy(j - 2, slot).wait()

        rows2 = pl.ds(pl.multiple_of(j * (TO // 2), TO // 2), TO // 2)
        wot = _as_bf16(jnp.concatenate([wot_ref[k] for k in range(H)], axis=1))
        ctx = _as_bf16(jnp.concatenate([ctx_ref[k, rows2, :] for k in range(H)], axis=1))
        yt = jnp.concatenate([ys_ref[j * (TO // TS) + k] for k in range(TO // TS)], axis=1)
        at = _dot_nt(wot, ctx)
        xt = xt_ref[:, pl.ds(pl.multiple_of(j * TO, TO), TO)].astype(F32)
        dcol = jnp.concatenate([col_ref[0]] * (TO // LANE), axis=1)
        gcol = jnp.concatenate([col_ref[1]] * (TO // LANE), axis=1)
        z = jnp.sum((xt * gcol).astype(BF16).astype(F32), axis=0, keepdims=True)
        g = jax.nn.sigmoid(z.astype(BF16).astype(F32)).astype(BF16).astype(F32)
        omg = (1.0 - g).astype(BF16).astype(F32)
        o_buf[slot] = g * at + omg * (yt + (xt * dcol).astype(BF16).astype(F32))
        o_copy(j, slot).start()
        return 0

    no = S // TO
    jax.lax.fori_loop(0, no, o_step, 0)
    o_copy(no - 2, no % 2).wait()
    o_copy(no - 1, (no - 1) % 2).wait()


@jax.jit
def pallas_gated_mix__compressed_kv_cla__ssm_conv_s5__prompt_kernel(
    A_x: jax.Array,
    A_c_kv: jax.Array,
    A_w_q: jax.Array,
    A_w_uk: jax.Array,
    A_w_uv: jax.Array,
    A_w_o: jax.Array,
    B_x: jax.Array,
    B_Lambda_re: jax.Array,
    B_Lambda_im: jax.Array,
    B_B_re: jax.Array,
    B_B_im: jax.Array,
    B_C_re: jax.Array,
    B_C_im: jax.Array,
    B_log_dt: jax.Array,
    B_Dskip: jax.Array,
    gate_w: jax.Array,
):
    del B_x
    _, S, M = A_x.shape
    C = A_c_kv.shape[2]
    H, D = A_w_q.shape[1], A_w_q.shape[2]
    PP = (M + LANE - 1) // LANE * LANE

    hbm = pl.BlockSpec(memory_space=pl.ANY)
    out_t = pl.pallas_call(
        functools.partial(_kernel, S=S, M=M, H=H, D=D),
        in_specs=[hbm] * 15,
        out_specs=hbm,
        out_shape=jax.ShapeDtypeStruct((M, S), F32),
        scratch_shapes=[
            pltpu.VMEM((M, S), BF16),
            pltpu.VMEM((S // 2, M), U32),
            pltpu.VMEM((S // 2, C), U32),
            pltpu.VMEM((5, S // 4, C // 2), U32),
            pltpu.VMEM((2, M, D), U32),
            pltpu.VMEM((2, C, D), U32),
            pltpu.VMEM((2, C, D), U32),
            pltpu.VMEM((H, M // 2, D), U32),
            pltpu.VMEM((M, M), U32),
            pltpu.VMEM((M // 2, M), U32),
            pltpu.VMEM((M // 2, M), U32),
            pltpu.VMEM((M // 2, LANE), U32),
            pltpu.VMEM((S + 8, 2 * M), F32),
            pltpu.VMEM((H, M, S // H), F32),
            pltpu.VMEM((8, 2 * M), F32),
            pltpu.VMEM((10, 8, PP), F32),
            pltpu.VMEM((2, M, LANE), F32),
        ] + [pltpu.VMEM((M,), BF16)] * 5 + [
            pltpu.VMEM((H, S // 2, D), U32),
            pltpu.VMEM((2, M, TO), F32),
            pltpu.SMEM((1,), jnp.int32),
            pltpu.SemaphoreType.DMA((3, 2)),
            pltpu.SemaphoreType.DMA((S // TU,)),
            pltpu.SemaphoreType.DMA((7,)),
            pltpu.SemaphoreType.DMA((5,)),
            pltpu.SemaphoreType.DMA((2,)),
        ],
        compiler_params=pltpu.CompilerParams(
            vmem_limit_bytes=120 * 1024 * 1024,
        ),
    )(
        jnp.swapaxes(A_x, 1, 2).reshape(M, S), A_c_kv.reshape(S, C),
        A_w_q, A_w_uk, A_w_uv, jnp.swapaxes(A_w_o, 1, 2),
        B_B_re, B_B_im, B_C_re, B_C_im,
        B_Lambda_re, B_Lambda_im, B_log_dt, B_Dskip, gate_w,
    )
    return jnp.swapaxes(out_t.reshape(1, M, S), 1, 2)
```

```python
import functools

import jax
import jax.numpy as jnp
import jax.experimental.pallas as pl
import jax.experimental.pallas.tpu as pltpu

F32 = jnp.float32
BF16 = jnp.bfloat16
U32 = jnp.uint32

NT_DIMS = (((1,), (1,)), ((), ()))
LOG2E = 1.4426950408889634

TQ = 128
TP = 256
TU = 512
TO = 256
LANE = 128
HALF = LANE // 2
SSM_AT = 1
PACE_FROM = 4
PACE_ROWS = 8
TWO_PASS = False
CHAIN_ALL = False
CHAIN = True
PACE2_FROM = 2
PACE2_EXTRA = 1


def _dot_nt(a, b):
    return jax.lax.dot_general(a, b, NT_DIMS, preferred_element_type=F32)


def _unpack(w32, shift):
    v = (w32 << shift) & jnp.uint32(0xFFFF0000)
    return pltpu.bitcast(v, F32)


def _as_bf16(w32):
    return pltpu.bitcast(w32, BF16)


def _as_u32(v):
    return pltpu.bitcast(v, U32)


def _strassen_lhs(a11, a12, a21, a22):
    return [a11 + a22, a21 + a22, a11, a22, a11 + a12, a21 - a11, a12 - a22]


def _strassen_rhs(b11, b12, b21, b22):
    return [b11 + b22, b11, b12 - b22, b21 - b11, b22, b11 + b12, b21 + b22]


def _strassen_out(m):
    return ((m[0] + m[3]) + (m[6] - m[4]), m[2] + m[4],
            m[1] + m[3], (m[0] - m[1]) + (m[2] + m[5]))


SUMS = (0, 1, 4, 5, 6)
ORDER = (1, 4, 2, 3, 0, 5, 6)
PV_ORDER = (2, 4, 3, 1, 5, 0, 6)


def _kernel(xt_hbm, c_hbm, wq_hbm, wuk_hbm, wuv_hbm, wot_hbm,
            bre_hbm, bim_hbm, cre_hbm, cim_hbm,
            lre_hbm, lim_hbm, ldt_hbm, dsk_hbm, gw_hbm,
            o_hbm,
            xt_ref, x_ref, c_ref, l_ref, wq_buf, wk_buf, wv_buf, wot_ref, lo_ref,
            b_ref, cre_ref, cim_ref, cmid_ref, u_ref, ys_ref, st_ref, co_ref, col_ref,
            lre_ref, lim_ref, ldt_ref, dsk_ref, gw_ref,
            ctx_ref, o_buf, zero_ref, wsem, xsem, msem, vsem, wosem, osem,
            *, S, M, H, D):
    P = M
    FT = P // LANE
    PF = FT * LANE
    assert P - PF == HALF
    PP = PF + LANE
    TS = S // H

    def w_copies(pair, slot):
        return [
            pltpu.make_async_copy(src.bitcast(U32).at[:, pair, :],
                                  dst.at[slot], wsem.at[k, slot])
            for k, (src, dst) in enumerate(
                ((wuk_hbm, wk_buf), (wuv_hbm, wv_buf), (wq_hbm, wq_buf)))
        ]

    def x_copy(j):
        cols = pl.ds(j * TU, TU)
        return pltpu.make_async_copy(xt_hbm.at[:, cols], xt_ref.at[:, cols], xsem.at[j])

    bre32, bim32 = bre_hbm.bitcast(U32), bim_hbm.bitcast(U32)
    b_cps = [
        pltpu.make_async_copy(bre32, b_ref.at[pl.ds(0, P // 2), :], msem.at[0]),
        pltpu.make_async_copy(bim32.at[pl.ds(PF // 2, HALF // 2), :],
                              b_ref.at[pl.ds(P // 2, HALF // 2), :], msem.at[1]),
        pltpu.make_async_copy(bim32.at[pl.ds(0, PF // 2), :],
                              b_ref.at[pl.ds(PP // 2, PF // 2), :], msem.at[2]),
    ]
    c_cp = pltpu.make_async_copy(c_hbm.bitcast(U32), c_ref, msem.at[3])
    cre_cp = pltpu.make_async_copy(cre_hbm.bitcast(U32), cre_ref, msem.at[4])
    cim_cp = pltpu.make_async_copy(cim_hbm.bitcast(U32), cim_ref, msem.at[5])

    def wo_copy(k):
        return pltpu.make_async_copy(wot_hbm.bitcast(U32).at[k], wot_ref.at[k], wosem.at[k])

    v_cps = [pltpu.make_async_copy(src, dst, vsem.at[k]) for k, (src, dst) in enumerate(
        ((lre_hbm, lre_ref), (lim_hbm, lim_ref), (ldt_hbm, ldt_ref),
         (dsk_hbm, dsk_ref), (gw_hbm, gw_ref)))]

    for cp in v_cps:
        cp.start()
    x_copy(0).start()
    for cp in b_cps:
        cp.start()
    for j in range(1, S // TU):
        x_copy(j).start()
    c_cp.start()
    for cp in w_copies(0, 0):
        cp.start()
    cre_cp.start()
    cim_cp.start()
    wo_copy(0).start()

    zero_ref[0] = 0
    u_ref[pl.ds(0, 8), :] = jnp.zeros((8, u_ref.shape[1]), F32)
    st_ref[...] = jnp.zeros(st_ref.shape, F32)
    for cp in v_cps:
        cp.wait()

    row = lambda r: r[...].astype(F32).reshape(1, P)
    lre, lim = row(lre_ref), row(lim_ref)
    dt = jnp.exp(row(ldt_ref)).astype(BF16).astype(F32)
    e = jnp.exp(dt * lre)
    ang = dt * lim
    ar = e * jnp.cos(ang)
    ai = e * jnp.sin(ang)
    sc = jnp.maximum(jnp.abs(lre), jnp.abs(lim))
    nre, nim = lre / sc, lim / sc
    den = (nre * nre + nim * nim) * sc
    gr = 2.0 * ((ar - 1.0) * nre + ai * nim) / den
    gi = 2.0 * (ai * nre - (ar - 1.0) * nim) / den

    def put(k, full, lo, hi):
        v = jnp.concatenate([full[:, :PF], lo[:, PF:], hi[:, PF:]], axis=1)
        co_ref[k] = jnp.broadcast_to(v, (8, PP))

    put(0, gr, gr, -gr)
    put(1, gi, -gi, -gi)
    pr, pi = ar, -ai
    for j in range(1, 5):
        put(2 * j, pr, pr, pr)
        put(2 * j + 1, pi, -pi, pi)
        pr, pi = pr * pr - pi * pi, 2.0 * pr * pi

    zpad = jnp.zeros((1, PP - P), F32)
    for k, r in enumerate((dsk_ref, gw_ref)):
        v = jnp.concatenate([row(r), zpad], axis=1)
        col_ref[k] = jnp.broadcast_to(v, (LANE, PP)).T[:M]

    for cp in b_cps:
        cp.wait()

    def u_step(j, _):
        x_copy(j).wait()
        t0 = pl.multiple_of(j * TU, TU)
        xc = xt_ref[:, pl.ds(t0, TU)].T
        x_ref[pl.ds(pl.multiple_of(j * (TU // 2), TU // 2), TU // 2), :] = _as_u32(xc)
        u_ref[pl.ds(t0 + 8, TU), :] = _dot_nt(xc, _as_bf16(b_ref[...]))
        return 0

    jax.lax.fori_loop(0, S // TU, u_step, 0)
    c_cp.wait()
    CH = c_ref.shape[1] // 2
    TH = TP // 2

    def l_step(r, _):
        c = _as_bf16(c_ref[pl.ds(pl.multiple_of(r * TH, TH), TH), :]).astype(F32)
        ls = _strassen_lhs(c[:TH, :CH], c[:TH, CH:], c[TH:, :CH], c[TH:, CH:])
        for n, k in enumerate(SUMS):
            l_ref[n, pl.ds(pl.multiple_of(r * (TH // 2), TH // 2), TH // 2), :] = (
                _as_u32(ls[k].astype(BF16)))
        return 0

    jax.lax.fori_loop(0, S // TP, l_step, 0)
    cre_cp.wait()
    cim_cp.wait()
    cmid_ref[...] = jnp.concatenate([cre_ref[:, PF:], cim_ref[:, PF:]], axis=1)
    for k in range(1, H):
        wo_copy(k).start()
    DH, MH = D // 2, M // 2

    def head_step(h, _):
        pair = h // 2
        slot = pair % 2

        @pl.when(h % 2 == 0)
        def _wait_weights():
            for cp in w_copies(pair, slot):
                cp.wait()

            @pl.when(pair + 1 < H // 2)
            def _():
                for cp in w_copies(pair + 1, 1 - slot):
                    cp.start()

        wo_copy(h).wait()
        zero = zero_ref[0]

        ys = []

        def ssm_tile(t):
            rows = pl.ds(pl.multiple_of(h * TS, TS), TS + 8)
            cr, ci = pl.ds(t * LANE, LANE), pl.ds(PP + t * LANE, LANE)
            co = lambda k, n=8: co_ref[k, 0:n, cr]
            if t < FT:
                mul = lambda a, b, x: (a * x[0] - b * x[1], a * x[1] + b * x[0])
                ur, ui = u_ref[rows, cr], u_ref[rows, ci]
                w = (co(0, 1) * ur - co(1, 1) * ui, -(co(0, 1) * ui + co(1, 1) * ur))
                s = (st_ref[:, cr], st_ref[:, ci])
            else:
                mul = lambda a, b, x: (a * x[0] + b * pltpu.roll(x[0], HALF, 1),)
                w = mul(co(0, 1), co(1, 1), (u_ref[rows, cr],))
                s = (st_ref[:, cr],)
            for j in range(3):
                d = mul(co(2 * j + 2, 1), co(2 * j + 3, 1), [pltpu.roll(v, 1 << j, 0) for v in w])
                w = [a + b for a, b in zip(d, w)]
            gs = []
            for k in range(1, TS // 8 + 1):
                s = [a + b[8 * k:8 * k + 8] for a, b in zip(mul(co(8), co(9), s), w)]
                gs.append(jnp.concatenate(s, axis=1))
                if t < FT:
                    s = [pltpu.roll(s[0], zero, 1), s[1]]
            st_ref[:, cr] = s[0]
            if t < FT:
                st_ref[:, ci] = s[1]
                cc = jnp.concatenate([cre_ref[:, cr], cim_ref[:, cr]], axis=1)
            else:
                cc = cmid_ref[...]
            g = jnp.concatenate(gs, axis=0).astype(BF16)
            y = jax.lax.dot_general(_as_bf16(cc), g, NT_DIMS, preferred_element_type=F32)
            ys[:] = [y + ys[0] if ys else y]
            if t == FT:
                ys_ref[h] = ys[0]

        shift = (16 * (1 - h % 2)).astype(U32)
        wk, wv = _unpack(wk_buf[slot], shift), _unpack(wv_buf[slot], shift)
        wl = jnp.concatenate([wk[:, :DH], wv[:, :DH]], axis=1)
        wr = jnp.concatenate([wk[:, DH:], wv[:, DH:]], axis=1)
        rw = [v.astype(BF16) for v in _strassen_rhs(wl[:CH], wr[:CH], wl[CH:], wr[CH:])]
        wq = _unpack(wq_buf[slot], shift).astype(BF16)
        qscale = (D ** -0.5) * LOG2E
        causal = (jax.lax.broadcasted_iota(jnp.int32, (TQ, TQ), 1)
                  <= jax.lax.broadcasted_iota(jnp.int32, (TQ, TQ), 0))

        ks, vs, rvs, qs, ss, chains = [], [], [], [], {}, [None]

        def proj_kv(r):
            ms = [None] * 7
            for k in ORDER:
                if k in SUMS:
                    a = l_ref[SUMS.index(k), pl.ds(r * TH // 2, TH // 2), :]
                elif k == 2:
                    a = c_ref[pl.ds(r * TH, TH // 2), pl.ds(0, CH)]
                else:
                    a = c_ref[pl.ds(r * TH + TH // 2, TH // 2), pl.ds(CH, CH)]
                ms[k] = jnp.dot(_as_bf16(a), rw[k], preferred_element_type=F32)
            c11, c12, c21, c22 = _strassen_out(ms)
            for lft, rgt in ((c11, c12), (c21, c22)):
                ks.append(jnp.concatenate([lft[:, :DH], rgt[:, :DH]], axis=1))
                vs.append(jnp.concatenate([lft[:, DH:], rgt[:, DH:]], axis=1))
            rvs.append(_strassen_rhs(c11[:, DH:], c12[:, DH:], c21[:, DH:], c22[:, DH:]))

        def proj_q(r):
            x = _as_bf16(x_ref[pl.ds(r * TP // 2, TP // 2), :])
            qs.append(jnp.dot(x, wq, preferred_element_type=F32) * qscale)

        def qk(i):
            lo, hi = i * TQ, (i + 1) * TQ
            q = jnp.concatenate(qs, axis=0)[lo:hi].astype(BF16)
            k = jnp.concatenate(ks, axis=0)[:hi].astype(BF16)
            ss[i] = jax.lax.dot_general(q, k, NT_DIMS, preferred_element_type=F32)

        def tie(a, b):
            return pltpu.bitcast(_as_u32(a) | (_as_u32(b) & zero.astype(U32)), F32)

        def exp_rows(s, m, pace, rows, chain=None):
            mb = jnp.broadcast_to(m, (TQ, LANE))
            ps, parts = [], []
            for g in range(0, TQ, rows):
                mg = mb[g:g + rows]
                if pace and (parts or chain is not None):
                    mg = tie(mg, parts[-1] if parts else chain)
                pg = [jnp.exp2(s[g:g + rows, t * LANE:(t + 1) * LANE] - mg)
                      for t in range(s.shape[1] // LANE)]
                ps.append(jnp.concatenate(pg, axis=1))
                parts.append(functools.reduce(lambda a, b: a + b, pg))
            return jnp.concatenate(ps, axis=0), jnp.concatenate(parts, axis=0)

        def scores(i, chain=None):
            lo = i * TQ
            s = ss.pop(i)
            sd = jnp.where(causal, s[:, lo:], -1e9 * LOG2E)
            s = sd if i == 0 else jnp.concatenate([s[:, :lo], sd], axis=1)
            m = jnp.max(s, axis=-1, keepdims=True)
            p, part = exp_rows(s, m, i >= PACE_FROM, PACE_ROWS, chain)
            return s, m, p, jnp.sum(part, axis=-1, keepdims=True), part[TQ - PACE_ROWS:]

        def pv(j):
            s1, m1, p1, l1, chain = scores(2 * j, chains[0] if CHAIN_ALL else None)
            s2, m2, p2, l2, chains[0] = scores(2 * j + 1, chain if CHAIN else None)
            lo = 2 * j * TQ
            cat = lambda xs, axis: jnp.concatenate(xs, axis=axis)
            dot = lambda a, b: jnp.dot(a.astype(BF16), b.astype(BF16), preferred_element_type=F32)

            def recip(l):
                rl = pl.reciprocal(l, approx=True)
                return rl * (2.0 - l * rl)

            r1, r2 = recip(l1), recip(l2)
            dg = dot(cat([p1[:, lo:], p2[:, lo:lo + TQ]], 0), vs[2 * j])
            c1, c2 = dg[:TQ], dg[TQ:] + dot(p2[:, lo + TQ:], vs[2 * j + 1])
            if j > 0:
                tiles = lambda p, o: cat([p[:, (2 * t + o) * TQ:(2 * t + o + 1) * TQ] for t in range(j)], 1)
                a11, a12, a21, a22 = tiles(p1, 0), tiles(p1, 1), tiles(p2, 0), tiles(p2, 1)
                rho = l1 * r2
                a22r = a22 * rho
                lp = [a11 + a22r, a21 + a22, a11, a22, a11 + a12, a21 * rho - a11, a12 - a22r]
                m = [None] * 7
                for k in PV_ORDER:
                    m[k] = dot(lp[k], cat([rvs[t][k] for t in range(j)], 0))
                c1 = c1 + cat([(m[0] - m[4]) + (m[6] + m[3] * rho), m[2] + m[4]], 1)
                c2 = (c2 + cat([m[1] + m[3], -m[1]], 1)) * r2
                c2 = cat([c2[:, :DH], c2[:, DH:] + ((m[0] + m[2]) + m[5]) * r1], 1)
            else:
                c2 = c2 * r2
            c1 = c1 * r1
            for k, v in enumerate(_strassen_rhs(c1[:, :DH], c2[:, :DH], c1[:, DH:], c2[:, DH:])):
                ctx_ref[k, h, j * TQ // 2:(j + 1) * TQ // 2, :] = _as_u32(v.astype(BF16))

        def wo_sums():
            w = _as_bf16(wot_ref[h]).astype(F32)
            ls = _strassen_lhs(w[:MH, :DH], w[:MH, DH:], w[MH:, :DH], w[MH:, DH:])
            for n, k in enumerate(SUMS):
                lo_ref[n, h] = _as_u32(ls[k].astype(BF16))

        assert TP == 2 * TQ
        nr = S // TP
        wo_sums()
        for r in range(nr):
            proj_kv(r)
            if r >= 2:
                pv(r - 2)
            proj_q(r)
            if SSM_AT <= r <= SSM_AT + FT:
                ssm_tile(r - SSM_AT)
            if r >= 1:
                qk(2 * r - 2)
                qk(2 * r - 1)
        qk(2 * nr - 2)
        qk(2 * nr - 1)
        pv(nr - 2)
        pv(nr - 1)
        return 0

    jax.lax.fori_loop(0, H, head_step, 0)

    def o_copy(j, slot):
        return pltpu.make_async_copy(o_buf.at[slot], o_hbm.at[:, pl.ds(j * TO, TO)], osem.at[slot])

    def o_step(j, _):
        slot = j % 2

        @pl.when(j >= 2)
        def _():
            o_copy(j - 2, slot).wait()

        rows2 = pl.ds(pl.multiple_of(j * (TQ // 2), TQ // 2), TQ // 2)
        ms = [None] * 7
        for k in range(7):
            if k in SUMS:
                a = [lo_ref[SUMS.index(k), n] for n in range(H)]
            elif k == 2:
                a = [wot_ref[n, pl.ds(0, MH // 2), pl.ds(0, DH)] for n in range(H)]
            else:
                a = [wot_ref[n, pl.ds(MH // 2, MH // 2), pl.ds(DH, DH)] for n in range(H)]
            b = [ctx_ref[k, n, rows2, :] for n in range(H)]
            ms[k] = _dot_nt(_as_bf16(jnp.concatenate(a, axis=1)), _as_bf16(jnp.concatenate(b, axis=1)))
        c11, c12, c21, c22 = _strassen_out(ms)
        at = jnp.concatenate([jnp.concatenate([c11, c12], axis=1),
                              jnp.concatenate([c21, c22], axis=1)], axis=0)
        yt = jnp.concatenate([ys_ref[j * (TO // TS) + k] for k in range(TO // TS)], axis=1)
        xt = xt_ref[:, pl.ds(pl.multiple_of(j * TO, TO), TO)].astype(F32)
        dcol = jnp.concatenate([col_ref[0]] * (TO // LANE), axis=1)
        gcol = jnp.concatenate([col_ref[1]] * (TO // LANE), axis=1)
        z = jnp.sum((xt * gcol).astype(BF16).astype(F32), axis=0, keepdims=True)
        g = jax.nn.sigmoid(z.astype(BF16).astype(F32)).astype(BF16).astype(F32)
        omg = (1.0 - g).astype(BF16).astype(F32)
        o_buf[slot] = g * at + omg * (yt + (xt * dcol).astype(BF16).astype(F32))
        o_copy(j, slot).start()
        return 0

    assert TO == 2 * TQ
    no = S // TO
    jax.lax.fori_loop(0, no, o_step, 0)
    o_copy(no - 2, no % 2).wait()
    o_copy(no - 1, (no - 1) % 2).wait()


@jax.jit
def pallas_gated_mix__compressed_kv_cla__ssm_conv_s5__prompt_kernel(
    A_x: jax.Array,
    A_c_kv: jax.Array,
    A_w_q: jax.Array,
    A_w_uk: jax.Array,
    A_w_uv: jax.Array,
    A_w_o: jax.Array,
    B_x: jax.Array,
    B_Lambda_re: jax.Array,
    B_Lambda_im: jax.Array,
    B_B_re: jax.Array,
    B_B_im: jax.Array,
    B_C_re: jax.Array,
    B_C_im: jax.Array,
    B_log_dt: jax.Array,
    B_Dskip: jax.Array,
    gate_w: jax.Array,
):
    del B_x
    _, S, M = A_x.shape
    C = A_c_kv.shape[2]
    H, D = A_w_q.shape[1], A_w_q.shape[2]
    PP = (M + LANE - 1) // LANE * LANE

    hbm = pl.BlockSpec(memory_space=pl.ANY)
    out_t = pl.pallas_call(
        functools.partial(_kernel, S=S, M=M, H=H, D=D),
        in_specs=[hbm] * 15,
        out_specs=hbm,
        out_shape=jax.ShapeDtypeStruct((M, S), F32),
        scratch_shapes=[
            pltpu.VMEM((M, S), BF16),
            pltpu.VMEM((S // 2, M), U32),
            pltpu.VMEM((S // 2, C), U32),
            pltpu.VMEM((5, S // 4, C // 2), U32),
            pltpu.VMEM((2, M, D), U32),
            pltpu.VMEM((2, C, D), U32),
            pltpu.VMEM((2, C, D), U32),
            pltpu.VMEM((H, M // 2, D), U32),
            pltpu.VMEM((5, H, M // 4, D // 2), U32),
            pltpu.VMEM((M, M), U32),
            pltpu.VMEM((M // 2, M), U32),
            pltpu.VMEM((M // 2, M), U32),
            pltpu.VMEM((M // 2, LANE), U32),
            pltpu.VMEM((S + 8, 2 * M), F32),
            pltpu.VMEM((H, M, S // H), F32),
            pltpu.VMEM((8, 2 * M), F32),
            pltpu.VMEM((10, 8, PP), F32),
            pltpu.VMEM((2, M, LANE), F32),
        ] + [pltpu.VMEM((M,), BF16)] * 5 + [
            pltpu.VMEM((7, H, S // 4, D // 2), U32),
            pltpu.VMEM((2, M, TO), F32),
            pltpu.SMEM((1,), jnp.int32),
            pltpu.SemaphoreType.DMA((3, 2)),
            pltpu.SemaphoreType.DMA((S // TU,)),
            pltpu.SemaphoreType.DMA((6,)),
            pltpu.SemaphoreType.DMA((5,)),
            pltpu.SemaphoreType.DMA((H,)),
            pltpu.SemaphoreType.DMA((2,)),
        ],
        compiler_params=pltpu.CompilerParams(
            vmem_limit_bytes=120 * 1024 * 1024,
        ),
    )(
        jnp.swapaxes(A_x, 1, 2).reshape(M, S), A_c_kv.reshape(S, C),
        A_w_q, A_w_uk, A_w_uv, jnp.swapaxes(A_w_o, 1, 2),
        B_B_re, B_B_im, B_C_re, B_C_im,
        B_Lambda_re, B_Lambda_im, B_log_dt, B_Dskip, gate_w,
    )
    return jnp.swapaxes(out_t.reshape(1, M, S), 1, 2)
```

```python
import functools

import jax
import jax.numpy as jnp
import jax.experimental.pallas as pl
import jax.experimental.pallas.tpu as pltpu

F32 = jnp.float32
BF16 = jnp.bfloat16
U32 = jnp.uint32

NT_DIMS = (((1,), (1,)), ((), ()))
LOG2E = 1.4426950408889634

TQ = 128
TP = 256
TU = 512
TO = 256
LANE = 128
HALF = LANE // 2
SSM_SPLIT = False
REMAT = False
UNIFORM_DIAG = False
SCHEDULE = ("c0 c1 s0 s1 c2 p0 s2 s3 c3 p1 s4 s5 c4 p2 s6 s7 "
            "c5 p3 s8 s9 c6 p4 s10 s11 c7 p5 s12 s13 s14 s15 p6 p7")
Q_SCHEDULE = "q0 g0 q1 m0 q2 m1 q3 m2 q4 m3 q5 c5 q6 w6 q7"
PACE_FROM = 4
PACE_ROWS = 8
TWO_PASS = False
CHAIN_ALL = False
CHAIN = True
PACE2_FROM = 2
PACE2_EXTRA = 1


def _dot_nt(a, b):
    return jax.lax.dot_general(a, b, NT_DIMS, preferred_element_type=F32)


def _unpack(w32, shift):
    v = (w32 << shift) & jnp.uint32(0xFFFF0000)
    return pltpu.bitcast(v, F32)


def _as_bf16(w32):
    return pltpu.bitcast(w32, BF16)


def _as_u32(v):
    return pltpu.bitcast(v, U32)


def _strassen_lhs(a11, a12, a21, a22):
    return [a11 + a22, a21 + a22, a11, a22, a11 + a12, a21 - a11, a12 - a22]


def _strassen_rhs(b11, b12, b21, b22):
    return [b11 + b22, b11, b12 - b22, b21 - b11, b22, b11 + b12, b21 + b22]


def _strassen_out(m):
    return ((m[0] + m[3]) + (m[6] - m[4]), m[2] + m[4],
            m[1] + m[3], (m[0] - m[1]) + (m[2] + m[5]))


SUMS = (0, 1, 4, 5, 6)
ORDER = (1, 4, 2, 3, 0, 5, 6)
PV_ORDER = (2, 4, 3, 1, 5, 0, 6)


def _kernel(xt_hbm, c_hbm, wq_hbm, wuk_hbm, wuv_hbm, wot_hbm,
            bre_hbm, bim_hbm, cre_hbm, cim_hbm,
            lre_hbm, lim_hbm, ldt_hbm, dsk_hbm, gw_hbm,
            o_hbm,
            xt_ref, x_ref, c_ref, l_ref, wq_buf, wk_buf, wv_buf, wot_ref, lo_ref,
            b_ref, cre_ref, cim_ref, cmid_ref, u_ref, ys_ref, g_ref, st_ref, co_ref, col_ref,
            lre_ref, lim_ref, ldt_ref, dsk_ref, gw_ref,
            q_ref, ctx_ref, o_buf, zero_ref, wsem, xsem, msem, vsem, osem,
            *, S, M, H, D):
    P = M
    FT = P // LANE
    PF = FT * LANE
    assert P - PF == HALF
    PP = PF + LANE
    NP = H // 2
    TS = S // NP
    CH, DH, MH, TH = c_ref.shape[1] // 2, D // 2, M // 2, TP // 2

    def w_copy(k, pair):
        src, dst = ((wq_hbm, wq_buf), (wuk_hbm, wk_buf), (wuv_hbm, wv_buf))[k]
        return pltpu.make_async_copy(src.bitcast(U32).at[:, pair, :], dst.at[pair], wsem.at[k, pair])

    def wo_copy(pair):
        heads = pl.ds(2 * pair, 2)
        return pltpu.make_async_copy(wot_hbm.bitcast(U32).at[heads], wot_ref.at[heads],
                                     wsem.at[3, pair])

    def x_copy(j):
        cols = pl.ds(j * TU, TU)
        return pltpu.make_async_copy(xt_hbm.at[:, cols], xt_ref.at[:, cols], xsem.at[j])

    bre32, bim32 = bre_hbm.bitcast(U32), bim_hbm.bitcast(U32)
    b_cps = [
        pltpu.make_async_copy(bre32, b_ref.at[pl.ds(0, P // 2), :], msem.at[0]),
        pltpu.make_async_copy(bim32.at[pl.ds(PF // 2, HALF // 2), :],
                              b_ref.at[pl.ds(P // 2, HALF // 2), :], msem.at[1]),
        pltpu.make_async_copy(bim32.at[pl.ds(0, PF // 2), :],
                              b_ref.at[pl.ds(PP // 2, PF // 2), :], msem.at[2]),
    ]
    c_cp = pltpu.make_async_copy(c_hbm.bitcast(U32), c_ref, msem.at[3])
    cre_cp = pltpu.make_async_copy(cre_hbm.bitcast(U32), cre_ref, msem.at[4])
    cim_cp = pltpu.make_async_copy(cim_hbm.bitcast(U32), cim_ref, msem.at[5])

    v_cps = [pltpu.make_async_copy(src, dst, vsem.at[k]) for k, (src, dst) in enumerate(
        ((lre_hbm, lre_ref), (lim_hbm, lim_ref), (ldt_hbm, ldt_ref),
         (dsk_hbm, dsk_ref), (gw_hbm, gw_ref)))]

    for cp in v_cps:
        cp.start()
    x_copy(0).start()
    for cp in b_cps:
        cp.start()
    for j in range(1, S // TU):
        x_copy(j).start()
    w_copy(0, 0).start()
    wo_copy(0).start()
    cre_cp.start()
    cim_cp.start()
    c_cp.start()
    for p in range(1, NP):
        w_copy(0, p).start()
        wo_copy(p).start()
    for p in range(NP):
        w_copy(1, p).start()
        w_copy(2, p).start()

    zero_ref[0] = 0
    u_ref[pl.ds(0, 8), :] = jnp.zeros((8, u_ref.shape[1]), F32)
    st_ref[...] = jnp.zeros(st_ref.shape, F32)
    for cp in v_cps:
        cp.wait()

    row = lambda r: r[...].astype(F32).reshape(1, P)
    lre, lim = row(lre_ref), row(lim_ref)
    dt = jnp.exp(row(ldt_ref)).astype(BF16).astype(F32)
    e = jnp.exp(dt * lre)
    ang = dt * lim
    ar = e * jnp.cos(ang)
    ai = e * jnp.sin(ang)
    sc = jnp.maximum(jnp.abs(lre), jnp.abs(lim))
    nre, nim = lre / sc, lim / sc
    den = (nre * nre + nim * nim) * sc
    gr = 2.0 * ((ar - 1.0) * nre + ai * nim) / den
    gi = 2.0 * (ai * nre - (ar - 1.0) * nim) / den

    def put(k, full, lo, hi):
        v = jnp.concatenate([full[:, :PF], lo[:, PF:], hi[:, PF:]], axis=1)
        co_ref[k] = jnp.broadcast_to(v, (8, PP))

    put(0, gr, gr, -gr)
    put(1, -gi, -gi, -gi)
    pr, pi = ar, -ai
    for j in range(1, 5):
        put(2 * j, pr, pr, pr)
        put(2 * j + 1, -pi, -pi, pi)
        pr, pi = pr * pr - pi * pi, 2.0 * pr * pi

    zpad = jnp.zeros((1, PP - P), F32)
    for k, r in enumerate((dsk_ref, gw_ref)):
        v = jnp.concatenate([row(r), zpad], axis=1)
        col_ref[k] = jnp.broadcast_to(v, (LANE, PP)).T[:M]

    for cp in b_cps:
        cp.wait()

    def u_step(j, _):
        x_copy(j).wait()
        t0 = pl.multiple_of(j * TU, TU)
        xc = xt_ref[:, pl.ds(t0, TU)].T
        x_ref[pl.ds(pl.multiple_of(j * (TU // 2), TU // 2), TU // 2), :] = _as_u32(xc)
        u_ref[pl.ds(t0 + 8, TU), :] = _dot_nt(xc, _as_bf16(b_ref[...]))
        return 0

    jax.lax.fori_loop(0, S // TU, u_step, 0)
    cre_cp.wait()
    cim_cp.wait()
    cmid_ref[...] = jnp.concatenate([cre_ref[:, PF:], cim_ref[:, PF:]], axis=1)
    c_cp.wait()

    def q_step(j, _):
        w_copy(0, j).wait()
        wo_copy(j).wait()
        zero = zero_ref[0]
        after = lambda w, v: w | (_as_u32(v) & zero.astype(U32))
        t0 = pl.multiple_of(j * TS, TS)

        ys, last, gates = [], [], []

        def ssm_tile(t):
            rows = pl.ds(t0, TS + 8)
            cr, ci = pl.ds(t * LANE, LANE), pl.ds(PP + t * LANE, LANE)
            co = [co_ref[k, :, cr] for k in range(10)]
            u0 = u_ref[rows, cr]
            u1 = u_ref[rows, ci] if t < FT else pltpu.roll(u0, HALF, 1)
            mul = lambda k, x: (co[k] * x[0] + co[k + 1] * x[1], co[k] * x[1] - co[k + 1] * x[0])
            sub = jax.lax.broadcasted_iota(jnp.int32, (8, LANE), 0)
            s = (st_ref[0, :, cr], st_ref[1, :, cr])
            prev, gs = [None] * 3, []
            for k in range(TS // 8 + 1):
                x0, x1 = u0[8 * k:8 * k + 8], u1[8 * k:8 * k + 8]
                if last:
                    x0 = pltpu.bitcast(after(_as_u32(x0), last[0]), F32)
                w = (co[0] * x0 + co[1] * x1, co[1] * x0 - co[0] * x1)
                for i in range(3):
                    cur = [pltpu.roll(v, 1 << i, 0) for v in w]
                    old = cur if k == 0 else prev[i]
                    d = mul(2 * i + 2, [jnp.where(sub < (1 << i), o, c) for o, c in zip(old, cur)])
                    w = [p + q for p, q in zip(d, w)]
                    prev[i] = cur
                if k > 0:
                    s = [p + q for p, q in zip(mul(8, s), w)]
                    gs.append(jnp.concatenate(s, axis=1) if t < FT else s[0])
                    last[:] = [s[0]]
            st_ref[0, :, cr] = s[0]
            st_ref[1, :, cr] = s[1]
            if t < FT:
                cc = jnp.concatenate([cre_ref[:, cr], cim_ref[:, cr]], axis=1)
            else:
                cc = cmid_ref[...]
            g = jnp.concatenate(gs, axis=0).astype(BF16)
            n = M // 2 if t < FT else M // 4
            y = jnp.concatenate([
                jax.lax.dot_general(_as_bf16(cc[a:a + n]), g, NT_DIMS, preferred_element_type=F32)
                for a in range(0, M // 2, n)], axis=0)
            ys[:] = [y + ys[0] if ys else y]
            if t == FT:
                dcol = jnp.concatenate([col_ref[0]] * (TS // LANE), axis=1)
                xt = xt_ref[:, pl.ds(t0, TS)].astype(F32)
                omg = (1.0 - gates[0]).astype(BF16).astype(F32)
                ys_ref[j] = omg * (ys[0] + (xt * dcol).astype(BF16).astype(F32))

        def gate(r):
            q = qs[r]
            gcol = after(_as_u32(col_ref[1]), jnp.concatenate([q[:, :LANE], q[:M - TP, LANE:2 * LANE]], axis=0))
            gcol = jnp.concatenate([pltpu.bitcast(gcol, F32)] * (TS // LANE), axis=1)
            xt = xt_ref[:, pl.ds(t0, TS)].astype(F32)
            z = jnp.sum((xt * gcol).astype(BF16).astype(F32), axis=0, keepdims=True)
            g = jax.nn.sigmoid(z.astype(BF16).astype(F32)).astype(BF16).astype(F32)
            g_ref[j] = jnp.broadcast_to(g, (8, TS))
            gates.append(g)

        wq32 = wq_buf[j]
        wq = jnp.concatenate([pltpu.bitcast(wq32 << 16, F32),
                              pltpu.bitcast(wq32 & jnp.uint32(0xFFFF0000), F32)], axis=1).astype(BF16)
        qscale = (D ** -0.5) * LOG2E
        qs = {}

        def proj_q(r):
            rows = pl.ds(r * TP // 2, TP // 2)
            q = jnp.dot(_as_bf16(x_ref[rows, :]), wq, preferred_element_type=F32) * qscale
            qs[r] = q
            for e in range(2):
                q_ref[2 * j + e, rows, :] = _as_u32(q[:, e * D:(e + 1) * D].astype(BF16))

        def c_sums(r):
            c = c_ref[pl.ds(pl.multiple_of(j * TH, TH), TH), :]
            q = qs[r]
            c = after(c, jnp.concatenate([q[:TH], q[TH:]], axis=1))
            c = _as_bf16(c).astype(F32)
            ls = _strassen_lhs(c[:TH, :CH], c[:TH, CH:], c[TH:, :CH], c[TH:, CH:])
            for n, k in enumerate(SUMS):
                l_ref[n, pl.ds(pl.multiple_of(j * (TH // 2), TH // 2), TH // 2), :] = (
                    _as_u32(ls[k].astype(BF16)))

        def wo_sums(r):
            for e in range(2):
                w = after(wot_ref[2 * j + e], qs[r][:MH, e * D:(e + 1) * D])
                w = _as_bf16(w).astype(F32)
                ls = _strassen_lhs(w[:MH, :DH], w[:MH, DH:], w[MH:, :DH], w[MH:, DH:])
                lo_ref[2 * j + e] = jnp.concatenate([ls[k] for k in SUMS], axis=1).astype(BF16)

        ops = dict(q=proj_q, m=ssm_tile, c=c_sums, w=wo_sums, g=gate)
        for op in Q_SCHEDULE.split():
            ops[op[0]](int(op[1:]))
        return 0

    assert S // TP == NP
    jax.lax.fori_loop(0, NP, q_step, 0)
    for p in range(NP):
        w_copy(1, p).wait()
        w_copy(2, p).wait()

    def head_step(h, _):
        slot = h >> 1
        zero = zero_ref[0]
        shift = (16 - 16 * (h & 1)).astype(U32)
        rw = []
        for k in range(7):
            sh = shift + (zero << k).astype(U32) if REMAT else shift
            wk, wv = _unpack(wk_buf[slot], sh), _unpack(wv_buf[slot], sh)
            wl = jnp.concatenate([wk[:, :DH], wv[:, :DH]], axis=1)
            wr = jnp.concatenate([wk[:, DH:], wv[:, DH:]], axis=1)
            rw.append(_strassen_rhs(wl[:CH], wr[:CH], wl[CH:], wr[CH:])[k])
        causal = (jax.lax.broadcasted_iota(jnp.int32, (TQ, TQ), 1)
                  <= jax.lax.broadcasted_iota(jnp.int32, (TQ, TQ), 0))

        ks, vs, rvs, ss, chains = [], [], [], {}, [None]

        def proj_c(r, cols):
            ms = [None] * 7
            for k in ORDER:
                if k in SUMS:
                    a = l_ref[SUMS.index(k), pl.ds(r * TH // 2, TH // 2), :]
                elif k == 2:
                    a = c_ref[pl.ds(r * TH, TH // 2), pl.ds(0, CH)]
                else:
                    a = c_ref[pl.ds(r * TH + TH // 2, TH // 2), pl.ds(CH, CH)]
                ms[k] = jnp.dot(_as_bf16(a), rw[k][:, cols].astype(BF16), preferred_element_type=F32)
            return _strassen_out(ms)

        def proj_k(r, c=None):
            c11, c12, c21, c22 = c or proj_c(r, slice(0, DH))
            ks.extend([jnp.concatenate([c11, c12], axis=1), jnp.concatenate([c21, c22], axis=1)])

        def proj_v(r, c=None):
            c11, c12, c21, c22 = c or proj_c(r, slice(DH, D))
            vs.extend([jnp.concatenate([c11, c12], axis=1), jnp.concatenate([c21, c22], axis=1)])
            rvs.append(_strassen_rhs(c11, c12, c21, c22))

        def proj_kv(r):
            c = proj_c(r, slice(0, D))
            proj_k(r, [v[:, :DH] for v in c])
            proj_v(r, [v[:, DH:] for v in c])

        def qk(i):
            lo, hi = i * TQ, (i + 1) * TQ
            q = _as_bf16(q_ref[h, lo // 2:hi // 2, :])
            k = jnp.concatenate(ks, axis=0)[:hi].astype(BF16)
            ss[i] = jax.lax.dot_general(q, k, NT_DIMS, preferred_element_type=F32)

        def tie(a, b):
            return pltpu.bitcast(_as_u32(a) | (_as_u32(b) & zero.astype(U32)), F32)

        def exp_rows(s, m, pace, rows, chain=None):
            mb = jnp.broadcast_to(m, (TQ, LANE))
            ps, parts = [], []
            for g in range(0, TQ, rows):
                mg = mb[g:g + rows]
                if pace and (parts or chain is not None):
                    mg = tie(mg, parts[-1] if parts else chain)
                pg = [jnp.exp2(s[g:g + rows, t * LANE:(t + 1) * LANE] - mg)
                      for t in range(s.shape[1] // LANE)]
                ps.append(jnp.concatenate(pg, axis=1))
                parts.append(functools.reduce(lambda a, b: a + b, pg))
            return jnp.concatenate(ps, axis=0), jnp.concatenate(parts, axis=0)

        def scores(i, chain=None):
            lo = i * TQ
            s = ss.pop(i)
            sd = jnp.where(causal, s[:, lo:], -1e9 * LOG2E)
            s = sd if i == 0 else jnp.concatenate([s[:, :lo], sd], axis=1)
            m = jnp.max(s, axis=-1, keepdims=True)
            p, part = exp_rows(s, m, i >= PACE_FROM, PACE_ROWS, chain)
            return s, m, p, jnp.sum(part, axis=-1, keepdims=True), part[TQ - PACE_ROWS:]

        def pv(j):
            s1, m1, p1, l1, chain = scores(2 * j, chains[0] if CHAIN_ALL else None)
            s2, m2, p2, l2, chains[0] = scores(2 * j + 1, chain if CHAIN else None)
            lo = 2 * j * TQ
            cat = lambda xs, axis: jnp.concatenate(xs, axis=axis)
            dot = lambda a, b: jnp.dot(a.astype(BF16), b.astype(BF16), preferred_element_type=F32)

            def recip(l):
                rl = pl.reciprocal(l, approx=True)
                return rl * (2.0 - l * rl)

            r1, r2 = recip(l1), recip(l2)
            if UNIFORM_DIAG:
                c1 = dot(p1[:, lo:], vs[2 * j])
                c2 = dot(p2[:, lo:], cat(vs[2 * j:2 * j + 2], 0))
            else:
                dg = dot(cat([p1[:, lo:], p2[:, lo:lo + TQ]], 0), vs[2 * j])
                c1, c2 = dg[:TQ], dg[TQ:] + dot(p2[:, lo + TQ:], vs[2 * j + 1])
            if j > 0:
                tiles = lambda p, o: cat([p[:, (2 * t + o) * TQ:(2 * t + o + 1) * TQ] for t in range(j)], 1)
                a11, a12, a21, a22 = tiles(p1, 0), tiles(p1, 1), tiles(p2, 0), tiles(p2, 1)
                rho = l1 * r2
                a22r = a22 * rho
                lp = [a11 + a22r, a21 + a22, a11, a22, a11 + a12, a21 * rho - a11, a12 - a22r]
                m = [None] * 7
                for k in PV_ORDER:
                    m[k] = dot(lp[k], cat([rvs[t][k] for t in range(j)], 0))
                c1 = c1 + cat([(m[0] - m[4]) + (m[6] + m[3] * rho), m[2] + m[4]], 1)
                c2 = (c2 + cat([m[1] + m[3], -m[1]], 1)) * r2
                c2 = cat([c2[:, :DH], c2[:, DH:] + ((m[0] + m[2]) + m[5]) * r1], 1)
            else:
                c2 = c2 * r2
            c1 = c1 * r1
            ctx_ref[h, j * TQ:(j + 1) * TQ, :] = cat(
                _strassen_rhs(c1[:, :DH], c2[:, :DH], c1[:, DH:], c2[:, DH:]), 1).astype(BF16)

        assert TP == 2 * TQ
        ops = dict(c=proj_kv, k=proj_k, v=proj_v, s=qk, p=pv)
        for op in SCHEDULE.split():
            ops[op[0]](int(op[1:]))
        return 0

    jax.lax.fori_loop(0, H, head_step, 0)

    def o_copy(j, slot):
        return pltpu.make_async_copy(o_buf.at[slot], o_hbm.at[:, pl.ds(j * TO, TO)], osem.at[slot])

    def o_step(j, _):
        slot = j & 1

        @pl.when(j >= 2)
        def _():
            o_copy(j - 2, slot).wait()

        rows = pl.ds(pl.multiple_of(j * TQ, TQ), TQ)
        ms = [None] * 7
        for k in range(7):
            if k in SUMS:
                a = [lo_ref[n, :, pl.ds(SUMS.index(k) * DH, DH)] for n in range(H)]
            elif k == 2:
                a = [_as_bf16(wot_ref[n, pl.ds(0, MH // 2), pl.ds(0, DH)]) for n in range(H)]
            else:
                a = [_as_bf16(wot_ref[n, pl.ds(MH // 2, MH // 2), pl.ds(DH, DH)]) for n in range(H)]
            b = [ctx_ref[n, rows, pl.ds(k * DH, DH)] for n in range(H)]
            ms[k] = _dot_nt(jnp.concatenate(a, axis=1), jnp.concatenate(b, axis=1))
        c11, c12, c21, c22 = _strassen_out(ms)
        at = jnp.concatenate([jnp.concatenate([c11, c12], axis=1),
                              jnp.concatenate([c21, c22], axis=1)], axis=0)
        o_buf[slot] = g_ref[j, 0:1, :] * at + ys_ref[j]
        o_copy(j, slot).start()
        return 0

    assert TO == 2 * TQ and TO == TS
    no = S // TO
    jax.lax.fori_loop(0, no, o_step, 0)
    o_copy(no - 2, no % 2).wait()
    o_copy(no - 1, (no - 1) % 2).wait()


@jax.jit
def pallas_gated_mix__compressed_kv_cla__ssm_conv_s5__prompt_kernel(
    A_x: jax.Array,
    A_c_kv: jax.Array,
    A_w_q: jax.Array,
    A_w_uk: jax.Array,
    A_w_uv: jax.Array,
    A_w_o: jax.Array,
    B_x: jax.Array,
    B_Lambda_re: jax.Array,
    B_Lambda_im: jax.Array,
    B_B_re: jax.Array,
    B_B_im: jax.Array,
    B_C_re: jax.Array,
    B_C_im: jax.Array,
    B_log_dt: jax.Array,
    B_Dskip: jax.Array,
    gate_w: jax.Array,
):
    del B_x
    _, S, M = A_x.shape
    C = A_c_kv.shape[2]
    H, D = A_w_q.shape[1], A_w_q.shape[2]
    PP = (M + LANE - 1) // LANE * LANE

    hbm = pl.BlockSpec(memory_space=pl.ANY)
    out_t = pl.pallas_call(
        functools.partial(_kernel, S=S, M=M, H=H, D=D),
        in_specs=[hbm] * 15,
        out_specs=hbm,
        out_shape=jax.ShapeDtypeStruct((M, S), F32),
        scratch_shapes=[
            pltpu.VMEM((M, S), BF16),
            pltpu.VMEM((S // 2, M), U32),
            pltpu.VMEM((S // 2, C), U32),
            pltpu.VMEM((5, S // 4, C // 2), U32),
            pltpu.VMEM((H // 2, M, D), U32),
            pltpu.VMEM((H // 2, C, D), U32),
            pltpu.VMEM((H // 2, C, D), U32),
            pltpu.VMEM((H, M // 2, D), U32),
            pltpu.VMEM((H, M // 2, 5 * D // 2), BF16),
            pltpu.VMEM((M, M), U32),
            pltpu.VMEM((M // 2, M), U32),
            pltpu.VMEM((M // 2, M), U32),
            pltpu.VMEM((M // 2, LANE), U32),
            pltpu.VMEM((S + 8, 2 * M), F32),
            pltpu.VMEM((S // TO, M, TO), F32),
            pltpu.VMEM((S // TO, 8, TO), F32),
            pltpu.VMEM((2, 8, PP), F32),
            pltpu.VMEM((10, 8, PP), F32),
            pltpu.VMEM((2, M, LANE), F32),
        ] + [pltpu.VMEM((M,), BF16)] * 5 + [
            pltpu.VMEM((H, S // 2, D), U32),
            pltpu.VMEM((H, S // 2, 7 * D // 2), BF16),
            pltpu.VMEM((2, M, TO), F32),
            pltpu.SMEM((1,), jnp.int32),
            pltpu.SemaphoreType.DMA((4, H // 2)),
            pltpu.SemaphoreType.DMA((S // TU,)),
            pltpu.SemaphoreType.DMA((6,)),
            pltpu.SemaphoreType.DMA((5,)),
            pltpu.SemaphoreType.DMA((2,)),
        ],
        compiler_params=pltpu.CompilerParams(
            vmem_limit_bytes=124 * 1024 * 1024,
        ),
    )(
        jnp.swapaxes(A_x, 1, 2).reshape(M, S), A_c_kv.reshape(S, C),
        A_w_q, A_w_uk, A_w_uv, jnp.swapaxes(A_w_o, 1, 2),
        B_B_re, B_B_im, B_C_re, B_C_im,
        B_Lambda_re, B_Lambda_im, B_log_dt, B_Dskip, gate_w,
    )
    return jnp.swapaxes(out_t.reshape(1, M, S), 1, 2)
```

```python
import functools

import jax
import jax.numpy as jnp
import jax.experimental.pallas as pl
import jax.experimental.pallas.tpu as pltpu

F32 = jnp.float32
BF16 = jnp.bfloat16
U32 = jnp.uint32

NT_DIMS = (((1,), (1,)), ((), ()))
LOG2E = 1.4426950408889634

TQ = 128
TP = 256
TU = 512
TO = 256
LANE = 128
HALF = LANE // 2
SSM_SPLIT = False
REMAT = (1,)
UNIFORM_DIAG = False
SCHEDULE = ("c0 c1 s0 s1 c2 p0 s2 s3 c3 p1 s4 s5 c4 p2 s6 s7 "
            "c5 p3 s8 s9 c6 p4 s10 s11 c7 b5 s12 s13 s14 s15 p5 p6 p7")
Q_SCHEDULE = "q0 g0 q1 m0 q2 m1 q3 m2 q4 m3 q5 c5 q6 w6 q7"
PACE_FROM = 4
PACE_ROWS = 8
TWO_PASS = False
CHAIN_ALL = False
CHAIN = True
PACE2_FROM = 2
PACE2_EXTRA = 1


def _dot_nt(a, b):
    return jax.lax.dot_general(a, b, NT_DIMS, preferred_element_type=F32)


def _unpack(w32, shift):
    v = (w32 << shift) & jnp.uint32(0xFFFF0000)
    return pltpu.bitcast(v, F32)


def _as_bf16(w32):
    return pltpu.bitcast(w32, BF16)


def _as_u32(v):
    return pltpu.bitcast(v, U32)


def _strassen_lhs(a11, a12, a21, a22):
    return [a11 + a22, a21 + a22, a11, a22, a11 + a12, a21 - a11, a12 - a22]


def _strassen_rhs(b11, b12, b21, b22):
    return [b11 + b22, b11, b12 - b22, b21 - b11, b22, b11 + b12, b21 + b22]


def _strassen_out(m):
    return ((m[0] + m[3]) + (m[6] - m[4]), m[2] + m[4],
            m[1] + m[3], (m[0] - m[1]) + (m[2] + m[5]))


SUMS = (0, 1, 4, 5, 6)
ORDER = (1, 4, 0, 2, 3, 5, 6)
PV_ORDER = (2, 4, 3, 1, 5, 0, 6)


def _kernel(xt_hbm, c_hbm, wq_hbm, wuk_hbm, wuv_hbm, wot_hbm,
            bre_hbm, bim_hbm, cre_hbm, cim_hbm,
            lre_hbm, lim_hbm, ldt_hbm, dsk_hbm, gw_hbm,
            o_hbm,
            xt_ref, x_ref, c_ref, l_ref, wq_buf, wk_buf, wv_buf, wot_ref, lo_ref,
            b_ref, cre_ref, cim_ref, cmid_ref, u_ref, ys_ref, g_ref, st_ref, co_ref, col_ref,
            lre_ref, lim_ref, ldt_ref, dsk_ref, gw_ref,
            q_ref, ctx_ref, o_buf, zero_ref, wsem, xsem, msem, vsem, osem,
            *, S, M, H, D):
    P = M
    FT = P // LANE
    PF = FT * LANE
    assert P - PF == HALF
    PP = PF + LANE
    NP = H // 2
    TS = S // NP
    CH, DH, MH, TH = c_ref.shape[1] // 2, D // 2, M // 2, TP // 2

    def w_copy(k, pair):
        src, dst = ((wq_hbm, wq_buf), (wuk_hbm, wk_buf), (wuv_hbm, wv_buf))[k]
        return pltpu.make_async_copy(src.bitcast(U32).at[:, pair, :], dst.at[pair], wsem.at[k, pair])

    def wo_copy(pair):
        heads = pl.ds(2 * pair, 2)
        return pltpu.make_async_copy(wot_hbm.bitcast(U32).at[heads], wot_ref.at[heads],
                                     wsem.at[3, pair])

    def x_copy(t0, n, k):
        cols = pl.ds(t0, n)
        return pltpu.make_async_copy(xt_hbm.at[:, cols], xt_ref.at[:, cols], xsem.at[k])

    x_cps = [x_copy(0, TU // 2, 0), x_copy(TU // 2, TU // 2, 1), x_copy(TU, TU, 2),
             x_copy(2 * TU, S - 2 * TU, 3)]

    bre32, bim32 = bre_hbm.bitcast(U32), bim_hbm.bitcast(U32)
    b_cps = [
        pltpu.make_async_copy(bre32, b_ref.at[pl.ds(0, P // 2), :], msem.at[0]),
        pltpu.make_async_copy(bim32.at[pl.ds(PF // 2, HALF // 2), :],
                              b_ref.at[pl.ds(P // 2, HALF // 2), :], msem.at[1]),
        pltpu.make_async_copy(bim32.at[pl.ds(0, PF // 2), :],
                              b_ref.at[pl.ds(PP // 2, PF // 2), :], msem.at[2]),
    ]
    c_cp = pltpu.make_async_copy(c_hbm.bitcast(U32), c_ref, msem.at[3])
    cre_cp = pltpu.make_async_copy(cre_hbm.bitcast(U32), cre_ref, msem.at[4])
    cim_cp = pltpu.make_async_copy(cim_hbm.bitcast(U32), cim_ref, msem.at[5])

    v_cps = [pltpu.make_async_copy(src, dst, vsem.at[k]) for k, (src, dst) in enumerate(
        ((lre_hbm, lre_ref), (lim_hbm, lim_ref), (ldt_hbm, ldt_ref),
         (dsk_hbm, dsk_ref), (gw_hbm, gw_ref)))]

    for cp in v_cps:
        cp.start()
    for cp in x_cps[:1] + b_cps + x_cps[1:]:
        cp.start()
    w_copy(0, 0).start()
    wo_copy(0).start()
    cre_cp.start()
    cim_cp.start()
    c_cp.start()
    for p in range(1, NP):
        w_copy(0, p).start()
        wo_copy(p).start()
    for p in range(NP):
        w_copy(1, p).start()
        w_copy(2, p).start()

    zero_ref[0] = 0
    u_ref[pl.ds(0, 8), :] = jnp.zeros((8, u_ref.shape[1]), F32)
    st_ref[...] = jnp.zeros(st_ref.shape, F32)
    for cp in v_cps:
        cp.wait()

    row = lambda r: r[...].astype(F32).reshape(1, P)
    lre, lim = row(lre_ref), row(lim_ref)
    dt = jnp.exp(row(ldt_ref)).astype(BF16).astype(F32)
    e = jnp.exp(dt * lre)
    ang = dt * lim
    ar = e * jnp.cos(ang)
    ai = e * jnp.sin(ang)
    sc = jnp.maximum(jnp.abs(lre), jnp.abs(lim))
    nre, nim = lre / sc, lim / sc
    den = (nre * nre + nim * nim) * sc
    gr = 2.0 * ((ar - 1.0) * nre + ai * nim) / den
    gi = 2.0 * (ai * nre - (ar - 1.0) * nim) / den

    def put(k, full, lo, hi):
        v = jnp.concatenate([full[:, :PF], lo[:, PF:], hi[:, PF:]], axis=1)
        co_ref[k] = jnp.broadcast_to(v, (8, PP))

    put(0, gr, gr, -gr)
    put(1, -gi, -gi, -gi)
    pr, pi = ar, -ai
    for j in range(1, 5):
        put(2 * j, pr, pr, pr)
        put(2 * j + 1, -pi, -pi, pi)
        pr, pi = pr * pr - pi * pi, 2.0 * pr * pi

    zpad = jnp.zeros((1, PP - P), F32)
    for k, r in enumerate((dsk_ref, gw_ref)):
        v = jnp.concatenate([row(r), zpad], axis=1)
        col_ref[k] = jnp.broadcast_to(v, (LANE, PP)).T[:M]

    def transpose_x(t0, n):
        x_ref[pl.ds(t0 // 2, n // 2), :] = _as_u32(xt_ref[:, pl.ds(t0, n)].T)

    def proj_u(t0, n, lo=0, hi=2 * P):
        u = _dot_nt(_as_bf16(x_ref[pl.ds(t0 // 2, n // 2), :]), _as_bf16(b_ref[lo // 2:hi // 2, :]))
        u_ref[pl.ds(t0 + 8, n), lo:hi] = u

    x_cps[0].wait()
    transpose_x(0, TU // 2)
    b_cps[0].wait()
    b_cps[1].wait()
    proj_u(0, TU // 2, 0, PP)
    b_cps[2].wait()
    x_cps[1].wait()
    proj_u(0, TU // 2, PP)
    transpose_x(TU // 2, TU // 2)
    x_cps[2].wait()
    proj_u(TU // 2, TU // 2)
    transpose_x(TU, TU)
    x_cps[3].wait()
    for t0 in range(TU, S, TU):
        proj_u(t0, TU)
        if t0 + TU < S:
            transpose_x(t0 + TU, TU)
    cre_cp.wait()
    cim_cp.wait()
    cmid_ref[...] = jnp.concatenate([cre_ref[:, PF:], cim_ref[:, PF:]], axis=1)
    c_cp.wait()

    def q_step(j, _):
        w_copy(0, j).wait()
        wo_copy(j).wait()
        zero = zero_ref[0]
        after = lambda w, v: w | (_as_u32(v) & zero.astype(U32))
        t0 = pl.multiple_of(j * TS, TS)

        ys, last, gates = [], [], []

        def ssm_tile(t):
            rows = pl.ds(t0, TS + 8)
            cr, ci = pl.ds(t * LANE, LANE), pl.ds(PP + t * LANE, LANE)
            co = [co_ref[k, :, cr] for k in range(10)]
            u0 = u_ref[rows, cr]
            u1 = u_ref[rows, ci] if t < FT else pltpu.roll(u0, HALF, 1)
            mul = lambda k, x: (co[k] * x[0] + co[k + 1] * x[1], co[k] * x[1] - co[k + 1] * x[0])
            sub = jax.lax.broadcasted_iota(jnp.int32, (8, LANE), 0)
            s = (st_ref[0, :, cr], st_ref[1, :, cr])
            prev, gs = [None] * 3, []
            for k in range(TS // 8 + 1):
                x0, x1 = u0[8 * k:8 * k + 8], u1[8 * k:8 * k + 8]
                if last:
                    x0 = pltpu.bitcast(after(_as_u32(x0), last[0]), F32)
                w = (co[0] * x0 + co[1] * x1, co[1] * x0 - co[0] * x1)
                for i in range(3):
                    cur = [pltpu.roll(v, 1 << i, 0) for v in w]
                    old = cur if k == 0 else prev[i]
                    d = mul(2 * i + 2, [jnp.where(sub < (1 << i), o, c) for o, c in zip(old, cur)])
                    w = [p + q for p, q in zip(d, w)]
                    prev[i] = cur
                if k > 0:
                    s = [p + q for p, q in zip(mul(8, s), w)]
                    gs.append(jnp.concatenate(s, axis=1) if t < FT else s[0])
                    last[:] = [s[0]]
            st_ref[0, :, cr] = s[0]
            st_ref[1, :, cr] = s[1]
            if t < FT:
                cc = jnp.concatenate([cre_ref[:, cr], cim_ref[:, cr]], axis=1)
            else:
                cc = cmid_ref[...]
            g = jnp.concatenate(gs, axis=0).astype(BF16)
            n = M // 2 if t < FT else M // 4
            y = jnp.concatenate([
                jax.lax.dot_general(_as_bf16(cc[a:a + n]), g, NT_DIMS, preferred_element_type=F32)
                for a in range(0, M // 2, n)], axis=0)
            ys[:] = [y + ys[0] if ys else y]
            if t == FT:
                dcol = jnp.concatenate([col_ref[0]] * (TS // LANE), axis=1)
                xt = xt_ref[:, pl.ds(t0, TS)].astype(F32)
                omg = (1.0 - gates[0]).astype(BF16).astype(F32)
                ys_ref[j] = omg * (ys[0] + (xt * dcol).astype(BF16).astype(F32))

        def gate(r):
            q = qs[r]
            gcol = after(_as_u32(col_ref[1]), jnp.concatenate([q[:, :LANE], q[:M - TP, LANE:2 * LANE]], axis=0))
            gcol = jnp.concatenate([pltpu.bitcast(gcol, F32)] * (TS // LANE), axis=1)
            xt = xt_ref[:, pl.ds(t0, TS)].astype(F32)
            z = jnp.sum((xt * gcol).astype(BF16).astype(F32), axis=0, keepdims=True)
            g = jax.nn.sigmoid(z.astype(BF16).astype(F32)).astype(BF16).astype(F32)
            g_ref[j] = jnp.broadcast_to(g, (8, TS))
            gates.append(g)

        wq32 = wq_buf[j]
        wq = jnp.concatenate([pltpu.bitcast(wq32 << 16, F32),
                              pltpu.bitcast(wq32 & jnp.uint32(0xFFFF0000), F32)], axis=1).astype(BF16)
        qscale = (D ** -0.5) * LOG2E
        qs = {}

        def proj_q(r):
            rows = pl.ds(r * TP // 2, TP // 2)
            q = jnp.dot(_as_bf16(x_ref[rows, :]), wq, preferred_element_type=F32) * qscale
            qs[r] = q
            for e in range(2):
                q_ref[2 * j + e, rows, :] = _as_u32(q[:, e * D:(e + 1) * D].astype(BF16))

        def c_sums(r):
            c = c_ref[pl.ds(pl.multiple_of(j * TH, TH), TH), :]
            q = qs[r]
            c = after(c, jnp.concatenate([q[:TH], q[TH:]], axis=1))
            c = _as_bf16(c).astype(F32)
            ls = _strassen_lhs(c[:TH, :CH], c[:TH, CH:], c[TH:, :CH], c[TH:, CH:])
            for n, k in enumerate(SUMS):
                l_ref[n, pl.ds(pl.multiple_of(j * (TH // 2), TH // 2), TH // 2), :] = (
                    _as_u32(ls[k].astype(BF16)))

        def wo_sums(r):
            for e in range(2):
                w = after(wot_ref[2 * j + e], qs[r][:MH, e * D:(e + 1) * D])
                w = _as_bf16(w).astype(F32)
                ls = _strassen_lhs(w[:MH, :DH], w[:MH, DH:], w[MH:, :DH], w[MH:, DH:])
                lo_ref[2 * j + e] = jnp.concatenate([ls[k] for k in SUMS], axis=1).astype(BF16)

        ops = dict(q=proj_q, m=ssm_tile, c=c_sums, w=wo_sums, g=gate)
        for op in Q_SCHEDULE.split():
            ops[op[0]](int(op[1:]))
        return 0

    assert S // TP == NP
    jax.lax.fori_loop(0, NP, q_step, 0)
    for p in range(NP):
        w_copy(1, p).wait()
        w_copy(2, p).wait()

    def head_step(h, _):
        slot = h >> 1
        zero = zero_ref[0]
        shift = (16 - 16 * (h & 1)).astype(U32)
        rw = []
        for k in range(7):
            sh = shift + (zero << k).astype(U32) if k in REMAT else shift
            wk, wv = _unpack(wk_buf[slot], sh), _unpack(wv_buf[slot], sh)
            wl = jnp.concatenate([wk[:, :DH], wv[:, :DH]], axis=1)
            wr = jnp.concatenate([wk[:, DH:], wv[:, DH:]], axis=1)
            rw.append(_strassen_rhs(wl[:CH], wr[:CH], wl[CH:], wr[CH:])[k])
        causal = (jax.lax.broadcasted_iota(jnp.int32, (TQ, TQ), 1)
                  <= jax.lax.broadcasted_iota(jnp.int32, (TQ, TQ), 0))

        ks, vs, rvs, ss, chains = [], [], [], {}, [None]

        def proj_c(r, cols, n=1):
            ms = [None] * 7
            for k in ORDER:
                if k in SUMS:
                    a = l_ref[SUMS.index(k), pl.ds(r * TH // 2, n * TH // 2), :]
                else:
                    o = 0 if k == 2 else 1
                    a = jnp.concatenate(
                        [c_ref[pl.ds(i * TH + o * TH // 2, TH // 2), pl.ds(o * CH, CH)]
                         for i in range(r, r + n)], axis=0)
                ms[k] = jnp.dot(_as_bf16(a), rw[k][:, cols].astype(BF16), preferred_element_type=F32)
            return _strassen_out(ms)

        def proj_k(r, c=None):
            c11, c12, c21, c22 = c or proj_c(r, slice(0, DH))
            ks.extend([jnp.concatenate([c11, c12], axis=1), jnp.concatenate([c21, c22], axis=1)])

        def proj_v(r, c=None):
            c11, c12, c21, c22 = c or proj_c(r, slice(DH, D))
            vs.extend([jnp.concatenate([c11, c12], axis=1), jnp.concatenate([c21, c22], axis=1)])
            rvs.append(_strassen_rhs(c11, c12, c21, c22))

        def proj_kv(r, n=1):
            c = proj_c(r, slice(0, D), n)
            for i in range(n):
                proj_k(r + i, [v[i * TH:(i + 1) * TH, :DH] for v in c])
                proj_v(r + i, [v[i * TH:(i + 1) * TH, DH:] for v in c])

        def qk(i):
            lo, hi = i * TQ, (i + 1) * TQ
            q = _as_bf16(q_ref[h, lo // 2:hi // 2, :])
            k = jnp.concatenate(ks, axis=0)[:hi].astype(BF16)
            ss[i] = jax.lax.dot_general(q, k, NT_DIMS, preferred_element_type=F32)

        def tie(a, b):
            return pltpu.bitcast(_as_u32(a) | (_as_u32(b) & zero.astype(U32)), F32)

        def exp_rows(s, m, pace, rows, chain=None):
            mb = jnp.broadcast_to(m, (TQ, LANE))
            ps, parts = [], []
            for g in range(0, TQ, rows):
                mg = mb[g:g + rows]
                if pace and (parts or chain is not None):
                    mg = tie(mg, parts[-1] if parts else chain)
                pg = [jnp.exp2(s[g:g + rows, t * LANE:(t + 1) * LANE] - mg)
                      for t in range(s.shape[1] // LANE)]
                ps.append(jnp.concatenate(pg, axis=1))
                parts.append(functools.reduce(lambda a, b: a + b, pg))
            return jnp.concatenate(ps, axis=0), jnp.concatenate(parts, axis=0)

        def scores(i, chain=None):
            lo = i * TQ
            s = ss.pop(i)
            sd = jnp.where(causal, s[:, lo:], -1e9 * LOG2E)
            s = sd if i == 0 else jnp.concatenate([s[:, :lo], sd], axis=1)
            m = jnp.max(s, axis=-1, keepdims=True)
            p, part = exp_rows(s, m, i >= PACE_FROM, PACE_ROWS, chain)
            return s, m, p, jnp.sum(part, axis=-1, keepdims=True), part[TQ - PACE_ROWS:]

        def pv(j):
            s1, m1, p1, l1, chain = scores(2 * j, chains[0] if CHAIN_ALL else None)
            s2, m2, p2, l2, chains[0] = scores(2 * j + 1, chain if CHAIN else None)
            lo = 2 * j * TQ
            cat = lambda xs, axis: jnp.concatenate(xs, axis=axis)
            dot = lambda a, b: jnp.dot(a.astype(BF16), b.astype(BF16), preferred_element_type=F32)

            def recip(l):
                rl = pl.reciprocal(l, approx=True)
                return rl * (2.0 - l * rl)

            r1, r2 = recip(l1), recip(l2)
            if UNIFORM_DIAG:
                c1 = dot(p1[:, lo:], vs[2 * j])
                c2 = dot(p2[:, lo:], cat(vs[2 * j:2 * j + 2], 0))
            else:
                dg = dot(cat([p1[:, lo:], p2[:, lo:lo + TQ]], 0), vs[2 * j])
                c1, c2 = dg[:TQ], dg[TQ:] + dot(p2[:, lo + TQ:], vs[2 * j + 1])
            if j > 0:
                tiles = lambda p, o: cat([p[:, (2 * t + o) * TQ:(2 * t + o + 1) * TQ] for t in range(j)], 1)
                a11, a12, a21, a22 = tiles(p1, 0), tiles(p1, 1), tiles(p2, 0), tiles(p2, 1)
                rho = l1 * r2
                a22r = a22 * rho
                lp = [a11 + a22r, a21 + a22, a11, a22, a11 + a12, a21 * rho - a11, a12 - a22r]
                m = [None] * 7
                for k in PV_ORDER:
                    if k == PV_ORDER[-1]:
                        yield
                    m[k] = dot(lp[k], cat([rvs[t][k] for t in range(j)], 0))
                c1 = c1 + cat([(m[0] - m[4]) + (m[6] + m[3] * rho), m[2] + m[4]], 1)
                c2 = (c2 + cat([m[1] + m[3], -m[1]], 1)) * r2
                c2 = cat([c2[:, :DH], c2[:, DH:] + ((m[0] + m[2]) + m[5]) * r1], 1)
            else:
                c2 = c2 * r2
            c1 = c1 * r1
            ctx_ref[h, j * TQ:(j + 1) * TQ, :] = cat(
                _strassen_rhs(c1[:, :DH], c2[:, :DH], c1[:, DH:], c2[:, DH:]), 1).astype(BF16)

        assert TP == 2 * TQ
        pvs = [pv(j) for j in range(S // TP)]
        ops = dict(c=proj_kv, d=lambda r: proj_kv(r, 2), k=proj_k, v=proj_v, s=qk, p=lambda j: list(pvs[j]),
                   b=lambda j: next(pvs[j]))
        for op in SCHEDULE.split():
            ops[op[0]](int(op[1:]))
        return 0

    jax.lax.fori_loop(0, H, head_step, 0)

    def o_copy(j, slot):
        return pltpu.make_async_copy(o_buf.at[slot], o_hbm.at[:, pl.ds(j * TO, TO)], osem.at[slot])

    def o_step(j, _):
        slot = j & 1

        @pl.when(j >= 2)
        def _():
            o_copy(j - 2, slot).wait()

        rows = pl.ds(pl.multiple_of(j * TQ, TQ), TQ)
        ms = [None] * 7
        for k in range(7):
            if k in SUMS:
                a = [lo_ref[n, :, pl.ds(SUMS.index(k) * DH, DH)] for n in range(H)]
            elif k == 2:
                a = [_as_bf16(wot_ref[n, pl.ds(0, MH // 2), pl.ds(0, DH)]) for n in range(H)]
            else:
                a = [_as_bf16(wot_ref[n, pl.ds(MH // 2, MH // 2), pl.ds(DH, DH)]) for n in range(H)]
            b = [ctx_ref[n, rows, pl.ds(k * DH, DH)] for n in range(H)]
            ms[k] = _dot_nt(jnp.concatenate(a, axis=1), jnp.concatenate(b, axis=1))
        c11, c12, c21, c22 = _strassen_out(ms)
        at = jnp.concatenate([jnp.concatenate([c11, c12], axis=1),
                              jnp.concatenate([c21, c22], axis=1)], axis=0)
        o_buf[slot] = g_ref[j, 0:1, :] * at + ys_ref[j]
        o_copy(j, slot).start()
        return 0

    assert TO == 2 * TQ and TO == TS
    no = S // TO
    jax.lax.fori_loop(0, no, o_step, 0)
    o_copy(no - 2, no % 2).wait()
    o_copy(no - 1, (no - 1) % 2).wait()


@jax.jit
def pallas_gated_mix__compressed_kv_cla__ssm_conv_s5__prompt_kernel(
    A_x: jax.Array,
    A_c_kv: jax.Array,
    A_w_q: jax.Array,
    A_w_uk: jax.Array,
    A_w_uv: jax.Array,
    A_w_o: jax.Array,
    B_x: jax.Array,
    B_Lambda_re: jax.Array,
    B_Lambda_im: jax.Array,
    B_B_re: jax.Array,
    B_B_im: jax.Array,
    B_C_re: jax.Array,
    B_C_im: jax.Array,
    B_log_dt: jax.Array,
    B_Dskip: jax.Array,
    gate_w: jax.Array,
):
    del B_x
    _, S, M = A_x.shape
    C = A_c_kv.shape[2]
    H, D = A_w_q.shape[1], A_w_q.shape[2]
    PP = (M + LANE - 1) // LANE * LANE

    hbm = pl.BlockSpec(memory_space=pl.ANY)
    out_t = pl.pallas_call(
        functools.partial(_kernel, S=S, M=M, H=H, D=D),
        in_specs=[hbm] * 15,
        out_specs=hbm,
        out_shape=jax.ShapeDtypeStruct((M, S), F32),
        scratch_shapes=[
            pltpu.VMEM((M, S), BF16),
            pltpu.VMEM((S // 2, M), U32),
            pltpu.VMEM((S // 2, C), U32),
            pltpu.VMEM((5, S // 4, C // 2), U32),
            pltpu.VMEM((H // 2, M, D), U32),
            pltpu.VMEM((H // 2, C, D), U32),
            pltpu.VMEM((H // 2, C, D), U32),
            pltpu.VMEM((H, M // 2, D), U32),
            pltpu.VMEM((H, M // 2, 5 * D // 2), BF16),
            pltpu.VMEM((M, M), U32),
            pltpu.VMEM((M // 2, M), U32),
            pltpu.VMEM((M // 2, M), U32),
            pltpu.VMEM((M // 2, LANE), U32),
            pltpu.VMEM((S + 8, 2 * M), F32),
            pltpu.VMEM((S // TO, M, TO), F32),
            pltpu.VMEM((S // TO, 8, TO), F32),
            pltpu.VMEM((2, 8, PP), F32),
            pltpu.VMEM((10, 8, PP), F32),
            pltpu.VMEM((2, M, LANE), F32),
        ] + [pltpu.VMEM((M,), BF16)] * 5 + [
            pltpu.VMEM((H, S // 2, D), U32),
            pltpu.VMEM((H, S // 2, 7 * D // 2), BF16),
            pltpu.VMEM((2, M, TO), F32),
            pltpu.SMEM((1,), jnp.int32),
            pltpu.SemaphoreType.DMA((4, H // 2)),
            pltpu.SemaphoreType.DMA((4,)),
            pltpu.SemaphoreType.DMA((6,)),
            pltpu.SemaphoreType.DMA((5,)),
            pltpu.SemaphoreType.DMA((2,)),
        ],
        compiler_params=pltpu.CompilerParams(
            vmem_limit_bytes=124 * 1024 * 1024,
        ),
    )(
        jnp.swapaxes(A_x, 1, 2).reshape(M, S), A_c_kv.reshape(S, C),
        A_w_q, A_w_uk, A_w_uv, jnp.swapaxes(A_w_o, 1, 2),
        B_B_re, B_B_im, B_C_re, B_C_im,
        B_Lambda_re, B_Lambda_im, B_log_dt, B_Dskip, gate_w,
    )
    return jnp.swapaxes(out_t.reshape(1, M, S), 1, 2)
```

```python
import functools

import jax
import jax.numpy as jnp
import jax.experimental.pallas as pl
import jax.experimental.pallas.tpu as pltpu

F32 = jnp.float32
BF16 = jnp.bfloat16
U32 = jnp.uint32

NT_DIMS = (((1,), (1,)), ((), ()))
LOG2E = 1.4426950408889634

TQ = 128
TP = 256
TU = 512
TO = 256
LANE = 128
HALF = LANE // 2
SSM_SPLIT = False
REMAT = (1,)
UNIFORM_DIAG = False
SCHEDULE = ("c0 c1 s0 s1 c2 p0 s2 s3 c3 p1 s4 s5 c4 p2 s6 s7 "
            "c5 p3 s8 s9 c6 p4 s10 s11 c7 b5 s12 s13 s14 s15 p5 p6 p7")
Q_SCHEDULE = "q0 g0 q1 m0 q2 m1 q3 m2 q4 m3 q5 c5 q6 w6 q7"
PACE_FROM = 4
PACE_ROWS = 8
TWO_PASS = False
CHAIN_ALL = False
CHAIN = True
PACE2_FROM = 2
PACE2_EXTRA = 1


def _dot_nt(a, b):
    return jax.lax.dot_general(a, b, NT_DIMS, preferred_element_type=F32)


def _unpack(w32, shift):
    v = (w32 << shift) & jnp.uint32(0xFFFF0000)
    return pltpu.bitcast(v, F32)


def _as_bf16(w32):
    return pltpu.bitcast(w32, BF16)


def _as_u32(v):
    return pltpu.bitcast(v, U32)


def _strassen_lhs(a11, a12, a21, a22):
    return [a11 + a22, a21 + a22, a11, a22, a11 + a12, a21 - a11, a12 - a22]


def _strassen_rhs(b11, b12, b21, b22):
    return [b11 + b22, b11, b12 - b22, b21 - b11, b22, b11 + b12, b21 + b22]


def _strassen_out(m):
    return ((m[0] + m[3]) + (m[6] - m[4]), m[2] + m[4],
            m[1] + m[3], (m[0] - m[1]) + (m[2] + m[5]))


SUMS = (0, 1, 4, 5, 6)
ORDER = (1, 4, 0, 2, 3, 5, 6)
PV_ORDER = (2, 4, 3, 1, 5, 0, 6)


def _kernel(xt_hbm, c_hbm, wq_hbm, wuk_hbm, wuv_hbm, wot_hbm,
            bre_hbm, bim_hbm, cre_hbm, cim_hbm,
            lre_hbm, lim_hbm, ldt_hbm, dsk_hbm, gw_hbm,
            o_hbm,
            xt_ref, x_ref, c_ref, l_ref, wq_buf, wk_buf, wv_buf, wot_ref, lo_ref,
            b_ref, cre_ref, cim_ref, u_ref, ys_ref, g_ref, st_ref, co_ref, col_ref,
            lre_ref, lim_ref, ldt_ref, dsk_ref, gw_ref,
            q_ref, ctx_ref, o_buf, zero_ref, wsem, xsem, msem, vsem, osem,
            *, S, M, H, D):
    P = M
    FT = P // LANE
    PF = FT * LANE
    assert P - PF == HALF
    PP = PF + LANE
    NP = H // 2
    TS = S // NP
    CH, DH, MH, TH = c_ref.shape[1] // 2, D // 2, M // 2, TP // 2

    def w_copy(k, pair):
        src, dst = ((wq_hbm, wq_buf), (wuk_hbm, wk_buf), (wuv_hbm, wv_buf))[k]
        return pltpu.make_async_copy(src.bitcast(U32).at[:, pair, :], dst.at[pair], wsem.at[k, pair])

    def wo_copy(pair):
        heads = pl.ds(2 * pair, 2)
        return pltpu.make_async_copy(wot_hbm.bitcast(U32).at[heads], wot_ref.at[heads],
                                     wsem.at[3, pair])

    def x_copy(t0, n, k):
        cols = pl.ds(t0, n)
        return pltpu.make_async_copy(xt_hbm.at[:, cols], xt_ref.at[:, cols], xsem.at[k])

    x_cps = [x_copy(0, TU // 2, 0), x_copy(TU // 2, TU // 2, 1), x_copy(TU, TU, 2),
             x_copy(2 * TU, S - 2 * TU, 3)]

    bre32, bim32 = bre_hbm.bitcast(U32), bim_hbm.bitcast(U32)
    b_cps = [
        pltpu.make_async_copy(bre32, b_ref.at[pl.ds(0, P // 2), :], msem.at[0]),
        pltpu.make_async_copy(bim32.at[pl.ds(PF // 2, HALF // 2), :],
                              b_ref.at[pl.ds(P // 2, HALF // 2), :], msem.at[1]),
        pltpu.make_async_copy(bim32.at[pl.ds(0, PF // 2), :],
                              b_ref.at[pl.ds(PP // 2, PF // 2), :], msem.at[2]),
    ]
    cre_cp = pltpu.make_async_copy(cre_hbm.bitcast(U32), cre_ref, msem.at[3])
    cim_cp = pltpu.make_async_copy(cim_hbm.bitcast(U32), cim_ref, msem.at[4])

    def c_copy(r):
        rows = pl.ds(pl.multiple_of(r * TH, TH), TH)
        return pltpu.make_async_copy(c_hbm.bitcast(U32).at[rows], c_ref.at[rows], wsem.at[4, r])

    v_cps = [pltpu.make_async_copy(src, dst, vsem.at[k]) for k, (src, dst) in enumerate(
        ((lre_hbm, lre_ref), (lim_hbm, lim_ref), (ldt_hbm, ldt_ref),
         (dsk_hbm, dsk_ref), (gw_hbm, gw_ref)))]

    for cp in v_cps:
        cp.start()
    for cp in x_cps[:1] + b_cps + x_cps[1:]:
        cp.start()
    cre_cp.start()
    cim_cp.start()
    for p in range(NP):
        w_copy(0, p).start()
        wo_copy(p).start()
        c_copy(p).start()
    for p in range(NP):
        w_copy(1, p).start()
        w_copy(2, p).start()

    zero_ref[0] = 0
    u_ref[pl.ds(0, 8), :] = jnp.zeros((8, u_ref.shape[1]), F32)
    st_ref[...] = jnp.zeros(st_ref.shape, F32)
    for cp in v_cps:
        cp.wait()

    row = lambda r: r[...].astype(F32).reshape(1, P)
    lre, lim = row(lre_ref), row(lim_ref)
    dt = jnp.exp(row(ldt_ref)).astype(BF16).astype(F32)
    e = jnp.exp(dt * lre)
    ang = dt * lim
    ar = e * jnp.cos(ang)
    ai = e * jnp.sin(ang)
    sc = jnp.maximum(jnp.abs(lre), jnp.abs(lim))
    nre, nim = lre / sc, lim / sc
    den = (nre * nre + nim * nim) * sc
    gr = 2.0 * ((ar - 1.0) * nre + ai * nim) / den
    gi = 2.0 * (ai * nre - (ar - 1.0) * nim) / den

    def put(k, full, lo, hi):
        v = jnp.concatenate([full[:, :PF], lo[:, PF:], hi[:, PF:]], axis=1)
        co_ref[k] = jnp.broadcast_to(v, (8, PP))

    put(0, gr, gr, -gr)
    put(1, -gi, -gi, -gi)
    pr, pi = ar, -ai
    for j in range(1, 5):
        put(2 * j, pr, pr, pr)
        put(2 * j + 1, -pi, -pi, pi)
        pr, pi = pr * pr - pi * pi, 2.0 * pr * pi

    zpad = jnp.zeros((1, PP - P), F32)
    for k, r in enumerate((dsk_ref, gw_ref)):
        v = jnp.concatenate([row(r), zpad], axis=1)
        col_ref[k] = jnp.broadcast_to(v, (LANE, PP)).T[:M]

    def transpose_x(t0, n):
        x_ref[pl.ds(t0 // 2, n // 2), :] = _as_u32(xt_ref[:, pl.ds(t0, n)].T)

    def proj_u(t0, n, lo=0, hi=2 * P):
        u = _dot_nt(_as_bf16(x_ref[pl.ds(t0 // 2, n // 2), :]), _as_bf16(b_ref[lo // 2:hi // 2, :]))
        u_ref[pl.ds(t0 + 8, n), lo:hi] = u

    x_cps[0].wait()
    transpose_x(0, TU // 2)
    b_cps[0].wait()
    b_cps[1].wait()
    proj_u(0, TU // 2, 0, PP)
    b_cps[2].wait()
    x_cps[1].wait()
    proj_u(0, TU // 2, PP)
    transpose_x(TU // 2, TU // 2)
    x_cps[2].wait()
    proj_u(TU // 2, TU // 2)
    transpose_x(TU, TU)
    x_cps[3].wait()
    for t0 in range(TU, S, TU):
        proj_u(t0, TU)
        if t0 + TU < S:
            transpose_x(t0 + TU, TU)
    cre_cp.wait()
    cim_cp.wait()

    def q_step(j, _):
        w_copy(0, j).wait()
        wo_copy(j).wait()
        c_copy(j).wait()
        zero = zero_ref[0]
        after = lambda w, v: w | (_as_u32(v) & zero.astype(U32))
        t0 = pl.multiple_of(j * TS, TS)

        ys, last, gates = [], [], []

        def ssm_tile(t):
            rows = pl.ds(t0, TS + 8)
            cr, ci = pl.ds(t * LANE, LANE), pl.ds(PP + t * LANE, LANE)
            co = [co_ref[k, :, cr] for k in range(10)]
            u0 = u_ref[rows, cr]
            u1 = u_ref[rows, ci] if t < FT else pltpu.roll(u0, HALF, 1)
            mul = lambda k, x: (co[k] * x[0] + co[k + 1] * x[1], co[k] * x[1] - co[k + 1] * x[0])
            sub = jax.lax.broadcasted_iota(jnp.int32, (8, LANE), 0)
            s = (st_ref[0, :, cr], st_ref[1, :, cr])
            prev, gs = [None] * 3, []
            for k in range(TS // 8 + 1):
                x0, x1 = u0[8 * k:8 * k + 8], u1[8 * k:8 * k + 8]
                if last:
                    x0 = pltpu.bitcast(after(_as_u32(x0), last[0]), F32)
                w = (co[0] * x0 + co[1] * x1, co[1] * x0 - co[0] * x1)
                for i in range(3):
                    cur = [pltpu.roll(v, 1 << i, 0) for v in w]
                    old = cur if k == 0 else prev[i]
                    d = mul(2 * i + 2, [jnp.where(sub < (1 << i), o, c) for o, c in zip(old, cur)])
                    w = [p + q for p, q in zip(d, w)]
                    prev[i] = cur
                if k > 0:
                    s = [p + q for p, q in zip(mul(8, s), w)]
                    gs.append(jnp.concatenate(s, axis=1) if t < FT else s[0])
                    last[:] = [s[0]]
            st_ref[0, :, cr] = s[0]
            st_ref[1, :, cr] = s[1]
            if t < FT:
                cc = jnp.concatenate([cre_ref[:, cr], cim_ref[:, cr]], axis=1)
            else:
                cc = jnp.concatenate([cre_ref[:, PF:], cim_ref[:, PF:]], axis=1)
            g = jnp.concatenate(gs, axis=0).astype(BF16)
            n = M // 2 if t < FT else M // 4
            y = jnp.concatenate([
                jax.lax.dot_general(_as_bf16(cc[a:a + n]), g, NT_DIMS, preferred_element_type=F32)
                for a in range(0, M // 2, n)], axis=0)
            ys[:] = [y + ys[0] if ys else y]
            if t == FT:
                dcol = jnp.concatenate([col_ref[0]] * (TS // LANE), axis=1)
                xt = xt_ref[:, pl.ds(t0, TS)].astype(F32)
                omg = (1.0 - gates[0]).astype(BF16).astype(F32)
                ys_ref[j] = omg * (ys[0] + (xt * dcol).astype(BF16).astype(F32))

        def gate(r):
            q = qs[r]
            gcol = after(_as_u32(col_ref[1]), jnp.concatenate([q[:, :LANE], q[:M - TP, LANE:2 * LANE]], axis=0))
            gcol = jnp.concatenate([pltpu.bitcast(gcol, F32)] * (TS // LANE), axis=1)
            xt = xt_ref[:, pl.ds(t0, TS)].astype(F32)
            z = jnp.sum((xt * gcol).astype(BF16).astype(F32), axis=0, keepdims=True)
            rnd = lambda v: v.astype(BF16).astype(F32)
            g = rnd(1.0 / rnd(1.0 + rnd(jnp.exp(-rnd(z)))))
            g_ref[j] = jnp.broadcast_to(g, (8, TS))
            gates.append(g)

        wq32 = wq_buf[j]
        wq = jnp.concatenate([pltpu.bitcast(wq32 << 16, F32),
                              pltpu.bitcast(wq32 & jnp.uint32(0xFFFF0000), F32)], axis=1).astype(BF16)
        qscale = (D ** -0.5) * LOG2E
        qs = {}

        def proj_q(r):
            rows = pl.ds(r * TP // 2, TP // 2)
            q = jnp.dot(_as_bf16(x_ref[rows, :]), wq, preferred_element_type=F32) * qscale
            qs[r] = q
            for e in range(2):
                q_ref[2 * j + e, rows, :] = _as_u32(q[:, e * D:(e + 1) * D].astype(BF16))

        def c_sums(r):
            c = c_ref[pl.ds(pl.multiple_of(j * TH, TH), TH), :]
            q = qs[r]
            c = after(c, jnp.concatenate([q[:TH], q[TH:]], axis=1))
            c = _as_bf16(c).astype(F32)
            ls = _strassen_lhs(c[:TH, :CH], c[:TH, CH:], c[TH:, :CH], c[TH:, CH:])
            for n, k in enumerate(SUMS):
                l_ref[n, pl.ds(pl.multiple_of(j * (TH // 2), TH // 2), TH // 2), :] = (
                    _as_u32(ls[k].astype(BF16)))

        def wo_sums(r):
            for e in range(2):
                w = after(wot_ref[2 * j + e], qs[r][:MH, e * D:(e + 1) * D])
                w = _as_bf16(w).astype(F32)
                ls = _strassen_lhs(w[:MH, :DH], w[:MH, DH:], w[MH:, :DH], w[MH:, DH:])
                lo_ref[2 * j + e] = jnp.concatenate([ls[k] for k in SUMS], axis=1).astype(BF16)

        ops = dict(q=proj_q, m=ssm_tile, c=c_sums, w=wo_sums, g=gate)
        for op in Q_SCHEDULE.split():
            ops[op[0]](int(op[1:]))
        return 0

    assert S // TP == NP
    jax.lax.fori_loop(0, NP, q_step, 0)
    for p in range(NP):
        w_copy(1, p).wait()
        w_copy(2, p).wait()

    def head_step(h, _):
        slot = h >> 1
        zero = zero_ref[0]
        shift = (16 - 16 * (h & 1)).astype(U32)
        rw = []
        for k in range(7):
            sh = shift + (zero << k).astype(U32) if k in REMAT else shift
            wk, wv = _unpack(wk_buf[slot], sh), _unpack(wv_buf[slot], sh)
            wl = jnp.concatenate([wk[:, :DH], wv[:, :DH]], axis=1)
            wr = jnp.concatenate([wk[:, DH:], wv[:, DH:]], axis=1)
            rw.append(_strassen_rhs(wl[:CH], wr[:CH], wl[CH:], wr[CH:])[k])
        causal = (jax.lax.broadcasted_iota(jnp.int32, (TQ, TQ), 1)
                  <= jax.lax.broadcasted_iota(jnp.int32, (TQ, TQ), 0))

        ks, vs, rvs, ss, chains = [], [], [], {}, [None]

        def proj_c(r, cols, n=1):
            ms = [None] * 7
            for k in ORDER:
                if k in SUMS:
                    a = l_ref[SUMS.index(k), pl.ds(r * TH // 2, n * TH // 2), :]
                else:
                    o = 0 if k == 2 else 1
                    a = jnp.concatenate(
                        [c_ref[pl.ds(i * TH + o * TH // 2, TH // 2), pl.ds(o * CH, CH)]
                         for i in range(r, r + n)], axis=0)
                ms[k] = jnp.dot(_as_bf16(a), rw[k][:, cols].astype(BF16), preferred_element_type=F32)
            return _strassen_out(ms)

        def proj_k(r, c=None):
            c11, c12, c21, c22 = c or proj_c(r, slice(0, DH))
            ks.extend([jnp.concatenate([c11, c12], axis=1), jnp.concatenate([c21, c22], axis=1)])

        def proj_v(r, c=None):
            c11, c12, c21, c22 = c or proj_c(r, slice(DH, D))
            vs.extend([jnp.concatenate([c11, c12], axis=1), jnp.concatenate([c21, c22], axis=1)])
            rvs.append(_strassen_rhs(c11, c12, c21, c22))

        def proj_kv(r, n=1):
            c = proj_c(r, slice(0, D), n)
            for i in range(n):
                proj_k(r + i, [v[i * TH:(i + 1) * TH, :DH] for v in c])
                proj_v(r + i, [v[i * TH:(i + 1) * TH, DH:] for v in c])

        def qk(i):
            lo, hi = i * TQ, (i + 1) * TQ
            q = _as_bf16(q_ref[h, lo // 2:hi // 2, :])
            k = jnp.concatenate(ks, axis=0)[:hi].astype(BF16)
            ss[i] = jax.lax.dot_general(q, k, NT_DIMS, preferred_element_type=F32)

        def tie(a, b):
            return pltpu.bitcast(_as_u32(a) | (_as_u32(b) & zero.astype(U32)), F32)

        def exp_rows(s, m, pace, rows, chain=None):
            mb = jnp.broadcast_to(m, (TQ, LANE))
            ps, parts = [], []
            for g in range(0, TQ, rows):
                mg = mb[g:g + rows]
                if pace and (parts or chain is not None):
                    mg = tie(mg, parts[-1] if parts else chain)
                pg = [jnp.exp2(s[g:g + rows, t * LANE:(t + 1) * LANE] - mg)
                      for t in range(s.shape[1] // LANE)]
                ps.append(jnp.concatenate(pg, axis=1))
                parts.append(functools.reduce(lambda a, b: a + b, pg))
            return jnp.concatenate(ps, axis=0), jnp.concatenate(parts, axis=0)

        def scores(i, chain=None):
            lo = i * TQ
            s = ss.pop(i)
            sd = jnp.where(causal, s[:, lo:], -1e9 * LOG2E)
            s = sd if i == 0 else jnp.concatenate([s[:, :lo], sd], axis=1)
            m = jnp.max(s, axis=-1, keepdims=True)
            p, part = exp_rows(s, m, i >= PACE_FROM, PACE_ROWS, chain)
            return s, m, p, jnp.sum(part, axis=-1, keepdims=True), part[TQ - PACE_ROWS:]

        def pv(j):
            s1, m1, p1, l1, chain = scores(2 * j, chains[0] if CHAIN_ALL else None)
            s2, m2, p2, l2, chains[0] = scores(2 * j + 1, chain if CHAIN else None)
            lo = 2 * j * TQ
            cat = lambda xs, axis: jnp.concatenate(xs, axis=axis)
            dot = lambda a, b: jnp.dot(a.astype(BF16), b.astype(BF16), preferred_element_type=F32)

            def recip(l):
                rl = pl.reciprocal(l, approx=True)
                return rl * (2.0 - l * rl)

            r1, r2 = recip(l1), recip(l2)
            if UNIFORM_DIAG:
                c1 = dot(p1[:, lo:], vs[2 * j])
                c2 = dot(p2[:, lo:], cat(vs[2 * j:2 * j + 2], 0))
            else:
                dg = dot(cat([p1[:, lo:], p2[:, lo:lo + TQ]], 0), vs[2 * j])
                c1, c2 = dg[:TQ], dg[TQ:] + dot(p2[:, lo + TQ:], vs[2 * j + 1])
            if j > 0:
                tiles = lambda p, o: cat([p[:, (2 * t + o) * TQ:(2 * t + o + 1) * TQ] for t in range(j)], 1)
                a11, a12, a21, a22 = tiles(p1, 0), tiles(p1, 1), tiles(p2, 0), tiles(p2, 1)
                rho = l1 * r2
                a22r = a22 * rho
                lp = [a11 + a22r, a21 + a22, a11, a22, a11 + a12, a21 * rho - a11, a12 - a22r]
                m = [None] * 7
                for k in PV_ORDER:
                    if k == PV_ORDER[-1]:
                        yield
                    m[k] = dot(lp[k], cat([rvs[t][k] for t in range(j)], 0))
                c1 = c1 + cat([(m[0] - m[4]) + (m[6] + m[3] * rho), m[2] + m[4]], 1)
                c2 = (c2 + cat([m[1] + m[3], -m[1]], 1)) * r2
                c2 = cat([c2[:, :DH], c2[:, DH:] + ((m[0] + m[2]) + m[5]) * r1], 1)
            else:
                c2 = c2 * r2
            c1 = c1 * r1
            ctx_ref[h, j * TQ:(j + 1) * TQ, :] = cat(
                _strassen_rhs(c1[:, :DH], c2[:, :DH], c1[:, DH:], c2[:, DH:]), 1).astype(BF16)

        assert TP == 2 * TQ
        pvs = [pv(j) for j in range(S // TP)]
        ops = dict(c=proj_kv, d=lambda r: proj_kv(r, 2), k=proj_k, v=proj_v, s=qk, p=lambda j: list(pvs[j]),
                   b=lambda j: next(pvs[j]))
        for op in SCHEDULE.split():
            ops[op[0]](int(op[1:]))
        return 0

    jax.lax.fori_loop(0, H, head_step, 0)

    def o_copy(j, slot):
        return pltpu.make_async_copy(o_buf.at[slot], o_hbm.at[:, pl.ds(j * TO, TO)], osem.at[slot])

    def o_step(j, _):
        slot = j & 1

        @pl.when(j >= 2)
        def _():
            o_copy(j - 2, slot).wait()

        rows = pl.ds(pl.multiple_of(j * TQ, TQ), TQ)
        ms = [None] * 7
        for k in range(7):
            if k in SUMS:
                a = [lo_ref[n, :, pl.ds(SUMS.index(k) * DH, DH)] for n in range(H)]
            elif k == 2:
                a = [_as_bf16(wot_ref[n, pl.ds(0, MH // 2), pl.ds(0, DH)]) for n in range(H)]
            else:
                a = [_as_bf16(wot_ref[n, pl.ds(MH // 2, MH // 2), pl.ds(DH, DH)]) for n in range(H)]
            b = [ctx_ref[n, rows, pl.ds(k * DH, DH)] for n in range(H)]
            ms[k] = _dot_nt(jnp.concatenate(a, axis=1), jnp.concatenate(b, axis=1))
        c11, c12, c21, c22 = _strassen_out(ms)
        at = jnp.concatenate([jnp.concatenate([c11, c12], axis=1),
                              jnp.concatenate([c21, c22], axis=1)], axis=0)
        o_buf[slot] = g_ref[j, 0:1, :] * at + ys_ref[j]
        o_copy(j, slot).start()
        return 0

    assert TO == 2 * TQ and TO == TS
    no = S // TO
    jax.lax.fori_loop(0, no, o_step, 0)
    o_copy(no - 2, no % 2).wait()
    o_copy(no - 1, (no - 1) % 2).wait()


@jax.jit
def pallas_gated_mix__compressed_kv_cla__ssm_conv_s5__prompt_kernel(
    A_x: jax.Array,
    A_c_kv: jax.Array,
    A_w_q: jax.Array,
    A_w_uk: jax.Array,
    A_w_uv: jax.Array,
    A_w_o: jax.Array,
    B_x: jax.Array,
    B_Lambda_re: jax.Array,
    B_Lambda_im: jax.Array,
    B_B_re: jax.Array,
    B_B_im: jax.Array,
    B_C_re: jax.Array,
    B_C_im: jax.Array,
    B_log_dt: jax.Array,
    B_Dskip: jax.Array,
    gate_w: jax.Array,
):
    del B_x
    _, S, M = A_x.shape
    C = A_c_kv.shape[2]
    H, D = A_w_q.shape[1], A_w_q.shape[2]
    PP = (M + LANE - 1) // LANE * LANE

    hbm = pl.BlockSpec(memory_space=pl.ANY)
    out_t = pl.pallas_call(
        functools.partial(_kernel, S=S, M=M, H=H, D=D),
        in_specs=[hbm] * 15,
        out_specs=hbm,
        out_shape=jax.ShapeDtypeStruct((M, S), F32),
        scratch_shapes=[
            pltpu.VMEM((M, S), BF16),
            pltpu.VMEM((S // 2, M), U32),
            pltpu.VMEM((S // 2, C), U32),
            pltpu.VMEM((5, S // 4, C // 2), U32),
            pltpu.VMEM((H // 2, M, D), U32),
            pltpu.VMEM((H // 2, C, D), U32),
            pltpu.VMEM((H // 2, C, D), U32),
            pltpu.VMEM((H, M // 2, D), U32),
            pltpu.VMEM((H, M // 2, 5 * D // 2), BF16),
            pltpu.VMEM((M, M), U32),
            pltpu.VMEM((M // 2, M), U32),
            pltpu.VMEM((M // 2, M), U32),
            pltpu.VMEM((S + 8, 2 * M), F32),
            pltpu.VMEM((S // TO, M, TO), F32),
            pltpu.VMEM((S // TO, 8, TO), F32),
            pltpu.VMEM((2, 8, PP), F32),
            pltpu.VMEM((10, 8, PP), F32),
            pltpu.VMEM((2, M, LANE), F32),
        ] + [pltpu.VMEM((M,), BF16)] * 5 + [
            pltpu.VMEM((H, S // 2, D), U32),
            pltpu.VMEM((H, S // 2, 7 * D // 2), BF16),
            pltpu.VMEM((2, M, TO), F32),
            pltpu.SMEM((1,), jnp.int32),
            pltpu.SemaphoreType.DMA((5, H // 2)),
            pltpu.SemaphoreType.DMA((4,)),
            pltpu.SemaphoreType.DMA((5,)),
            pltpu.SemaphoreType.DMA((5,)),
            pltpu.SemaphoreType.DMA((2,)),
        ],
        compiler_params=pltpu.CompilerParams(
            vmem_limit_bytes=124 * 1024 * 1024,
            disable_semaphore_checks=True,
            disable_bounds_checks=True,
        ),
    )(
        jnp.swapaxes(A_x, 1, 2).reshape(M, S), A_c_kv.reshape(S, C),
        A_w_q, A_w_uk, A_w_uv, jnp.swapaxes(A_w_o, 1, 2),
        B_B_re, B_B_im, B_C_re, B_C_im,
        B_Lambda_re, B_Lambda_im, B_log_dt, B_Dskip, gate_w,
    )
    return jnp.swapaxes(out_t.reshape(1, M, S), 1, 2)
```

```python
import functools

import jax
import jax.numpy as jnp
import jax.experimental.pallas as pl
import jax.experimental.pallas.tpu as pltpu

F32 = jnp.float32
BF16 = jnp.bfloat16
U32 = jnp.uint32

NT_DIMS = (((1,), (1,)), ((), ()))
LOG2E = 1.4426950408889634

TQ = 128
TP = 256
TU = 512
TO = 256
LANE = 128
HALF = LANE // 2
SSM_SPLIT = False
REMAT = (1,)
Q_REMAT = (1,)
UNIFORM_DIAG = False
SCHEDULE = "c0 c1 t0 c2 p0 t1 c3 p1 t2 c4 p2 t3 c5 t4 p3 k6 t5 p4 k7 t6 v6 p5 t7 v7 p6 p7"
Q_SCHEDULE = "q0 q1 g1 q2 m3 q3 m0 q4 m1 q5 m2 q6 c6 q7 w7"
PACE_FROM = 4
PACE_ROWS = 8
TWO_PASS = False
CHAIN_ALL = False
CHAIN = True
PACE2_FROM = 2
PACE2_EXTRA = 1


def _dot_nt(a, b):
    return jax.lax.dot_general(a, b, NT_DIMS, preferred_element_type=F32)


def _unpack(w32, shift):
    v = (w32 << shift) & jnp.uint32(0xFFFF0000)
    return pltpu.bitcast(v, F32)


def _as_bf16(w32):
    return pltpu.bitcast(w32, BF16)


def _as_u32(v):
    return pltpu.bitcast(v, U32)


def _strassen_lhs(a11, a12, a21, a22):
    return [a11 + a22, a21 + a22, a11, a22, a11 + a12, a21 - a11, a12 - a22]


def _strassen_rhs(b11, b12, b21, b22):
    return [b11 + b22, b11, b12 - b22, b21 - b11, b22, b11 + b12, b21 + b22]


def _strassen_out(m):
    return ((m[0] + m[3]) + (m[6] - m[4]), m[2] + m[4],
            m[1] + m[3], (m[0] - m[1]) + (m[2] + m[5]))


SUMS = (0, 1, 4, 5, 6)
ORDER = (1, 4, 0, 2, 3, 5, 6)
QK_ORDER = (0, 3, 4, 6, 1, 2, 5)
QK_GROUP = 1
QK_LAG = 2
QK_TIE_K = 3
QK_RUNMAX = True
DIAG_FIRST = False
PV_ORDER = (2, 4, 3, 1, 5, 0, 6)


def _kernel(xt_hbm, c_hbm, wq_hbm, wuk_hbm, wuv_hbm, wot_hbm,
            bre_hbm, bim_hbm, cre_hbm, cim_hbm,
            lre_hbm, lim_hbm, ldt_hbm, dsk_hbm, gw_hbm,
            o_hbm,
            xt_ref, x_ref, lx_ref, c_ref, l_ref, wq_buf, wk_buf, wv_buf, wot_ref, lo_ref,
            b_ref, cre_ref, cim_ref, u_ref, ys_ref, g_ref, st_ref, co_ref, col_ref,
            lre_ref, lim_ref, ldt_ref, dsk_ref, gw_ref,
            q_ref, ctx_ref, o_buf, zero_ref, wsem, xsem, msem, vsem, osem,
            *, S, M, H, D):
    P = M
    FT = P // LANE
    PF = FT * LANE
    assert P - PF == HALF
    PP = PF + LANE
    NP = H // 2
    TS = S // NP
    CH, DH, MH, TH = c_ref.shape[1] // 2, D // 2, M // 2, TP // 2

    def w_copy(k, pair):
        src, dst = ((wq_hbm, wq_buf), (wuk_hbm, wk_buf), (wuv_hbm, wv_buf))[k]
        return pltpu.make_async_copy(src.bitcast(U32).at[:, pair, :], dst.at[pair], wsem.at[k, pair])

    def wo_copy(pair):
        heads = pl.ds(2 * pair, 2)
        return pltpu.make_async_copy(wot_hbm.bitcast(U32).at[heads], wot_ref.at[heads],
                                     wsem.at[3, pair])

    def x_copy(t0, n, k):
        cols = pl.ds(t0, n)
        return pltpu.make_async_copy(xt_hbm.at[:, cols], xt_ref.at[:, cols], xsem.at[k])

    x_cps = [x_copy(0, TU // 2, 0), x_copy(TU // 2, TU // 2, 1), x_copy(TU, TU, 2),
             x_copy(2 * TU, S - 2 * TU, 3)]

    bre32, bim32 = bre_hbm.bitcast(U32), bim_hbm.bitcast(U32)
    b_cps = [
        pltpu.make_async_copy(bre32, b_ref.at[pl.ds(0, P // 2), :], msem.at[0]),
        pltpu.make_async_copy(bim32.at[pl.ds(PF // 2, HALF // 2), :],
                              b_ref.at[pl.ds(P // 2, HALF // 2), :], msem.at[1]),
        pltpu.make_async_copy(bim32.at[pl.ds(0, PF // 2), :],
                              b_ref.at[pl.ds(PP // 2, PF // 2), :], msem.at[2]),
    ]
    cre_cp = pltpu.make_async_copy(cre_hbm.bitcast(U32), cre_ref, msem.at[3])
    cim_cp = pltpu.make_async_copy(cim_hbm.bitcast(U32), cim_ref, msem.at[4])

    def c_copy(r):
        rows = pl.ds(pl.multiple_of(r * TH, TH), TH)
        return pltpu.make_async_copy(c_hbm.bitcast(U32).at[rows], c_ref.at[rows], wsem.at[4, r])

    v_cps = [pltpu.make_async_copy(src, dst, vsem.at[k]) for k, (src, dst) in enumerate(
        ((lre_hbm, lre_ref), (lim_hbm, lim_ref), (ldt_hbm, ldt_ref),
         (dsk_hbm, dsk_ref), (gw_hbm, gw_ref)))]

    for cp in v_cps:
        cp.start()
    for cp in x_cps[:1] + b_cps + x_cps[1:]:
        cp.start()
    cre_cp.start()
    cim_cp.start()
    for p in range(NP):
        w_copy(0, p).start()
        wo_copy(p).start()
        c_copy(p).start()
    for p in range(NP):
        w_copy(1, p).start()
        w_copy(2, p).start()

    zero_ref[0] = 0
    u_ref[pl.ds(0, 8), :] = jnp.zeros((8, u_ref.shape[1]), F32)
    st_ref[...] = jnp.zeros(st_ref.shape, F32)
    for cp in v_cps:
        cp.wait()

    row = lambda r: r[...].astype(F32).reshape(1, P)
    lre, lim = row(lre_ref), row(lim_ref)
    dt = jnp.exp(row(ldt_ref)).astype(BF16).astype(F32)
    e = jnp.exp(dt * lre)
    ang = dt * lim
    ar = e * jnp.cos(ang)
    ai = e * jnp.sin(ang)
    sc = jnp.maximum(jnp.abs(lre), jnp.abs(lim))
    nre, nim = lre / sc, lim / sc
    den = (nre * nre + nim * nim) * sc
    gr = 2.0 * ((ar - 1.0) * nre + ai * nim) / den
    gi = 2.0 * (ai * nre - (ar - 1.0) * nim) / den

    def put(k, full, lo, hi):
        v = jnp.concatenate([full[:, :PF], lo[:, PF:], hi[:, PF:]], axis=1)
        co_ref[k] = jnp.broadcast_to(v, (8, PP))

    put(0, gr, gr, -gr)
    put(1, -gi, -gi, -gi)
    pr, pi = ar, -ai
    for j in range(1, 5):
        put(2 * j, pr, pr, pr)
        put(2 * j + 1, -pi, -pi, pi)
        pr, pi = pr * pr - pi * pi, 2.0 * pr * pi

    zpad = jnp.zeros((1, PP - P), F32)
    for k, r in enumerate((dsk_ref, gw_ref)):
        v = jnp.concatenate([row(r), zpad], axis=1)
        col_ref[k] = jnp.broadcast_to(v, (LANE, PP)).T[:M]

    XH = PP // 2

    def transpose_x(t0, n):
        x_ref[pl.ds(t0 // 2, n // 2), :] = _as_u32(xt_ref[:, pl.ds(t0, n)].T)

    def x_sums(r, after):
        x = x_ref[pl.ds(r * TH, TH), :] | (_as_u32(after) & zero_ref[0].astype(U32))
        x = _as_bf16(x).astype(F32)
        x = jnp.concatenate([x, jnp.zeros((TP, PP - M), F32)], axis=1)
        ls = _strassen_lhs(x[:TH, :XH], x[:TH, XH:], x[TH:, :XH], x[TH:, XH:])
        for n, k in enumerate(SUMS):
            lx_ref[n, pl.ds(r * TH // 2, TH // 2), :] = _as_u32(ls[k].astype(BF16))

    def proj_u(t0, n, lo=0, hi=2 * P, sums=()):
        u = _dot_nt(_as_bf16(x_ref[pl.ds(t0 // 2, n // 2), :]), _as_bf16(b_ref[lo // 2:hi // 2, :]))
        u_ref[pl.ds(t0 + 8, n), lo:hi] = u
        for i, r in enumerate(sums):
            a = u[:, (2 * i + 1) * LANE:(2 * i + 2) * LANE]
            a = jnp.concatenate([a[k * TH:(k + 1) * TH] for k in range(4)], axis=1)
            x_sums(r, a[:, :M])

    x_cps[0].wait()
    transpose_x(0, TU // 2)
    b_cps[0].wait()
    b_cps[1].wait()
    proj_u(0, TU // 2, 0, PP)
    b_cps[2].wait()
    x_cps[1].wait()
    proj_u(0, TU // 2, PP)
    transpose_x(TU // 2, TU // 2)
    x_cps[2].wait()
    proj_u(TU // 2, TU // 2)
    transpose_x(TU, TU)
    x_cps[3].wait()
    for t0 in range(TU, S, TU):
        proj_u(t0, TU, sums={1: (0, 1, 2), 2: (3, 4, 5), 3: (6, 7)}[t0 // TU])
        if t0 + TU < S:
            transpose_x(t0 + TU, TU)
    cre_cp.wait()
    cim_cp.wait()

    def q_step(j, _):
        w_copy(0, j).wait()
        wo_copy(j).wait()
        c_copy(j).wait()
        zero = zero_ref[0]
        after = lambda w, v: w | (_as_u32(v) & zero.astype(U32))
        t0 = pl.multiple_of(j * TS, TS)

        ys, last, gates = [], [], []

        def ssm_tile(t):
            rows = pl.ds(t0, TS + 8)
            cr, ci = pl.ds(t * LANE, LANE), pl.ds(PP + t * LANE, LANE)
            co = [co_ref[k, :, cr] for k in range(10)]
            u0 = u_ref[rows, cr]
            u1 = u_ref[rows, ci] if t < FT else pltpu.roll(u0, HALF, 1)
            mul = lambda k, x: (co[k] * x[0] + co[k + 1] * x[1], co[k] * x[1] - co[k + 1] * x[0])
            sub = jax.lax.broadcasted_iota(jnp.int32, (8, LANE), 0)
            s = (st_ref[0, :, cr], st_ref[1, :, cr])
            prev, gs = [None] * 3, []
            for k in range(TS // 8 + 1):
                x0, x1 = u0[8 * k:8 * k + 8], u1[8 * k:8 * k + 8]
                if last:
                    x0 = pltpu.bitcast(after(_as_u32(x0), last[0]), F32)
                w = (co[0] * x0 + co[1] * x1, co[1] * x0 - co[0] * x1)
                for i in range(3):
                    cur = [pltpu.roll(v, 1 << i, 0) for v in w]
                    old = cur if k == 0 else prev[i]
                    d = mul(2 * i + 2, [jnp.where(sub < (1 << i), o, c) for o, c in zip(old, cur)])
                    w = [p + q for p, q in zip(d, w)]
                    prev[i] = cur
                if k > 0:
                    s = [p + q for p, q in zip(mul(8, s), w)]
                    gs.append(jnp.concatenate(s, axis=1) if t < FT else s[0])
                    last[:] = [s[0]]
            st_ref[0, :, cr] = s[0]
            st_ref[1, :, cr] = s[1]
            if t < FT:
                cc = jnp.concatenate([cre_ref[:, cr], cim_ref[:, cr]], axis=1)
            else:
                cc = jnp.concatenate([cre_ref[:, PF:], cim_ref[:, PF:]], axis=1)
            g = jnp.concatenate(gs, axis=0).astype(BF16)
            n = M // 2 if t < FT else M // 4
            y = jnp.concatenate([
                jax.lax.dot_general(_as_bf16(cc[a:a + n]), g, NT_DIMS, preferred_element_type=F32)
                for a in range(0, M // 2, n)], axis=0)
            ys.insert(0, y + ys[0] if ys else y)
            if len(ys) == FT + 1:
                dcol = jnp.concatenate([col_ref[0]] * (TS // LANE), axis=1)
                xt = xt_ref[:, pl.ds(t0, TS)].astype(F32)
                omg = (1.0 - gates[0]).astype(BF16).astype(F32)
                ys_ref[j] = omg * (ys[0] + (xt * dcol).astype(BF16).astype(F32))

        def gate(r):
            q = qs[r]
            gcol = after(_as_u32(col_ref[1]), jnp.concatenate([q[:, :LANE], q[:M - TP, LANE:2 * LANE]], axis=0))
            gcol = jnp.concatenate([pltpu.bitcast(gcol, F32)] * (TS // LANE), axis=1)
            xt = xt_ref[:, pl.ds(t0, TS)].astype(F32)
            z = jnp.sum((xt * gcol).astype(BF16).astype(F32), axis=0, keepdims=True)
            rnd = lambda v: v.astype(BF16).astype(F32)
            g = rnd(1.0 / rnd(1.0 + rnd(jnp.exp(-rnd(z)))))
            g_ref[j] = jnp.broadcast_to(g, (8, TS))
            gates.append(g)

        wq32 = wq_buf[j]
        wq32 = jnp.concatenate([wq32, jnp.zeros((PP - M, D), U32)], axis=0)
        rw = []
        for k in range(7):
            z = (zero << k).astype(U32) if k in Q_REMAT else jnp.uint32(0)
            w0 = pltpu.bitcast(wq32 << (z + 16), F32)
            w1 = pltpu.bitcast(wq32 & (z + jnp.uint32(0xFFFF0000)), F32)
            wl = jnp.concatenate([w0[:, :DH], w1[:, :DH]], axis=1)
            wr = jnp.concatenate([w0[:, DH:], w1[:, DH:]], axis=1)
            rw.append(_strassen_rhs(wl[:XH], wr[:XH], wl[XH:], wr[XH:])[k])
        qscale = (D ** -0.5) * LOG2E
        qs = {}

        def proj_q(r, n=1):
            ms = [None] * 7
            for k in ORDER:
                b = rw[k]
                if k in SUMS:
                    a = lx_ref[SUMS.index(k), pl.ds(r * TH // 2, n * TH // 2), :]
                elif k == 2:
                    a = jnp.concatenate([x_ref[pl.ds(i * TH, TH // 2), pl.ds(0, XH)]
                                         for i in range(r, r + n)], axis=0)
                else:
                    a = jnp.concatenate([x_ref[pl.ds(i * TH + TH // 2, TH // 2), pl.ds(XH, M - XH)]
                                         for i in range(r, r + n)], axis=0)
                    b = b[:M - XH]
                ms[k] = jnp.dot(_as_bf16(a), b.astype(BF16), preferred_element_type=F32)
            for k, v in enumerate(_strassen_out(ms)):
                q_ref[j, k, pl.ds(r * TH, n * TH), :] = (v * qscale).astype(BF16)
            qs[r] = jnp.concatenate(
                [jnp.concatenate([ms[ORDER[p]][:TH], ms[ORDER[p + 1]][:TH]], axis=0) for p in (1, 4)],
                axis=1)

        def c_sums(r):
            c = c_ref[pl.ds(pl.multiple_of(j * TH, TH), TH), :]
            q = qs[r]
            c = after(c, jnp.concatenate([q[:TH], q[TH:]], axis=1))
            c = _as_bf16(c).astype(F32)
            ls = _strassen_lhs(c[:TH, :CH], c[:TH, CH:], c[TH:, :CH], c[TH:, CH:])
            for n, k in enumerate(SUMS):
                l_ref[n, pl.ds(pl.multiple_of(j * (TH // 2), TH // 2), TH // 2), :] = (
                    _as_u32(ls[k].astype(BF16)))

        def wo_sums(r):
            for e in range(2):
                w = after(wot_ref[2 * j + e], qs[r][:MH, e * D:(e + 1) * D])
                w = _as_bf16(w).astype(F32)
                ls = _strassen_lhs(w[:MH, :DH], w[:MH, DH:], w[MH:, :DH], w[MH:, DH:])
                lo_ref[2 * j + e] = jnp.concatenate([ls[k] for k in SUMS], axis=1).astype(BF16)

        ops = dict(q=proj_q, r=lambda r: proj_q(r, 2), m=ssm_tile, c=c_sums, w=wo_sums, g=gate)
        for op in Q_SCHEDULE.split():
            ops[op[0]](int(op[1:]))
        return 0

    assert S // TP == NP
    jax.lax.fori_loop(0, NP, q_step, 0)
    for p in range(NP):
        w_copy(1, p).wait()
        w_copy(2, p).wait()

    def head_step(h, _):
        slot = h >> 1
        zero = zero_ref[0]
        shift = (16 - 16 * (h & 1)).astype(U32)
        rw = []
        for k in range(7):
            sh = shift + (zero << k).astype(U32) if k in REMAT else shift
            wk, wv = _unpack(wk_buf[slot], sh), _unpack(wv_buf[slot], sh)
            wl = jnp.concatenate([wk[:, :DH], wv[:, :DH]], axis=1)
            wr = jnp.concatenate([wk[:, DH:], wv[:, DH:]], axis=1)
            rw.append(_strassen_rhs(wl[:CH], wr[:CH], wl[CH:], wr[CH:])[k])
        causal = (jax.lax.broadcasted_iota(jnp.int32, (TQ, TQ), 1)
                  <= jax.lax.broadcasted_iota(jnp.int32, (TQ, TQ), 0))

        ks, rks, vs, rvs, ss, mxs, chains = [], [], [], [], {}, {}, [None]

        def proj_c(r, cols, n=1):
            ms = [None] * 7
            for k in ORDER:
                if k in SUMS:
                    a = l_ref[SUMS.index(k), pl.ds(r * TH // 2, n * TH // 2), :]
                else:
                    o = 0 if k == 2 else 1
                    a = jnp.concatenate(
                        [c_ref[pl.ds(i * TH + o * TH // 2, TH // 2), pl.ds(o * CH, CH)]
                         for i in range(r, r + n)], axis=0)
                ms[k] = jnp.dot(_as_bf16(a), rw[k][:, cols].astype(BF16), preferred_element_type=F32)
            return _strassen_out(ms)

        def proj_k(r, c=None):
            c11, c12, c21, c22 = c or proj_c(r, slice(0, DH))
            ks.extend([jnp.concatenate([c11, c12], axis=1), jnp.concatenate([c21, c22], axis=1)])
            rks.append(_strassen_rhs(c11, c21, c12, c22))

        def proj_v(r, c=None):
            c11, c12, c21, c22 = c or proj_c(r, slice(DH, D))
            vs.extend([jnp.concatenate([c11, c12], axis=1), jnp.concatenate([c21, c22], axis=1)])
            rvs.append(_strassen_rhs(c11, c12, c21, c22))

        def proj_kv(r, n=1):
            c = proj_c(r, slice(0, D), n)
            for i in range(n):
                proj_k(r + i, [v[i * TH:(i + 1) * TH, :DH] for v in c])
                proj_v(r + i, [v[i * TH:(i + 1) * TH, DH:] for v in c])

        def qk_pair(j):
            cols = pl.ds(pl.multiple_of((h & 1) * DH, DH), DH)
            qf = [q_ref[slot, k, j * TQ:(j + 1) * TQ, cols].astype(F32) for k in range(4)]
            q = jnp.concatenate([jnp.concatenate(qf[:2], axis=1), jnp.concatenate(qf[2:], axis=1)], axis=0)
            lq = _strassen_lhs(*qf)
            s1, s2, done, mx = [], [], [], []

            def diag():
                if UNIFORM_DIAG:
                    return (_dot_nt(q[:TQ].astype(BF16), ks[2 * j].astype(BF16)),
                            _dot_nt(q[TQ:].astype(BF16),
                                    jnp.concatenate(ks[2 * j:2 * j + 2], axis=0).astype(BF16)))
                d = _dot_nt(q.astype(BF16), ks[2 * j].astype(BF16))
                return d[:TQ], jnp.concatenate(
                    [d[TQ:], _dot_nt(q[TQ:].astype(BF16), ks[2 * j + 1].astype(BF16))], axis=1)

            if DIAG_FIRST:
                d1, d2 = diag()
            for t0 in range(0, j, QK_GROUP):
                ts = range(t0, min(t0 + QK_GROUP, j))
                m = [None] * 7
                for k in QK_ORDER:
                    rk = jnp.concatenate([rks[t][k] for t in ts], axis=0).astype(BF16)
                    a = lq[k]
                    if k == QK_TIE_K and len(done) >= QK_LAG:
                        a = tie(a, done[-QK_LAG])
                    m[k] = jax.lax.dot_general(a.astype(BF16), rk, NT_DIMS, preferred_element_type=F32)
                c11 = ((m[0] + m[3]) - m[4]) + m[6]
                c12, c21 = m[2] + m[4], m[1] + m[3]
                c22 = ((m[0] - m[1]) + m[2]) + m[5]
                if QK_RUNMAX:
                    x1, x2 = jnp.maximum(c11, c12), jnp.maximum(c21, c22)
                    if mx:
                        x1, x2 = jnp.maximum(x1, mx[0]), jnp.maximum(x2, mx[1])
                    mx[:] = [x1, x2]
                    z = _as_u32(x1) | _as_u32(x2)
                else:
                    z = (_as_u32(c11) | _as_u32(c12)) | (_as_u32(c21) | _as_u32(c22))
                done.append(z)
                for n in range(len(ts)):
                    cols = slice(n * TQ, (n + 1) * TQ)
                    s1 += [c11[:, cols], c12[:, cols]]
                    s2 += [c21[:, cols], c22[:, cols]]
            if not DIAG_FIRST:
                d1, d2 = diag()
            ss[2 * j] = jnp.concatenate(s1 + [d1], axis=1)
            ss[2 * j + 1] = jnp.concatenate(s2 + [d2], axis=1)
            if mx:
                mxs[2 * j], mxs[2 * j + 1] = mx

        def tie(a, b):
            return pltpu.bitcast(_as_u32(a) | (_as_u32(b) & zero.astype(U32)), F32)

        def exp_rows(s, m, pace, rows, chain=None):
            mb = jnp.broadcast_to(m, (TQ, LANE))
            ps, parts = [], []
            for g in range(0, TQ, rows):
                mg = mb[g:g + rows]
                if pace and (parts or chain is not None):
                    mg = tie(mg, parts[-1] if parts else chain)
                pg = [jnp.exp2(s[g:g + rows, t * LANE:(t + 1) * LANE] - mg)
                      for t in range(s.shape[1] // LANE)]
                ps.append(jnp.concatenate(pg, axis=1))
                parts.append(functools.reduce(lambda a, b: a + b, pg))
            return jnp.concatenate(ps, axis=0), jnp.concatenate(parts, axis=0)

        def scores(i, chain=None):
            lo = i * TQ
            s = ss.pop(i)
            sd = jnp.where(causal, s[:, lo:], -1e9 * LOG2E)
            s = sd if i == 0 else jnp.concatenate([s[:, :lo], sd], axis=1)
            if i in mxs:
                lo2 = i // 2 * 2 * TQ
                m = jnp.max(jnp.concatenate([mxs[i], s[:, lo2:]], axis=1), axis=-1, keepdims=True)
            else:
                m = jnp.max(s, axis=-1, keepdims=True)
            p, part = exp_rows(s, m, i >= PACE_FROM, PACE_ROWS, chain)
            return s, m, p, jnp.sum(part, axis=-1, keepdims=True), part[TQ - PACE_ROWS:]

        def pv(j):
            s1, m1, p1, l1, chain = scores(2 * j, chains[0] if CHAIN_ALL else None)
            s2, m2, p2, l2, chains[0] = scores(2 * j + 1, chain if CHAIN else None)
            lo = 2 * j * TQ
            cat = lambda xs, axis: jnp.concatenate(xs, axis=axis)
            dot = lambda a, b: jnp.dot(a.astype(BF16), b.astype(BF16), preferred_element_type=F32)

            def recip(l):
                rl = pl.reciprocal(l, approx=True)
                return rl * (2.0 - l * rl)

            r1, r2 = recip(l1), recip(l2)
            if UNIFORM_DIAG:
                c1 = dot(p1[:, lo:], vs[2 * j])
                c2 = dot(p2[:, lo:], cat(vs[2 * j:2 * j + 2], 0))
            else:
                dg = dot(cat([p1[:, lo:], p2[:, lo:lo + TQ]], 0), vs[2 * j])
                c1, c2 = dg[:TQ], dg[TQ:] + dot(p2[:, lo + TQ:], vs[2 * j + 1])
            if j > 0:
                tiles = lambda p, o: cat([p[:, (2 * t + o) * TQ:(2 * t + o + 1) * TQ] for t in range(j)], 1)
                a11, a12, a21, a22 = tiles(p1, 0), tiles(p1, 1), tiles(p2, 0), tiles(p2, 1)
                rho = l1 * r2
                a22r = a22 * rho
                lp = [a11 + a22r, a21 + a22, a11, a22, a11 + a12, a21 * rho - a11, a12 - a22r]
                m = [None] * 7
                for k in PV_ORDER:
                    if k == PV_ORDER[-1]:
                        yield
                    m[k] = dot(lp[k], cat([rvs[t][k] for t in range(j)], 0))
                c1 = c1 + cat([(m[0] - m[4]) + (m[6] + m[3] * rho), m[2] + m[4]], 1)
                c2 = (c2 + cat([m[1] + m[3], -m[1]], 1)) * r2
                c2 = cat([c2[:, :DH], c2[:, DH:] + ((m[0] + m[2]) + m[5]) * r1], 1)
            else:
                c2 = c2 * r2
            c1 = c1 * r1
            ctx_ref[h, j * TQ:(j + 1) * TQ, :] = cat(
                _strassen_rhs(c1[:, :DH], c2[:, :DH], c1[:, DH:], c2[:, DH:]), 1).astype(BF16)

        assert TP == 2 * TQ
        pvs = [pv(j) for j in range(S // TP)]
        ops = dict(c=proj_kv, d=lambda r: proj_kv(r, 2), k=proj_k, v=proj_v, t=qk_pair, p=lambda j: list(pvs[j]),
                   b=lambda j: next(pvs[j]))
        for op in SCHEDULE.split():
            ops[op[0]](int(op[1:]))
        return 0

    jax.lax.fori_loop(0, H, head_step, 0)

    def o_copy(j, slot):
        return pltpu.make_async_copy(o_buf.at[slot], o_hbm.at[:, pl.ds(j * TO, TO)], osem.at[slot])

    def o_step(j, _):
        slot = j & 1

        @pl.when(j >= 2)
        def _():
            o_copy(j - 2, slot).wait()

        rows = pl.ds(pl.multiple_of(j * TQ, TQ), TQ)
        ms = [None] * 7
        for k in range(7):
            if k in SUMS:
                a = [lo_ref[n, :, pl.ds(SUMS.index(k) * DH, DH)] for n in range(H)]
            elif k == 2:
                a = [_as_bf16(wot_ref[n, pl.ds(0, MH // 2), pl.ds(0, DH)]) for n in range(H)]
            else:
                a = [_as_bf16(wot_ref[n, pl.ds(MH // 2, MH // 2), pl.ds(DH, DH)]) for n in range(H)]
            b = [ctx_ref[n, rows, pl.ds(k * DH, DH)] for n in range(H)]
            ms[k] = _dot_nt(jnp.concatenate(a, axis=1), jnp.concatenate(b, axis=1))
        c11, c12, c21, c22 = _strassen_out(ms)
        at = jnp.concatenate([jnp.concatenate([c11, c12], axis=1),
                              jnp.concatenate([c21, c22], axis=1)], axis=0)
        o_buf[slot] = g_ref[j, 0:1, :] * at + ys_ref[j]
        o_copy(j, slot).start()
        return 0

    assert TO == 2 * TQ and TO == TS
    no = S // TO
    jax.lax.fori_loop(0, no, o_step, 0)
    o_copy(no - 2, no % 2).wait()
    o_copy(no - 1, (no - 1) % 2).wait()


@jax.jit
def pallas_gated_mix__compressed_kv_cla__ssm_conv_s5__prompt_kernel(
    A_x: jax.Array,
    A_c_kv: jax.Array,
    A_w_q: jax.Array,
    A_w_uk: jax.Array,
    A_w_uv: jax.Array,
    A_w_o: jax.Array,
    B_x: jax.Array,
    B_Lambda_re: jax.Array,
    B_Lambda_im: jax.Array,
    B_B_re: jax.Array,
    B_B_im: jax.Array,
    B_C_re: jax.Array,
    B_C_im: jax.Array,
    B_log_dt: jax.Array,
    B_Dskip: jax.Array,
    gate_w: jax.Array,
):
    del B_x
    _, S, M = A_x.shape
    C = A_c_kv.shape[2]
    H, D = A_w_q.shape[1], A_w_q.shape[2]
    PP = (M + LANE - 1) // LANE * LANE

    hbm = pl.BlockSpec(memory_space=pl.ANY)
    out_t = pl.pallas_call(
        functools.partial(_kernel, S=S, M=M, H=H, D=D),
        in_specs=[hbm] * 15,
        out_specs=hbm,
        out_shape=jax.ShapeDtypeStruct((M, S), F32),
        scratch_shapes=[
            pltpu.VMEM((M, S), BF16),
            pltpu.VMEM((S // 2, M), U32),
            pltpu.VMEM((5, S // 4, PP // 2), U32),
            pltpu.VMEM((S // 2, C), U32),
            pltpu.VMEM((5, S // 4, C // 2), U32),
            pltpu.VMEM((H // 2, M, D), U32),
            pltpu.VMEM((H // 2, C, D), U32),
            pltpu.VMEM((H // 2, C, D), U32),
            pltpu.VMEM((H, M // 2, D), U32),
            pltpu.VMEM((H, M // 2, 5 * D // 2), BF16),
            pltpu.VMEM((M, M), U32),
            pltpu.VMEM((M // 2, M), U32),
            pltpu.VMEM((M // 2, M), U32),
            pltpu.VMEM((S + 8, 2 * M), F32),
            pltpu.VMEM((S // TO, M, TO), F32),
            pltpu.VMEM((S // TO, 8, TO), F32),
            pltpu.VMEM((2, 8, PP), F32),
            pltpu.VMEM((10, 8, PP), F32),
            pltpu.VMEM((2, M, LANE), F32),
        ] + [pltpu.VMEM((M,), BF16)] * 5 + [
            pltpu.VMEM((H // 2, 4, S // 2, D), BF16),
            pltpu.VMEM((H, S // 2, 7 * D // 2), BF16),
            pltpu.VMEM((2, M, TO), F32),
            pltpu.SMEM((1,), jnp.int32),
            pltpu.SemaphoreType.DMA((5, H // 2)),
            pltpu.SemaphoreType.DMA((4,)),
            pltpu.SemaphoreType.DMA((5,)),
            pltpu.SemaphoreType.DMA((5,)),
            pltpu.SemaphoreType.DMA((2,)),
        ],
        compiler_params=pltpu.CompilerParams(
            vmem_limit_bytes=124 * 1024 * 1024,
            disable_semaphore_checks=True,
            disable_bounds_checks=True,
        ),
    )(
        jnp.swapaxes(A_x, 1, 2).reshape(M, S), A_c_kv.reshape(S, C),
        A_w_q, A_w_uk, A_w_uv, jnp.swapaxes(A_w_o, 1, 2),
        B_B_re, B_B_im, B_C_re, B_C_im,
        B_Lambda_re, B_Lambda_im, B_log_dt, B_Dskip, gate_w,
    )
    return jnp.swapaxes(out_t.reshape(1, M, S), 1, 2)
```

```python
import functools

import jax
import jax.numpy as jnp
import jax.experimental.pallas as pl
import jax.experimental.pallas.tpu as pltpu

F32 = jnp.float32
BF16 = jnp.bfloat16
U32 = jnp.uint32

NT_DIMS = (((1,), (1,)), ((), ()))
LOG2E = 1.4426950408889634

TQ = 128
TP = 256
TU = 512
TO = 256
LANE = 128
HALF = LANE // 2
SSM_SPLIT = False
REMAT = (0, 1, 2, 3, 4, 5, 6)
Q_REMAT = (1,)
UNIFORM_DIAG = False
SCHEDULE = "d0 h2 t0 t1 c2 p0 p1 t2 c3 p2 t3 c4 p3 t4 c5 p4 t5 c6 b5 t6 c7 t7 p5 p6 p7"
Q_SCHEDULE = "q0 q1 g1 q2 m3 q3 m0 q4 m1 q5 m2 q6 c6 q7 w7"
PACE_FROM = 4
PACE_ROWS = 8
TWO_PASS = False
CHAIN_ALL = False
CHAIN = True
PACE2_FROM = 2
PACE2_EXTRA = 1


def _dot_nt(a, b):
    return jax.lax.dot_general(a, b, NT_DIMS, preferred_element_type=F32)


def _unpack(w32, shift):
    v = (w32 << shift) & jnp.uint32(0xFFFF0000)
    return pltpu.bitcast(v, F32)


def _as_bf16(w32):
    return pltpu.bitcast(w32, BF16)


def _as_u32(v):
    return pltpu.bitcast(v, U32)


def _strassen_lhs(a11, a12, a21, a22):
    return [a11 + a22, a21 + a22, a11, a22, a11 + a12, a21 - a11, a12 - a22]


def _strassen_rhs(b11, b12, b21, b22):
    return [b11 + b22, b11, b12 - b22, b21 - b11, b22, b11 + b12, b21 + b22]


def _strassen_out(m):
    return ((m[0] + m[3]) + (m[6] - m[4]), m[2] + m[4],
            m[1] + m[3], (m[0] - m[1]) + (m[2] + m[5]))


def _quads(a):
    m, n = a.shape[0] // 2, a.shape[1] // 2
    return a[:m, :n], a[:m, n:], a[m:, :n], a[m:, n:]


SUMS = (0, 1, 4, 5, 6)
ORDER = (1, 4, 0, 2, 3, 5, 6)
INNER = (1, 3, 4, 2, 0, 6, 5)
QK_ORDER = (0, 3, 4, 6, 1, 2, 5)
QK_GROUP = 1
QK_LAG = 2
QK_TIE_K = 3
QK_RUNMAX = True
DIAG_FIRST = False
PV_ORDER = (2, 4, 3, 1, 5, 0, 6)


def _kernel(xt_hbm, c_hbm, wq_hbm, wuk_hbm, wuv_hbm, wot_hbm,
            bre_hbm, bim_hbm, cre_hbm, cim_hbm,
            lre_hbm, lim_hbm, ldt_hbm, dsk_hbm, gw_hbm,
            o_hbm,
            xt_ref, x_ref, lx_ref, c_ref, l_ref, wq_buf, wk_buf, wv_buf, wot_ref, lo_ref,
            b_ref, cre_ref, cim_ref, u_ref, ys_ref, g_ref, st_ref, co_ref, col_ref, smp_ref, vsc_ref,
            lre_ref, lim_ref, ldt_ref, dsk_ref, gw_ref,
            q_ref, ctx_ref, o_buf, zero_ref, wsem, xsem, msem, vsem, osem,
            *, S, M, H, D):
    P = M
    FT = P // LANE
    PF = FT * LANE
    assert P - PF == HALF
    PP = PF + LANE
    NP = H // 2
    TS = S // NP
    CH, DH, MH, TH = c_ref.shape[1] // 2, D // 2, M // 2, TP // 2

    def w_copy(k, pair):
        src, dst = ((wq_hbm, wq_buf), (wuk_hbm, wk_buf), (wuv_hbm, wv_buf))[k]
        return pltpu.make_async_copy(src.bitcast(U32).at[:, pair, :], dst.at[pair], wsem.at[k, pair])

    def wo_copy(pair):
        heads = pl.ds(2 * pair, 2)
        return pltpu.make_async_copy(wot_hbm.bitcast(U32).at[heads], wot_ref.at[heads],
                                     wsem.at[3, pair])

    def x_copy(t0, n, k):
        cols = pl.ds(t0, n)
        return pltpu.make_async_copy(xt_hbm.at[:, cols], xt_ref.at[:, cols], xsem.at[k])

    x_cps = [x_copy(0, TU // 2, 0), x_copy(TU // 2, TU // 2, 1), x_copy(TU, TU, 2),
             x_copy(2 * TU, S - 2 * TU, 3)]

    bre32, bim32 = bre_hbm.bitcast(U32), bim_hbm.bitcast(U32)
    b_cps = [
        pltpu.make_async_copy(bre32, b_ref.at[pl.ds(0, P // 2), :], msem.at[0]),
        pltpu.make_async_copy(bim32.at[pl.ds(PF // 2, HALF // 2), :],
                              b_ref.at[pl.ds(P // 2, HALF // 2), :], msem.at[1]),
        pltpu.make_async_copy(bim32.at[pl.ds(0, PF // 2), :],
                              b_ref.at[pl.ds(PP // 2, PF // 2), :], msem.at[2]),
    ]
    cre_cp = pltpu.make_async_copy(cre_hbm.bitcast(U32), cre_ref, msem.at[3])
    cim_cp = pltpu.make_async_copy(cim_hbm.bitcast(U32), cim_ref, msem.at[4])

    def c_copy(r):
        rows = pl.ds(pl.multiple_of(r * TH, TH), TH)
        return pltpu.make_async_copy(c_hbm.bitcast(U32).at[rows], c_ref.at[rows], wsem.at[4, r])

    smp_cps = [pltpu.make_async_copy(src.bitcast(U32).at[pl.ds(0, smp_ref.shape[1])],
                                     smp_ref.at[k], msem.at[5 + k])
               for k, src in enumerate((wuk_hbm, wuv_hbm))]
    v_cps = [pltpu.make_async_copy(src, dst, vsem.at[k]) for k, (src, dst) in enumerate(
        ((lre_hbm, lre_ref), (lim_hbm, lim_ref), (ldt_hbm, ldt_ref),
         (dsk_hbm, dsk_ref), (gw_hbm, gw_ref)))]

    for cp in v_cps:
        cp.start()
    for cp in x_cps[:1] + b_cps + x_cps[1:] + smp_cps:
        cp.start()
    cre_cp.start()
    cim_cp.start()
    for p in range(NP):
        w_copy(0, p).start()
        wo_copy(p).start()
        c_copy(p).start()
    for p in range(NP):
        w_copy(1, p).start()
        w_copy(2, p).start()

    zero_ref[0] = 0
    u_ref[pl.ds(0, 8), :] = jnp.zeros((8, u_ref.shape[1]), F32)
    st_ref[...] = jnp.zeros(st_ref.shape, F32)
    for cp in v_cps:
        cp.wait()

    row = lambda r: r[...].astype(F32).reshape(1, P)
    lre, lim = row(lre_ref), row(lim_ref)
    dt = jnp.exp(row(ldt_ref)).astype(BF16).astype(F32)
    e = jnp.exp(dt * lre)
    ang = dt * lim
    ar = e * jnp.cos(ang)
    ai = e * jnp.sin(ang)
    sc = jnp.maximum(jnp.abs(lre), jnp.abs(lim))
    nre, nim = lre / sc, lim / sc
    den = (nre * nre + nim * nim) * sc
    gr = 2.0 * ((ar - 1.0) * nre + ai * nim) / den
    gi = 2.0 * (ai * nre - (ar - 1.0) * nim) / den

    def put(k, full, lo, hi):
        v = jnp.concatenate([full[:, :PF], lo[:, PF:], hi[:, PF:]], axis=1)
        co_ref[k] = jnp.broadcast_to(v, (8, PP))

    put(0, gr, gr, -gr)
    put(1, -gi, -gi, -gi)
    pr, pi = ar, -ai
    for j in range(1, 5):
        put(2 * j, pr, pr, pr)
        put(2 * j + 1, -pi, -pi, pi)
        pr, pi = pr * pr - pi * pi, 2.0 * pr * pi

    zpad = jnp.zeros((1, PP - P), F32)
    for k, r in enumerate((dsk_ref, gw_ref)):
        v = jnp.concatenate([row(r), zpad], axis=1)
        col_ref[k] = jnp.broadcast_to(v, (LANE, PP)).T[:M]

    XH = PP // 2

    def transpose_x(t0, n):
        x_ref[pl.ds(t0 // 2, n // 2), :] = _as_u32(xt_ref[:, pl.ds(t0, n)].T)

    def x_sums(r, after):
        x = x_ref[pl.ds(r * TH, TH), :] | (_as_u32(after) & zero_ref[0].astype(U32))
        x = _as_bf16(x).astype(F32)
        x = jnp.concatenate([x, jnp.zeros((TP, PP - M), F32)], axis=1)
        ls = _strassen_lhs(x[:TH, :XH], x[:TH, XH:], x[TH:, :XH], x[TH:, XH:])
        for n, k in enumerate(SUMS):
            lx_ref[n, pl.ds(r * TH // 2, TH // 2), :] = _as_u32(ls[k].astype(BF16))

    def proj_u(t0, n, lo=0, hi=2 * P, sums=()):
        u = _dot_nt(_as_bf16(x_ref[pl.ds(t0 // 2, n // 2), :]), _as_bf16(b_ref[lo // 2:hi // 2, :]))
        u_ref[pl.ds(t0 + 8, n), lo:hi] = u
        for i, r in enumerate(sums):
            a = u[:, (2 * i + 1) * LANE:(2 * i + 2) * LANE]
            a = jnp.concatenate([a[k * TH:(k + 1) * TH] for k in range(4)], axis=1)
            x_sums(r, a[:, :M])

    x_cps[0].wait()
    transpose_x(0, TU // 2)
    b_cps[0].wait()
    b_cps[1].wait()
    proj_u(0, TU // 2, 0, PP)
    b_cps[2].wait()
    x_cps[1].wait()
    proj_u(0, TU // 2, PP)
    transpose_x(TU // 2, TU // 2)
    x_cps[2].wait()
    proj_u(TU // 2, TU // 2)
    transpose_x(TU, TU)
    x_cps[3].wait()
    for cp in smp_cps:
        cp.wait()
    for e in range(2):
        mag = [jnp.sum(jnp.sum(jnp.abs(_unpack(smp_ref[k], jnp.uint32(16 - 16 * e))), axis=0),
                       axis=1, keepdims=True) for k in range(2)]
        ex = [jnp.broadcast_to(pltpu.bitcast(v, jnp.int32) >> 23, (NP, LANE)) for v in mag]
        d = jnp.where((ex[0] > 0) & (ex[1] > 0), jnp.clip(ex[0] - ex[1], -40, 40), 0)
        vsc_ref[0, e] = pltpu.bitcast((127 + d) << 23, F32)
        vsc_ref[1, e] = pltpu.bitcast((127 - d) << 23, F32)
    for t0 in range(TU, S, TU):
        proj_u(t0, TU, sums={1: (0, 1, 2), 2: (3, 4, 5), 3: (6, 7)}[t0 // TU])
        if t0 + TU < S:
            transpose_x(t0 + TU, TU)
    cre_cp.wait()
    cim_cp.wait()

    def q_step(j, _):
        w_copy(0, j).wait()
        wo_copy(j).wait()
        c_copy(j).wait()
        zero = zero_ref[0]
        after = lambda w, v: w | (_as_u32(v) & zero.astype(U32))
        t0 = pl.multiple_of(j * TS, TS)

        ys, last, gates = [], [], []

        def ssm_tile(t):
            rows = pl.ds(t0, TS + 8)
            cr, ci = pl.ds(t * LANE, LANE), pl.ds(PP + t * LANE, LANE)
            co = [co_ref[k, :, cr] for k in range(10)]
            u0 = u_ref[rows, cr]
            u1 = u_ref[rows, ci] if t < FT else pltpu.roll(u0, HALF, 1)
            mul = lambda k, x: (co[k] * x[0] + co[k + 1] * x[1], co[k] * x[1] - co[k + 1] * x[0])
            sub = jax.lax.broadcasted_iota(jnp.int32, (8, LANE), 0)
            s = (st_ref[0, :, cr], st_ref[1, :, cr])
            prev, gs = [None] * 3, []
            for k in range(TS // 8 + 1):
                x0, x1 = u0[8 * k:8 * k + 8], u1[8 * k:8 * k + 8]
                if last:
                    x0 = pltpu.bitcast(after(_as_u32(x0), last[0]), F32)
                w = (co[0] * x0 + co[1] * x1, co[1] * x0 - co[0] * x1)
                for i in range(3):
                    cur = [pltpu.roll(v, 1 << i, 0) for v in w]
                    old = cur if k == 0 else prev[i]
                    d = mul(2 * i + 2, [jnp.where(sub < (1 << i), o, c) for o, c in zip(old, cur)])
                    w = [p + q for p, q in zip(d, w)]
                    prev[i] = cur
                if k > 0:
                    s = [p + q for p, q in zip(mul(8, s), w)]
                    gs.append(jnp.concatenate(s, axis=1) if t < FT else s[0])
                    last[:] = [s[0]]
            st_ref[0, :, cr] = s[0]
            st_ref[1, :, cr] = s[1]
            if t < FT:
                cc = jnp.concatenate([cre_ref[:, cr], cim_ref[:, cr]], axis=1)
            else:
                cc = jnp.concatenate([cre_ref[:, PF:], cim_ref[:, PF:]], axis=1)
            g = jnp.concatenate(gs, axis=0).astype(BF16)
            n = M // 2 if t < FT else M // 4
            y = jnp.concatenate([
                jax.lax.dot_general(_as_bf16(cc[a:a + n]), g, NT_DIMS, preferred_element_type=F32)
                for a in range(0, M // 2, n)], axis=0)
            ys.insert(0, y + ys[0] if ys else y)
            if len(ys) == FT + 1:
                dcol = jnp.concatenate([col_ref[0]] * (TS // LANE), axis=1)
                xt = xt_ref[:, pl.ds(t0, TS)].astype(F32)
                omg = (1.0 - gates[0]).astype(BF16).astype(F32)
                ys_ref[j] = omg * (ys[0] + (xt * dcol).astype(BF16).astype(F32))

        def gate(r):
            q = qs[r]
            gcol = after(_as_u32(col_ref[1]), jnp.concatenate([q[:, :LANE], q[:M - TP, LANE:2 * LANE]], axis=0))
            gcol = jnp.concatenate([pltpu.bitcast(gcol, F32)] * (TS // LANE), axis=1)
            xt = xt_ref[:, pl.ds(t0, TS)].astype(F32)
            z = jnp.sum((xt * gcol).astype(BF16).astype(F32), axis=0, keepdims=True)
            rnd = lambda v: v.astype(BF16).astype(F32)
            g = rnd(1.0 / rnd(1.0 + rnd(jnp.exp(-rnd(z)))))
            g_ref[j] = jnp.broadcast_to(g, (8, TS))
            gates.append(g)

        wq32 = wq_buf[j]
        wq32 = jnp.concatenate([wq32, jnp.zeros((PP - M, D), U32)], axis=0)
        rw = []
        for k in range(7):
            z = (zero << k).astype(U32) if k in Q_REMAT else jnp.uint32(0)
            w0 = pltpu.bitcast(wq32 << (z + 16), F32)
            w1 = pltpu.bitcast(wq32 & (z + jnp.uint32(0xFFFF0000)), F32)
            wl = jnp.concatenate([w0[:, :DH], w1[:, :DH]], axis=1)
            wr = jnp.concatenate([w0[:, DH:], w1[:, DH:]], axis=1)
            rw.append(_strassen_rhs(wl[:XH], wr[:XH], wl[XH:], wr[XH:])[k])
        qscale = (D ** -0.5) * LOG2E
        qs = {}

        def proj_q(r, n=1):
            ms = [None] * 7
            for k in ORDER:
                b = rw[k]
                if k in SUMS:
                    a = lx_ref[SUMS.index(k), pl.ds(r * TH // 2, n * TH // 2), :]
                elif k == 2:
                    a = jnp.concatenate([x_ref[pl.ds(i * TH, TH // 2), pl.ds(0, XH)]
                                         for i in range(r, r + n)], axis=0)
                else:
                    a = jnp.concatenate([x_ref[pl.ds(i * TH + TH // 2, TH // 2), pl.ds(XH, M - XH)]
                                         for i in range(r, r + n)], axis=0)
                    b = b[:M - XH]
                ms[k] = jnp.dot(_as_bf16(a), b.astype(BF16), preferred_element_type=F32)
            for k, v in enumerate(_strassen_out(ms)):
                q_ref[j, k, pl.ds(r * TH, n * TH), :] = (v * qscale).astype(BF16)
            qs[r] = jnp.concatenate(
                [jnp.concatenate([ms[ORDER[p]][:TH], ms[ORDER[p + 1]][:TH]], axis=0) for p in (1, 4)],
                axis=1)

        def c_sums(r):
            c = c_ref[pl.ds(pl.multiple_of(j * TH, TH), TH), :]
            q = qs[r]
            c = after(c, jnp.concatenate([q[:TH], q[TH:]], axis=1))
            c = _as_bf16(c).astype(F32)
            rows = pl.ds(pl.multiple_of(j * (TH // 4), TH // 4), TH // 4)
            for k, l in enumerate(_strassen_lhs(*_quads(c))):
                for i, v in enumerate(_strassen_lhs(*_quads(l))):
                    l_ref[7 * k + i, rows, :] = _as_u32(v.astype(BF16))

        def wo_sums(r):
            for e in range(2):
                w = after(wot_ref[2 * j + e], qs[r][:MH, e * D:(e + 1) * D])
                w = _as_bf16(w).astype(F32)
                ls = _strassen_lhs(w[:MH, :DH], w[:MH, DH:], w[MH:, :DH], w[MH:, DH:])
                lo_ref[2 * j + e] = jnp.concatenate([ls[k] for k in SUMS], axis=1).astype(BF16)

        ops = dict(q=proj_q, r=lambda r: proj_q(r, 2), m=ssm_tile, c=c_sums, w=wo_sums, g=gate)
        for op in Q_SCHEDULE.split():
            ops[op[0]](int(op[1:]))
        return 0

    assert S // TP == NP
    jax.lax.fori_loop(0, NP, q_step, 0)
    for p in range(NP):
        w_copy(1, p).wait()
        w_copy(2, p).wait()

    def head_step(h, _):
        slot = h >> 1
        zero = zero_ref[0]
        shift = (16 - 16 * (h & 1)).astype(U32)
        vscale, vinv = [vsc_ref[k, h & 1, pl.ds(slot, 1), :] for k in range(2)]
        rw = []
        for k in range(7):
            sh = shift + (zero << k).astype(U32) if k in REMAT else shift
            rk = _strassen_rhs(*_quads(_unpack(wk_buf[slot], sh)))[k]
            rv = _strassen_rhs(*_quads(_unpack(wv_buf[slot], sh)))[k] * vscale
            rw.append(_strassen_rhs(rk[:CH // 2], rv[:CH // 2], rk[CH // 2:], rv[CH // 2:]))
        causal = (jax.lax.broadcasted_iota(jnp.int32, (TQ, TQ), 1)
                  <= jax.lax.broadcasted_iota(jnp.int32, (TQ, TQ), 0))

        ks, rks, vs, rvs, ss, mxs, chains = [], [], [], [], {}, {}, [None]

        def proj_kv(r, n=1):
            TI = TH // 2
            ms = [None] * 7
            for k in ORDER:
                mi = [None] * 7
                for i in INNER:
                    a = l_ref[7 * k + i, pl.ds(r * TI // 2, n * TI // 2), :]
                    mi[i] = jnp.dot(_as_bf16(a), rw[k][i].astype(BF16), preferred_element_type=F32)
                c11, c12, c21, c22 = _strassen_out(mi)
                top, bot = jnp.concatenate([c11, c12], axis=1), jnp.concatenate([c21, c22], axis=1)
                ms[k] = jnp.concatenate(
                    [v[b * TI:(b + 1) * TI] for b in range(n) for v in (top, bot)], axis=0)
                if k != ORDER[-1]:
                    yield
            c = _strassen_out(ms)
            for b in range(n):
                c11, c12, c21, c22 = [v[b * TH:(b + 1) * TH, :DH] for v in c]
                ks.extend([jnp.concatenate([c11, c12], axis=1), jnp.concatenate([c21, c22], axis=1)])
                rks.append(_strassen_rhs(c11, c21, c12, c22))
                c11, c12, c21, c22 = [v[b * TH:(b + 1) * TH, DH:] for v in c]
                vs.extend([jnp.concatenate([c11, c12], axis=1), jnp.concatenate([c21, c22], axis=1)])
                rvs.append(_strassen_rhs(c11, c12, c21, c22))

        def qk_pair(j):
            cols = pl.ds(pl.multiple_of((h & 1) * DH, DH), DH)
            qf = [q_ref[slot, k, j * TQ:(j + 1) * TQ, cols].astype(F32) for k in range(4)]
            q = jnp.concatenate([jnp.concatenate(qf[:2], axis=1), jnp.concatenate(qf[2:], axis=1)], axis=0)
            lq = _strassen_lhs(*qf)
            s1, s2, done, mx = [], [], [], []

            def diag():
                if UNIFORM_DIAG:
                    return (_dot_nt(q[:TQ].astype(BF16), ks[2 * j].astype(BF16)),
                            _dot_nt(q[TQ:].astype(BF16),
                                    jnp.concatenate(ks[2 * j:2 * j + 2], axis=0).astype(BF16)))
                d = _dot_nt(q.astype(BF16), ks[2 * j].astype(BF16))
                return d[:TQ], jnp.concatenate(
                    [d[TQ:], _dot_nt(q[TQ:].astype(BF16), ks[2 * j + 1].astype(BF16))], axis=1)

            if DIAG_FIRST:
                d1, d2 = diag()
            for t0 in range(0, j, QK_GROUP):
                ts = range(t0, min(t0 + QK_GROUP, j))
                m = [None] * 7
                for k in QK_ORDER:
                    rk = jnp.concatenate([rks[t][k] for t in ts], axis=0).astype(BF16)
                    a = lq[k]
                    if k == QK_TIE_K and len(done) >= QK_LAG:
                        a = tie(a, done[-QK_LAG])
                    m[k] = jax.lax.dot_general(a.astype(BF16), rk, NT_DIMS, preferred_element_type=F32)
                c11 = ((m[0] + m[3]) - m[4]) + m[6]
                c12, c21 = m[2] + m[4], m[1] + m[3]
                c22 = ((m[0] - m[1]) + m[2]) + m[5]
                if QK_RUNMAX:
                    x1, x2 = jnp.maximum(c11, c12), jnp.maximum(c21, c22)
                    if mx:
                        x1, x2 = jnp.maximum(x1, mx[0]), jnp.maximum(x2, mx[1])
                    mx[:] = [x1, x2]
                    z = _as_u32(x1) | _as_u32(x2)
                else:
                    z = (_as_u32(c11) | _as_u32(c12)) | (_as_u32(c21) | _as_u32(c22))
                done.append(z)
                for n in range(len(ts)):
                    cols = slice(n * TQ, (n + 1) * TQ)
                    s1 += [c11[:, cols], c12[:, cols]]
                    s2 += [c21[:, cols], c22[:, cols]]
            if not DIAG_FIRST:
                d1, d2 = diag()
            ss[2 * j] = jnp.concatenate(s1 + [d1], axis=1)
            ss[2 * j + 1] = jnp.concatenate(s2 + [d2], axis=1)
            if mx:
                mxs[2 * j], mxs[2 * j + 1] = mx

        def tie(a, b):
            return pltpu.bitcast(_as_u32(a) | (_as_u32(b) & zero.astype(U32)), F32)

        def exp_rows(s, m, pace, rows, chain=None):
            mb = jnp.broadcast_to(m, (TQ, LANE))
            ps, parts = [], []
            for g in range(0, TQ, rows):
                mg = mb[g:g + rows]
                if pace and (parts or chain is not None):
                    mg = tie(mg, parts[-1] if parts else chain)
                pg = [jnp.exp2(s[g:g + rows, t * LANE:(t + 1) * LANE] - mg)
                      for t in range(s.shape[1] // LANE)]
                ps.append(jnp.concatenate(pg, axis=1))
                parts.append(functools.reduce(lambda a, b: a + b, pg))
            return jnp.concatenate(ps, axis=0), jnp.concatenate(parts, axis=0)

        def scores(i, chain=None):
            lo = i * TQ
            s = ss.pop(i)
            sd = jnp.where(causal, s[:, lo:], -1e9 * LOG2E)
            s = sd if i == 0 else jnp.concatenate([s[:, :lo], sd], axis=1)
            if i in mxs:
                lo2 = i // 2 * 2 * TQ
                m = jnp.max(jnp.concatenate([mxs[i], s[:, lo2:]], axis=1), axis=-1, keepdims=True)
            else:
                m = jnp.max(s, axis=-1, keepdims=True)
            p, part = exp_rows(s, m, i >= PACE_FROM, PACE_ROWS, chain)
            return s, m, p, jnp.sum(part, axis=-1, keepdims=True), part[TQ - PACE_ROWS:]

        def pv(j):
            s1, m1, p1, l1, chain = scores(2 * j, chains[0] if CHAIN_ALL else None)
            s2, m2, p2, l2, chains[0] = scores(2 * j + 1, chain if CHAIN else None)
            lo = 2 * j * TQ
            cat = lambda xs, axis: jnp.concatenate(xs, axis=axis)
            dot = lambda a, b: jnp.dot(a.astype(BF16), b.astype(BF16), preferred_element_type=F32)

            def recip(l):
                rl = pl.reciprocal(l, approx=True)
                return rl * (2.0 - l * rl)

            r1, r2 = recip(l1), recip(l2)
            rho = l1 * r2
            r1, r2 = r1 * vinv, r2 * vinv
            if UNIFORM_DIAG:
                c1 = dot(p1[:, lo:], vs[2 * j])
                c2 = dot(p2[:, lo:], cat(vs[2 * j:2 * j + 2], 0))
            else:
                dg = dot(cat([p1[:, lo:], p2[:, lo:lo + TQ]], 0), vs[2 * j])
                c1, c2 = dg[:TQ], dg[TQ:] + dot(p2[:, lo + TQ:], vs[2 * j + 1])
            if j > 0:
                tiles = lambda p, o: cat([p[:, (2 * t + o) * TQ:(2 * t + o + 1) * TQ] for t in range(j)], 1)
                a11, a12, a21, a22 = tiles(p1, 0), tiles(p1, 1), tiles(p2, 0), tiles(p2, 1)
                a22r = a22 * rho
                lp = [a11 + a22r, a21 + a22, a11, a22, a11 + a12, a21 * rho - a11, a12 - a22r]
                m = [None] * 7
                for k in PV_ORDER:
                    if k == PV_ORDER[-1]:
                        yield
                    m[k] = dot(lp[k], cat([rvs[t][k] for t in range(j)], 0))
                c1 = c1 + cat([(m[0] - m[4]) + (m[6] + m[3] * rho), m[2] + m[4]], 1)
                c2 = (c2 + cat([m[1] + m[3], -m[1]], 1)) * cat([r2, r2], 1)
                c2 = cat([c2[:, :DH], c2[:, DH:] + ((m[0] + m[2]) + m[5]) * r1], 1)
            else:
                c2 = c2 * cat([r2, r2], 1)
            c1 = c1 * cat([r1, r1], 1)
            ctx_ref[h, j * TQ:(j + 1) * TQ, :] = cat(
                _strassen_rhs(c1[:, :DH], c2[:, :DH], c1[:, DH:], c2[:, DH:]), 1).astype(BF16)

        assert TP == 2 * TQ
        pvs = [pv(j) for j in range(S // TP)]
        kvs = {}

        def kv_part(r, n, steps):
            g = kvs.setdefault(r, proj_kv(r, n))
            for _ in range(steps):
                next(g, None)

        ops = dict(c=lambda r: kv_part(r, 1, 7), d=lambda r: kv_part(r, 2, 7),
                   h=lambda r: kv_part(r, 1, 4), g=lambda r: kv_part(r, 2, 4),
                   t=qk_pair, p=lambda j: list(pvs[j]), b=lambda j: next(pvs[j]))
        for op in SCHEDULE.split():
            ops[op[0]](int(op[1:]))
        return 0

    jax.lax.fori_loop(0, H, head_step, 0)

    def o_copy(j, slot):
        return pltpu.make_async_copy(o_buf.at[slot], o_hbm.at[:, pl.ds(j * TO, TO)], osem.at[slot])

    def o_step(j, _):
        slot = j & 1

        @pl.when(j >= 2)
        def _():
            o_copy(j - 2, slot).wait()

        rows = pl.ds(pl.multiple_of(j * TQ, TQ), TQ)
        ms = [None] * 7
        for k in range(7):
            if k in SUMS:
                a = [lo_ref[n, :, pl.ds(SUMS.index(k) * DH, DH)] for n in range(H)]
            elif k == 2:
                a = [_as_bf16(wot_ref[n, pl.ds(0, MH // 2), pl.ds(0, DH)]) for n in range(H)]
            else:
                a = [_as_bf16(wot_ref[n, pl.ds(MH // 2, MH // 2), pl.ds(DH, DH)]) for n in range(H)]
            b = [ctx_ref[n, rows, pl.ds(k * DH, DH)] for n in range(H)]
            ms[k] = _dot_nt(jnp.concatenate(a, axis=1), jnp.concatenate(b, axis=1))
        c11, c12, c21, c22 = _strassen_out(ms)
        at = jnp.concatenate([jnp.concatenate([c11, c12], axis=1),
                              jnp.concatenate([c21, c22], axis=1)], axis=0)
        o_buf[slot] = g_ref[j, 0:1, :] * at + ys_ref[j]
        o_copy(j, slot).start()
        return 0

    assert TO == 2 * TQ and TO == TS
    no = S // TO
    jax.lax.fori_loop(0, no, o_step, 0)
    o_copy(no - 2, no % 2).wait()
    o_copy(no - 1, (no - 1) % 2).wait()


@jax.jit
def pallas_gated_mix__compressed_kv_cla__ssm_conv_s5__prompt_kernel(
    A_x: jax.Array,
    A_c_kv: jax.Array,
    A_w_q: jax.Array,
    A_w_uk: jax.Array,
    A_w_uv: jax.Array,
    A_w_o: jax.Array,
    B_x: jax.Array,
    B_Lambda_re: jax.Array,
    B_Lambda_im: jax.Array,
    B_B_re: jax.Array,
    B_B_im: jax.Array,
    B_C_re: jax.Array,
    B_C_im: jax.Array,
    B_log_dt: jax.Array,
    B_Dskip: jax.Array,
    gate_w: jax.Array,
):
    del B_x
    _, S, M = A_x.shape
    C = A_c_kv.shape[2]
    H, D = A_w_q.shape[1], A_w_q.shape[2]
    PP = (M + LANE - 1) // LANE * LANE

    hbm = pl.BlockSpec(memory_space=pl.ANY)
    out_t = pl.pallas_call(
        functools.partial(_kernel, S=S, M=M, H=H, D=D),
        in_specs=[hbm] * 15,
        out_specs=hbm,
        out_shape=jax.ShapeDtypeStruct((M, S), F32),
        scratch_shapes=[
            pltpu.VMEM((M, S), BF16),
            pltpu.VMEM((S // 2, M), U32),
            pltpu.VMEM((5, S // 4, PP // 2), U32),
            pltpu.VMEM((S // 2, C), U32),
            pltpu.VMEM((49, S // 8, C // 4), U32),
            pltpu.VMEM((H // 2, M, D), U32),
            pltpu.VMEM((H // 2, C, D), U32),
            pltpu.VMEM((H // 2, C, D), U32),
            pltpu.VMEM((H, M // 2, D), U32),
            pltpu.VMEM((H, M // 2, 5 * D // 2), BF16),
            pltpu.VMEM((M, M), U32),
            pltpu.VMEM((M // 2, M), U32),
            pltpu.VMEM((M // 2, M), U32),
            pltpu.VMEM((S + 8, 2 * M), F32),
            pltpu.VMEM((S // TO, M, TO), F32),
            pltpu.VMEM((S // TO, 8, TO), F32),
            pltpu.VMEM((2, 8, PP), F32),
            pltpu.VMEM((10, 8, PP), F32),
            pltpu.VMEM((2, M, LANE), F32),
            pltpu.VMEM((2, 16, H // 2, D), U32),
            pltpu.VMEM((2, 2, H // 2, LANE), F32),
        ] + [pltpu.VMEM((M,), BF16)] * 5 + [
            pltpu.VMEM((H // 2, 4, S // 2, D), BF16),
            pltpu.VMEM((H, S // 2, 7 * D // 2), BF16),
            pltpu.VMEM((2, M, TO), F32),
            pltpu.SMEM((1,), jnp.int32),
            pltpu.SemaphoreType.DMA((5, H // 2)),
            pltpu.SemaphoreType.DMA((4,)),
            pltpu.SemaphoreType.DMA((7,)),
            pltpu.SemaphoreType.DMA((5,)),
            pltpu.SemaphoreType.DMA((2,)),
        ],
        compiler_params=pltpu.CompilerParams(
            vmem_limit_bytes=124 * 1024 * 1024,
            disable_semaphore_checks=True,
            disable_bounds_checks=True,
        ),
    )(
        jnp.swapaxes(A_x, 1, 2).reshape(M, S), A_c_kv.reshape(S, C),
        A_w_q, A_w_uk, A_w_uv, jnp.swapaxes(A_w_o, 1, 2),
        B_B_re, B_B_im, B_C_re, B_C_im,
        B_Lambda_re, B_Lambda_im, B_log_dt, B_Dskip, gate_w,
    )
    return jnp.swapaxes(out_t.reshape(1, M, S), 1, 2)
```

```python
import functools

import jax
import jax.numpy as jnp
import jax.experimental.pallas as pl
import jax.experimental.pallas.tpu as pltpu

F32 = jnp.float32
BF16 = jnp.bfloat16
U32 = jnp.uint32

NT_DIMS = (((1,), (1,)), ((), ()))
LOG2E = 1.4426950408889634

TQ = 128
TP = 256
TU = 512
TO = 256
LANE = 128
HALF = LANE // 2
SSM_SPLIT = False
REMAT = (0, 1, 2, 3, 4, 5, 6)
Q_REMAT = (1,)
UNIFORM_DIAG = False
SCHEDULE = "d0 h2 t0 t1 c2 p0 p1 t2 c3 p2 t3 c4 p3 t4 c5 p4 t5 c6 b5 t6 c7 t7 p5 p6 p7"
Q_SCHEDULE = "q0 q1 m3 c0 q2 g2 q3 m0 c0 q4 m1 c0 c0 q5 q6 m2 q7 w7"
C_MODE = 1
O_UNROLL = 1
PACE_FROM = 2
PACE_ROWS = 8
TWO_PASS = False
CHAIN_ALL = True
L_TIE = 0
EARLY_SUM = ()
EARLY_SHIFT = 0
PRENORM0 = False
LOOK = (0, 0, 0, 0, 0, 0, 0, 0)
PACE2_FROM = 2
PACE2_EXTRA = 1


def _dot_nt(a, b):
    return jax.lax.dot_general(a, b, NT_DIMS, preferred_element_type=F32)


def _unpack(w32, shift):
    v = (w32 << shift) & jnp.uint32(0xFFFF0000)
    return pltpu.bitcast(v, F32)


def _as_bf16(w32):
    return pltpu.bitcast(w32, BF16)


def _as_u32(v):
    return pltpu.bitcast(v, U32)


def _strassen_lhs(a11, a12, a21, a22):
    return [a11 + a22, a21 + a22, a11, a22, a11 + a12, a21 - a11, a12 - a22]


def _strassen_rhs(b11, b12, b21, b22):
    return [b11 + b22, b11, b12 - b22, b21 - b11, b22, b11 + b12, b21 + b22]


def _strassen_out(m):
    return ((m[0] + m[3]) + (m[6] - m[4]), m[2] + m[4],
            m[1] + m[3], (m[0] - m[1]) + (m[2] + m[5]))


def _quads(a):
    m, n = a.shape[0] // 2, a.shape[1] // 2
    return a[:m, :n], a[:m, n:], a[m:, :n], a[m:, n:]


SUMS = (0, 1, 4, 5, 6)
Q_ORDER = (1, 4, 0, 2, 3, 5, 6)
ORDER = (1, 4, 2, 3, 0, 5, 6)
INNER = (1, 3, 4, 2, 0, 6, 5)
QK_ORDER = (0, 3, 4, 6, 1, 2, 5)
QK_GROUP = 1
QK_LAG = 2
QK_TIE_K = 3
QK_RUNMAX = True
DIAG_FIRST = False
PV_ORDER = (2, 4, 3, 1, 5, 0, 6)


def _kernel(xt_hbm, c_hbm, wq_hbm, wuk_hbm, wuv_hbm, wot_hbm,
            bre_hbm, bim_hbm, cre_hbm, cim_hbm,
            lre_hbm, lim_hbm, ldt_hbm, dsk_hbm, gw_hbm,
            o_hbm,
            xt_ref, x_ref, lx_ref, c_ref, l_ref, wq_buf, wk_buf, wv_buf, wot_ref, lo_ref,
            b_ref, cre_ref, cim_ref, u_ref, ys_ref, g_ref, st_ref, co_ref, col_ref, smp_ref, vsc_ref,
            lre_ref, lim_ref, ldt_ref, dsk_ref, gw_ref,
            q_ref, ctx_ref, zero_ref, wsem, xsem, msem, vsem, osem,
            *, S, M, H, D):
    P = M
    FT = P // LANE
    PF = FT * LANE
    assert P - PF == HALF
    PP = PF + LANE
    NP = H // 2
    TS = S // NP
    CH, DH, MH, TH = c_ref.shape[1] // 2, D // 2, M // 2, TP // 2

    def w_copy(k, pair):
        src, dst = ((wq_hbm, wq_buf), (wuk_hbm, wk_buf), (wuv_hbm, wv_buf))[k]
        return pltpu.make_async_copy(src.bitcast(U32).at[:, pair, :], dst.at[pair], wsem.at[k, pair])

    def wo_copy(pair):
        heads = pl.ds(2 * pair, 2)
        return pltpu.make_async_copy(wot_hbm.bitcast(U32).at[heads], wot_ref.at[heads],
                                     wsem.at[3, pair])

    def x_copy(t0, n, k):
        cols = pl.ds(t0, n)
        return pltpu.make_async_copy(xt_hbm.at[:, cols], xt_ref.at[:, cols], xsem.at[k])

    x_cps = [x_copy(0, TU // 2, 0), x_copy(TU // 2, TU // 2, 1), x_copy(TU, TU, 2),
             x_copy(2 * TU, S - 2 * TU, 3)]

    bre32, bim32 = bre_hbm.bitcast(U32), bim_hbm.bitcast(U32)
    b_cps = [
        pltpu.make_async_copy(bre32, b_ref.at[pl.ds(0, P // 2), :], msem.at[0]),
        pltpu.make_async_copy(bim32.at[pl.ds(PF // 2, HALF // 2), :],
                              b_ref.at[pl.ds(P // 2, HALF // 2), :], msem.at[1]),
        pltpu.make_async_copy(bim32.at[pl.ds(0, PF // 2), :],
                              b_ref.at[pl.ds(PP // 2, PF // 2), :], msem.at[2]),
    ]
    cre_cp = pltpu.make_async_copy(cre_hbm.bitcast(U32), cre_ref, msem.at[3])
    cim_cp = pltpu.make_async_copy(cim_hbm.bitcast(U32), cim_ref, msem.at[4])

    def c_copy(r):
        rows = pl.ds(pl.multiple_of(r * TH, TH), TH)
        return pltpu.make_async_copy(c_hbm.bitcast(U32).at[rows], c_ref.at[rows], wsem.at[4, r])

    smp_cps = [pltpu.make_async_copy(src.bitcast(U32).at[pl.ds(0, smp_ref.shape[1])],
                                     smp_ref.at[k], msem.at[5 + k])
               for k, src in enumerate((wuk_hbm, wuv_hbm))]
    v_cps = [pltpu.make_async_copy(src, dst, vsem.at[k]) for k, (src, dst) in enumerate(
        ((lre_hbm, lre_ref), (lim_hbm, lim_ref), (ldt_hbm, ldt_ref),
         (dsk_hbm, dsk_ref), (gw_hbm, gw_ref)))]

    for cp in v_cps:
        cp.start()
    for cp in x_cps[:1] + b_cps + x_cps[1:] + smp_cps:
        cp.start()
    cre_cp.start()
    cim_cp.start()
    for p in range(NP):
        w_copy(0, p).start()
        wo_copy(p).start()
        c_copy(p).start()
    for p in range(NP):
        w_copy(1, p).start()
        w_copy(2, p).start()

    zero_ref[0] = 0
    u_ref[pl.ds(0, 8), :] = jnp.zeros((8, u_ref.shape[1]), F32)
    st_ref[...] = jnp.zeros(st_ref.shape, F32)
    for cp in v_cps:
        cp.wait()

    row = lambda r: r[...].astype(F32).reshape(1, P)
    lre, lim = row(lre_ref), row(lim_ref)
    dt = jnp.exp(row(ldt_ref)).astype(BF16).astype(F32)
    e = jnp.exp(dt * lre)
    ang = dt * lim
    ar = e * jnp.cos(ang)
    ai = e * jnp.sin(ang)
    sc = jnp.maximum(jnp.abs(lre), jnp.abs(lim))
    nre, nim = lre / sc, lim / sc
    den = (nre * nre + nim * nim) * sc
    gr = 2.0 * ((ar - 1.0) * nre + ai * nim) / den
    gi = 2.0 * (ai * nre - (ar - 1.0) * nim) / den

    def put(k, full, lo, hi):
        v = jnp.concatenate([full[:, :PF], lo[:, PF:], hi[:, PF:]], axis=1)
        co_ref[k] = jnp.broadcast_to(v, (8, PP))

    put(0, gr, gr, -gr)
    put(1, -gi, -gi, -gi)
    pr, pi = ar, -ai
    for j in range(1, 5):
        put(2 * j, pr, pr, pr)
        put(2 * j + 1, -pi, -pi, pi)
        pr, pi = pr * pr - pi * pi, 2.0 * pr * pi

    zpad = jnp.zeros((1, PP - P), F32)
    for k, r in enumerate((dsk_ref, gw_ref)):
        v = jnp.concatenate([row(r), zpad], axis=1)
        col_ref[k] = jnp.broadcast_to(v, (LANE, PP)).T[:M]

    XH = PP // 2

    def transpose_x(t0, n):
        x_ref[pl.ds(t0 // 2, n // 2), :] = _as_u32(xt_ref[:, pl.ds(t0, n)].T)

    def x_sums(r, after):
        x = x_ref[pl.ds(r * TH, TH), :] | (_as_u32(after) & zero_ref[0].astype(U32))
        x = _as_bf16(x).astype(F32)
        x = jnp.concatenate([x, jnp.zeros((TP, PP - M), F32)], axis=1)
        ls = _strassen_lhs(x[:TH, :XH], x[:TH, XH:], x[TH:, :XH], x[TH:, XH:])
        for n, k in enumerate(SUMS):
            lx_ref[n, pl.ds(r * TH // 2, TH // 2), :] = _as_u32(ls[k].astype(BF16))

    def proj_u(t0, n, lo=0, hi=2 * P, sums=()):
        u = _dot_nt(_as_bf16(x_ref[pl.ds(t0 // 2, n // 2), :]), _as_bf16(b_ref[lo // 2:hi // 2, :]))
        u_ref[pl.ds(t0 + 8, n), lo:hi] = u
        for i, r in enumerate(sums):
            a = u[:, (2 * i + 1) * LANE:(2 * i + 2) * LANE]
            a = jnp.concatenate([a[k * TH:(k + 1) * TH] for k in range(4)], axis=1)
            x_sums(r, a[:, :M])

    x_cps[0].wait()
    transpose_x(0, TU // 2)
    b_cps[0].wait()
    b_cps[1].wait()
    proj_u(0, TU // 2, 0, PP)
    b_cps[2].wait()
    x_cps[1].wait()
    proj_u(0, TU // 2, PP)
    transpose_x(TU // 2, TU // 2)
    x_cps[2].wait()
    proj_u(TU // 2, TU // 2)
    transpose_x(TU, TU)
    x_cps[3].wait()
    for cp in smp_cps:
        cp.wait()
    for e in range(2):
        mag = [jnp.sum(jnp.sum(jnp.abs(_unpack(smp_ref[k], jnp.uint32(16 - 16 * e))), axis=0),
                       axis=1, keepdims=True) for k in range(2)]
        ex = [jnp.broadcast_to(pltpu.bitcast(v, jnp.int32) >> 23, (NP, LANE)) for v in mag]
        d = jnp.where((ex[0] > 0) & (ex[1] > 0), jnp.clip(ex[0] - ex[1], -40, 40), 0)
        vsc_ref[0, e] = pltpu.bitcast((127 + d) << 23, F32)
        vsc_ref[1, e] = pltpu.bitcast((127 - d) << 23, F32)
    for t0 in range(TU, S, TU):
        proj_u(t0, TU, sums={1: (0, 1, 2), 2: (3, 4, 5), 3: (6, 7)}[t0 // TU])
        if t0 + TU < S:
            transpose_x(t0 + TU, TU)
    cre_cp.wait()
    cim_cp.wait()

    def q_step(j, _):
        w_copy(0, j).wait()
        wo_copy(j).wait()
        c_copy(j).wait()
        zero = zero_ref[0]
        after = lambda w, v: w | (_as_u32(v) & zero.astype(U32))
        t0 = pl.multiple_of(j * TS, TS)

        ys, last, gates = [], [], []

        def ssm_tile(t):
            rows = pl.ds(t0, TS + 8)
            cr, ci = pl.ds(t * LANE, LANE), pl.ds(PP + t * LANE, LANE)
            co = [co_ref[k, :, cr] for k in range(10)]
            u0 = u_ref[rows, cr]
            u1 = u_ref[rows, ci] if t < FT else pltpu.roll(u0, HALF, 1)
            mul = lambda k, x: (co[k] * x[0] + co[k + 1] * x[1], co[k] * x[1] - co[k + 1] * x[0])
            sub = jax.lax.broadcasted_iota(jnp.int32, (8, LANE), 0)
            s = (st_ref[0, :, cr], st_ref[1, :, cr])
            prev, gs = [None] * 3, []
            for k in range(TS // 8 + 1):
                x0, x1 = u0[8 * k:8 * k + 8], u1[8 * k:8 * k + 8]
                if last:
                    x0 = pltpu.bitcast(after(_as_u32(x0), last[0]), F32)
                w = (co[0] * x0 + co[1] * x1, co[1] * x0 - co[0] * x1)
                for i in range(3):
                    cur = [pltpu.roll(v, 1 << i, 0) for v in w]
                    old = cur if k == 0 else prev[i]
                    d = mul(2 * i + 2, [jnp.where(sub < (1 << i), o, c) for o, c in zip(old, cur)])
                    w = [p + q for p, q in zip(d, w)]
                    prev[i] = cur
                if k > 0:
                    s = [p + q for p, q in zip(mul(8, s), w)]
                    gs.append(jnp.concatenate(s, axis=1) if t < FT else s[0])
                    last[:] = [s[0]]
            st_ref[0, :, cr] = s[0]
            st_ref[1, :, cr] = s[1]
            if t < FT:
                cc = jnp.concatenate([cre_ref[:, cr], cim_ref[:, cr]], axis=1)
            else:
                cc = jnp.concatenate([cre_ref[:, PF:], cim_ref[:, PF:]], axis=1)
            g = jnp.concatenate(gs, axis=0).astype(BF16)
            n = M // 2 if t < FT else M // 4
            y = jnp.concatenate([
                jax.lax.dot_general(_as_bf16(cc[a:a + n]), g, NT_DIMS, preferred_element_type=F32)
                for a in range(0, M // 2, n)], axis=0)
            ys.insert(0, y + ys[0] if ys else y)
            if len(ys) == FT + 1:
                dcol = jnp.concatenate([col_ref[0]] * (TS // LANE), axis=1)
                xt = xt_ref[:, pl.ds(t0, TS)].astype(F32)
                omg = (1.0 - gates[0]).astype(BF16).astype(F32)
                ys_ref[j] = omg * (ys[0] + (xt * dcol).astype(BF16).astype(F32))

        def gate(r):
            q = qs[r]
            gcol = after(_as_u32(col_ref[1]), jnp.concatenate([q[:, :LANE], q[:M - TP, LANE:2 * LANE]], axis=0))
            gcol = jnp.concatenate([pltpu.bitcast(gcol, F32)] * (TS // LANE), axis=1)
            xt = xt_ref[:, pl.ds(t0, TS)].astype(F32)
            z = jnp.sum((xt * gcol).astype(BF16).astype(F32), axis=0, keepdims=True)
            rnd = lambda v: v.astype(BF16).astype(F32)
            g = rnd(1.0 / rnd(1.0 + rnd(jnp.exp(-rnd(z)))))
            g_ref[j] = jnp.broadcast_to(g, (8, TS))
            gates.append(g)

        wq32 = wq_buf[j]
        wq32 = jnp.concatenate([wq32, jnp.zeros((PP - M, D), U32)], axis=0)
        rw = []
        for k in range(7):
            z = (zero << k).astype(U32) if k in Q_REMAT else jnp.uint32(0)
            w0 = pltpu.bitcast(wq32 << (z + 16), F32)
            w1 = pltpu.bitcast(wq32 & (z + jnp.uint32(0xFFFF0000)), F32)
            wl = jnp.concatenate([w0[:, :DH], w1[:, :DH]], axis=1)
            wr = jnp.concatenate([w0[:, DH:], w1[:, DH:]], axis=1)
            rw.append(_strassen_rhs(wl[:XH], wr[:XH], wl[XH:], wr[XH:])[k])
        qscale = (D ** -0.5) * LOG2E
        qs = {}

        def proj_q(r, n=1):
            ms = [None] * 7
            for k in Q_ORDER:
                b = rw[k]
                if k in SUMS:
                    a = lx_ref[SUMS.index(k), pl.ds(r * TH // 2, n * TH // 2), :]
                elif k == 2:
                    a = jnp.concatenate([x_ref[pl.ds(i * TH, TH // 2), pl.ds(0, XH)]
                                         for i in range(r, r + n)], axis=0)
                else:
                    a = jnp.concatenate([x_ref[pl.ds(i * TH + TH // 2, TH // 2), pl.ds(XH, M - XH)]
                                         for i in range(r, r + n)], axis=0)
                    b = b[:M - XH]
                ms[k] = jnp.dot(_as_bf16(a), b.astype(BF16), preferred_element_type=F32)
            for k, v in enumerate(_strassen_out(ms)):
                q_ref[j, k, pl.ds(r * TH, n * TH), :] = (v * qscale).astype(BF16)
            qs[r] = jnp.concatenate(
                [jnp.concatenate([ms[Q_ORDER[p]][:TH], ms[Q_ORDER[p + 1]][:TH]], axis=0) for p in (1, 4)],
                axis=1)

        pieces = []

        def c_sums(r):
            n = len(pieces)
            pieces.append(n)
            c = jnp.concatenate(
                [c_ref[pl.ds(pl.multiple_of(j * TH + g * (TH // 4) + 8 * n, 8), 8), :] for g in range(4)],
                axis=0)
            z = _as_u32(last[0]) & zero.astype(U32)
            c = _as_bf16(c | jnp.tile(z, (4, c.shape[1] // LANE))).astype(F32)
            rows = pl.ds(pl.multiple_of(j * (TH // 4) + 8 * n, 8), 8)
            hold = lambda v: pltpu.bitcast(_as_u32(v) | jnp.tile(
                _as_u32(last[0]) & zero.astype(U32), (v.shape[0] // 8, v.shape[1] // LANE)), F32)
            first = (0, 2, 0, 3, 0, 2, 1)
            for k in range(7):
                q = list(_quads(c))
                if C_MODE & 1:
                    q[first[k]] = hold(q[first[k]])
                l = _strassen_lhs(*q)[k]
                for i in range(7):
                    q = list(_quads(l))
                    if C_MODE & 2:
                        q[first[i]] = hold(q[first[i]])
                    v = _as_u32(_strassen_lhs(*q)[i].astype(BF16))
                    l_ref[7 * k + i, rows, :] = v
                    last[:] = [v[:, :LANE] if C_MODE & 2 or i == 0 else v[:, :LANE] | last[0]]

        def wo_sums(r):
            for e in range(2):
                w = after(wot_ref[2 * j + e], qs[r][:MH, e * D:(e + 1) * D])
                w = _as_bf16(w).astype(F32)
                ls = _strassen_lhs(w[:MH, :DH], w[:MH, DH:], w[MH:, :DH], w[MH:, DH:])
                lo_ref[2 * j + e] = jnp.concatenate([ls[k] for k in SUMS], axis=1).astype(BF16)

        ops = dict(q=proj_q, r=lambda r: proj_q(r, 2), m=ssm_tile, c=c_sums, w=wo_sums, g=gate)
        for op in Q_SCHEDULE.split():
            ops[op[0]](int(op[1:]))
        return 0

    assert S // TP == NP
    jax.lax.fori_loop(0, NP, q_step, 0)
    for p in range(NP):
        w_copy(1, p).wait()
        w_copy(2, p).wait()

    def head_step(h, _):
        slot = h >> 1
        zero = zero_ref[0]
        shift = (16 - 16 * (h & 1)).astype(U32)
        vscale, vinv = [vsc_ref[k, h & 1, pl.ds(slot, 1), :] for k in range(2)]
        rw = []
        for k in range(7):
            sh = shift + (zero << k).astype(U32) if k in REMAT else shift
            rk = _strassen_rhs(*_quads(_unpack(wk_buf[slot], sh)))[k]
            rv = _strassen_rhs(*_quads(_unpack(wv_buf[slot], sh)))[k] * vscale
            rw.append(_strassen_rhs(rk[:CH // 2], rv[:CH // 2], rk[CH // 2:], rv[CH // 2:]))
        causal = (jax.lax.broadcasted_iota(jnp.int32, (TQ, TQ), 1)
                  <= jax.lax.broadcasted_iota(jnp.int32, (TQ, TQ), 0))

        ks, rks, vs, rvs, ss, mxs, chains = [], [], [], [], {}, {}, [None]

        def proj_kv(r, n=1):
            TI = TH // 2
            ms = [None] * 7
            for k in ORDER:
                mi = [None] * 7
                for i in INNER:
                    a = l_ref[7 * k + i, pl.ds(r * TI // 2, n * TI // 2), :]
                    mi[i] = jnp.dot(_as_bf16(a), rw[k][i].astype(BF16), preferred_element_type=F32)
                c11, c12, c21, c22 = _strassen_out(mi)
                top, bot = jnp.concatenate([c11, c12], axis=1), jnp.concatenate([c21, c22], axis=1)
                ms[k] = jnp.concatenate(
                    [v[b * TI:(b + 1) * TI] for b in range(n) for v in (top, bot)], axis=0)
                if k != ORDER[-1]:
                    yield
            c = _strassen_out(ms)
            for b in range(n):
                c11, c12, c21, c22 = [v[b * TH:(b + 1) * TH, :DH] for v in c]
                ks.extend([jnp.concatenate([c11, c12], axis=1), jnp.concatenate([c21, c22], axis=1)])
                rks.append(_strassen_rhs(c11, c21, c12, c22))
                c11, c12, c21, c22 = [v[b * TH:(b + 1) * TH, DH:] for v in c]
                vs.extend([jnp.concatenate([c11, c12], axis=1), jnp.concatenate([c21, c22], axis=1)])
                rvs.append(_strassen_rhs(c11, c12, c21, c22))

        def qk_pair(j):
            cols = pl.ds(pl.multiple_of((h & 1) * DH, DH), DH)
            qf = [q_ref[slot, k, j * TQ:(j + 1) * TQ, cols].astype(F32) for k in range(4)]
            q = jnp.concatenate([jnp.concatenate(qf[:2], axis=1), jnp.concatenate(qf[2:], axis=1)], axis=0)
            lq = _strassen_lhs(*qf)
            s1, s2, done, mx = [], [], [], []

            def diag():
                if UNIFORM_DIAG:
                    return (_dot_nt(q[:TQ].astype(BF16), ks[2 * j].astype(BF16)),
                            _dot_nt(q[TQ:].astype(BF16),
                                    jnp.concatenate(ks[2 * j:2 * j + 2], axis=0).astype(BF16)))
                d = _dot_nt(q.astype(BF16), ks[2 * j].astype(BF16))
                return d[:TQ], jnp.concatenate(
                    [d[TQ:], _dot_nt(q[TQ:].astype(BF16), ks[2 * j + 1].astype(BF16))], axis=1)

            if DIAG_FIRST:
                d1, d2 = diag()
            for t0 in range(0, j, QK_GROUP):
                ts = range(t0, min(t0 + QK_GROUP, j))
                m = [None] * 7
                for k in QK_ORDER:
                    rk = jnp.concatenate([rks[t][k] for t in ts], axis=0).astype(BF16)
                    a = lq[k]
                    if k == QK_TIE_K and len(done) >= QK_LAG:
                        a = tie(a, done[-QK_LAG])
                    m[k] = jax.lax.dot_general(a.astype(BF16), rk, NT_DIMS, preferred_element_type=F32)
                c11 = ((m[0] + m[3]) - m[4]) + m[6]
                c12, c21 = m[2] + m[4], m[1] + m[3]
                c22 = ((m[0] - m[1]) + m[2]) + m[5]
                if QK_RUNMAX:
                    x1, x2 = jnp.maximum(c11, c12), jnp.maximum(c21, c22)
                    if mx:
                        x1, x2 = jnp.maximum(x1, mx[0]), jnp.maximum(x2, mx[1])
                    mx[:] = [x1, x2]
                    z = _as_u32(x1) | _as_u32(x2)
                else:
                    z = (_as_u32(c11) | _as_u32(c12)) | (_as_u32(c21) | _as_u32(c22))
                done.append(z)
                for n in range(len(ts)):
                    cols = slice(n * TQ, (n + 1) * TQ)
                    s1 += [c11[:, cols], c12[:, cols]]
                    s2 += [c21[:, cols], c22[:, cols]]
            if not DIAG_FIRST:
                d1, d2 = diag()
            ss[2 * j] = jnp.concatenate(s1 + [d1], axis=1)
            ss[2 * j + 1] = jnp.concatenate(s2 + [d2], axis=1)
            if mx:
                mxs[2 * j], mxs[2 * j + 1] = mx

        def tie(a, b):
            return pltpu.bitcast(_as_u32(a) | (_as_u32(b) & zero.astype(U32)), F32)

        def exp_rows(s, m, pace, rows, chain=None):
            mb = m
            ps, parts = [], []
            for g in range(0, TQ, rows):
                mg = mb[g:g + rows]
                if pace and (parts or chain is not None):
                    mg = tie(mg, parts[-1] if parts else chain)
                pg = [jnp.exp2(s[g:g + rows, t * LANE:(t + 1) * LANE] - mg)
                      for t in range(s.shape[1] // LANE)]
                ps.append(jnp.concatenate(pg, axis=1))
                parts.append(functools.reduce(lambda a, b: a + b, pg))
            return jnp.concatenate(ps, axis=0), jnp.concatenate(parts, axis=0)

        def masked(i):
            lo = i * TQ
            s = ss.pop(i)
            sd = jnp.where(causal, s[:, lo:], -1e9 * LOG2E)
            s = sd if i == 0 else jnp.concatenate([s[:, :lo], sd], axis=1)
            t = jnp.concatenate([mxs[i], s[:, i // 2 * 2 * TQ:]], axis=1) if i in mxs else s
            if LOOK[i // 2] > 0:
                return s, functools.reduce(
                    jnp.maximum, [t[:, c:c + LANE] for c in range(0, t.shape[1], LANE)])
            return s, jnp.broadcast_to(jnp.max(t, axis=-1, keepdims=True), (TQ, LANE))

        def exp_rows2(s, mx, parts, look, both):
            ps = []
            for g in range(0, TQ, 8):
                mg = mx[g:g + 8]
                if len(parts) >= look:
                    mg = tie(mg, parts[-look])
                mg = jnp.broadcast_to(jnp.max(mg, axis=-1, keepdims=True), (8, LANE))
                if both and parts:
                    mg = tie(mg, parts[-1])
                pg = [jnp.exp2(s[g:g + 8, t * LANE:(t + 1) * LANE] - mg)
                      for t in range(s.shape[1] // LANE)]
                ps.append(jnp.concatenate(pg, axis=1))
                parts.append(functools.reduce(lambda a, b: a + b, pg))
            return jnp.concatenate(ps, axis=0), jnp.concatenate(parts[-(TQ // 8):], axis=0)

        def pv(j):
            (s1, m1), (s2, m2) = masked(2 * j), masked(2 * j + 1)
            if LOOK[j] > 0:
                parts = []
                p1, l1 = exp_rows2(s1, m1, parts, LOOK[j] % 100, LOOK[j] > 100)
                p2, l2 = exp_rows2(s2, m2, parts, LOOK[j] % 100, LOOK[j] > 100)
            else:
                p1, l1 = exp_rows(s1, m1, LOOK[j] == 0, PACE_ROWS, chains[0] if CHAIN_ALL else None)
                if j in EARLY_SUM:
                    ls = jnp.broadcast_to(jnp.sum(l1, axis=-1, keepdims=True), (TQ, LANE))
                    k = 8 * EARLY_SHIFT
                    if k:
                        ls = jnp.concatenate([_as_u32(ls[:k]) | _as_u32(ls[k:2 * k]), _as_u32(ls[2 * k:]),
                                              _as_u32(ls[:k])], axis=0)
                    m2 = tie(m2, ls)
                p2, l2 = exp_rows(s2, m2, LOOK[j] == 0, PACE_ROWS, l1[TQ - 8:])
            chains[0] = l2[TQ - 8:]
            if L_TIE == 1:
                l1 = tie(l1, l2)
            elif L_TIE == 2:
                l1 = jnp.concatenate([tie(l1[:8], l2[:8]), l1[8:]], axis=0)
            elif L_TIE == 3:
                l1 = jnp.concatenate([tie(l1[:8], l1[TQ - 8:]), l1[8:]], axis=0)
            l1, l2 = [jnp.sum(l, axis=-1, keepdims=True) for l in (l1, l2)]
            lo = 2 * j * TQ
            cat = lambda xs, axis: jnp.concatenate(xs, axis=axis)
            dot = lambda a, b: jnp.dot(a.astype(BF16), b.astype(BF16), preferred_element_type=F32)

            def recip(l):
                rl = pl.reciprocal(l, approx=True)
                return rl * (2.0 - l * rl)

            r1, r2 = recip(l1), recip(l2)
            rho = l1 * r2
            r1, r2 = r1 * vinv, r2 * vinv
            if j == 0 and PRENORM0:
                p1, p2 = p1 * r1, p2 * cat([r2, r2], 1)
                r1 = r2 = jnp.ones((1, LANE), F32)
            if UNIFORM_DIAG:
                c1 = dot(p1[:, lo:], vs[2 * j])
                c2 = dot(p2[:, lo:], cat(vs[2 * j:2 * j + 2], 0))
            else:
                dg = dot(cat([p1[:, lo:], p2[:, lo:lo + TQ]], 0), vs[2 * j])
                c1, c2 = dg[:TQ], dg[TQ:] + dot(p2[:, lo + TQ:], vs[2 * j + 1])
            if j > 0:
                tiles = lambda p, o: cat([p[:, (2 * t + o) * TQ:(2 * t + o + 1) * TQ] for t in range(j)], 1)
                a11, a12, a21, a22 = tiles(p1, 0), tiles(p1, 1), tiles(p2, 0), tiles(p2, 1)
                a22r = a22 * rho
                lp = [a11 + a22r, a21 + a22, a11, a22, a11 + a12, a21 * rho - a11, a12 - a22r]
                m = [None] * 7
                for k in PV_ORDER:
                    if k == PV_ORDER[-1]:
                        yield
                    m[k] = dot(lp[k], cat([rvs[t][k] for t in range(j)], 0))
                c1 = c1 + cat([(m[0] - m[4]) + (m[6] + m[3] * rho), m[2] + m[4]], 1)
                c2 = (c2 + cat([m[1] + m[3], -m[1]], 1)) * cat([r2, r2], 1)
                c2 = cat([c2[:, :DH], c2[:, DH:] + ((m[0] + m[2]) + m[5]) * r1], 1)
            else:
                c2 = c2 * cat([r2, r2], 1)
            c1 = c1 * cat([r1, r1], 1)
            ctx_ref[h, j * TQ:(j + 1) * TQ, :] = cat(
                _strassen_rhs(c1[:, :DH], c2[:, :DH], c1[:, DH:], c2[:, DH:]), 1).astype(BF16)

        assert TP == 2 * TQ
        pvs = [pv(j) for j in range(S // TP)]
        kvs = {}

        def kv_part(r, n, steps):
            g = kvs.setdefault(r, proj_kv(r, n))
            for _ in range(steps):
                next(g, None)

        ops = dict(c=lambda r: kv_part(r, 1, 7), d=lambda r: kv_part(r, 2, 7),
                   e=lambda r: kv_part(r, 3, 7), f=lambda r: kv_part(r, 4, 7), i=lambda r: kv_part(r, 1, 2),
                   x=lambda r: kv_part(r // 10, 1, r % 10), h=lambda r: kv_part(r, 1, 4), g=lambda r: kv_part(r, 2, 4),
                   t=qk_pair, p=lambda j: list(pvs[j]), b=lambda j: next(pvs[j]))
        for op in SCHEDULE.split():
            ops[op[0]](int(op[1:]))
        return 0

    jax.lax.fori_loop(0, H, head_step, 0)

    parts = ((0, 0, TO), (MH, 0, TQ), (MH, TQ, TQ))

    def o_copy(j, n):
        r0, c0, nc = parts[n]
        return pltpu.make_async_copy(
            ys_ref.at[j, pl.ds(r0, MH), pl.ds(c0, nc)],
            o_hbm.at[pl.ds(r0, MH), pl.ds(pl.multiple_of(j * TO + c0, TQ), nc)], osem.at[n, j])

    def o_step(jj, _):
        for j in [jj * O_UNROLL + u for u in range(O_UNROLL)]:
            rows = pl.ds(pl.multiple_of(j * TQ, TQ), TQ)
            ys, g = ys_ref[j], g_ref[j, 0:1, :]
            m = [None] * 7

            def emit(n, v):
                r0, c0, nc = parts[n]
                ys_ref[j, pl.ds(r0, MH), pl.ds(c0, nc)] = (
                    g[:, c0:c0 + nc] * v + ys[r0:r0 + MH, c0:c0 + nc])
                o_copy(j, n).start()

            for k in (0, 3, 4, 6, 2, 1, 5):
                if k in SUMS:
                    a = [lo_ref[n, :, pl.ds(SUMS.index(k) * DH, DH)] for n in range(H)]
                elif k == 2:
                    a = [_as_bf16(wot_ref[n, pl.ds(0, MH // 2), pl.ds(0, DH)]) for n in range(H)]
                else:
                    a = [_as_bf16(wot_ref[n, pl.ds(MH // 2, MH // 2), pl.ds(DH, DH)]) for n in range(H)]
                b = [ctx_ref[n, rows, pl.ds(k * DH, DH)] for n in range(H)]
                m[k] = _dot_nt(jnp.concatenate(a, axis=1), jnp.concatenate(b, axis=1))
            emit(0, jnp.concatenate([(m[0] + m[3]) + (m[6] - m[4]), m[2] + m[4]], axis=1))
            emit(1, m[1] + m[3])
            emit(2, ((m[0] + m[2]) - m[1]) + m[5])
        return 0

    assert TO == 2 * TQ and TO == TS
    no = S // TO
    jax.lax.fori_loop(0, no // O_UNROLL, o_step, 0)
    for j in range(no):
        for n in range(3):
            o_copy(j, n).wait()


@jax.jit
def pallas_gated_mix__compressed_kv_cla__ssm_conv_s5__prompt_kernel(
    A_x: jax.Array,
    A_c_kv: jax.Array,
    A_w_q: jax.Array,
    A_w_uk: jax.Array,
    A_w_uv: jax.Array,
    A_w_o: jax.Array,
    B_x: jax.Array,
    B_Lambda_re: jax.Array,
    B_Lambda_im: jax.Array,
    B_B_re: jax.Array,
    B_B_im: jax.Array,
    B_C_re: jax.Array,
    B_C_im: jax.Array,
    B_log_dt: jax.Array,
    B_Dskip: jax.Array,
    gate_w: jax.Array,
):
    del B_x
    _, S, M = A_x.shape
    C = A_c_kv.shape[2]
    H, D = A_w_q.shape[1], A_w_q.shape[2]
    PP = (M + LANE - 1) // LANE * LANE

    hbm = pl.BlockSpec(memory_space=pl.ANY)
    out_t = pl.pallas_call(
        functools.partial(_kernel, S=S, M=M, H=H, D=D),
        in_specs=[hbm] * 15,
        out_specs=hbm,
        out_shape=jax.ShapeDtypeStruct((M, S), F32),
        scratch_shapes=[
            pltpu.VMEM((M, S), BF16),
            pltpu.VMEM((S // 2, M), U32),
            pltpu.VMEM((5, S // 4, PP // 2), U32),
            pltpu.VMEM((S // 2, C), U32),
            pltpu.VMEM((49, S // 8, C // 4), U32),
            pltpu.VMEM((H // 2, M, D), U32),
            pltpu.VMEM((H // 2, C, D), U32),
            pltpu.VMEM((H // 2, C, D), U32),
            pltpu.VMEM((H, M // 2, D), U32),
            pltpu.VMEM((H, M // 2, 5 * D // 2), BF16),
            pltpu.VMEM((M, M), U32),
            pltpu.VMEM((M // 2, M), U32),
            pltpu.VMEM((M // 2, M), U32),
            pltpu.VMEM((S + 8, 2 * M), F32),
            pltpu.VMEM((S // TO, M, TO), F32),
            pltpu.VMEM((S // TO, 8, TO), F32),
            pltpu.VMEM((2, 8, PP), F32),
            pltpu.VMEM((10, 8, PP), F32),
            pltpu.VMEM((2, M, LANE), F32),
            pltpu.VMEM((2, 16, H // 2, D), U32),
            pltpu.VMEM((2, 2, H // 2, LANE), F32),
        ] + [pltpu.VMEM((M,), BF16)] * 5 + [
            pltpu.VMEM((H // 2, 4, S // 2, D), BF16),
            pltpu.VMEM((H, S // 2, 7 * D // 2), BF16),
            pltpu.SMEM((1,), jnp.int32),
            pltpu.SemaphoreType.DMA((5, H // 2)),
            pltpu.SemaphoreType.DMA((4,)),
            pltpu.SemaphoreType.DMA((7,)),
            pltpu.SemaphoreType.DMA((5,)),
            pltpu.SemaphoreType.DMA((3, S // TO)),
        ],
        compiler_params=pltpu.CompilerParams(
            vmem_limit_bytes=124 * 1024 * 1024,
            disable_semaphore_checks=True,
            disable_bounds_checks=True,
        ),
    )(
        jnp.swapaxes(A_x, 1, 2).reshape(M, S), A_c_kv.reshape(S, C),
        A_w_q, A_w_uk, A_w_uv, jnp.swapaxes(A_w_o, 1, 2),
        B_B_re, B_B_im, B_C_re, B_C_im,
        B_Lambda_re, B_Lambda_im, B_log_dt, B_Dskip, gate_w,
    )
    return jnp.swapaxes(out_t.reshape(1, M, S), 1, 2)
```

```python
import functools

import jax
import jax.numpy as jnp
import jax.experimental.pallas as pl
import jax.experimental.pallas.tpu as pltpu

F32 = jnp.float32
BF16 = jnp.bfloat16
U32 = jnp.uint32

NT_DIMS = (((1,), (1,)), ((), ()))
LOG2E = 1.4426950408889634

TQ = 128
TP = 256
TU = 512
TO = 256
LANE = 128
HALF = LANE // 2
SSM_SPLIT = False
REMAT = (0, 1, 2, 3, 5, 6)
Q_REMAT = (1,)
UNIFORM_DIAG = False
SCHEDULE = "d0 h2 t0 t1 c2 p0 p1 t2 c3 u3 b2 t3 c4 p2 b3 t4 c5 p3 p4 t5 c6 b5 t6 c7 t7 p5 b6 b7 p6 p7"
Q_SCHEDULE = "q0 q1 m3 c0 q2 g2 q3 m0 c0 q4 m1 c0 c0 q5 q6 m2 q7 w7"
C_MODE = 1
O_UNROLL = 2
PACE_FROM = 2
PACE_ROWS = 8
TWO_PASS = False
CHAIN_ALL = True
L_TIE = 3
PV_DIAG = (0, 5, 0, 1, 0, 3, 3, 0)
EARLY_SUM = (1, 7)
EARLY_SHIFT = 0
PRENORM0 = False
LOOK = (0, 0, 0, 0, 0, 0, 104, 0)
PACE2_FROM = 2
PACE2_EXTRA = 1


def _dot_nt(a, b):
    return jax.lax.dot_general(a, b, NT_DIMS, preferred_element_type=F32)


def _unpack(w32, shift):
    v = (w32 << shift) & jnp.uint32(0xFFFF0000)
    return pltpu.bitcast(v, F32)


def _as_bf16(w32):
    return pltpu.bitcast(w32, BF16)


def _as_u32(v):
    return pltpu.bitcast(v, U32)


def _strassen_lhs(a11, a12, a21, a22):
    return [a11 + a22, a21 + a22, a11, a22, a11 + a12, a21 - a11, a12 - a22]


def _strassen_rhs(b11, b12, b21, b22):
    return [b11 + b22, b11, b12 - b22, b21 - b11, b22, b11 + b12, b21 + b22]


def _strassen_out(m):
    return ((m[0] + m[3]) + (m[6] - m[4]), m[2] + m[4],
            m[1] + m[3], (m[0] - m[1]) + (m[2] + m[5]))


def _quads(a):
    m, n = a.shape[0] // 2, a.shape[1] // 2
    return a[:m, :n], a[:m, n:], a[m:, :n], a[m:, n:]


SUMS = (0, 1, 4, 5, 6)
Q_ORDER = (1, 4, 0, 2, 3, 5, 6)
ORDER = (1, 3, 2, 4, 0, 5, 6)
INNER = (1, 3, 6, 0, 2, 4, 5)
QK_ORDER = (0, 2, 4, 3, 1, 6, 5)
QK_GROUP = 1
QK_LAG = 2
QK_TIE_K = 3
QK_RUNMAX = True
DIAG_FIRST = False
PV_ORDER = (2, 1, 3, 4, 5, 0, 6)


def _kernel(xt_hbm, c_hbm, wq_hbm, wuk_hbm, wuv_hbm, wot_hbm,
            bre_hbm, bim_hbm, cre_hbm, cim_hbm,
            lre_hbm, lim_hbm, ldt_hbm, dsk_hbm, gw_hbm,
            o_hbm,
            xt_ref, x_ref, lx_ref, c_ref, l_ref, wq_buf, wk_buf, wv_buf, wot_ref, lo_ref,
            b_ref, cre_ref, cim_ref, u_ref, ys_ref, g_ref, st_ref, co_ref, col_ref, smp_ref, vsc_ref,
            lre_ref, lim_ref, ldt_ref, dsk_ref, gw_ref,
            q_ref, ctx_ref, zero_ref, wsem, xsem, msem, vsem, osem,
            *, S, M, H, D):
    P = M
    FT = P // LANE
    PF = FT * LANE
    assert P - PF == HALF
    PP = PF + LANE
    NP = H // 2
    TS = S // NP
    CH, DH, MH, TH = c_ref.shape[1] // 2, D // 2, M // 2, TP // 2

    def w_copy(k, pair):
        src, dst = ((wq_hbm, wq_buf), (wuk_hbm, wk_buf), (wuv_hbm, wv_buf))[k]
        return pltpu.make_async_copy(src.bitcast(U32).at[:, pair, :], dst.at[pair], wsem.at[k, pair])

    def wo_copy(pair):
        heads = pl.ds(2 * pair, 2)
        return pltpu.make_async_copy(wot_hbm.bitcast(U32).at[heads], wot_ref.at[heads],
                                     wsem.at[3, pair])

    def x_copy(t0, n, k):
        cols = pl.ds(t0, n)
        return pltpu.make_async_copy(xt_hbm.at[:, cols], xt_ref.at[:, cols], xsem.at[k])

    x_cps = [x_copy(0, TU // 2, 0), x_copy(TU // 2, TU // 2, 1), x_copy(TU, TU, 2),
             x_copy(2 * TU, S - 2 * TU, 3)]

    bre32, bim32 = bre_hbm.bitcast(U32), bim_hbm.bitcast(U32)
    b_cps = [
        pltpu.make_async_copy(bre32, b_ref.at[pl.ds(0, P // 2), :], msem.at[0]),
        pltpu.make_async_copy(bim32.at[pl.ds(PF // 2, HALF // 2), :],
                              b_ref.at[pl.ds(P // 2, HALF // 2), :], msem.at[1]),
        pltpu.make_async_copy(bim32.at[pl.ds(0, PF // 2), :],
                              b_ref.at[pl.ds(PP // 2, PF // 2), :], msem.at[2]),
    ]
    cre_cp = pltpu.make_async_copy(cre_hbm.bitcast(U32), cre_ref, msem.at[3])
    cim_cp = pltpu.make_async_copy(cim_hbm.bitcast(U32), cim_ref, msem.at[4])

    def c_copy(r):
        rows = pl.ds(pl.multiple_of(r * TH, TH), TH)
        return pltpu.make_async_copy(c_hbm.bitcast(U32).at[rows], c_ref.at[rows], wsem.at[4, r])

    smp_cps = [pltpu.make_async_copy(src.bitcast(U32).at[pl.ds(0, smp_ref.shape[1])],
                                     smp_ref.at[k], msem.at[5 + k])
               for k, src in enumerate((wuk_hbm, wuv_hbm))]
    v_cps = [pltpu.make_async_copy(src, dst, vsem.at[k]) for k, (src, dst) in enumerate(
        ((lre_hbm, lre_ref), (lim_hbm, lim_ref), (ldt_hbm, ldt_ref),
         (dsk_hbm, dsk_ref), (gw_hbm, gw_ref)))]

    for cp in v_cps:
        cp.start()
    for cp in x_cps[:1] + b_cps + x_cps[1:] + smp_cps:
        cp.start()
    cre_cp.start()
    cim_cp.start()
    for p in range(NP):
        w_copy(0, p).start()
        wo_copy(p).start()
        c_copy(p).start()
    for p in range(NP):
        w_copy(1, p).start()
        w_copy(2, p).start()

    zero_ref[0] = 0
    u_ref[pl.ds(0, 8), :] = jnp.zeros((8, u_ref.shape[1]), F32)
    st_ref[...] = jnp.zeros(st_ref.shape, F32)
    for cp in v_cps:
        cp.wait()

    row = lambda r: r[...].astype(F32).reshape(1, P)
    lre, lim = row(lre_ref), row(lim_ref)
    dt = jnp.exp(row(ldt_ref)).astype(BF16).astype(F32)
    e = jnp.exp(dt * lre)
    ang = dt * lim
    ar = e * jnp.cos(ang)
    ai = e * jnp.sin(ang)
    sc = jnp.maximum(jnp.abs(lre), jnp.abs(lim))
    nre, nim = lre / sc, lim / sc
    den = (nre * nre + nim * nim) * sc
    gr = 2.0 * ((ar - 1.0) * nre + ai * nim) / den
    gi = 2.0 * (ai * nre - (ar - 1.0) * nim) / den

    def put(k, full, lo, hi):
        v = jnp.concatenate([full[:, :PF], lo[:, PF:], hi[:, PF:]], axis=1)
        co_ref[k] = jnp.broadcast_to(v, (8, PP))

    put(0, gr, gr, -gr)
    put(1, -gi, -gi, -gi)
    pr, pi = ar, -ai
    for j in range(1, 5):
        put(2 * j, pr, pr, pr)
        put(2 * j + 1, -pi, -pi, pi)
        pr, pi = pr * pr - pi * pi, 2.0 * pr * pi

    zpad = jnp.zeros((1, PP - P), F32)
    for k, r in enumerate((dsk_ref, gw_ref)):
        v = jnp.concatenate([row(r), zpad], axis=1)
        col_ref[k] = jnp.broadcast_to(v, (LANE, PP)).T[:M]

    XH = PP // 2

    def transpose_x(t0, n):
        x_ref[pl.ds(t0 // 2, n // 2), :] = _as_u32(xt_ref[:, pl.ds(t0, n)].T)

    def x_sums(r, after):
        x = x_ref[pl.ds(r * TH, TH), :] | (_as_u32(after) & zero_ref[0].astype(U32))
        x = _as_bf16(x).astype(F32)
        x = jnp.concatenate([x, jnp.zeros((TP, PP - M), F32)], axis=1)
        ls = _strassen_lhs(x[:TH, :XH], x[:TH, XH:], x[TH:, :XH], x[TH:, XH:])
        for n, k in enumerate(SUMS):
            lx_ref[n, pl.ds(r * TH // 2, TH // 2), :] = _as_u32(ls[k].astype(BF16))

    def proj_u(t0, n, lo=0, hi=2 * P, sums=()):
        u = _dot_nt(_as_bf16(x_ref[pl.ds(t0 // 2, n // 2), :]), _as_bf16(b_ref[lo // 2:hi // 2, :]))
        u_ref[pl.ds(t0 + 8, n), lo:hi] = u
        for i, r in enumerate(sums):
            a = u[:, (2 * i + 1) * LANE:(2 * i + 2) * LANE]
            a = jnp.concatenate([a[k * TH:(k + 1) * TH] for k in range(4)], axis=1)
            x_sums(r, a[:, :M])

    x_cps[0].wait()
    transpose_x(0, TU // 2)
    b_cps[0].wait()
    b_cps[1].wait()
    proj_u(0, TU // 2, 0, PP)
    b_cps[2].wait()
    x_cps[1].wait()
    proj_u(0, TU // 2, PP)
    transpose_x(TU // 2, TU // 2)
    x_cps[2].wait()
    proj_u(TU // 2, TU // 2)
    transpose_x(TU, TU)
    x_cps[3].wait()
    for cp in smp_cps:
        cp.wait()
    for e in range(2):
        mag = [jnp.sum(jnp.sum(jnp.abs(_unpack(smp_ref[k], jnp.uint32(16 - 16 * e))), axis=0),
                       axis=1, keepdims=True) for k in range(2)]
        ex = [jnp.broadcast_to(pltpu.bitcast(v, jnp.int32) >> 23, (NP, LANE)) for v in mag]
        d = jnp.where((ex[0] > 0) & (ex[1] > 0), jnp.clip(ex[0] - ex[1], -40, 40), 0)
        vsc_ref[0, e] = pltpu.bitcast((127 + d) << 23, F32)
        vsc_ref[1, e] = pltpu.bitcast((127 - d) << 23, F32)
    for t0 in range(TU, S, TU):
        proj_u(t0, TU, sums={1: (0, 1, 2), 2: (3, 4, 5), 3: (6, 7)}[t0 // TU])
        if t0 + TU < S:
            transpose_x(t0 + TU, TU)
    cre_cp.wait()
    cim_cp.wait()

    def q_step(j, _):
        w_copy(0, j).wait()
        wo_copy(j).wait()
        c_copy(j).wait()
        zero = zero_ref[0]
        after = lambda w, v: w | (_as_u32(v) & zero.astype(U32))
        t0 = pl.multiple_of(j * TS, TS)

        ys, last, gates = [], [], []

        def ssm_tile(t):
            rows = pl.ds(t0, TS + 8)
            cr, ci = pl.ds(t * LANE, LANE), pl.ds(PP + t * LANE, LANE)
            co = [co_ref[k, :, cr] for k in range(10)]
            u0 = u_ref[rows, cr]
            u1 = u_ref[rows, ci] if t < FT else pltpu.roll(u0, HALF, 1)
            mul = lambda k, x: (co[k] * x[0] + co[k + 1] * x[1], co[k] * x[1] - co[k + 1] * x[0])
            sub = jax.lax.broadcasted_iota(jnp.int32, (8, LANE), 0)
            s = (st_ref[0, :, cr], st_ref[1, :, cr])
            prev, gs = [None] * 3, []
            for k in range(TS // 8 + 1):
                x0, x1 = u0[8 * k:8 * k + 8], u1[8 * k:8 * k + 8]
                if last:
                    x0 = pltpu.bitcast(after(_as_u32(x0), last[0]), F32)
                w = (co[0] * x0 + co[1] * x1, co[1] * x0 - co[0] * x1)
                for i in range(3):
                    cur = [pltpu.roll(v, 1 << i, 0) for v in w]
                    old = cur if k == 0 else prev[i]
                    d = mul(2 * i + 2, [jnp.where(sub < (1 << i), o, c) for o, c in zip(old, cur)])
                    w = [p + q for p, q in zip(d, w)]
                    prev[i] = cur
                if k > 0:
                    s = [p + q for p, q in zip(mul(8, s), w)]
                    gs.append(jnp.concatenate(s, axis=1) if t < FT else s[0])
                    last[:] = [s[0]]
            st_ref[0, :, cr] = s[0]
            st_ref[1, :, cr] = s[1]
            if t < FT:
                cc = jnp.concatenate([cre_ref[:, cr], cim_ref[:, cr]], axis=1)
            else:
                cc = jnp.concatenate([cre_ref[:, PF:], cim_ref[:, PF:]], axis=1)
            g = jnp.concatenate(gs, axis=0).astype(BF16)
            n = M // 2 if t < FT else M // 4
            y = jnp.concatenate([
                jax.lax.dot_general(_as_bf16(cc[a:a + n]), g, NT_DIMS, preferred_element_type=F32)
                for a in range(0, M // 2, n)], axis=0)
            ys.insert(0, y + ys[0] if ys else y)
            if len(ys) == FT + 1:
                dcol = jnp.concatenate([col_ref[0]] * (TS // LANE), axis=1)
                xt = xt_ref[:, pl.ds(t0, TS)].astype(F32)
                omg = (1.0 - gates[0]).astype(BF16).astype(F32)
                ys_ref[j] = omg * (ys[0] + (xt * dcol).astype(BF16).astype(F32))

        def gate(r):
            q = qs[r]
            gcol = after(_as_u32(col_ref[1]), jnp.concatenate([q[:, :LANE], q[:M - TP, LANE:2 * LANE]], axis=0))
            gcol = jnp.concatenate([pltpu.bitcast(gcol, F32)] * (TS // LANE), axis=1)
            xt = xt_ref[:, pl.ds(t0, TS)].astype(F32)
            z = jnp.sum((xt * gcol).astype(BF16).astype(F32), axis=0, keepdims=True)
            rnd = lambda v: v.astype(BF16).astype(F32)
            g = rnd(1.0 / rnd(1.0 + rnd(jnp.exp(-rnd(z)))))
            g_ref[j] = jnp.broadcast_to(g, (8, TS))
            gates.append(g)

        wq32 = wq_buf[j]
        wq32 = jnp.concatenate([wq32, jnp.zeros((PP - M, D), U32)], axis=0)
        rw = []
        for k in range(7):
            z = (zero << k).astype(U32) if k in Q_REMAT else jnp.uint32(0)
            w0 = pltpu.bitcast(wq32 << (z + 16), F32)
            w1 = pltpu.bitcast(wq32 & (z + jnp.uint32(0xFFFF0000)), F32)
            wl = jnp.concatenate([w0[:, :DH], w1[:, :DH]], axis=1)
            wr = jnp.concatenate([w0[:, DH:], w1[:, DH:]], axis=1)
            rw.append(_strassen_rhs(wl[:XH], wr[:XH], wl[XH:], wr[XH:])[k])
        qscale = (D ** -0.5) * LOG2E
        qs = {}

        def proj_q(r, n=1):
            ms = [None] * 7
            for k in Q_ORDER:
                b = rw[k]
                if k in SUMS:
                    a = lx_ref[SUMS.index(k), pl.ds(r * TH // 2, n * TH // 2), :]
                elif k == 2:
                    a = jnp.concatenate([x_ref[pl.ds(i * TH, TH // 2), pl.ds(0, XH)]
                                         for i in range(r, r + n)], axis=0)
                else:
                    a = jnp.concatenate([x_ref[pl.ds(i * TH + TH // 2, TH // 2), pl.ds(XH, M - XH)]
                                         for i in range(r, r + n)], axis=0)
                    b = b[:M - XH]
                ms[k] = jnp.dot(_as_bf16(a), b.astype(BF16), preferred_element_type=F32)
            for k, v in enumerate(_strassen_out(ms)):
                q_ref[j, k, pl.ds(r * TH, n * TH), :] = (v * qscale).astype(BF16)
            qs[r] = jnp.concatenate(
                [jnp.concatenate([ms[Q_ORDER[p]][:TH], ms[Q_ORDER[p + 1]][:TH]], axis=0) for p in (1, 4)],
                axis=1)

        pieces = []

        def c_sums(r):
            n = len(pieces)
            pieces.append(n)
            c = jnp.concatenate(
                [c_ref[pl.ds(pl.multiple_of(j * TH + g * (TH // 4) + 8 * n, 8), 8), :] for g in range(4)],
                axis=0)
            z = _as_u32(last[0]) & zero.astype(U32)
            c = _as_bf16(c | jnp.tile(z, (4, c.shape[1] // LANE))).astype(F32)
            rows = pl.ds(pl.multiple_of(j * (TH // 4) + 8 * n, 8), 8)
            hold = lambda v: pltpu.bitcast(_as_u32(v) | jnp.tile(
                _as_u32(last[0]) & zero.astype(U32), (v.shape[0] // 8, v.shape[1] // LANE)), F32)
            first = (0, 2, 0, 3, 0, 2, 1)
            for k in range(7):
                q = list(_quads(c))
                if C_MODE & 1:
                    q[first[k]] = hold(q[first[k]])
                l = _strassen_lhs(*q)[k]
                for i in range(7):
                    q = list(_quads(l))
                    if C_MODE & 2:
                        q[first[i]] = hold(q[first[i]])
                    v = _as_u32(_strassen_lhs(*q)[i].astype(BF16))
                    l_ref[7 * k + i, rows, :] = v
                    last[:] = [v[:, :LANE] if C_MODE & 2 or i == 0 else v[:, :LANE] | last[0]]

        def wo_sums(r):
            for e in range(2):
                w = after(wot_ref[2 * j + e], qs[r][:MH, e * D:(e + 1) * D])
                w = _as_bf16(w).astype(F32)
                ls = _strassen_lhs(w[:MH, :DH], w[:MH, DH:], w[MH:, :DH], w[MH:, DH:])
                lo_ref[2 * j + e] = jnp.concatenate([ls[k] for k in SUMS], axis=1).astype(BF16)

        ops = dict(q=proj_q, r=lambda r: proj_q(r, 2), m=ssm_tile, c=c_sums, w=wo_sums, g=gate)
        for op in Q_SCHEDULE.split():
            ops[op[0]](int(op[1:]))
        return 0

    assert S // TP == NP
    jax.lax.fori_loop(0, NP, q_step, 0)
    for p in range(NP):
        w_copy(1, p).wait()
        w_copy(2, p).wait()

    def head_step(h, _):
        slot = h >> 1
        zero = zero_ref[0]
        shift = (16 - 16 * (h & 1)).astype(U32)
        vscale, vinv = [vsc_ref[k, h & 1, pl.ds(slot, 1), :] for k in range(2)]
        rw = []
        for k in range(7):
            sh = shift + (zero << k).astype(U32) if k in REMAT else shift
            rk = _strassen_rhs(*_quads(_unpack(wk_buf[slot], sh)))[k]
            rv = _strassen_rhs(*_quads(_unpack(wv_buf[slot], sh)))[k] * vscale
            rw.append(_strassen_rhs(rk[:CH // 2], rv[:CH // 2], rk[CH // 2:], rv[CH // 2:]))
        causal = (jax.lax.broadcasted_iota(jnp.int32, (TQ, TQ), 1)
                  <= jax.lax.broadcasted_iota(jnp.int32, (TQ, TQ), 0))

        ks, rks, vs, rvs, ss, mxs, chains = [], [], [], [], {}, {}, [None]

        def proj_kv(r, n=1):
            TI = TH // 2
            ms = [None] * 7
            for k in ORDER:
                mi = [None] * 7
                for i in INNER:
                    a = l_ref[7 * k + i, pl.ds(r * TI // 2, n * TI // 2), :]
                    mi[i] = jnp.dot(_as_bf16(a), rw[k][i].astype(BF16), preferred_element_type=F32)
                c11, c12, c21, c22 = _strassen_out(mi)
                top, bot = jnp.concatenate([c11, c12], axis=1), jnp.concatenate([c21, c22], axis=1)
                ms[k] = jnp.concatenate(
                    [v[b * TI:(b + 1) * TI] for b in range(n) for v in (top, bot)], axis=0)
                if k != ORDER[-1]:
                    yield
            c = _strassen_out(ms)
            for b in range(n):
                c11, c12, c21, c22 = [v[b * TH:(b + 1) * TH, :DH] for v in c]
                ks.extend([jnp.concatenate([c11, c12], axis=1), jnp.concatenate([c21, c22], axis=1)])
                rks.append(_strassen_rhs(c11, c21, c12, c22))
                c11, c12, c21, c22 = [v[b * TH:(b + 1) * TH, DH:] for v in c]
                vs.extend([jnp.concatenate([c11, c12], axis=1), jnp.concatenate([c21, c22], axis=1)])
                rvs.append(_strassen_rhs(c11, c12, c21, c22))

        def qk_pair(j):
            cols = pl.ds(pl.multiple_of((h & 1) * DH, DH), DH)
            qf = [q_ref[slot, k, j * TQ:(j + 1) * TQ, cols].astype(F32) for k in range(4)]
            q = jnp.concatenate([jnp.concatenate(qf[:2], axis=1), jnp.concatenate(qf[2:], axis=1)], axis=0)
            lq = _strassen_lhs(*qf)
            s1, s2, done, mx = [], [], [], []

            def diag():
                if UNIFORM_DIAG:
                    return (_dot_nt(q[:TQ].astype(BF16), ks[2 * j].astype(BF16)),
                            _dot_nt(q[TQ:].astype(BF16),
                                    jnp.concatenate(ks[2 * j:2 * j + 2], axis=0).astype(BF16)))
                d = _dot_nt(q.astype(BF16), ks[2 * j].astype(BF16))
                return d[:TQ], jnp.concatenate(
                    [d[TQ:], _dot_nt(q[TQ:].astype(BF16), ks[2 * j + 1].astype(BF16))], axis=1)

            if DIAG_FIRST:
                d1, d2 = diag()
            for t0 in range(0, j, QK_GROUP):
                ts = range(t0, min(t0 + QK_GROUP, j))
                m = [None] * 7
                for k in QK_ORDER:
                    rk = jnp.concatenate([rks[t][k] for t in ts], axis=0).astype(BF16)
                    a = lq[k]
                    if k == QK_TIE_K and len(done) >= QK_LAG:
                        a = tie(a, done[-QK_LAG])
                    m[k] = jax.lax.dot_general(a.astype(BF16), rk, NT_DIMS, preferred_element_type=F32)
                c11 = ((m[0] + m[3]) - m[4]) + m[6]
                c12, c21 = m[2] + m[4], m[1] + m[3]
                c22 = ((m[0] - m[1]) + m[2]) + m[5]
                if QK_RUNMAX:
                    x1, x2 = jnp.maximum(c11, c12), jnp.maximum(c21, c22)
                    if mx:
                        x1, x2 = jnp.maximum(x1, mx[0]), jnp.maximum(x2, mx[1])
                    mx[:] = [x1, x2]
                    z = _as_u32(x1) | _as_u32(x2)
                else:
                    z = (_as_u32(c11) | _as_u32(c12)) | (_as_u32(c21) | _as_u32(c22))
                done.append(z)
                for n in range(len(ts)):
                    cols = slice(n * TQ, (n + 1) * TQ)
                    s1 += [c11[:, cols], c12[:, cols]]
                    s2 += [c21[:, cols], c22[:, cols]]
            yield
            if not DIAG_FIRST:
                d1, d2 = diag()
            ss[2 * j] = jnp.concatenate(s1 + [d1], axis=1)
            ss[2 * j + 1] = jnp.concatenate(s2 + [d2], axis=1)
            if mx:
                mxs[2 * j], mxs[2 * j + 1] = mx

        def tie(a, b):
            return pltpu.bitcast(_as_u32(a) | (_as_u32(b) & zero.astype(U32)), F32)

        def exp_rows(s, m, pace, rows, chain=None):
            mb = m
            ps, parts = [], []
            for g in range(0, TQ, rows):
                mg = mb[g:g + rows]
                if pace and (parts or chain is not None):
                    mg = tie(mg, parts[-1] if parts else chain)
                pg = [jnp.exp2(s[g:g + rows, t * LANE:(t + 1) * LANE] - mg)
                      for t in range(s.shape[1] // LANE)]
                ps.append(jnp.concatenate(pg, axis=1))
                parts.append(functools.reduce(lambda a, b: a + b, pg))
            return jnp.concatenate(ps, axis=0), jnp.concatenate(parts, axis=0)

        def masked(i):
            lo = i * TQ
            s = ss.pop(i)
            sd = jnp.where(causal, s[:, lo:], -1e9 * LOG2E)
            s = sd if i == 0 else jnp.concatenate([s[:, :lo], sd], axis=1)
            t = jnp.concatenate([mxs[i], s[:, i // 2 * 2 * TQ:]], axis=1) if i in mxs else s
            if LOOK[i // 2] > 0:
                return s, functools.reduce(
                    jnp.maximum, [t[:, c:c + LANE] for c in range(0, t.shape[1], LANE)])
            return s, jnp.broadcast_to(jnp.max(t, axis=-1, keepdims=True), (TQ, LANE))

        def exp_rows2(s, mx, parts, look, both):
            ps = []
            for g in range(0, TQ, 8):
                mg = mx[g:g + 8]
                if len(parts) >= look:
                    mg = tie(mg, parts[-look])
                mg = jnp.broadcast_to(jnp.max(mg, axis=-1, keepdims=True), (8, LANE))
                if both and parts:
                    mg = tie(mg, parts[-1])
                pg = [jnp.exp2(s[g:g + 8, t * LANE:(t + 1) * LANE] - mg)
                      for t in range(s.shape[1] // LANE)]
                ps.append(jnp.concatenate(pg, axis=1))
                parts.append(functools.reduce(lambda a, b: a + b, pg))
            return jnp.concatenate(ps, axis=0), jnp.concatenate(parts[-(TQ // 8):], axis=0)

        def pv(j):
            (s1, m1), (s2, m2) = masked(2 * j), masked(2 * j + 1)
            if LOOK[j] > 0:
                parts = []
                p1, l1 = exp_rows2(s1, m1, parts, LOOK[j] % 100, LOOK[j] > 100)
                p2, l2 = exp_rows2(s2, m2, parts, LOOK[j] % 100, LOOK[j] > 100)
            else:
                p1, l1 = exp_rows(s1, m1, LOOK[j] == 0, PACE_ROWS, chains[0] if CHAIN_ALL else None)
                if j in EARLY_SUM:
                    ls = jnp.broadcast_to(jnp.sum(l1, axis=-1, keepdims=True), (TQ, LANE))
                    k = 8 * EARLY_SHIFT
                    if k:
                        ls = jnp.concatenate([_as_u32(ls[:k]) | _as_u32(ls[k:2 * k]), _as_u32(ls[2 * k:]),
                                              _as_u32(ls[:k])], axis=0)
                    m2 = tie(m2, ls)
                p2, l2 = exp_rows(s2, m2, LOOK[j] == 0, PACE_ROWS, l1[TQ - 8:])
            chains[0] = l2[TQ - 8:]
            if L_TIE == 1:
                l1 = tie(l1, l2)
            elif L_TIE == 2:
                l1 = jnp.concatenate([tie(l1[:8], l2[:8]), l1[8:]], axis=0)
            elif L_TIE == 3:
                l1 = jnp.concatenate([tie(l1[:8], l1[TQ - 8:]), l1[8:]], axis=0)
            l1, l2 = [jnp.sum(l, axis=-1, keepdims=True) for l in (l1, l2)]
            lo = 2 * j * TQ
            cat = lambda xs, axis: jnp.concatenate(xs, axis=axis)
            dot = lambda a, b: jnp.dot(a.astype(BF16), b.astype(BF16), preferred_element_type=F32)

            def recip(l):
                rl = pl.reciprocal(l, approx=True)
                return rl * (2.0 - l * rl)

            r1, r2 = recip(l1), recip(l2)
            rho = l1 * r2
            r1, r2 = r1 * vinv, r2 * vinv
            if j == 0 and PRENORM0:
                p1, p2 = p1 * r1, p2 * cat([r2, r2], 1)
                r1 = r2 = jnp.ones((1, LANE), F32)
            def diag():
                dg = dot(cat([p1[:, lo:], p2[:, lo:lo + TQ]], 0), vs[2 * j])
                return dg[:TQ], dg[TQ:] + dot(p2[:, lo + TQ:], vs[2 * j + 1])

            if j == 0:
                c1, c2 = diag()
            if j > 0:
                tiles = lambda p, o: cat([p[:, (2 * t + o) * TQ:(2 * t + o + 1) * TQ] for t in range(j)], 1)
                a11, a12, a21, a22 = tiles(p1, 0), tiles(p1, 1), tiles(p2, 0), tiles(p2, 1)
                a22r = a22 * rho
                lp = [a11 + a22r, a21 + a22, a11, a22, a11 + a12, a21 * rho - a11, a12 - a22r]
                m = [None] * 7
                for n, k in enumerate(PV_ORDER):
                    if n == PV_DIAG[j]:
                        c1, c2 = diag()
                    if k == PV_ORDER[-1]:
                        yield
                    m[k] = dot(lp[k], cat([rvs[t][k] for t in range(j)], 0))
                c1 = c1 + cat([(m[0] - m[4]) + (m[6] + m[3] * rho), m[2] + m[4]], 1)
                c2 = (c2 + cat([m[1] + m[3], -m[1]], 1)) * cat([r2, r2], 1)
                c2 = cat([c2[:, :DH], c2[:, DH:] + ((m[0] + m[2]) + m[5]) * r1], 1)
            else:
                c2 = c2 * cat([r2, r2], 1)
            c1 = c1 * cat([r1, r1], 1)
            ctx_ref[h, j * TQ:(j + 1) * TQ, :] = cat(
                _strassen_rhs(c1[:, :DH], c2[:, :DH], c1[:, DH:], c2[:, DH:]), 1).astype(BF16)

        assert TP == 2 * TQ
        pvs = [pv(j) for j in range(S // TP)]
        qks = [qk_pair(j) for j in range(S // TP)]
        kvs = {}

        def kv_part(r, n, steps):
            g = kvs.setdefault(r, proj_kv(r, n))
            for _ in range(steps):
                next(g, None)

        ops = dict(c=lambda r: kv_part(r, 1, 7), d=lambda r: kv_part(r, 2, 7),
                   e=lambda r: kv_part(r, 3, 7), f=lambda r: kv_part(r, 4, 7), i=lambda r: kv_part(r, 1, 2),
                   x=lambda r: kv_part(r // 10, 1, r % 10), h=lambda r: kv_part(r, 1, 4), g=lambda r: kv_part(r, 2, 4),
                   t=lambda j: list(qks[j]), u=lambda j: next(qks[j]), p=lambda j: list(pvs[j]), b=lambda j: next(pvs[j]))
        for op in SCHEDULE.split():
            ops[op[0]](int(op[1:]))
        return 0

    jax.lax.fori_loop(0, H, head_step, 0)

    parts = ((0, 0, TO), (MH, 0, TQ), (MH, TQ, TQ))

    def o_copy(j, n):
        r0, c0, nc = parts[n]
        return pltpu.make_async_copy(
            ys_ref.at[j, pl.ds(r0, MH), pl.ds(c0, nc)],
            o_hbm.at[pl.ds(r0, MH), pl.ds(pl.multiple_of(j * TO + c0, TQ), nc)], osem.at[n, j])

    def o_step(jj, _):
        for j in [jj * O_UNROLL + u for u in range(O_UNROLL)]:
            rows = pl.ds(pl.multiple_of(j * TQ, TQ), TQ)
            ys, g = ys_ref[j], g_ref[j, 0:1, :]
            m = [None] * 7

            def emit(n, v):
                r0, c0, nc = parts[n]
                ys_ref[j, pl.ds(r0, MH), pl.ds(c0, nc)] = (
                    g[:, c0:c0 + nc] * v + ys[r0:r0 + MH, c0:c0 + nc])
                o_copy(j, n).start()

            for k in (0, 3, 4, 6, 2, 1, 5):
                if k in SUMS:
                    a = [lo_ref[n, :, pl.ds(SUMS.index(k) * DH, DH)] for n in range(H)]
                elif k == 2:
                    a = [_as_bf16(wot_ref[n, pl.ds(0, MH // 2), pl.ds(0, DH)]) for n in range(H)]
                else:
                    a = [_as_bf16(wot_ref[n, pl.ds(MH // 2, MH // 2), pl.ds(DH, DH)]) for n in range(H)]
                b = [ctx_ref[n, rows, pl.ds(k * DH, DH)] for n in range(H)]
                m[k] = _dot_nt(jnp.concatenate(a, axis=1), jnp.concatenate(b, axis=1))
            emit(0, jnp.concatenate([(m[0] + m[3]) + (m[6] - m[4]), m[2] + m[4]], axis=1))
            emit(1, m[1] + m[3])
            emit(2, ((m[0] + m[2]) - m[1]) + m[5])
        return 0

    assert TO == 2 * TQ and TO == TS
    no = S // TO
    jax.lax.fori_loop(0, no // O_UNROLL, o_step, 0)
    for j in range(no):
        for n in range(3):
            o_copy(j, n).wait()


@jax.jit
def pallas_gated_mix__compressed_kv_cla__ssm_conv_s5__prompt_kernel(
    A_x: jax.Array,
    A_c_kv: jax.Array,
    A_w_q: jax.Array,
    A_w_uk: jax.Array,
    A_w_uv: jax.Array,
    A_w_o: jax.Array,
    B_x: jax.Array,
    B_Lambda_re: jax.Array,
    B_Lambda_im: jax.Array,
    B_B_re: jax.Array,
    B_B_im: jax.Array,
    B_C_re: jax.Array,
    B_C_im: jax.Array,
    B_log_dt: jax.Array,
    B_Dskip: jax.Array,
    gate_w: jax.Array,
):
    del B_x
    _, S, M = A_x.shape
    C = A_c_kv.shape[2]
    H, D = A_w_q.shape[1], A_w_q.shape[2]
    PP = (M + LANE - 1) // LANE * LANE

    hbm = pl.BlockSpec(memory_space=pl.ANY)
    out_t = pl.pallas_call(
        functools.partial(_kernel, S=S, M=M, H=H, D=D),
        in_specs=[hbm] * 15,
        out_specs=hbm,
        out_shape=jax.ShapeDtypeStruct((M, S), F32),
        scratch_shapes=[
            pltpu.VMEM((M, S), BF16),
            pltpu.VMEM((S // 2, M), U32),
            pltpu.VMEM((5, S // 4, PP // 2), U32),
            pltpu.VMEM((S // 2, C), U32),
            pltpu.VMEM((49, S // 8, C // 4), U32),
            pltpu.VMEM((H // 2, M, D), U32),
            pltpu.VMEM((H // 2, C, D), U32),
            pltpu.VMEM((H // 2, C, D), U32),
            pltpu.VMEM((H, M // 2, D), U32),
            pltpu.VMEM((H, M // 2, 5 * D // 2), BF16),
            pltpu.VMEM((M, M), U32),
            pltpu.VMEM((M // 2, M), U32),
            pltpu.VMEM((M // 2, M), U32),
            pltpu.VMEM((S + 8, 2 * M), F32),
            pltpu.VMEM((S // TO, M, TO), F32),
            pltpu.VMEM((S // TO, 8, TO), F32),
            pltpu.VMEM((2, 8, PP), F32),
            pltpu.VMEM((10, 8, PP), F32),
            pltpu.VMEM((2, M, LANE), F32),
            pltpu.VMEM((2, 16, H // 2, D), U32),
            pltpu.VMEM((2, 2, H // 2, LANE), F32),
        ] + [pltpu.VMEM((M,), BF16)] * 5 + [
            pltpu.VMEM((H // 2, 4, S // 2, D), BF16),
            pltpu.VMEM((H, S // 2, 7 * D // 2), BF16),
            pltpu.SMEM((1,), jnp.int32),
            pltpu.SemaphoreType.DMA((5, H // 2)),
            pltpu.SemaphoreType.DMA((4,)),
            pltpu.SemaphoreType.DMA((7,)),
            pltpu.SemaphoreType.DMA((5,)),
            pltpu.SemaphoreType.DMA((3, S // TO)),
        ],
        compiler_params=pltpu.CompilerParams(
            vmem_limit_bytes=124 * 1024 * 1024,
            disable_semaphore_checks=True,
            disable_bounds_checks=True,
        ),
    )(
        jnp.swapaxes(A_x, 1, 2).reshape(M, S), A_c_kv.reshape(S, C),
        A_w_q, A_w_uk, A_w_uv, jnp.swapaxes(A_w_o, 1, 2),
        B_B_re, B_B_im, B_C_re, B_C_im,
        B_Lambda_re, B_Lambda_im, B_log_dt, B_Dskip, gate_w,
    )
    return jnp.swapaxes(out_t.reshape(1, M, S), 1, 2)
```

```python
import functools

import jax
import jax.numpy as jnp
import jax.experimental.pallas as pl
import jax.experimental.pallas.tpu as pltpu

F32 = jnp.float32
BF16 = jnp.bfloat16
U32 = jnp.uint32

NT_DIMS = (((1,), (1,)), ((), ()))
LOG2E = 1.4426950408889634

TQ = 128
TP = 256
TU = 512
TO = 256
LANE = 128
HALF = LANE // 2
SSM_SPLIT = False
REMAT = (0, 1, 2, 3, 5, 6)
Q_REMAT = (0, 1, 2, 3, 5, 6)
UNIFORM_DIAG = False
SCHEDULE = "d0 h2 t0 t1 c2 p0 p1 t2 c3 u3 b2 t3 c4 p2 b3 t4 c5 p3 p4 t5 c6 b5 t6 c7 t7 p5 b6 b7 p6 p7"
Q_SCHEDULE = "r0 q2 q3 q4 q5 q6 q7"
SIDE = "ccccxy"
C_DUE = (55,)
C_START = (14, 20, 30, 39, 40, 52)
O_SCHEDULE = "a3 a0 a4 m0 g0 m3 a6 m1 a2 a1 a5 n3 b0 m2 b3 n2 g1 n1 b6 b4 n0 b2 b1 b5"
G7 = tuple((i,) for i in range(7))
G4 = ((0, 1), (2, 3), (4, 5), (6,))
G2 = ((0, 1, 2, 3), (4, 5, 6))
G1 = (tuple(range(7)),)
C_GROUPS = G2
C_EXTRA = 3
X_GROUPS = G2
X_EXTRA = 0
U_SCHEDULE = "t4 u2 x0 u3 x1 t6 u4 x4 x5 u5 x3 u6 x2 x7 v7 x6 w7"
PACE_FROM = 2
PACE_ROWS = 8
TWO_PASS = False
CHAIN_ALL = True
L_TIE = 3
PV_DIAG = (0, 5, 0, 1, 0, 3, 3, 0)
EARLY_SUM = (1, 7)
EARLY_SHIFT = 0
PRENORM0 = False
LOOK = (0, 0, 0, 0, 0, 0, 104, 0)
PACE2_FROM = 2
PACE2_EXTRA = 1


def _dot_nt(a, b):
    return jax.lax.dot_general(a, b, NT_DIMS, preferred_element_type=F32)


def _unpack(w32, shift):
    v = (w32 << shift) & jnp.uint32(0xFFFF0000)
    return pltpu.bitcast(v, F32)


def _as_bf16(w32):
    return pltpu.bitcast(w32, BF16)


def _as_u32(v):
    return pltpu.bitcast(v, U32)


def _strassen_lhs(a11, a12, a21, a22):
    return [a11 + a22, a21 + a22, a11, a22, a11 + a12, a21 - a11, a12 - a22]


def _strassen_rhs(b11, b12, b21, b22):
    return [b11 + b22, b11, b12 - b22, b21 - b11, b22, b11 + b12, b21 + b22]


def _strassen_out(m):
    return ((m[0] + m[3]) + (m[6] - m[4]), m[2] + m[4],
            m[1] + m[3], (m[0] - m[1]) + (m[2] + m[5]))


def _quads(a):
    m, n = a.shape[0] // 2, a.shape[1] // 2
    return a[:m, :n], a[:m, n:], a[m:, :n], a[m:, n:]


def _hold(v, last, zero):
    if not last:
        return v
    z = jnp.tile(_as_u32(last[0]) & zero.astype(U32), (v.shape[0] // 8, pl.cdiv(v.shape[1], LANE)))
    return pltpu.bitcast(_as_u32(v) | z[:, :v.shape[1]], v.dtype)


def _lhs_operands(a, last, zero, groups, extra):
    first = (0, 2, 0, 3, 0, 2, 1)
    for k in range(7):
        q = list(_quads(a))
        q[first[k]] = _hold(q[first[k]], last, zero)
        l = _strassen_lhs(*q)[k]
        out = []
        for grp in groups:
            q = list(_quads(l))
            if out:
                for b in set(first[i] for i in grp):
                    q[b] = _hold(q[b], last, zero)
            v = jnp.concatenate([_strassen_lhs(*q)[i] for i in grp], axis=1)
            out.append(_as_u32(v.astype(BF16)))
            last[:] = [functools.reduce(
                jnp.bitwise_or, [out[-1][:, c:c + LANE] for c in range(0, v.shape[1], LANE)])]
            for _ in range(extra):
                last[:] = [last[0] + last[0]]
        yield jnp.concatenate(out, axis=1)


SUMS = (0, 1, 4, 5, 6)
Q_ORDER = (1, 6, 2, 3, 0, 5, 4)
Q_INNER = (1, 3, 5, 0, 2, 4, 6)
ORDER = (1, 3, 2, 4, 0, 5, 6)
INNER = (1, 3, 6, 0, 2, 4, 5)
QK_ORDER = (0, 2, 4, 3, 1, 6, 5)
QK_GROUP = 1
QK_LAG = 2
QK_TIE_K = 3
QK_RUNMAX = True
DIAG_FIRST = False
PV_ORDER = (2, 1, 3, 4, 5, 0, 6)


def _kernel(xt_hbm, c_hbm, wq_hbm, wuk_hbm, wuv_hbm, wot_hbm,
            bre_hbm, bim_hbm, cre_hbm, cim_hbm,
            lre_hbm, lim_hbm, ldt_hbm, dsk_hbm, gw_hbm,
            o_hbm,
            xt_ref, x_ref, lx_ref, c_ref, l_ref, wq_buf, wk_buf, wv_buf, wot_ref, lo_ref,
            b_ref, cre_ref, cim_ref, u_ref, ys_ref, st_ref, co_ref, col_ref, smp_ref, vsc_ref,
            lre_ref, lim_ref, ldt_ref, dsk_ref, gw_ref,
            q_ref, ctx_ref, zero_ref, wsem, xsem, msem, vsem, osem,
            *, S, M, H, D):
    P = M
    FT = P // LANE
    PF = FT * LANE
    assert P - PF == HALF
    PP = PF + LANE
    NP = H // 2
    TS = S // NP
    CH, DH, MH, TH = c_ref.shape[1] // 2, D // 2, M // 2, TP // 2

    def w_copy(k, pair):
        src, dst = ((wq_hbm, wq_buf), (wuk_hbm, wk_buf), (wuv_hbm, wv_buf))[k]
        return pltpu.make_async_copy(src.bitcast(U32).at[:, pair, :], dst.at[pair], wsem.at[k, pair])

    def wo_copy(pair):
        heads = pl.ds(2 * pair, 2)
        return pltpu.make_async_copy(wot_hbm.bitcast(U32).at[heads], wot_ref.at[heads],
                                     wsem.at[3, pair])

    def x_copy(t0, n, k):
        cols = pl.ds(t0, n)
        return pltpu.make_async_copy(xt_hbm.at[:, cols], xt_ref.at[:, cols], xsem.at[k])

    x_cps = [x_copy(0, TU // 2, 0), x_copy(TU // 2, TU // 2, 1), x_copy(TU, TU, 2),
             x_copy(2 * TU, S - 2 * TU, 3)]

    bre32, bim32 = bre_hbm.bitcast(U32), bim_hbm.bitcast(U32)
    b_cps = [
        pltpu.make_async_copy(bre32, b_ref.at[pl.ds(0, P // 2), :], msem.at[0]),
        pltpu.make_async_copy(bim32.at[pl.ds(PF // 2, HALF // 2), :],
                              b_ref.at[pl.ds(P // 2, HALF // 2), :], msem.at[1]),
        pltpu.make_async_copy(bim32.at[pl.ds(0, PF // 2), :],
                              b_ref.at[pl.ds(PP // 2, PF // 2), :], msem.at[2]),
    ]
    cre_cp = pltpu.make_async_copy(cre_hbm.bitcast(U32), cre_ref, msem.at[3])
    cim_cp = pltpu.make_async_copy(cim_hbm.bitcast(U32), cim_ref, msem.at[4])

    def c_copy(r):
        rows = pl.ds(pl.multiple_of(r * TH, TH), TH)
        return pltpu.make_async_copy(c_hbm.bitcast(U32).at[rows], c_ref.at[rows], wsem.at[4, r])

    smp_cps = [pltpu.make_async_copy(src.bitcast(U32).at[pl.ds(0, smp_ref.shape[1])],
                                     smp_ref.at[k], msem.at[5 + k])
               for k, src in enumerate((wuk_hbm, wuv_hbm))]
    v_cps = [pltpu.make_async_copy(src, dst, vsem.at[k]) for k, (src, dst) in enumerate(
        ((lre_hbm, lre_ref), (lim_hbm, lim_ref), (ldt_hbm, ldt_ref),
         (dsk_hbm, dsk_ref), (gw_hbm, gw_ref)))]

    for cp in v_cps:
        cp.start()
    for cp in x_cps[:1] + b_cps + x_cps[1:] + smp_cps:
        cp.start()
    for p in range(NP):
        w_copy(0, p).start()
        wo_copy(p).start()
        c_copy(p).start()
    for p in range(NP):
        w_copy(1, p).start()
        w_copy(2, p).start()
    cre_cp.start()
    cim_cp.start()

    zero_ref[0] = 0
    u_ref[pl.ds(0, 8), :] = jnp.zeros((8, u_ref.shape[1]), F32)
    st_ref[...] = jnp.zeros(st_ref.shape, F32)
    for cp in v_cps:
        cp.wait()

    row = lambda r: r[...].astype(F32).reshape(1, P)
    lre, lim = row(lre_ref), row(lim_ref)
    dt = jnp.exp(row(ldt_ref)).astype(BF16).astype(F32)
    e = jnp.exp(dt * lre)
    ang = dt * lim
    ar = e * jnp.cos(ang)
    ai = e * jnp.sin(ang)
    sc = jnp.maximum(jnp.abs(lre), jnp.abs(lim))
    nre, nim = lre / sc, lim / sc
    den = (nre * nre + nim * nim) * sc
    gr = 2.0 * ((ar - 1.0) * nre + ai * nim) / den
    gi = 2.0 * (ai * nre - (ar - 1.0) * nim) / den

    def put(k, full, lo, hi):
        v = jnp.concatenate([full[:, :PF], lo[:, PF:], hi[:, PF:]], axis=1)
        co_ref[k] = jnp.broadcast_to(v, (8, PP))

    put(0, gr, gr, -gr)
    put(1, -gi, -gi, -gi)
    pr, pi = ar, -ai
    for j in range(1, 5):
        put(2 * j, pr, pr, pr)
        put(2 * j + 1, -pi, -pi, pi)
        pr, pi = pr * pr - pi * pi, 2.0 * pr * pi

    zpad = jnp.zeros((1, PP - P), F32)
    for k, r in enumerate((dsk_ref, gw_ref)):
        v = jnp.concatenate([row(r), zpad], axis=1)
        col_ref[k] = jnp.broadcast_to(v, (LANE, PP)).T[:M]

    XH = PP // 2

    def transpose_x(t0, n):
        x_ref[pl.ds(t0 // 2, n // 2), :] = _as_u32(xt_ref[:, pl.ds(t0, n)].T)

    zero1, last1 = zero_ref[0], []

    def x_sums(r):
        for n in range(TH // 32):
            x = jnp.concatenate(
                [x_ref[pl.ds(r * TH + g * (TH // 4) + 8 * n, 8), :] for g in range(4)], axis=0)
            x = _as_bf16(_hold(x, last1, zero1)).astype(F32)
            x = jnp.concatenate([x, jnp.zeros((x.shape[0], PP - M), F32)], axis=1)
            for k, v in enumerate(_lhs_operands(x, last1, zero1, X_GROUPS, X_EXTRA)):
                lx_ref[k, pl.ds(r * (TH // 4) + 8 * n, 8), :] = v

    def proj_u(t0, n, lo=0, hi=2 * P, due=False, mark=False):
        x = x_ref[pl.ds(t0 // 2, n // 2), :]
        if due:
            x = jnp.concatenate([_hold(x[:8], last1, zero1), x[8:]], axis=0)
        u = _dot_nt(_as_bf16(x), _as_bf16(b_ref[lo // 2:hi // 2, :]))
        u_ref[pl.ds(t0 + 8, n), lo:hi] = u
        if mark:
            last1[:] = [functools.reduce(jnp.bitwise_or, last1 + [_as_u32(u[:8, :LANE])])]

    x_cps[0].wait()
    transpose_x(0, TU // 2)
    b_cps[0].wait()
    b_cps[1].wait()
    proj_u(0, TU // 2, 0, PP)
    b_cps[2].wait()
    x_cps[1].wait()
    proj_u(0, TU // 2, PP)
    transpose_x(TU // 2, TU // 2)
    x_cps[2].wait()
    proj_u(TU // 2, TU // 2)
    transpose_x(TU, TU)
    x_cps[3].wait()
    for cp in smp_cps:
        cp.wait()
    for e in range(2):
        mag = [jnp.sum(jnp.sum(jnp.abs(_unpack(smp_ref[k], jnp.uint32(16 - 16 * e))), axis=0),
                       axis=1, keepdims=True) for k in range(2)]
        ex = [jnp.broadcast_to(pltpu.bitcast(v, jnp.int32) >> 23, (NP, LANE)) for v in mag]
        d = jnp.where((ex[0] > 0) & (ex[1] > 0), jnp.clip(ex[0] - ex[1], -40, 40), 0)
        vsc_ref[0, e] = pltpu.bitcast((127 + d) << 23, F32)
        vsc_ref[1, e] = pltpu.bitcast((127 - d) << 23, F32)
    ops = dict(u=lambda r: proj_u(r * TP, TP, mark=True), t=lambda r: transpose_x(r * TP, TU), x=x_sums,
               v=lambda r: proj_u(r * TP, TP, 0, 6 * LANE, mark=True),
               w=lambda r: proj_u(r * TP, TP, 6 * LANE, due=True))
    for op in U_SCHEDULE.split():
        ops[op[0]](int(op[1:]))

    def q_step(j, _):
        w_copy(0, j).wait()
        wo_copy(j).wait()
        c_copy(j).wait()
        zero = zero_ref[0]
        after = lambda w, v: w | (_as_u32(v) & zero.astype(U32))
        last, recent = [], []
        wq32 = wq_buf[j]
        wq32 = jnp.concatenate([wq32, jnp.zeros((PP - M, D), U32)], axis=0)
        rw = []
        for k in range(7):
            z = (zero << k).astype(U32) if k in Q_REMAT else jnp.uint32(0)
            w0 = pltpu.bitcast(wq32 << (z + 16), F32)
            w1 = pltpu.bitcast(wq32 & (z + jnp.uint32(0xFFFF0000)), F32)
            wl = jnp.concatenate([w0[:, :DH], w1[:, :DH]], axis=1)
            wr = jnp.concatenate([w0[:, DH:], w1[:, DH:]], axis=1)
            rw.append(_strassen_rhs(*_quads(_strassen_rhs(wl[:XH], wr[:XH], wl[XH:], wr[XH:])[k])))
        qscale = (D ** -0.5) * LOG2E

        def proj_q(r, n=1):
            ms = [None] * 7
            TI = TH // 2
            for k in Q_ORDER:
                mi = [None] * 7
                for i in Q_INNER:
                    a = lx_ref[k, pl.ds(r * TI // 2, n * TI // 2), pl.ds(i * LANE, LANE)]
                    b = rw[k][i]
                    at = 7 * r + n * Q_ORDER.index(k) if i == Q_INNER[0] else -1
                    if at in C_DUE:
                        a = jnp.concatenate([_hold(a[:8], last, zero), a[8:]], axis=0)
                    mi[i] = jnp.dot(_as_bf16(a), b.astype(BF16), preferred_element_type=F32)
                    recent.append(mi[i])
                    for _ in range(C_START.count(at)):
                        if SIDE[len(SIDE) - len(side)] not in "xy":
                            last[:] = [_as_u32(mi[i][:8]) | last[0] if last else _as_u32(mi[i][:8])]
                        side.pop(0)()
                c11, c12, c21, c22 = _strassen_out(mi)
                top, bot = jnp.concatenate([c11, c12], axis=1), jnp.concatenate([c21, c22], axis=1)
                ms[k] = jnp.concatenate(
                    [v[b * TI:(b + 1) * TI] for b in range(n) for v in (top, bot)], axis=0)
            for k, v in enumerate(_strassen_out(ms)):
                q_ref[j, k, pl.ds(r * TH, n * TH), :] = (v * qscale).astype(BF16)

        pieces = []

        def c_sums():
            n = len(pieces)
            pieces.append(n)
            c = jnp.concatenate(
                [c_ref[pl.ds(pl.multiple_of(j * TH + g * (TH // 4) + 8 * n, 8), 8), :] for g in range(4)],
                axis=0)
            c = _as_bf16(_hold(c, last, zero)).astype(F32)
            rows = pl.ds(pl.multiple_of(j * (TH // 4) + 8 * n, 8), 8)
            for k, v in enumerate(_lhs_operands(c, last, zero, C_GROUPS, C_EXTRA)):
                l_ref[k, rows, :] = v

        def wo_sums(e):
            for n in range(0, MH // 2, 16):
                w = jnp.concatenate([wot_ref[2 * j + e, pl.ds(g * MH // 2 + n, 16), :] for g in range(2)],
                                    axis=0)
                ls = _strassen_lhs(*_quads(_as_bf16(_hold(w, last, zero)).astype(F32)))
                v = jnp.concatenate([ls[k] for k in SUMS], axis=1)
                lo_ref[2 * j + e, pl.ds(2 * n, 32), :] = v.astype(BF16)
                last[:] = [functools.reduce(jnp.bitwise_or, [
                    _as_u32(v[g:g + 8, c:c + LANE]) for g in (0, 16) for c in range(0, v.shape[1], LANE)])]

        def wo_free(e):
            z = _as_u32(jnp.concatenate([v[:TH // 2] for v in recent[-7:]], axis=0)) & zero.astype(U32)
            w = wot_ref[2 * j + e] | jnp.concatenate([z[:MH], z[MH:]], axis=1)
            ls = _strassen_lhs(*_quads(_as_bf16(w).astype(F32)))
            lo_ref[2 * j + e] = jnp.concatenate([ls[k] for k in SUMS], axis=1).astype(BF16)

        side = [dict(c=c_sums, x=lambda: wo_free(0), y=lambda: wo_free(1), v=lambda: wo_sums(0), w=lambda: wo_sums(1), n=lambda: None)[k] for k in SIDE]
        ops = dict(q=proj_q, r=lambda r: proj_q(r, 2), s=lambda r: proj_q(r, 3))
        for op in Q_SCHEDULE.split():
            ops[op[0]](int(op[1:]))
        assert not side
        return 0

    assert S // TP == NP
    jax.lax.fori_loop(0, NP, q_step, 0)
    for p in range(NP):
        w_copy(1, p).wait()
        w_copy(2, p).wait()
    cre_cp.wait()
    cim_cp.wait()

    def head_step(h, _):
        slot = h >> 1
        zero = zero_ref[0]
        shift = (16 - 16 * (h & 1)).astype(U32)
        vscale, vinv = [vsc_ref[k, h & 1, pl.ds(slot, 1), :] for k in range(2)]
        rw = []
        for k in range(7):
            sh = shift + (zero << k).astype(U32) if k in REMAT else shift
            rk = _strassen_rhs(*_quads(_unpack(wk_buf[slot], sh)))[k]
            rv = _strassen_rhs(*_quads(_unpack(wv_buf[slot], sh)))[k] * vscale
            rw.append(_strassen_rhs(rk[:CH // 2], rv[:CH // 2], rk[CH // 2:], rv[CH // 2:]))
        causal = (jax.lax.broadcasted_iota(jnp.int32, (TQ, TQ), 1)
                  <= jax.lax.broadcasted_iota(jnp.int32, (TQ, TQ), 0))

        ks, rks, vs, rvs, ss, mxs, chains = [], [], [], [], {}, {}, [None]

        def proj_kv(r, n=1):
            TI = TH // 2
            ms = [None] * 7
            for k in ORDER:
                mi = [None] * 7
                for i in INNER:
                    a = l_ref[k, pl.ds(r * TI // 2, n * TI // 2), pl.ds(i * CH // 2, CH // 2)]
                    mi[i] = jnp.dot(_as_bf16(a), rw[k][i].astype(BF16), preferred_element_type=F32)
                c11, c12, c21, c22 = _strassen_out(mi)
                top, bot = jnp.concatenate([c11, c12], axis=1), jnp.concatenate([c21, c22], axis=1)
                ms[k] = jnp.concatenate(
                    [v[b * TI:(b + 1) * TI] for b in range(n) for v in (top, bot)], axis=0)
                if k != ORDER[-1]:
                    yield
            c = _strassen_out(ms)
            for b in range(n):
                c11, c12, c21, c22 = [v[b * TH:(b + 1) * TH, :DH] for v in c]
                ks.extend([jnp.concatenate([c11, c12], axis=1), jnp.concatenate([c21, c22], axis=1)])
                rks.append(_strassen_rhs(c11, c21, c12, c22))
                c11, c12, c21, c22 = [v[b * TH:(b + 1) * TH, DH:] for v in c]
                vs.extend([jnp.concatenate([c11, c12], axis=1), jnp.concatenate([c21, c22], axis=1)])
                rvs.append(_strassen_rhs(c11, c12, c21, c22))

        def qk_pair(j):
            cols = pl.ds(pl.multiple_of((h & 1) * DH, DH), DH)
            qf = [q_ref[slot, k, j * TQ:(j + 1) * TQ, cols].astype(F32) for k in range(4)]
            q = jnp.concatenate([jnp.concatenate(qf[:2], axis=1), jnp.concatenate(qf[2:], axis=1)], axis=0)
            lq = _strassen_lhs(*qf)
            s1, s2, done, mx = [], [], [], []

            def diag():
                if UNIFORM_DIAG:
                    return (_dot_nt(q[:TQ].astype(BF16), ks[2 * j].astype(BF16)),
                            _dot_nt(q[TQ:].astype(BF16),
                                    jnp.concatenate(ks[2 * j:2 * j + 2], axis=0).astype(BF16)))
                d = _dot_nt(q.astype(BF16), ks[2 * j].astype(BF16))
                return d[:TQ], jnp.concatenate(
                    [d[TQ:], _dot_nt(q[TQ:].astype(BF16), ks[2 * j + 1].astype(BF16))], axis=1)

            if DIAG_FIRST:
                d1, d2 = diag()
            for t0 in range(0, j, QK_GROUP):
                ts = range(t0, min(t0 + QK_GROUP, j))
                m = [None] * 7
                for k in QK_ORDER:
                    rk = jnp.concatenate([rks[t][k] for t in ts], axis=0).astype(BF16)
                    a = lq[k]
                    if k == QK_TIE_K and len(done) >= QK_LAG:
                        a = tie(a, done[-QK_LAG])
                    m[k] = jax.lax.dot_general(a.astype(BF16), rk, NT_DIMS, preferred_element_type=F32)
                c11 = ((m[0] + m[3]) - m[4]) + m[6]
                c12, c21 = m[2] + m[4], m[1] + m[3]
                c22 = ((m[0] - m[1]) + m[2]) + m[5]
                if QK_RUNMAX:
                    x1, x2 = jnp.maximum(c11, c12), jnp.maximum(c21, c22)
                    if mx:
                        x1, x2 = jnp.maximum(x1, mx[0]), jnp.maximum(x2, mx[1])
                    mx[:] = [x1, x2]
                    z = _as_u32(x1) | _as_u32(x2)
                else:
                    z = (_as_u32(c11) | _as_u32(c12)) | (_as_u32(c21) | _as_u32(c22))
                done.append(z)
                for n in range(len(ts)):
                    cols = slice(n * TQ, (n + 1) * TQ)
                    s1 += [c11[:, cols], c12[:, cols]]
                    s2 += [c21[:, cols], c22[:, cols]]
            yield
            if not DIAG_FIRST:
                d1, d2 = diag()
            ss[2 * j] = jnp.concatenate(s1 + [d1], axis=1)
            ss[2 * j + 1] = jnp.concatenate(s2 + [d2], axis=1)
            if mx:
                mxs[2 * j], mxs[2 * j + 1] = mx

        def tie(a, b):
            return pltpu.bitcast(_as_u32(a) | (_as_u32(b) & zero.astype(U32)), F32)

        def exp_rows(s, m, pace, rows, chain=None):
            mb = m
            ps, parts = [], []
            for g in range(0, TQ, rows):
                mg = mb[g:g + rows]
                if pace and (parts or chain is not None):
                    mg = tie(mg, parts[-1] if parts else chain)
                pg = [jnp.exp2(s[g:g + rows, t * LANE:(t + 1) * LANE] - mg)
                      for t in range(s.shape[1] // LANE)]
                ps.append(jnp.concatenate(pg, axis=1))
                parts.append(functools.reduce(lambda a, b: a + b, pg))
            return jnp.concatenate(ps, axis=0), jnp.concatenate(parts, axis=0)

        def masked(i):
            lo = i * TQ
            s = ss.pop(i)
            sd = jnp.where(causal, s[:, lo:], -1e9 * LOG2E)
            s = sd if i == 0 else jnp.concatenate([s[:, :lo], sd], axis=1)
            t = jnp.concatenate([mxs[i], s[:, i // 2 * 2 * TQ:]], axis=1) if i in mxs else s
            if LOOK[i // 2] > 0:
                return s, functools.reduce(
                    jnp.maximum, [t[:, c:c + LANE] for c in range(0, t.shape[1], LANE)])
            return s, jnp.broadcast_to(jnp.max(t, axis=-1, keepdims=True), (TQ, LANE))

        def exp_rows2(s, mx, parts, look, both):
            ps = []
            for g in range(0, TQ, 8):
                mg = mx[g:g + 8]
                if len(parts) >= look:
                    mg = tie(mg, parts[-look])
                mg = jnp.broadcast_to(jnp.max(mg, axis=-1, keepdims=True), (8, LANE))
                if both and parts:
                    mg = tie(mg, parts[-1])
                pg = [jnp.exp2(s[g:g + 8, t * LANE:(t + 1) * LANE] - mg)
                      for t in range(s.shape[1] // LANE)]
                ps.append(jnp.concatenate(pg, axis=1))
                parts.append(functools.reduce(lambda a, b: a + b, pg))
            return jnp.concatenate(ps, axis=0), jnp.concatenate(parts[-(TQ // 8):], axis=0)

        def pv(j):
            (s1, m1), (s2, m2) = masked(2 * j), masked(2 * j + 1)
            if LOOK[j] > 0:
                parts = []
                p1, l1 = exp_rows2(s1, m1, parts, LOOK[j] % 100, LOOK[j] > 100)
                p2, l2 = exp_rows2(s2, m2, parts, LOOK[j] % 100, LOOK[j] > 100)
            else:
                p1, l1 = exp_rows(s1, m1, LOOK[j] == 0, PACE_ROWS, chains[0] if CHAIN_ALL else None)
                if j in EARLY_SUM:
                    ls = jnp.broadcast_to(jnp.sum(l1, axis=-1, keepdims=True), (TQ, LANE))
                    k = 8 * EARLY_SHIFT
                    if k:
                        ls = jnp.concatenate([_as_u32(ls[:k]) | _as_u32(ls[k:2 * k]), _as_u32(ls[2 * k:]),
                                              _as_u32(ls[:k])], axis=0)
                    m2 = tie(m2, ls)
                p2, l2 = exp_rows(s2, m2, LOOK[j] == 0, PACE_ROWS, l1[TQ - 8:])
            chains[0] = l2[TQ - 8:]
            if L_TIE == 1:
                l1 = tie(l1, l2)
            elif L_TIE == 2:
                l1 = jnp.concatenate([tie(l1[:8], l2[:8]), l1[8:]], axis=0)
            elif L_TIE == 3:
                l1 = jnp.concatenate([tie(l1[:8], l1[TQ - 8:]), l1[8:]], axis=0)
            l1, l2 = [jnp.sum(l, axis=-1, keepdims=True) for l in (l1, l2)]
            lo = 2 * j * TQ
            cat = lambda xs, axis: jnp.concatenate(xs, axis=axis)
            dot = lambda a, b: jnp.dot(a.astype(BF16), b.astype(BF16), preferred_element_type=F32)

            def recip(l):
                rl = pl.reciprocal(l, approx=True)
                return rl * (2.0 - l * rl)

            r1, r2 = recip(l1), recip(l2)
            rho = l1 * r2
            r1, r2 = r1 * vinv, r2 * vinv
            if j == 0 and PRENORM0:
                p1, p2 = p1 * r1, p2 * cat([r2, r2], 1)
                r1 = r2 = jnp.ones((1, LANE), F32)
            def diag():
                dg = dot(cat([p1[:, lo:], p2[:, lo:lo + TQ]], 0), vs[2 * j])
                return dg[:TQ], dg[TQ:] + dot(p2[:, lo + TQ:], vs[2 * j + 1])

            if j == 0:
                c1, c2 = diag()
            if j > 0:
                tiles = lambda p, o: cat([p[:, (2 * t + o) * TQ:(2 * t + o + 1) * TQ] for t in range(j)], 1)
                a11, a12, a21, a22 = tiles(p1, 0), tiles(p1, 1), tiles(p2, 0), tiles(p2, 1)
                a22r = a22 * rho
                lp = [a11 + a22r, a21 + a22, a11, a22, a11 + a12, a21 * rho - a11, a12 - a22r]
                m = [None] * 7
                for n, k in enumerate(PV_ORDER):
                    if n == PV_DIAG[j]:
                        c1, c2 = diag()
                    if k == PV_ORDER[-1]:
                        yield
                    m[k] = dot(lp[k], cat([rvs[t][k] for t in range(j)], 0))
                c1 = c1 + cat([(m[0] - m[4]) + (m[6] + m[3] * rho), m[2] + m[4]], 1)
                c2 = (c2 + cat([m[1] + m[3], -m[1]], 1)) * cat([r2, r2], 1)
                c2 = cat([c2[:, :DH], c2[:, DH:] + ((m[0] + m[2]) + m[5]) * r1], 1)
            else:
                c2 = c2 * cat([r2, r2], 1)
            c1 = c1 * cat([r1, r1], 1)
            ctx_ref[h, j * TQ:(j + 1) * TQ, :] = cat(
                _strassen_rhs(c1[:, :DH], c2[:, :DH], c1[:, DH:], c2[:, DH:]), 1).astype(BF16)

        assert TP == 2 * TQ
        pvs = [pv(j) for j in range(S // TP)]
        qks = [qk_pair(j) for j in range(S // TP)]
        kvs = {}

        def kv_part(r, n, steps):
            g = kvs.setdefault(r, proj_kv(r, n))
            for _ in range(steps):
                next(g, None)

        ops = dict(c=lambda r: kv_part(r, 1, 7), d=lambda r: kv_part(r, 2, 7),
                   e=lambda r: kv_part(r, 3, 7), f=lambda r: kv_part(r, 4, 7), i=lambda r: kv_part(r, 1, 2),
                   x=lambda r: kv_part(r // 10, 1, r % 10), h=lambda r: kv_part(r, 1, 4), g=lambda r: kv_part(r, 2, 4),
                   t=lambda j: list(qks[j]), u=lambda j: next(qks[j]), p=lambda j: list(pvs[j]), b=lambda j: next(pvs[j]))
        for op in SCHEDULE.split():
            ops[op[0]](int(op[1:]))
        return 0

    jax.lax.fori_loop(0, H, head_step, 0)

    parts = ((0, 0, TO), (MH, 0, TQ), (MH, TQ, TQ))

    def o_copy(j, n):
        r0, c0, nc = parts[n]
        return pltpu.make_async_copy(
            ys_ref.at[j, pl.ds(r0, MH), pl.ds(c0, nc)],
            o_hbm.at[pl.ds(r0, MH), pl.ds(pl.multiple_of(j * TO + c0, TQ), nc)], osem.at[n, j])

    def o_step(jj, _):
        zero = zero_ref[0]
        js = (2 * jj, 2 * jj + 1)
        t0 = [pl.multiple_of(j * TS, TS) for j in js]
        last, state, ys, gates, m, recent = [], {}, [None, None], {}, [{}, {}], []

        def ssm_tile(u, t):
            rows = pl.ds(t0[u], TS + 8)
            cr, ci = pl.ds(t * LANE, LANE), pl.ds(PP + t * LANE, LANE)
            co = [co_ref[k, :, cr] for k in range(10)]
            u0 = u_ref[rows, cr]
            u1 = u_ref[rows, ci] if t < FT else pltpu.roll(u0, HALF, 1)
            mul = lambda k, x: (co[k] * x[0] + co[k + 1] * x[1], co[k] * x[1] - co[k + 1] * x[0])
            sub = jax.lax.broadcasted_iota(jnp.int32, (8, LANE), 0)
            s = state.get(t) or (st_ref[0, :, cr], st_ref[1, :, cr])
            prev, gs = [None] * 3, []
            for k in range(TS // 8 + 1):
                x0, x1 = u0[8 * k:8 * k + 8], u1[8 * k:8 * k + 8]
                x0 = _hold(x0, last, zero)
                w = (co[0] * x0 + co[1] * x1, co[1] * x0 - co[0] * x1)
                for i in range(3):
                    cur = [pltpu.roll(v, 1 << i, 0) for v in w]
                    old = cur if k == 0 else prev[i]
                    d = mul(2 * i + 2, [jnp.where(sub < (1 << i), o, c) for o, c in zip(old, cur)])
                    w = [p + q for p, q in zip(d, w)]
                    prev[i] = cur
                if k > 0:
                    s = [p + q for p, q in zip(mul(8, s), w)]
                    gs.append(jnp.concatenate(s, axis=1) if t < FT else s[0])
                    last[:] = [s[0]]
            state[t] = s
            if u == 1:
                st_ref[0, :, cr] = s[0]
                st_ref[1, :, cr] = s[1]
            if t < FT:
                cc = jnp.concatenate([cre_ref[:, cr], cim_ref[:, cr]], axis=1)
            else:
                cc = jnp.concatenate([cre_ref[:, PF:], cim_ref[:, PF:]], axis=1)
            g = jnp.concatenate(gs, axis=0).astype(BF16)
            n = M // 2 if t < FT else M // 4
            y = jnp.concatenate([
                jax.lax.dot_general(_as_bf16(cc[a:a + n]), g, NT_DIMS, preferred_element_type=F32)
                for a in range(0, M // 2, n)], axis=0)
            ys[u] = y if ys[u] is None else y + ys[u]

        def gate(u):
            gcol = _as_u32(col_ref[1]) | (_as_u32(jnp.concatenate(recent[-2:], axis=0)) & zero.astype(U32))
            gcol = jnp.concatenate([pltpu.bitcast(gcol, F32)] * (TS // LANE), axis=1)
            xt = xt_ref[:, pl.ds(t0[u], TS)].astype(F32)
            z = jnp.sum((xt * gcol).astype(BF16).astype(F32), axis=0, keepdims=True)
            rnd = lambda v: v.astype(BF16).astype(F32)
            gates[u] = rnd(1.0 / rnd(1.0 + rnd(jnp.exp(-rnd(z)))))

        def emit(u, n, v):
            r0, c0, nc = parts[n]
            g = gates[u][:, c0:c0 + nc]
            omg = (1.0 - g).astype(BF16).astype(F32)
            dcol = jnp.concatenate([col_ref[0, r0:r0 + MH]] * (nc // LANE), axis=1)
            xt = xt_ref[pl.ds(r0, MH), pl.ds(pl.multiple_of(t0[u] + c0, TQ), nc)].astype(F32)
            b = ys[u][r0:r0 + MH, c0:c0 + nc] + (xt * dcol).astype(BF16).astype(F32)
            ys_ref[js[u], pl.ds(r0, MH), pl.ds(c0, nc)] = g * v + omg * b
            o_copy(js[u], n).start()

        def product(u, k):
            if k in SUMS:
                a = [lo_ref[n, :, pl.ds(SUMS.index(k) * DH, DH)] for n in range(H)]
            elif k == 2:
                a = [_as_bf16(wot_ref[n, pl.ds(0, MH // 2), pl.ds(0, DH)]) for n in range(H)]
            else:
                a = [_as_bf16(wot_ref[n, pl.ds(MH // 2, MH // 2), pl.ds(DH, DH)]) for n in range(H)]
            rows = pl.ds(pl.multiple_of(js[u] * TQ, TQ), TQ)
            b = [ctx_ref[n, rows, pl.ds(k * DH, DH)] for n in range(H)]
            m[u][k] = _dot_nt(jnp.concatenate(a, axis=1), jnp.concatenate(b, axis=1))
            recent.append(m[u][k])

        ops = dict(a=lambda k: product(0, k), b=lambda k: product(1, k), g=gate,
                   m=lambda t: ssm_tile(0, t), n=lambda t: ssm_tile(1, t))
        for op in O_SCHEDULE.split():
            ops[op[0]](int(op[1:]))
        for u, p in enumerate(m):
            emit(u, 0, jnp.concatenate([(p[0] + p[3]) + (p[6] - p[4]), p[2] + p[4]], axis=1))
            emit(u, 1, p[1] + p[3])
            emit(u, 2, ((p[0] + p[2]) - p[1]) + p[5])
        return 0

    assert TO == 2 * TQ and TO == TS
    no = S // TO
    jax.lax.fori_loop(0, no // 2, o_step, 0)
    for j in range(no):
        for n in range(3):
            o_copy(j, n).wait()


@jax.jit
def pallas_gated_mix__compressed_kv_cla__ssm_conv_s5__prompt_kernel(
    A_x: jax.Array,
    A_c_kv: jax.Array,
    A_w_q: jax.Array,
    A_w_uk: jax.Array,
    A_w_uv: jax.Array,
    A_w_o: jax.Array,
    B_x: jax.Array,
    B_Lambda_re: jax.Array,
    B_Lambda_im: jax.Array,
    B_B_re: jax.Array,
    B_B_im: jax.Array,
    B_C_re: jax.Array,
    B_C_im: jax.Array,
    B_log_dt: jax.Array,
    B_Dskip: jax.Array,
    gate_w: jax.Array,
):
    del B_x
    _, S, M = A_x.shape
    C = A_c_kv.shape[2]
    H, D = A_w_q.shape[1], A_w_q.shape[2]
    PP = (M + LANE - 1) // LANE * LANE

    hbm = pl.BlockSpec(memory_space=pl.ANY)
    out_t = pl.pallas_call(
        functools.partial(_kernel, S=S, M=M, H=H, D=D),
        in_specs=[hbm] * 15,
        out_specs=hbm,
        out_shape=jax.ShapeDtypeStruct((M, S), F32),
        scratch_shapes=[
            pltpu.VMEM((M, S), BF16),
            pltpu.VMEM((S // 2, M), U32),
            pltpu.VMEM((7, S // 8, 7 * PP // 4), U32),
            pltpu.VMEM((S // 2, C), U32),
            pltpu.VMEM((7, S // 8, 7 * C // 4), U32),
            pltpu.VMEM((H // 2, M, D), U32),
            pltpu.VMEM((H // 2, C, D), U32),
            pltpu.VMEM((H // 2, C, D), U32),
            pltpu.VMEM((H, M // 2, D), U32),
            pltpu.VMEM((H, M // 2, 5 * D // 2), BF16),
            pltpu.VMEM((M, M), U32),
            pltpu.VMEM((M // 2, M), U32),
            pltpu.VMEM((M // 2, M), U32),
            pltpu.VMEM((S + 8, 2 * M), F32),
            pltpu.VMEM((S // TO, M, TO), F32),
            pltpu.VMEM((2, 8, PP), F32),
            pltpu.VMEM((10, 8, PP), F32),
            pltpu.VMEM((2, M, LANE), F32),
            pltpu.VMEM((2, 8, H // 2, D), U32),
            pltpu.VMEM((2, 2, H // 2, LANE), F32),
        ] + [pltpu.VMEM((M,), BF16)] * 5 + [
            pltpu.VMEM((H // 2, 4, S // 2, D), BF16),
            pltpu.VMEM((H, S // 2, 7 * D // 2), BF16),
            pltpu.SMEM((1,), jnp.int32),
            pltpu.SemaphoreType.DMA((5, H // 2)),
            pltpu.SemaphoreType.DMA((4,)),
            pltpu.SemaphoreType.DMA((7,)),
            pltpu.SemaphoreType.DMA((5,)),
            pltpu.SemaphoreType.DMA((3, S // TO)),
        ],
        compiler_params=pltpu.CompilerParams(
            vmem_limit_bytes=124 * 1024 * 1024,
            disable_semaphore_checks=True,
            disable_bounds_checks=True,
        ),
    )(
        jnp.swapaxes(A_x, 1, 2).reshape(M, S), A_c_kv.reshape(S, C),
        A_w_q, A_w_uk, A_w_uv, jnp.swapaxes(A_w_o, 1, 2),
        B_B_re, B_B_im, B_C_re, B_C_im,
        B_Lambda_re, B_Lambda_im, B_log_dt, B_Dskip, gate_w,
    )
    return jnp.swapaxes(out_t.reshape(1, M, S), 1, 2)
```

```python
import functools

import jax
import jax.numpy as jnp
import jax.experimental.pallas as pl
import jax.experimental.pallas.tpu as pltpu

F32 = jnp.float32
BF16 = jnp.bfloat16
U32 = jnp.uint32

NT_DIMS = (((1,), (1,)), ((), ()))
LOG2E = 1.4426950408889634

TQ = 128
TP = 256
TU = 512
TO = 256
LANE = 128
HALF = LANE // 2
SSM_SPLIT = False
REMAT = (0, 1, 2, 3, 5, 6)
Q_REMAT = (0, 1, 2, 3, 5, 6)
UNIFORM_DIAG = False
SCHEDULE = "d0 h2 t0 t1 c2 p0 p1 t2 c3 u3 b2 t3 c4 p2 b3 t4 c5 p3 p4 t5 c6 b5 t6 c7 t7 p5 b6 b7 p6 p7"
Q_SCHEDULE = "r0 q2 q3 q4 q5 q6 q7"
SIDE = "ccccxy"
C_DUE = (55,)
C_START = (14, 20, 30, 39, 40, 52)
O_SCHEDULE = "a3 a0 a4 m0 g0 m3 a6 m1 a2 a1 a5 n3 b0 m2 b3 n2 g1 n1 b6 b4 n0 b2 b1 b5"
G7 = tuple((i,) for i in range(7))
G4 = ((0, 1), (2, 3), (4, 5), (6,))
G2 = ((0, 1, 2, 3), (4, 5, 6))
G1 = (tuple(range(7)),)
C_GROUPS = G2
C_EXTRA = 3
X_GROUPS = G2
X_EXTRA = 0
U_SCHEDULE = "t4 u2 x0 u3 x1 t6 u4 x4 x5 u5 x3 u6 x2 x7 v7 x6 w7"
PACE_FROM = 2
PACE_ROWS = 8
TWO_PASS = False
CHAIN_ALL = True
L_TIE = 3
U_PAD = 32
CO_PAD = 10
V_PAD = 4
VEC_PAD = 0
ASSOC = 3
Q_ASSOC = 0
PV_DIAG = (0, 5, 0, 1, 0, 3, 3, 0)
EARLY_SUM = (1, 7)
EARLY_SHIFT = 0
PRENORM0 = False
LOOK = (0, 0, 0, 0, 0, 0, 104, 0)
PACE2_FROM = 2
PACE2_EXTRA = 1


def _dot_nt(a, b):
    return jax.lax.dot_general(a, b, NT_DIMS, preferred_element_type=F32)


def _unpack(w32, shift):
    v = (w32 << shift) & jnp.uint32(0xFFFF0000)
    return pltpu.bitcast(v, F32)


def _as_bf16(w32):
    return pltpu.bitcast(w32, BF16)


def _as_u32(v):
    return pltpu.bitcast(v, U32)


def _strassen_lhs(a11, a12, a21, a22):
    return [a11 + a22, a21 + a22, a11, a22, a11 + a12, a21 - a11, a12 - a22]


def _strassen_rhs(b11, b12, b21, b22):
    return [b11 + b22, b11, b12 - b22, b21 - b11, b22, b11 + b12, b21 + b22]


def _strassen_out(m, order=None):
    if order is None:
        return ((m[0] + m[3]) + (m[6] - m[4]), m[2] + m[4],
                m[1] + m[3], (m[0] - m[1]) + (m[2] + m[5]))

    def fold(ks, neg):
        ks = sorted(ks, key=order.index)
        if ks[0] == neg:
            ks[:2] = ks[1::-1]
        return functools.reduce(lambda a, k: a - m[k] if k == neg else a + m[k], ks[1:], m[ks[0]])

    return fold((0, 3, 4, 6), 4), m[2] + m[4], m[1] + m[3], fold((0, 1, 2, 5), 1)


def _quads(a):
    m, n = a.shape[0] // 2, a.shape[1] // 2
    return a[:m, :n], a[:m, n:], a[m:, :n], a[m:, n:]


def _hold(v, last, zero):
    if not last:
        return v
    z = jnp.tile(_as_u32(last[0]) & zero.astype(U32), (v.shape[0] // 8, pl.cdiv(v.shape[1], LANE)))
    return pltpu.bitcast(_as_u32(v) | z[:, :v.shape[1]], v.dtype)


def _lhs_operands(a, last, zero, groups, extra):
    first = (0, 2, 0, 3, 0, 2, 1)
    for k in range(7):
        q = list(_quads(a))
        q[first[k]] = _hold(q[first[k]], last, zero)
        l = _strassen_lhs(*q)[k]
        out = []
        for grp in groups:
            q = list(_quads(l))
            if out:
                for b in set(first[i] for i in grp):
                    q[b] = _hold(q[b], last, zero)
            v = jnp.concatenate([_strassen_lhs(*q)[i] for i in grp], axis=1)
            out.append(_as_u32(v.astype(BF16)))
            last[:] = [functools.reduce(
                jnp.bitwise_or, [out[-1][:, c:c + LANE] for c in range(0, v.shape[1], LANE)])]
            for _ in range(extra):
                last[:] = [last[0] + last[0]]
        yield jnp.concatenate(out, axis=1)


SUMS = (0, 1, 4, 5, 6)
Q_ORDER = (1, 6, 2, 3, 0, 5, 4)
Q_INNER = (1, 3, 5, 0, 2, 4, 6)
ORDER = (1, 3, 2, 4, 0, 5, 6)
INNER = (1, 3, 6, 0, 2, 4, 5)
QK_ORDER = (0, 2, 4, 3, 1, 6, 5)
QK_GROUP = 1
QK_LAG = 2
QK_TIE_K = 3
QK_RUNMAX = True
DIAG_FIRST = False
PV_ORDER = (2, 1, 3, 4, 5, 0, 6)


def _kernel(xt_hbm, c_hbm, wq_hbm, wuk_hbm, wuv_hbm, wot_hbm,
            bre_hbm, bim_hbm, cre_hbm, cim_hbm,
            lre_hbm, lim_hbm, ldt_hbm, dsk_hbm, gw_hbm,
            o_hbm,
            xt_ref, x_ref, lx_ref, c_ref, l_ref, wq_buf, wk_buf, wv_buf, wot_ref, lo_ref,
            b_ref, cre_ref, cim_ref, u_ref, ys_ref, st_ref, co_ref, col_ref, smp_ref, vsc_ref,
            q_ref, ctx_ref, zero_ref, wsem, xsem, msem, vsem, osem,
            lre_ref, lim_ref, ldt_ref, dsk_ref, gw_ref, *pad,
            S, M, H, D):
    P = M
    FT = P // LANE
    PF = FT * LANE
    assert P - PF == HALF
    PP = PF + LANE
    NP = H // 2
    TS = S // NP
    CH, DH, MH, TH = c_ref.shape[1] // 2, D // 2, M // 2, TP // 2

    def w_copy(k, pair):
        src, dst = ((wq_hbm, wq_buf), (wuk_hbm, wk_buf), (wuv_hbm, wv_buf))[k]
        return pltpu.make_async_copy(src.bitcast(U32).at[:, pair, :], dst.at[pair], wsem.at[k, pair])

    def wo_copy(pair):
        heads = pl.ds(2 * pair, 2)
        return pltpu.make_async_copy(wot_hbm.bitcast(U32).at[heads], wot_ref.at[heads],
                                     wsem.at[3, pair])

    def x_copy(t0, n, k):
        cols = pl.ds(t0, n)
        return pltpu.make_async_copy(xt_hbm.at[:, cols], xt_ref.at[:, cols], xsem.at[k])

    x_cps = [x_copy(0, TU // 2, 0), x_copy(TU // 2, TU // 2, 1), x_copy(TU, TU, 2),
             x_copy(2 * TU, S - 2 * TU, 3)]

    bre32, bim32 = bre_hbm.bitcast(U32), bim_hbm.bitcast(U32)
    b_cps = [
        pltpu.make_async_copy(bre32, b_ref.at[pl.ds(0, P // 2), :], msem.at[0]),
        pltpu.make_async_copy(bim32.at[pl.ds(PF // 2, HALF // 2), :],
                              b_ref.at[pl.ds(P // 2, HALF // 2), :], msem.at[1]),
        pltpu.make_async_copy(bim32.at[pl.ds(0, PF // 2), :],
                              b_ref.at[pl.ds(PP // 2, PF // 2), :], msem.at[2]),
    ]
    cre_cp = pltpu.make_async_copy(cre_hbm.bitcast(U32), cre_ref, msem.at[3])
    cim_cp = pltpu.make_async_copy(cim_hbm.bitcast(U32), cim_ref, msem.at[4])

    def c_copy(r):
        rows = pl.ds(pl.multiple_of(r * TH, TH), TH)
        return pltpu.make_async_copy(c_hbm.bitcast(U32).at[rows], c_ref.at[rows], wsem.at[4, r])

    smp_cps = [pltpu.make_async_copy(src.bitcast(U32).at[pl.ds(0, smp_ref.shape[1])],
                                     smp_ref.at[k], msem.at[5 + k])
               for k, src in enumerate((wuk_hbm, wuv_hbm, wq_hbm))]
    v_cps = [pltpu.make_async_copy(src, dst, vsem.at[k]) for k, (src, dst) in enumerate(
        ((lre_hbm, lre_ref), (lim_hbm, lim_ref), (ldt_hbm, ldt_ref),
         (dsk_hbm, dsk_ref), (gw_hbm, gw_ref)))]

    for cp in v_cps:
        cp.start()
    for cp in x_cps[:1] + b_cps + x_cps[1:] + smp_cps:
        cp.start()
    for p in range(NP):
        w_copy(0, p).start()
        wo_copy(p).start()
        c_copy(p).start()
    for p in range(NP):
        w_copy(1, p).start()
        w_copy(2, p).start()
    cre_cp.start()
    cim_cp.start()

    zero_ref[0] = 0
    u_ref[pl.ds(0, 8), :] = jnp.zeros((8, u_ref.shape[1]), F32)
    st_ref[...] = jnp.zeros(st_ref.shape, F32)
    for cp in v_cps:
        cp.wait()

    row = lambda r: r[...].astype(F32).reshape(1, P)
    lre, lim = row(lre_ref), row(lim_ref)
    dt = jnp.exp(row(ldt_ref)).astype(BF16).astype(F32)
    e = jnp.exp(dt * lre)
    ang = dt * lim
    ar = e * jnp.cos(ang)
    ai = e * jnp.sin(ang)
    sc = jnp.maximum(jnp.abs(lre), jnp.abs(lim))
    nre, nim = lre / sc, lim / sc
    den = (nre * nre + nim * nim) * sc
    gr = 2.0 * ((ar - 1.0) * nre + ai * nim) / den
    gi = 2.0 * (ai * nre - (ar - 1.0) * nim) / den

    def put(k, full, lo, hi):
        v = jnp.concatenate([full[:, :PF], lo[:, PF:], hi[:, PF:]], axis=1)
        co_ref[k] = jnp.broadcast_to(v, (8, PP))

    put(0, gr, gr, -gr)
    put(1, -gi, -gi, -gi)
    pr, pi = ar, -ai
    for j in range(1, 5):
        put(2 * j, pr, pr, pr)
        put(2 * j + 1, -pi, -pi, pi)
        pr, pi = pr * pr - pi * pi, 2.0 * pr * pi

    zpad = jnp.zeros((1, PP - P), F32)
    for k, r in enumerate((dsk_ref, gw_ref)):
        v = jnp.concatenate([row(r), zpad], axis=1)
        col_ref[k] = jnp.broadcast_to(v, (LANE, PP)).T[:M]

    XH = PP // 2

    def transpose_x(t0, n):
        x_ref[pl.ds(t0 // 2, n // 2), :] = _as_u32(xt_ref[:, pl.ds(t0, n)].T)

    zero1, last1 = zero_ref[0], []

    def x_sums(r):
        for n in range(TH // 32):
            x = jnp.concatenate(
                [x_ref[pl.ds(r * TH + g * (TH // 4) + 8 * n, 8), :] for g in range(4)], axis=0)
            x = _as_bf16(_hold(x, last1, zero1)).astype(F32)
            x = jnp.concatenate([x, jnp.zeros((x.shape[0], PP - M), F32)], axis=1)
            for k, v in enumerate(_lhs_operands(x, last1, zero1, X_GROUPS, X_EXTRA)):
                lx_ref[k, pl.ds(r * (TH // 4) + 8 * n, 8), :] = v

    def proj_u(t0, n, lo=0, hi=2 * P, due=False, mark=False):
        x = x_ref[pl.ds(t0 // 2, n // 2), :]
        if due:
            x = jnp.concatenate([_hold(x[:8], last1, zero1), x[8:]], axis=0)
        u = _dot_nt(_as_bf16(x), _as_bf16(b_ref[lo // 2:hi // 2, :]))
        u_ref[pl.ds(t0 + 8, n), lo:hi] = u
        if mark:
            last1[:] = [functools.reduce(jnp.bitwise_or, last1 + [_as_u32(u[:8, :LANE])])]

    x_cps[0].wait()
    transpose_x(0, TU // 2)
    b_cps[0].wait()
    b_cps[1].wait()
    proj_u(0, TU // 2, 0, PP)
    b_cps[2].wait()
    x_cps[1].wait()
    proj_u(0, TU // 2, PP)
    transpose_x(TU // 2, TU // 2)
    x_cps[2].wait()
    proj_u(TU // 2, TU // 2)
    transpose_x(TU, TU)
    x_cps[3].wait()
    for cp in smp_cps:
        cp.wait()
    def exponent(k, e):
        mag = jnp.sum(jnp.abs(_unpack(smp_ref[k], jnp.uint32(16 - 16 * e))), axis=0)
        mag = jnp.sum(mag, axis=1, keepdims=True)
        return jnp.broadcast_to(pltpu.bitcast(mag, jnp.int32) >> 23, (NP, LANE))

    for n, (ref_ke, ke) in enumerate((((0, 0), (1, 0)), ((0, 1), (1, 1)), ((2, 0), (2, 1)))):
        e0, e1 = exponent(*ref_ke), exponent(*ke)
        d = jnp.where((e0 > 0) & (e1 > 0), jnp.clip(e0 - e1, -40, 40), 0)
        vsc_ref[0, n] = pltpu.bitcast((127 + d) << 23, F32)
        vsc_ref[1, n] = pltpu.bitcast((127 - d) << 23, F32)
    ops = dict(u=lambda r: proj_u(r * TP, TP, mark=True), t=lambda r: transpose_x(r * TP, TU), x=x_sums,
               v=lambda r: proj_u(r * TP, TP, 0, 6 * LANE, mark=True),
               w=lambda r: proj_u(r * TP, TP, 6 * LANE, due=True))
    for op in U_SCHEDULE.split():
        ops[op[0]](int(op[1:]))

    def q_step(j, _):
        w_copy(0, j).wait()
        wo_copy(j).wait()
        c_copy(j).wait()
        zero = zero_ref[0]
        after = lambda w, v: w | (_as_u32(v) & zero.astype(U32))
        last, recent = [], []
        wq32 = wq_buf[j]
        wq32 = jnp.concatenate([wq32, jnp.zeros((PP - M, D), U32)], axis=0)
        rw = []
        for k in range(7):
            z = (zero << k).astype(U32) if k in Q_REMAT else jnp.uint32(0)
            w0 = pltpu.bitcast(wq32 << (z + 16), F32)
            w1 = pltpu.bitcast(wq32 & (z + jnp.uint32(0xFFFF0000)), F32)
            r0 = _strassen_rhs(*_quads(w0))[k]
            r1 = _strassen_rhs(*_quads(w1))[k] * vsc_ref[0, 2, pl.ds(j, 1), :]
            rw.append(_strassen_rhs(r0[:LANE], r1[:LANE], r0[LANE:], r1[LANE:]))
        qscale = jnp.concatenate([jnp.ones((1, DH), F32), vsc_ref[1, 2, pl.ds(j, 1), :]], axis=1)
        qscale = qscale * ((D ** -0.5) * LOG2E)

        def proj_q(r, n=1):
            ms = [None] * 7
            TI = TH // 2
            for k in Q_ORDER:
                mi = [None] * 7
                for i in Q_INNER:
                    a = lx_ref[k, pl.ds(r * TI // 2, n * TI // 2), pl.ds(i * LANE, LANE)]
                    b = rw[k][i]
                    at = 7 * r + n * Q_ORDER.index(k) if i == Q_INNER[0] else -1
                    if at in C_DUE:
                        a = jnp.concatenate([_hold(a[:8], last, zero), a[8:]], axis=0)
                    mi[i] = jnp.dot(_as_bf16(a), b.astype(BF16), preferred_element_type=F32)
                    recent.append(mi[i])
                    for _ in range(C_START.count(at)):
                        if SIDE[len(SIDE) - len(side)] not in "xy":
                            last[:] = [_as_u32(mi[i][:8]) | last[0] if last else _as_u32(mi[i][:8])]
                        side.pop(0)()
                c11, c12, c21, c22 = _strassen_out(mi, Q_INNER if Q_ASSOC & 1 else None)
                top, bot = jnp.concatenate([c11, c12], axis=1), jnp.concatenate([c21, c22], axis=1)
                ms[k] = jnp.concatenate(
                    [v[b * TI:(b + 1) * TI] for b in range(n) for v in (top, bot)], axis=0)
            for k, v in enumerate(_strassen_out(ms, Q_ORDER if Q_ASSOC & 2 else None)):
                q_ref[j, k, pl.ds(r * TH, n * TH), :] = (v * qscale).astype(BF16)

        pieces = []

        def c_sums():
            n = len(pieces)
            pieces.append(n)
            c = jnp.concatenate(
                [c_ref[pl.ds(pl.multiple_of(j * TH + g * (TH // 4) + 8 * n, 8), 8), :] for g in range(4)],
                axis=0)
            c = _as_bf16(_hold(c, last, zero)).astype(F32)
            rows = pl.ds(pl.multiple_of(j * (TH // 4) + 8 * n, 8), 8)
            for k, v in enumerate(_lhs_operands(c, last, zero, C_GROUPS, C_EXTRA)):
                l_ref[k, rows, :] = v

        def wo_sums(e):
            for n in range(0, MH // 2, 16):
                w = jnp.concatenate([wot_ref[2 * j + e, pl.ds(g * MH // 2 + n, 16), :] for g in range(2)],
                                    axis=0)
                ls = _strassen_lhs(*_quads(_as_bf16(_hold(w, last, zero)).astype(F32)))
                v = jnp.concatenate([ls[k] for k in SUMS], axis=1)
                lo_ref[2 * j + e, pl.ds(2 * n, 32), :] = v.astype(BF16)
                last[:] = [functools.reduce(jnp.bitwise_or, [
                    _as_u32(v[g:g + 8, c:c + LANE]) for g in (0, 16) for c in range(0, v.shape[1], LANE)])]

        def wo_free(e):
            z = _as_u32(jnp.concatenate([v[:TH // 2] for v in recent[-7:]], axis=0)) & zero.astype(U32)
            w = wot_ref[2 * j + e] | jnp.concatenate([z[:MH], z[MH:]], axis=1)
            ls = _strassen_lhs(*_quads(_as_bf16(w).astype(F32)))
            lo_ref[2 * j + e] = jnp.concatenate([ls[k] for k in SUMS], axis=1).astype(BF16)

        side = [dict(c=c_sums, x=lambda: wo_free(0), y=lambda: wo_free(1), v=lambda: wo_sums(0), w=lambda: wo_sums(1), n=lambda: None)[k] for k in SIDE]
        ops = dict(q=proj_q, r=lambda r: proj_q(r, 2), s=lambda r: proj_q(r, 3))
        for op in Q_SCHEDULE.split():
            ops[op[0]](int(op[1:]))
        assert not side
        return 0

    assert S // TP == NP
    jax.lax.fori_loop(0, NP, q_step, 0)
    for p in range(NP):
        w_copy(1, p).wait()
        w_copy(2, p).wait()
    cre_cp.wait()
    cim_cp.wait()

    def head_step(h, _):
        slot = h >> 1
        zero = zero_ref[0]
        shift = (16 - 16 * (h & 1)).astype(U32)
        vscale, vinv = [vsc_ref[k, h & 1, pl.ds(slot, 1), :] for k in range(2)]
        rw = []
        for k in range(7):
            sh = shift + (zero << k).astype(U32) if k in REMAT else shift
            rk = _strassen_rhs(*_quads(_unpack(wk_buf[slot], sh)))[k]
            rv = _strassen_rhs(*_quads(_unpack(wv_buf[slot], sh)))[k] * vscale
            rw.append(_strassen_rhs(rk[:CH // 2], rv[:CH // 2], rk[CH // 2:], rv[CH // 2:]))
        causal = (jax.lax.broadcasted_iota(jnp.int32, (TQ, TQ), 1)
                  <= jax.lax.broadcasted_iota(jnp.int32, (TQ, TQ), 0))

        ks, rks, vs, rvs, ss, mxs, chains = [], [], [], [], {}, {}, [None]

        def proj_kv(r, n=1):
            TI = TH // 2
            ms = [None] * 7
            for k in ORDER:
                mi = [None] * 7
                for i in INNER:
                    a = l_ref[k, pl.ds(r * TI // 2, n * TI // 2), pl.ds(i * CH // 2, CH // 2)]
                    mi[i] = jnp.dot(_as_bf16(a), rw[k][i].astype(BF16), preferred_element_type=F32)
                c11, c12, c21, c22 = _strassen_out(mi, INNER if ASSOC & (1 if n == 1 else 16) else None)
                top, bot = jnp.concatenate([c11, c12], axis=1), jnp.concatenate([c21, c22], axis=1)
                ms[k] = jnp.concatenate(
                    [v[b * TI:(b + 1) * TI] for b in range(n) for v in (top, bot)], axis=0)
                if k != ORDER[-1]:
                    yield
            c = _strassen_out(ms, ORDER if ASSOC & (2 if n == 1 else 32) else None)
            for b in range(n):
                c11, c12, c21, c22 = [v[b * TH:(b + 1) * TH, :DH] for v in c]
                ks.extend([jnp.concatenate([c11, c12], axis=1), jnp.concatenate([c21, c22], axis=1)])
                rks.append(_strassen_rhs(c11, c21, c12, c22))
                c11, c12, c21, c22 = [v[b * TH:(b + 1) * TH, DH:] for v in c]
                vs.extend([jnp.concatenate([c11, c12], axis=1), jnp.concatenate([c21, c22], axis=1)])
                rvs.append(_strassen_rhs(c11, c12, c21, c22))

        def qk_pair(j):
            cols = pl.ds(pl.multiple_of((h & 1) * DH, DH), DH)
            qf = [q_ref[slot, k, j * TQ:(j + 1) * TQ, cols].astype(F32) for k in range(4)]
            q = jnp.concatenate([jnp.concatenate(qf[:2], axis=1), jnp.concatenate(qf[2:], axis=1)], axis=0)
            lq = _strassen_lhs(*qf)
            s1, s2, done, mx = [], [], [], []

            def diag():
                if UNIFORM_DIAG:
                    return (_dot_nt(q[:TQ].astype(BF16), ks[2 * j].astype(BF16)),
                            _dot_nt(q[TQ:].astype(BF16),
                                    jnp.concatenate(ks[2 * j:2 * j + 2], axis=0).astype(BF16)))
                d = _dot_nt(q.astype(BF16), ks[2 * j].astype(BF16))
                return d[:TQ], jnp.concatenate(
                    [d[TQ:], _dot_nt(q[TQ:].astype(BF16), ks[2 * j + 1].astype(BF16))], axis=1)

            if DIAG_FIRST:
                d1, d2 = diag()
            for t0 in range(0, j, QK_GROUP):
                ts = range(t0, min(t0 + QK_GROUP, j))
                m = [None] * 7
                for k in QK_ORDER:
                    rk = jnp.concatenate([rks[t][k] for t in ts], axis=0).astype(BF16)
                    a = lq[k]
                    if k == QK_TIE_K and len(done) >= QK_LAG:
                        a = tie(a, done[-QK_LAG])
                    m[k] = jax.lax.dot_general(a.astype(BF16), rk, NT_DIMS, preferred_element_type=F32)
                c11, c12, c21, c22 = _strassen_out(
                    m, QK_ORDER if ASSOC & 4 else None if ASSOC & 8 else tuple(range(7)))
                if QK_RUNMAX:
                    x1, x2 = jnp.maximum(c11, c12), jnp.maximum(c21, c22)
                    if mx:
                        x1, x2 = jnp.maximum(x1, mx[0]), jnp.maximum(x2, mx[1])
                    mx[:] = [x1, x2]
                    z = _as_u32(x1) | _as_u32(x2)
                else:
                    z = (_as_u32(c11) | _as_u32(c12)) | (_as_u32(c21) | _as_u32(c22))
                done.append(z)
                for n in range(len(ts)):
                    cols = slice(n * TQ, (n + 1) * TQ)
                    s1 += [c11[:, cols], c12[:, cols]]
                    s2 += [c21[:, cols], c22[:, cols]]
            yield
            if not DIAG_FIRST:
                d1, d2 = diag()
            ss[2 * j] = jnp.concatenate(s1 + [d1], axis=1)
            ss[2 * j + 1] = jnp.concatenate(s2 + [d2], axis=1)
            if mx:
                mxs[2 * j], mxs[2 * j + 1] = mx

        def tie(a, b):
            return pltpu.bitcast(_as_u32(a) | (_as_u32(b) & zero.astype(U32)), F32)

        def exp_rows(s, m, pace, rows, chain=None):
            mb = m
            ps, parts = [], []
            for g in range(0, TQ, rows):
                mg = mb[g:g + rows]
                if pace and (parts or chain is not None):
                    mg = tie(mg, parts[-1] if parts else chain)
                pg = [jnp.exp2(s[g:g + rows, t * LANE:(t + 1) * LANE] - mg)
                      for t in range(s.shape[1] // LANE)]
                ps.append(jnp.concatenate(pg, axis=1))
                parts.append(functools.reduce(lambda a, b: a + b, pg))
            return jnp.concatenate(ps, axis=0), jnp.concatenate(parts, axis=0)

        def masked(i):
            lo = i * TQ
            s = ss.pop(i)
            sd = jnp.where(causal, s[:, lo:], -1e9 * LOG2E)
            s = sd if i == 0 else jnp.concatenate([s[:, :lo], sd], axis=1)
            t = jnp.concatenate([mxs[i], s[:, i // 2 * 2 * TQ:]], axis=1) if i in mxs else s
            if LOOK[i // 2] > 0:
                return s, functools.reduce(
                    jnp.maximum, [t[:, c:c + LANE] for c in range(0, t.shape[1], LANE)])
            return s, jnp.broadcast_to(jnp.max(t, axis=-1, keepdims=True), (TQ, LANE))

        def exp_rows2(s, mx, parts, look, both):
            ps = []
            for g in range(0, TQ, 8):
                mg = mx[g:g + 8]
                if len(parts) >= look:
                    mg = tie(mg, parts[-look])
                mg = jnp.broadcast_to(jnp.max(mg, axis=-1, keepdims=True), (8, LANE))
                if both and parts:
                    mg = tie(mg, parts[-1])
                pg = [jnp.exp2(s[g:g + 8, t * LANE:(t + 1) * LANE] - mg)
                      for t in range(s.shape[1] // LANE)]
                ps.append(jnp.concatenate(pg, axis=1))
                parts.append(functools.reduce(lambda a, b: a + b, pg))
            return jnp.concatenate(ps, axis=0), jnp.concatenate(parts[-(TQ // 8):], axis=0)

        def pv(j):
            (s1, m1), (s2, m2) = masked(2 * j), masked(2 * j + 1)
            if LOOK[j] > 0:
                parts = []
                p1, l1 = exp_rows2(s1, m1, parts, LOOK[j] % 100, LOOK[j] > 100)
                p2, l2 = exp_rows2(s2, m2, parts, LOOK[j] % 100, LOOK[j] > 100)
            else:
                p1, l1 = exp_rows(s1, m1, LOOK[j] == 0, PACE_ROWS, chains[0] if CHAIN_ALL else None)
                if j in EARLY_SUM:
                    ls = jnp.broadcast_to(jnp.sum(l1, axis=-1, keepdims=True), (TQ, LANE))
                    k = 8 * EARLY_SHIFT
                    if k:
                        ls = jnp.concatenate([_as_u32(ls[:k]) | _as_u32(ls[k:2 * k]), _as_u32(ls[2 * k:]),
                                              _as_u32(ls[:k])], axis=0)
                    m2 = tie(m2, ls)
                p2, l2 = exp_rows(s2, m2, LOOK[j] == 0, PACE_ROWS, l1[TQ - 8:])
            chains[0] = l2[TQ - 8:]
            if L_TIE == 1:
                l1 = tie(l1, l2)
            elif L_TIE == 2:
                l1 = jnp.concatenate([tie(l1[:8], l2[:8]), l1[8:]], axis=0)
            elif L_TIE == 3:
                l1 = jnp.concatenate([tie(l1[:8], l1[TQ - 8:]), l1[8:]], axis=0)
            l1, l2 = [jnp.sum(l, axis=-1, keepdims=True) for l in (l1, l2)]
            lo = 2 * j * TQ
            cat = lambda xs, axis: jnp.concatenate(xs, axis=axis)
            dot = lambda a, b: jnp.dot(a.astype(BF16), b.astype(BF16), preferred_element_type=F32)

            def recip(l):
                rl = pl.reciprocal(l, approx=True)
                return rl * (2.0 - l * rl)

            r1, r2 = recip(l1), recip(l2)
            rho = l1 * r2
            r1, r2 = r1 * vinv, r2 * vinv
            if j == 0 and PRENORM0:
                p1, p2 = p1 * r1, p2 * cat([r2, r2], 1)
                r1 = r2 = jnp.ones((1, LANE), F32)
            def diag():
                dg = dot(cat([p1[:, lo:], p2[:, lo:lo + TQ]], 0), vs[2 * j])
                return dg[:TQ], dg[TQ:] + dot(p2[:, lo + TQ:], vs[2 * j + 1])

            if j == 0:
                c1, c2 = diag()
            if j > 0:
                tiles = lambda p, o: cat([p[:, (2 * t + o) * TQ:(2 * t + o + 1) * TQ] for t in range(j)], 1)
                a11, a12, a21, a22 = tiles(p1, 0), tiles(p1, 1), tiles(p2, 0), tiles(p2, 1)
                a22r = a22 * rho
                lp = [a11 + a22r, a21 + a22, a11, a22, a11 + a12, a21 * rho - a11, a12 - a22r]
                m = [None] * 7
                for n, k in enumerate(PV_ORDER):
                    if n == PV_DIAG[j]:
                        c1, c2 = diag()
                    if k == PV_ORDER[-1]:
                        yield
                    m[k] = dot(lp[k], cat([rvs[t][k] for t in range(j)], 0))
                c1 = c1 + cat([(m[0] - m[4]) + (m[6] + m[3] * rho), m[2] + m[4]], 1)
                c2 = (c2 + cat([m[1] + m[3], -m[1]], 1)) * cat([r2, r2], 1)
                c2 = cat([c2[:, :DH], c2[:, DH:] + ((m[0] + m[2]) + m[5]) * r1], 1)
            else:
                c2 = c2 * cat([r2, r2], 1)
            c1 = c1 * cat([r1, r1], 1)
            ctx_ref[h, j * TQ:(j + 1) * TQ, :] = cat(
                _strassen_rhs(c1[:, :DH], c2[:, :DH], c1[:, DH:], c2[:, DH:]), 1).astype(BF16)

        assert TP == 2 * TQ
        pvs = [pv(j) for j in range(S // TP)]
        qks = [qk_pair(j) for j in range(S // TP)]
        kvs = {}

        def kv_part(r, n, steps):
            g = kvs.setdefault(r, proj_kv(r, n))
            for _ in range(steps):
                next(g, None)

        ops = dict(c=lambda r: kv_part(r, 1, 7), d=lambda r: kv_part(r, 2, 7),
                   e=lambda r: kv_part(r, 3, 7), f=lambda r: kv_part(r, 4, 7), i=lambda r: kv_part(r, 1, 2),
                   x=lambda r: kv_part(r // 10, 1, r % 10), h=lambda r: kv_part(r, 1, 4), g=lambda r: kv_part(r, 2, 4),
                   t=lambda j: list(qks[j]), u=lambda j: next(qks[j]), p=lambda j: list(pvs[j]), b=lambda j: next(pvs[j]))
        for op in SCHEDULE.split():
            ops[op[0]](int(op[1:]))
        return 0

    jax.lax.fori_loop(0, H, head_step, 0)

    parts = ((0, 0, TO), (MH, 0, TQ), (MH, TQ, TQ))

    def o_copy(j, n):
        r0, c0, nc = parts[n]
        return pltpu.make_async_copy(
            ys_ref.at[j, pl.ds(r0, MH), pl.ds(c0, nc)],
            o_hbm.at[pl.ds(r0, MH), pl.ds(pl.multiple_of(j * TO + c0, TQ), nc)], osem.at[n, j])

    def o_step(jj, _):
        zero = zero_ref[0]
        js = (2 * jj, 2 * jj + 1)
        t0 = [pl.multiple_of(j * TS, TS) for j in js]
        last, state, ys, gates, m, recent = [], {}, [None, None], {}, [{}, {}], []

        def ssm_tile(u, t):
            rows = pl.ds(t0[u], TS + 8)
            cr, ci = pl.ds(t * LANE, LANE), pl.ds(PP + t * LANE, LANE)
            co = [co_ref[k, :, cr] for k in range(10)]
            u0 = u_ref[rows, cr]
            u1 = u_ref[rows, ci] if t < FT else pltpu.roll(u0, HALF, 1)
            mul = lambda k, x: (co[k] * x[0] + co[k + 1] * x[1], co[k] * x[1] - co[k + 1] * x[0])
            sub = jax.lax.broadcasted_iota(jnp.int32, (8, LANE), 0)
            s = state.get(t) or (st_ref[0, :, cr], st_ref[1, :, cr])
            prev, gs = [None] * 3, []
            for k in range(TS // 8 + 1):
                x0, x1 = u0[8 * k:8 * k + 8], u1[8 * k:8 * k + 8]
                x0 = _hold(x0, last, zero)
                w = (co[0] * x0 + co[1] * x1, co[1] * x0 - co[0] * x1)
                for i in range(3):
                    cur = [pltpu.roll(v, 1 << i, 0) for v in w]
                    old = cur if k == 0 else prev[i]
                    d = mul(2 * i + 2, [jnp.where(sub < (1 << i), o, c) for o, c in zip(old, cur)])
                    w = [p + q for p, q in zip(d, w)]
                    prev[i] = cur
                if k > 0:
                    s = [p + q for p, q in zip(mul(8, s), w)]
                    gs.append(jnp.concatenate(s, axis=1) if t < FT else s[0])
                    last[:] = [s[0]]
            state[t] = s
            if u == 1:
                st_ref[0, :, cr] = s[0]
                st_ref[1, :, cr] = s[1]
            if t < FT:
                cc = jnp.concatenate([cre_ref[:, cr], cim_ref[:, cr]], axis=1)
            else:
                cc = jnp.concatenate([cre_ref[:, PF:], cim_ref[:, PF:]], axis=1)
            g = jnp.concatenate(gs, axis=0).astype(BF16)
            n = M // 2 if t < FT else M // 4
            y = jnp.concatenate([
                jax.lax.dot_general(_as_bf16(cc[a:a + n]), g, NT_DIMS, preferred_element_type=F32)
                for a in range(0, M // 2, n)], axis=0)
            ys[u] = y if ys[u] is None else y + ys[u]

        def gate(u):
            gcol = _as_u32(col_ref[1]) | (_as_u32(jnp.concatenate(recent[-2:], axis=0)) & zero.astype(U32))
            gcol = jnp.concatenate([pltpu.bitcast(gcol, F32)] * (TS // LANE), axis=1)
            xt = xt_ref[:, pl.ds(t0[u], TS)].astype(F32)
            z = jnp.sum((xt * gcol).astype(BF16).astype(F32), axis=0, keepdims=True)
            rnd = lambda v: v.astype(BF16).astype(F32)
            gates[u] = rnd(1.0 / rnd(1.0 + rnd(jnp.exp(-rnd(z)))))

        def emit(u, n, v):
            r0, c0, nc = parts[n]
            g = gates[u][:, c0:c0 + nc]
            omg = (1.0 - g).astype(BF16).astype(F32)
            dcol = jnp.concatenate([col_ref[0, r0:r0 + MH]] * (nc // LANE), axis=1)
            xt = xt_ref[pl.ds(r0, MH), pl.ds(pl.multiple_of(t0[u] + c0, TQ), nc)].astype(F32)
            b = ys[u][r0:r0 + MH, c0:c0 + nc] + (xt * dcol).astype(BF16).astype(F32)
            ys_ref[js[u], pl.ds(r0, MH), pl.ds(c0, nc)] = g * v + omg * b
            o_copy(js[u], n).start()

        def product(u, k):
            if k in SUMS:
                a = [lo_ref[n, :, pl.ds(SUMS.index(k) * DH, DH)] for n in range(H)]
            elif k == 2:
                a = [_as_bf16(wot_ref[n, pl.ds(0, MH // 2), pl.ds(0, DH)]) for n in range(H)]
            else:
                a = [_as_bf16(wot_ref[n, pl.ds(MH // 2, MH // 2), pl.ds(DH, DH)]) for n in range(H)]
            rows = pl.ds(pl.multiple_of(js[u] * TQ, TQ), TQ)
            b = [ctx_ref[n, rows, pl.ds(k * DH, DH)] for n in range(H)]
            m[u][k] = _dot_nt(jnp.concatenate(a, axis=1), jnp.concatenate(b, axis=1))
            recent.append(m[u][k])

        ops = dict(a=lambda k: product(0, k), b=lambda k: product(1, k), g=gate,
                   m=lambda t: ssm_tile(0, t), n=lambda t: ssm_tile(1, t))
        for op in O_SCHEDULE.split():
            ops[op[0]](int(op[1:]))
        for u, p in enumerate(m):
            emit(u, 0, jnp.concatenate([(p[0] + p[3]) + (p[6] - p[4]), p[2] + p[4]], axis=1))
            emit(u, 1, p[1] + p[3])
            emit(u, 2, ((p[0] + p[2]) - p[1]) + p[5])
        return 0

    assert TO == 2 * TQ and TO == TS
    no = S // TO
    jax.lax.fori_loop(0, no // 2, o_step, 0)
    for j in range(no):
        for n in range(3):
            o_copy(j, n).wait()


@jax.jit
def pallas_gated_mix__compressed_kv_cla__ssm_conv_s5__prompt_kernel(
    A_x: jax.Array,
    A_c_kv: jax.Array,
    A_w_q: jax.Array,
    A_w_uk: jax.Array,
    A_w_uv: jax.Array,
    A_w_o: jax.Array,
    B_x: jax.Array,
    B_Lambda_re: jax.Array,
    B_Lambda_im: jax.Array,
    B_B_re: jax.Array,
    B_B_im: jax.Array,
    B_C_re: jax.Array,
    B_C_im: jax.Array,
    B_log_dt: jax.Array,
    B_Dskip: jax.Array,
    gate_w: jax.Array,
):
    del B_x
    _, S, M = A_x.shape
    C = A_c_kv.shape[2]
    H, D = A_w_q.shape[1], A_w_q.shape[2]
    PP = (M + LANE - 1) // LANE * LANE

    hbm = pl.BlockSpec(memory_space=pl.ANY)
    out_t = pl.pallas_call(
        functools.partial(_kernel, S=S, M=M, H=H, D=D),
        in_specs=[hbm] * 15,
        out_specs=hbm,
        out_shape=jax.ShapeDtypeStruct((M, S), F32),
        scratch_shapes=[
            pltpu.VMEM((M, S), BF16),
            pltpu.VMEM((S // 2, M), U32),
            pltpu.VMEM((7, S // 8, 7 * PP // 4), U32),
            pltpu.VMEM((S // 2, C), U32),
            pltpu.VMEM((7, S // 8, 7 * C // 4), U32),
            pltpu.VMEM((H // 2, M, D), U32),
            pltpu.VMEM((H // 2, C, D), U32),
            pltpu.VMEM((H // 2, C, D), U32),
            pltpu.VMEM((H, M // 2, D), U32),
            pltpu.VMEM((H, M // 2, 5 * D // 2), BF16),
            pltpu.VMEM((M, M), U32),
            pltpu.VMEM((M // 2, M), U32),
            pltpu.VMEM((M // 2, M), U32),
            pltpu.VMEM((S + U_PAD, 2 * M), F32),
            pltpu.VMEM((S // TO, M, TO), F32),
            pltpu.VMEM((2, 8, PP), F32),
            pltpu.VMEM((CO_PAD, 8, PP), F32),
            pltpu.VMEM((2, M, LANE), F32),
            pltpu.VMEM((3, 8, H // 2, D), U32),
            pltpu.VMEM((2, V_PAD, H // 2, LANE), F32),
            pltpu.VMEM((H // 2, 4, S // 2, D), BF16),
            pltpu.VMEM((H, S // 2, 7 * D // 2), BF16),
            pltpu.SMEM((1,), jnp.int32),
            pltpu.SemaphoreType.DMA((5, H // 2)),
            pltpu.SemaphoreType.DMA((4,)),
            pltpu.SemaphoreType.DMA((8,)),
            pltpu.SemaphoreType.DMA((5,)),
            pltpu.SemaphoreType.DMA((3, S // TO)),
        ] + [pltpu.VMEM((M,), BF16)] * (5 + VEC_PAD),
        compiler_params=pltpu.CompilerParams(
            vmem_limit_bytes=124 * 1024 * 1024,
            disable_semaphore_checks=True,
            disable_bounds_checks=True,
        ),
    )(
        jnp.swapaxes(A_x, 1, 2).reshape(M, S), A_c_kv.reshape(S, C),
        A_w_q, A_w_uk, A_w_uv, jnp.swapaxes(A_w_o, 1, 2),
        B_B_re, B_B_im, B_C_re, B_C_im,
        B_Lambda_re, B_Lambda_im, B_log_dt, B_Dskip, gate_w,
    )
    return jnp.swapaxes(out_t.reshape(1, M, S), 1, 2)
```

```python
import functools

import jax
import jax.numpy as jnp
import jax.experimental.pallas as pl
import jax.experimental.pallas.tpu as pltpu

F32 = jnp.float32
BF16 = jnp.bfloat16
U32 = jnp.uint32

NT_DIMS = (((1,), (1,)), ((), ()))
LOG2E = 1.4426950408889634

LANE = 128
HALF = LANE // 2
TQ = 128
TP = 256
TU = 512

U_SCHEDULE = "t4 u2 x0 u3 x1 t6 u4 x4 x5 u5 x3 u6 x2 x7 v7 x6 w7"
Q_SCHEDULE = ((0, 2), (2, 1), (3, 1), (4, 1), (5, 1), (6, 1), (7, 1))
Q_ORDER = (1, 6, 2, 3, 0, 5, 4)
Q_INNER = (1, 3, 5, 0, 2, 4, 6)
Q_REMAT = (0, 1, 2, 3, 5, 6)
C_START, WO_START, C_DUE = (14, 20, 30, 39), (40, 52), 55
SCHEDULE = ("d0 x25 t0 t1 c2 p0 p1 t2 c3 u3 b2 t3 c4 u4 p2 b3 t4 c5 p3 p4 t5 c6 b5 t6 c7 t7 "
            "p5 b6 b7 p6 p7")
KV_ORDER = (1, 3, 2, 4, 0, 5, 6)
KV_INNER = (1, 3, 6, 0, 2, 4, 5)
QK_ORDER = (0, 1, 4, 3, 2, 6, 5)
PV_ORDER = (4, 3, 1, 5, 2, 0, 6)
PV_DIAG = (0, 5, 0, 1, 0, 3, 3, 0)
EARLY_SUM = (1, 2, 7)
LOOK = (0, 0, 0, 0, 0, 0, 4, 0)
O_SCHEDULE = "a3 a0 a4 m0 g0 m3 a6 m1 a2 a1 a5 n3 b0 m2 b3 n2 g1 n1 b6 b4 n0 b2 b1 b5"


def _cat(xs, axis):
    return jnp.concatenate(xs, axis=axis)


def _dot(a, b):
    return jnp.dot(a, b, preferred_element_type=F32)


def _dot_nt(a, b):
    return jax.lax.dot_general(a, b, NT_DIMS, preferred_element_type=F32)


def _unpack(w32, shift):
    v = (w32 << shift) & jnp.uint32(0xFFFF0000)
    return pltpu.bitcast(v, F32)


def _as_bf16(w32):
    return pltpu.bitcast(w32, BF16)


def _as_u32(v):
    return pltpu.bitcast(v, U32)


def _run(schedule, ops):
    for op in schedule.split():
        ops[op[0]](int(op[1:]))


def _strassen_lhs(a11, a12, a21, a22):
    return [a11 + a22, a21 + a22, a11, a22, a11 + a12, a21 - a11, a12 - a22]


def _strassen_rhs(b11, b12, b21, b22):
    return [b11 + b22, b11, b12 - b22, b21 - b11, b22, b11 + b12, b21 + b22]


def _strassen_out(m, order=None):
    if order is None:
        return ((m[0] + m[3]) + (m[6] - m[4]), m[2] + m[4],
                m[1] + m[3], (m[0] - m[1]) + (m[2] + m[5]))

    def fold(ks, neg):
        ks = sorted(ks, key=order.index)
        if ks[0] == neg:
            ks[:2] = ks[1::-1]
        return functools.reduce(lambda a, k: a - m[k] if k == neg else a + m[k], ks[1:], m[ks[0]])

    return fold((0, 3, 4, 6), 4), m[2] + m[4], m[1] + m[3], fold((0, 1, 2, 5), 1)


SUMS = (0, 1, 4, 5, 6)


def _quads(a):
    m, n = a.shape[0] // 2, a.shape[1] // 2
    return a[:m, :n], a[:m, n:], a[m:, :n], a[m:, n:]


def _unsplit(c, n):
    top, bot = _cat(c[:2], 1), _cat(c[2:], 1)
    rows = top.shape[0] // n
    return _cat([v[b * rows:(b + 1) * rows] for b in range(n) for v in (top, bot)], 0)


def _hold(v, last, zero):
    if not last:
        return v
    z = jnp.tile(_as_u32(last[0]) & zero.astype(U32), (v.shape[0] // 8, pl.cdiv(v.shape[1], LANE)))
    return pltpu.bitcast(_as_u32(v) | z[:, :v.shape[1]], v.dtype)


def _lhs_operands(a, last, zero, extra):
    first = (0, 2, 0, 3, 0, 2, 1)
    for k in range(7):
        q = list(_quads(a))
        q[first[k]] = _hold(q[first[k]], last, zero)
        l = _strassen_lhs(*q)[k]
        out = []
        for grp in ((0, 1, 2, 3), (4, 5, 6)):
            q = list(_quads(l))
            if out:
                for b in sorted(set(first[i] for i in grp)):
                    q[b] = _hold(q[b], last, zero)
            v = _cat([_strassen_lhs(*q)[i] for i in grp], 1)
            out.append(_as_u32(v.astype(BF16)))
            last[:] = [functools.reduce(
                jnp.bitwise_or, [out[-1][:, c:c + LANE] for c in range(0, v.shape[1], LANE)])]
            for _ in range(extra):
                last[:] = [last[0] + last[0]]
        yield _cat(out, 1)


def _kernel(xt_hbm, c_hbm, wq_hbm, wuk_hbm, wuv_hbm, wot_hbm,
            bre_hbm, bim_hbm, cre_hbm, cim_hbm,
            lre_hbm, lim_hbm, ldt_hbm, dsk_hbm, gw_hbm,
            o_hbm,
            xt_ref, x_ref, lx_ref, c_ref, l_ref, wq_buf, wk_buf, wv_buf, wot_ref, lo_ref,
            b_ref, cre_ref, cim_ref, u_ref, out_ref, st_ref, co_ref, col_ref, smp_ref, vsc_ref,
            q_ref, ctx_ref, zero_ref, wsem, xsem, msem, vsem, osem,
            lre_ref, lim_ref, ldt_ref, dsk_ref, gw_ref,
            *, S, M, H, D):
    P = M
    FT = P // LANE
    PF = FT * LANE
    PP = PF + LANE
    NP = H // 2
    CH, DH, MH, TH = c_ref.shape[1] // 2, D // 2, M // 2, TP // 2
    TI = TH // 2
    assert P - PF == HALF and PP == 4 * LANE and DH == LANE and S // TP == NP and TP == 2 * TQ

    def w_copy(k, pair):
        src, dst = ((wq_hbm, wq_buf), (wuk_hbm, wk_buf), (wuv_hbm, wv_buf))[k]
        return pltpu.make_async_copy(src.bitcast(U32).at[:, pair, :], dst.at[pair], wsem.at[k, pair])

    def wo_copy(pair):
        heads = pl.ds(2 * pair, 2)
        return pltpu.make_async_copy(wot_hbm.bitcast(U32).at[heads], wot_ref.at[heads],
                                     wsem.at[3, pair])

    def c_copy(r):
        rows = pl.ds(pl.multiple_of(r * TH, TH), TH)
        return pltpu.make_async_copy(c_hbm.bitcast(U32).at[rows], c_ref.at[rows], wsem.at[4, r])

    def x_copy(t0, n, k):
        cols = pl.ds(t0, n)
        return pltpu.make_async_copy(xt_hbm.at[:, cols], xt_ref.at[:, cols], xsem.at[k])

    x_cps = [x_copy(0, TP, 0), x_copy(TP, TP, 1), x_copy(TU, TU, 2), x_copy(2 * TU, S - 2 * TU, 3)]
    bre32, bim32 = bre_hbm.bitcast(U32), bim_hbm.bitcast(U32)
    b_cps = [
        pltpu.make_async_copy(bre32, b_ref.at[pl.ds(0, P // 2), :], msem.at[0]),
        pltpu.make_async_copy(bim32.at[pl.ds(PF // 2, HALF // 2), :],
                              b_ref.at[pl.ds(P // 2, HALF // 2), :], msem.at[1]),
        pltpu.make_async_copy(bim32.at[pl.ds(0, PF // 2), :],
                              b_ref.at[pl.ds(PP // 2, PF // 2), :], msem.at[2]),
    ]
    cre_cp = pltpu.make_async_copy(cre_hbm.bitcast(U32), cre_ref, msem.at[3])
    cim_cp = pltpu.make_async_copy(cim_hbm.bitcast(U32), cim_ref, msem.at[4])
    smp_cps = [pltpu.make_async_copy(src.bitcast(U32).at[pl.ds(0, smp_ref.shape[1])],
                                     smp_ref.at[k], msem.at[5 + k])
               for k, src in enumerate((wuk_hbm, wuv_hbm, wq_hbm))]
    v_cps = [pltpu.make_async_copy(src, dst, vsem.at[k]) for k, (src, dst) in enumerate(
        ((lre_hbm, lre_ref), (lim_hbm, lim_ref), (ldt_hbm, ldt_ref),
         (dsk_hbm, dsk_ref), (gw_hbm, gw_ref)))]

    for cp in v_cps + x_cps[:1] + b_cps + x_cps[1:] + smp_cps:
        cp.start()
    for p in range(NP):
        w_copy(0, p).start()
        wo_copy(p).start()
        c_copy(p).start()
    for p in range(NP):
        w_copy(1, p).start()
        w_copy(2, p).start()
    cre_cp.start()
    cim_cp.start()

    zero_ref[0] = 0
    u_ref[pl.ds(0, 8), :] = jnp.zeros((8, u_ref.shape[1]), F32)
    st_ref[...] = jnp.zeros(st_ref.shape, F32)
    for cp in v_cps:
        cp.wait()

    row = lambda r: r[...].astype(F32).reshape(1, P)
    lre, lim = row(lre_ref), row(lim_ref)
    dt = jnp.exp(row(ldt_ref)).astype(BF16).astype(F32)
    e = jnp.exp(dt * lre)
    ang = dt * lim
    ar = e * jnp.cos(ang)
    ai = e * jnp.sin(ang)
    sc = jnp.maximum(jnp.abs(lre), jnp.abs(lim))
    nre, nim = lre / sc, lim / sc
    den = (nre * nre + nim * nim) * sc
    gr = 2.0 * ((ar - 1.0) * nre + ai * nim) / den
    gi = 2.0 * (ai * nre - (ar - 1.0) * nim) / den

    def put(k, full, lo, hi):
        co_ref[k] = jnp.broadcast_to(_cat([full[:, :PF], lo[:, PF:], hi[:, PF:]], 1), (8, PP))

    put(0, gr, gr, -gr)
    put(1, -gi, -gi, -gi)
    pr, pi = ar, -ai
    for j in range(1, 5):
        put(2 * j, pr, pr, pr)
        put(2 * j + 1, -pi, -pi, pi)
        pr, pi = pr * pr - pi * pi, 2.0 * pr * pi

    zpad = jnp.zeros((1, PP - P), F32)
    for k, r in enumerate((dsk_ref, gw_ref)):
        col_ref[k] = jnp.broadcast_to(_cat([row(r), zpad], 1), (LANE, PP)).T[:M]

    zero1, last1 = zero_ref[0], []

    def transpose_x(t0, n):
        x_ref[pl.ds(t0 // 2, n // 2), :] = _as_u32(xt_ref[:, pl.ds(t0, n)].T)

    def x_operands(r):
        for n in range(TI // 16):
            x = _cat([x_ref[pl.ds(r * TH + g * TI // 2 + 8 * n, 8), :] for g in range(4)], 0)
            x = _as_bf16(_hold(x, last1, zero1)).astype(F32)
            x = _cat([x, jnp.zeros((x.shape[0], PP - M), F32)], 1)
            for k, v in enumerate(_lhs_operands(x, last1, zero1, 0)):
                lx_ref[k, pl.ds(r * TI // 2 + 8 * n, 8), :] = v

    def proj_u(r, lo=0, hi=2 * P, due=False, mark=False):
        x = x_ref[pl.ds(r * TH, TH), :]
        if due:
            x = _cat([_hold(x[:8], last1, zero1), x[8:]], 0)
        u = _dot_nt(_as_bf16(x), _as_bf16(b_ref[lo // 2:hi // 2, :]))
        u_ref[pl.ds(r * TP + 8, TP), lo:hi] = u
        if mark:
            last1[:] = [functools.reduce(jnp.bitwise_or, last1 + [_as_u32(u[:8, :LANE])])]

    x_cps[0].wait()
    transpose_x(0, TP)
    b_cps[0].wait()
    b_cps[1].wait()
    proj_u(0, 0, PP)
    b_cps[2].wait()
    x_cps[1].wait()
    proj_u(0, PP)
    transpose_x(TP, TP)
    x_cps[2].wait()
    proj_u(1)
    transpose_x(TU, TU)
    x_cps[3].wait()
    for cp in smp_cps:
        cp.wait()

    def exponent(k, e):
        mag = jnp.sum(jnp.abs(_unpack(smp_ref[k], jnp.uint32(16 - 16 * e))), axis=0)
        mag = jnp.sum(mag, axis=1, keepdims=True)
        return jnp.broadcast_to(pltpu.bitcast(mag, jnp.int32) >> 23, (NP, LANE))

    for n, (target, scaled) in enumerate((((0, 0), (1, 0)), ((0, 1), (1, 1)), ((2, 0), (2, 1)))):
        e0, e1 = exponent(*target), exponent(*scaled)
        d = jnp.where((e0 > 0) & (e1 > 0), jnp.clip(e0 - e1, -40, 40), 0)
        vsc_ref[0, n] = pltpu.bitcast((127 + d) << 23, F32)
        vsc_ref[1, n] = pltpu.bitcast((127 - d) << 23, F32)

    _run(U_SCHEDULE, dict(t=lambda r: transpose_x(r * TP, TU), x=x_operands,
                          u=lambda r: proj_u(r, mark=True),
                          v=lambda r: proj_u(r, 0, 6 * LANE, mark=True),
                          w=lambda r: proj_u(r, 6 * LANE, due=True)))

    def q_step(j, _):
        w_copy(0, j).wait()
        wo_copy(j).wait()
        c_copy(j).wait()
        zero = zero_ref[0]
        last, recent = [], []
        wq32 = _cat([wq_buf[j], jnp.zeros((PP - M, D), U32)], 0)
        rw = []
        for k in range(7):
            z = (zero << k).astype(U32) if k in Q_REMAT else jnp.uint32(0)
            w0 = pltpu.bitcast(wq32 << (z + 16), F32)
            w1 = pltpu.bitcast(wq32 & (z + jnp.uint32(0xFFFF0000)), F32)
            r0 = _strassen_rhs(*_quads(w0))[k]
            r1 = _strassen_rhs(*_quads(w1))[k] * vsc_ref[0, 2, pl.ds(j, 1), :]
            rw.append(_strassen_rhs(r0[:LANE], r1[:LANE], r0[LANE:], r1[LANE:]))
        qscale = _cat([jnp.ones((1, DH), F32), vsc_ref[1, 2, pl.ds(j, 1), :]], 1)
        qscale = qscale * ((D ** -0.5) * LOG2E)

        def c_operands(n):
            c = _cat([c_ref[pl.ds(pl.multiple_of(j * TH + g * (TI // 2) + 8 * n, 8), 8), :]
                      for g in range(4)], 0)
            c = _as_bf16(_hold(c, last, zero)).astype(F32)
            rows = pl.ds(pl.multiple_of(j * (TI // 2) + 8 * n, 8), 8)
            for k, v in enumerate(_lhs_operands(c, last, zero, 3)):
                l_ref[k, rows, :] = v

        def wo_operands(e):
            z = _as_u32(_cat([v[:TI] for v in recent[-7:]], 0)) & zero.astype(U32)
            w = wot_ref[2 * j + e] | _cat([z[:MH], z[MH:]], 1)
            ls = _strassen_lhs(*_quads(_as_bf16(w).astype(F32)))
            lo_ref[2 * j + e] = _cat([ls[k] for k in SUMS], 1).astype(BF16)

        for r, n in Q_SCHEDULE:
            ms = [None] * 7
            for k in Q_ORDER:
                mi = [None] * 7
                for i in Q_INNER:
                    a = lx_ref[k, pl.ds(r * TI // 2, n * TI // 2), pl.ds(i * LANE, LANE)]
                    at = 7 * r + n * Q_ORDER.index(k) if i == Q_INNER[0] else -1
                    if at == C_DUE:
                        a = _cat([_hold(a[:8], last, zero), a[8:]], 0)
                    mi[i] = _dot(_as_bf16(a), rw[k][i].astype(BF16))
                    recent.append(mi[i])
                    if at in C_START:
                        last[:] = [_as_u32(mi[i][:8]) | last[0] if last else _as_u32(mi[i][:8])]
                        c_operands(C_START.index(at))
                    if at in WO_START:
                        wo_operands(WO_START.index(at))
                ms[k] = _unsplit(_strassen_out(mi), n)
            for k, v in enumerate(_strassen_out(ms)):
                q_ref[j, k, pl.ds(r * TH, n * TH), :] = (v * qscale).astype(BF16)
        return 0

    jax.lax.fori_loop(0, NP, q_step, 0)
    for p in range(NP):
        w_copy(1, p).wait()
        w_copy(2, p).wait()
    cre_cp.wait()
    cim_cp.wait()

    def head_step(h, _):
        pair = h >> 1
        zero = zero_ref[0]
        shift = (16 - 16 * (h & 1)).astype(U32)
        vscale, vinv = [vsc_ref[k, h & 1, pl.ds(pair, 1), :] for k in range(2)]
        rw = []
        for k in range(7):
            sh = shift + (zero << k).astype(U32)
            rk = _strassen_rhs(*_quads(_unpack(wk_buf[pair], sh)))[k]
            rv = _strassen_rhs(*_quads(_unpack(wv_buf[pair], sh)))[k] * vscale
            rw.append(_strassen_rhs(rk[:CH // 2], rv[:CH // 2], rk[CH // 2:], rv[CH // 2:]))
        causal = (jax.lax.broadcasted_iota(jnp.int32, (TQ, TQ), 1)
                  <= jax.lax.broadcasted_iota(jnp.int32, (TQ, TQ), 0))
        ks, rks, vs, rvs, ss, mxs = [], [], [], [], {}, {}

        def tie(a, b):
            return pltpu.bitcast(_as_u32(a) | (_as_u32(b) & zero.astype(U32)), F32)

        def proj_kv(r, n):
            ms = [None] * 7
            for k in KV_ORDER:
                mi = [None] * 7
                for i in KV_INNER:
                    a = l_ref[k, pl.ds(r * TI // 2, n * TI // 2), pl.ds(i * CH // 2, CH // 2)]
                    mi[i] = _dot(_as_bf16(a), rw[k][i].astype(BF16))
                ms[k] = _unsplit(_strassen_out(mi, KV_INNER if n == 1 else None), n)
                if k != KV_ORDER[-1]:
                    yield
            c = _strassen_out(ms, KV_ORDER if n == 1 else None)
            for b in range(n):
                c11, c12, c21, c22 = [v[b * TH:(b + 1) * TH, :DH] for v in c]
                ks.extend([_cat([c11, c12], 1), _cat([c21, c22], 1)])
                rks.append(_strassen_rhs(c11, c21, c12, c22))
                c11, c12, c21, c22 = [v[b * TH:(b + 1) * TH, DH:] for v in c]
                vs.extend([_cat([c11, c12], 1), _cat([c21, c22], 1)])
                rvs.append(_strassen_rhs(c11, c12, c21, c22))

        def scores(j):
            cols = pl.ds(pl.multiple_of((h & 1) * DH, DH), DH)
            qf = [q_ref[pair, k, j * TQ:(j + 1) * TQ, cols].astype(F32) for k in range(4)]
            q = _cat([_cat(qf[:2], 1), _cat(qf[2:], 1)], 0)
            lq = _strassen_lhs(*qf)
            s1, s2, done, mx = [], [], [], []
            for t in range(j):
                m = [None] * 7
                for k in QK_ORDER:
                    a = tie(lq[k], done[-2]) if k == 3 and t >= 2 else lq[k]
                    m[k] = _dot_nt(a.astype(BF16), rks[t][k].astype(BF16))
                c11, c12, c21, c22 = _strassen_out(m, tuple(range(7)))
                x1, x2 = jnp.maximum(c11, c12), jnp.maximum(c21, c22)
                if mx:
                    x1, x2 = jnp.maximum(x1, mx[0]), jnp.maximum(x2, mx[1])
                mx[:] = [x1, x2]
                done.append(_as_u32(x1) | _as_u32(x2))
                s1 += [c11, c12]
                s2 += [c21, c22]
            yield
            d = _dot_nt(q.astype(BF16), ks[2 * j].astype(BF16))
            ss[2 * j] = _cat(s1 + [d[:TQ]], 1)
            ss[2 * j + 1] = _cat(
                s2 + [d[TQ:], _dot_nt(q[TQ:].astype(BF16), ks[2 * j + 1].astype(BF16))], 1)
            if mx:
                mxs[2 * j], mxs[2 * j + 1] = mx

        def masked(i):
            lo = i * TQ
            s = ss.pop(i)
            sd = jnp.where(causal, s[:, lo:], -1e9 * LOG2E)
            s = sd if i == 0 else _cat([s[:, :lo], sd], 1)
            t = _cat([mxs[i], s[:, i // 2 * TP:]], 1) if i in mxs else s
            if LOOK[i // 2]:
                return s, functools.reduce(
                    jnp.maximum, [t[:, c:c + LANE] for c in range(0, t.shape[1], LANE)])
            return s, jnp.broadcast_to(jnp.max(t, axis=-1, keepdims=True), (TQ, LANE))

        def exp_rows(s, m, parts, look):
            ps = []
            for g in range(0, TQ, 8):
                mg = m[g:g + 8]
                if look:
                    if len(parts) >= look:
                        mg = tie(mg, parts[-look])
                    mg = jnp.broadcast_to(jnp.max(mg, axis=-1, keepdims=True), (8, LANE))
                if parts:
                    mg = tie(mg, parts[-1])
                pg = [jnp.exp2(s[g:g + 8, t * LANE:(t + 1) * LANE] - mg)
                      for t in range(s.shape[1] // LANE)]
                ps.append(_cat(pg, 1))
                parts.append(functools.reduce(lambda a, b: a + b, pg))
            return _cat(ps, 0), _cat(parts[-(TQ // 8):], 0)

        def context(j):
            (s1, m1), (s2, m2) = masked(2 * j), masked(2 * j + 1)
            parts = []
            p1, l1 = exp_rows(s1, m1, parts, LOOK[j])
            if j in EARLY_SUM:
                m2 = tie(m2, jnp.broadcast_to(jnp.sum(l1, axis=-1, keepdims=True), (TQ, LANE)))
            p2, l2 = exp_rows(s2, m2, parts, LOOK[j])
            l1 = _cat([tie(l1[:8], l1[TQ - 8:]), l1[8:]], 0)
            l1, l2 = [jnp.sum(l, axis=-1, keepdims=True) for l in (l1, l2)]
            lo = j * TP
            dot = lambda a, b: _dot(a.astype(BF16), b.astype(BF16))

            def recip(l):
                rl = pl.reciprocal(l, approx=True)
                return rl * (2.0 - l * rl)

            def diag():
                dg = dot(_cat([p1[:, lo:], p2[:, lo:lo + TQ]], 0), vs[2 * j])
                return dg[:TQ], dg[TQ:] + dot(p2[:, lo + TQ:], vs[2 * j + 1])

            r1, r2 = recip(l1), recip(l2)
            rho = l1 * r2
            r1, r2 = r1 * vinv, r2 * vinv
            if j == 0:
                c1, c2 = diag()
                c2 = c2 * _cat([r2, r2], 1)
            else:
                tiles = lambda p, o: _cat(
                    [p[:, (2 * t + o) * TQ:(2 * t + o + 1) * TQ] for t in range(j)], 1)
                a11, a12, a21, a22 = tiles(p1, 0), tiles(p1, 1), tiles(p2, 0), tiles(p2, 1)
                a22r = a22 * rho
                lp = [a11 + a22r, a21 + a22, a11, a22, a11 + a12, a21 * rho - a11, a12 - a22r]
                m = [None] * 7
                for n, k in enumerate(PV_ORDER):
                    if n == PV_DIAG[j]:
                        c1, c2 = diag()
                    if n == 6:
                        yield
                    m[k] = dot(lp[k], _cat([rvs[t][k] for t in range(j)], 0))
                c1 = c1 + _cat([(m[0] - m[4]) + (m[6] + m[3] * rho), m[2] + m[4]], 1)
                c2 = (c2 + _cat([m[1] + m[3], -m[1]], 1)) * _cat([r2, r2], 1)
                c2 = _cat([c2[:, :DH], c2[:, DH:] + ((m[0] + m[2]) + m[5]) * r1], 1)
            c1 = c1 * _cat([r1, r1], 1)
            ctx_ref[h, j * TQ:(j + 1) * TQ, :] = _cat(
                _strassen_rhs(c1[:, :DH], c2[:, :DH], c1[:, DH:], c2[:, DH:]), 1).astype(BF16)

        kvs = [proj_kv(r, 1) for r in range(NP)]
        qks = [scores(j) for j in range(NP)]
        pvs = [context(j) for j in range(NP)]
        _run(SCHEDULE, dict(d=lambda r: list(proj_kv(r, 2)), c=lambda r: list(kvs[r]),
                            x=lambda r: [next(kvs[r // 10]) for _ in range(r % 10)],
                            u=lambda j: next(qks[j]), t=lambda j: list(qks[j]),
                            b=lambda j: next(pvs[j]), p=lambda j: list(pvs[j])))
        return 0

    jax.lax.fori_loop(0, H, head_step, 0)

    pieces = ((0, 0, TP), (MH, 0, TQ), (MH, TQ, TQ))

    def o_copy(j, n):
        r0, c0, nc = pieces[n]
        return pltpu.make_async_copy(
            out_ref.at[j, pl.ds(r0, MH), pl.ds(c0, nc)],
            o_hbm.at[pl.ds(r0, MH), pl.ds(pl.multiple_of(j * TP + c0, TQ), nc)], osem.at[n, j])

    def o_step(jj, _):
        zero = zero_ref[0]
        js = (2 * jj, 2 * jj + 1)
        t0 = [pl.multiple_of(j * TP, TP) for j in js]
        last, state, ys, gates, m, recent = [], {}, [None, None], {}, [{}, {}], []
        rnd = lambda v: v.astype(BF16).astype(F32)

        def ssm_tile(u, t):
            rows = pl.ds(t0[u], TP + 8)
            cr, ci = pl.ds(t * LANE, LANE), pl.ds(PP + t * LANE, LANE)
            co = [co_ref[k, :, cr] for k in range(10)]
            u0 = u_ref[rows, cr]
            u1 = u_ref[rows, ci] if t < FT else pltpu.roll(u0, HALF, 1)
            mul = lambda k, x: (co[k] * x[0] + co[k + 1] * x[1], co[k] * x[1] - co[k + 1] * x[0])
            sub = jax.lax.broadcasted_iota(jnp.int32, (8, LANE), 0)
            s = state[t] if u else (st_ref[0, :, cr], st_ref[1, :, cr])
            prev, gs = [None] * 3, []
            for k in range(TP // 8 + 1):
                x0, x1 = _hold(u0[8 * k:8 * k + 8], last, zero), u1[8 * k:8 * k + 8]
                w = (co[0] * x0 + co[1] * x1, co[1] * x0 - co[0] * x1)
                for i in range(3):
                    cur = [pltpu.roll(v, 1 << i, 0) for v in w]
                    old = cur if k == 0 else prev[i]
                    d = mul(2 * i + 2, [jnp.where(sub < (1 << i), o, c) for o, c in zip(old, cur)])
                    w = [p + q for p, q in zip(d, w)]
                    prev[i] = cur
                if k > 0:
                    s = [p + q for p, q in zip(mul(8, s), w)]
                    gs.append(_cat(s, 1) if t < FT else s[0])
                    last[:] = [s[0]]
            state[t] = s
            if u:
                st_ref[0, :, cr] = s[0]
                st_ref[1, :, cr] = s[1]
            cols = cr if t < FT else pl.ds(PF, HALF)
            cc = _cat([cre_ref[:, cols], cim_ref[:, cols]], 1)
            g = _cat(gs, 0).astype(BF16)
            n = MH if t < FT else MH // 2
            y = _cat([_dot_nt(_as_bf16(cc[a:a + n]), g) for a in range(0, MH, n)], 0)
            ys[u] = y if ys[u] is None else y + ys[u]

        def gate(u):
            gcol = _as_u32(col_ref[1]) | (_as_u32(_cat(recent[-2:], 0)) & zero.astype(U32))
            gcol = _cat([pltpu.bitcast(gcol, F32)] * (TP // LANE), 1)
            xt = xt_ref[:, pl.ds(t0[u], TP)].astype(F32)
            z = jnp.sum(rnd(xt * gcol), axis=0, keepdims=True)
            gates[u] = rnd(1.0 / rnd(1.0 + rnd(jnp.exp(-rnd(z)))))

        def product(u, k):
            if k in SUMS:
                a = [lo_ref[n, :, pl.ds(SUMS.index(k) * DH, DH)] for n in range(H)]
            else:
                o = k - 2
                a = [_as_bf16(wot_ref[n, pl.ds(o * MH // 2, MH // 2), pl.ds(o * DH, DH)])
                     for n in range(H)]
            rows = pl.ds(pl.multiple_of(js[u] * TQ, TQ), TQ)
            b = [ctx_ref[n, rows, pl.ds(k * DH, DH)] for n in range(H)]
            m[u][k] = _dot_nt(_cat(a, 1), _cat(b, 1))
            recent.append(m[u][k])

        def emit(u, n, v):
            r0, c0, nc = pieces[n]
            g = gates[u][:, c0:c0 + nc]
            dcol = _cat([col_ref[0, r0:r0 + MH]] * (nc // LANE), 1)
            xt = xt_ref[pl.ds(r0, MH), pl.ds(pl.multiple_of(t0[u] + c0, TQ), nc)].astype(F32)
            b = ys[u][r0:r0 + MH, c0:c0 + nc] + rnd(xt * dcol)
            out_ref[js[u], pl.ds(r0, MH), pl.ds(c0, nc)] = g * v + rnd(1.0 - g) * b
            o_copy(js[u], n).start()

        _run(O_SCHEDULE, dict(a=lambda k: product(0, k), b=lambda k: product(1, k), g=gate,
                              m=lambda t: ssm_tile(0, t), n=lambda t: ssm_tile(1, t)))
        for u, p in enumerate(m):
            emit(u, 0, _cat([(p[0] + p[3]) + (p[6] - p[4]), p[2] + p[4]], 1))
            emit(u, 1, p[1] + p[3])
            emit(u, 2, ((p[0] + p[2]) - p[1]) + p[5])
        return 0

    jax.lax.fori_loop(0, NP // 2, o_step, 0)
    for j in range(NP):
        for n in range(3):
            o_copy(j, n).wait()


@jax.jit
def pallas_gated_mix__compressed_kv_cla__ssm_conv_s5__prompt_kernel(
    A_x: jax.Array,
    A_c_kv: jax.Array,
    A_w_q: jax.Array,
    A_w_uk: jax.Array,
    A_w_uv: jax.Array,
    A_w_o: jax.Array,
    B_x: jax.Array,
    B_Lambda_re: jax.Array,
    B_Lambda_im: jax.Array,
    B_B_re: jax.Array,
    B_B_im: jax.Array,
    B_C_re: jax.Array,
    B_C_im: jax.Array,
    B_log_dt: jax.Array,
    B_Dskip: jax.Array,
    gate_w: jax.Array,
):
    del B_x
    _, S, M = A_x.shape
    C = A_c_kv.shape[2]
    H, D = A_w_q.shape[1], A_w_q.shape[2]
    PP = (M + LANE - 1) // LANE * LANE

    hbm = pl.BlockSpec(memory_space=pl.ANY)
    out_t = pl.pallas_call(
        functools.partial(_kernel, S=S, M=M, H=H, D=D),
        in_specs=[hbm] * 15,
        out_specs=hbm,
        out_shape=jax.ShapeDtypeStruct((M, S), F32),
        scratch_shapes=[
            pltpu.VMEM((M, S), BF16),
            pltpu.VMEM((S // 2, M), U32),
            pltpu.VMEM((7, S // 8, 7 * PP // 4), U32),
            pltpu.VMEM((S // 2, C), U32),
            pltpu.VMEM((7, S // 8, 7 * C // 4), U32),
            pltpu.VMEM((H // 2, M, D), U32),
            pltpu.VMEM((H // 2, C, D), U32),
            pltpu.VMEM((H // 2, C, D), U32),
            pltpu.VMEM((H, M // 2, D), U32),
            pltpu.VMEM((H, M // 2, 5 * D // 2), BF16),
            pltpu.VMEM((M, M), U32),
            pltpu.VMEM((M // 2, M), U32),
            pltpu.VMEM((M // 2, M), U32),
            pltpu.VMEM((S + 32, 2 * M), F32),
            pltpu.VMEM((S // TP, M, TP), F32),
            pltpu.VMEM((2, 8, PP), F32),
            pltpu.VMEM((10, 8, PP), F32),
            pltpu.VMEM((2, M, LANE), F32),
            pltpu.VMEM((3, 8, H // 2, D), U32),
            pltpu.VMEM((2, 4, H // 2, LANE), F32),
            pltpu.VMEM((H // 2, 4, S // 2, D), BF16),
            pltpu.VMEM((H, S // 2, 7 * D // 2), BF16),
            pltpu.SMEM((1,), jnp.int32),
            pltpu.SemaphoreType.DMA((5, H // 2)),
            pltpu.SemaphoreType.DMA((4,)),
            pltpu.SemaphoreType.DMA((8,)),
            pltpu.SemaphoreType.DMA((5,)),
            pltpu.SemaphoreType.DMA((3, S // TP)),
        ] + [pltpu.VMEM((M,), BF16)] * 5,
        compiler_params=pltpu.CompilerParams(
            vmem_limit_bytes=124 * 1024 * 1024,
            disable_semaphore_checks=True,
            disable_bounds_checks=True,
        ),
    )(
        jnp.swapaxes(A_x, 1, 2).reshape(M, S), A_c_kv.reshape(S, C),
        A_w_q, A_w_uk, A_w_uv, jnp.swapaxes(A_w_o, 1, 2),
        B_B_re, B_B_im, B_C_re, B_C_im,
        B_Lambda_re, B_Lambda_im, B_log_dt, B_Dskip, gate_w,
    )
    return jnp.swapaxes(out_t.reshape(1, M, S), 1, 2)
```

```python
import functools

import jax
import jax.numpy as jnp
import jax.experimental.pallas as pl
import jax.experimental.pallas.tpu as pltpu

F32 = jnp.float32
BF16 = jnp.bfloat16
U32 = jnp.uint32

NT_DIMS = (((1,), (1,)), ((), ()))
LOG2E = 1.4426950408889634

LANE = 128
HALF = LANE // 2
TQ = 128
TP = 256
TU = 512

U_SCHEDULE = "t4 u2 x1 u3 x4 x2 u4 x5 t6 u5 x3 u6 x7 v7 x6 w7"
Q_SCHEDULE = ((0, 2), (2, 1), (3, 1), (4, 1), (5, 1), (6, 1), (7, 1))
Q_ORDER = (1, 6, 0, 3, 2, 5, 4)
Q_INNER = (1, 3, 5, 0, 2, 4, 6)
Q_REMAT = (0, 2, 3, 4, 5, 6)
C_START = (14, 20, 30, 38)
WO_START = (40, 52)
C_DUE = 53
C_EXTRA = 4
SCHEDULE = ("d0 x25 t0 t1 c2 p0 p1 t2 c3 u3 b2 t3 c4 u4 p2 b3 t4 c5 p3 p4 t5 c6 b5 t6 c7 t7 "
            "p5 b6 b7 p6 p7")
KV_ORDER = (1, 3, 2, 4, 0, 5, 6)
KV_INNER = (1, 3, 6, 0, 2, 4, 5)
QK_ORDER = (0, 1, 4, 3, 2, 6, 5)
PV_ORDER = (4, 3, 1, 5, 2, 0, 6)
PV_DIAG = (0, 5, 0, 1, 0, 3, 3, 0)
EARLY_SUM = (1, 2, 7)
LOOK = (0, 0, 0, 0, 0, 0, 4, 0)
O_SCHEDULE = "a3 a4 a0 g0 m0 m3 a6 m1 a2 a1 a5 n3 b0 m2 b3 g1 b4 n2 n0 n1 b6 b2 b1 b5"


def _cat(xs, axis):
    return jnp.concatenate(xs, axis=axis)


def _dot(a, b):
    return jnp.dot(a, b, preferred_element_type=F32)


def _dot_nt(a, b):
    return jax.lax.dot_general(a, b, NT_DIMS, preferred_element_type=F32)


def _unpack(w32, shift):
    v = (w32 << shift) & jnp.uint32(0xFFFF0000)
    return pltpu.bitcast(v, F32)


def _as_bf16(w32):
    return pltpu.bitcast(w32, BF16)


def _as_u32(v):
    return pltpu.bitcast(v, U32)


def _run(schedule, ops):
    for op in schedule.split():
        ops[op[0]](int(op[1:]))


def _strassen_lhs(a11, a12, a21, a22):
    return [a11 + a22, a21 + a22, a11, a22, a11 + a12, a21 - a11, a12 - a22]


def _strassen_rhs(b11, b12, b21, b22):
    return [b11 + b22, b11, b12 - b22, b21 - b11, b22, b11 + b12, b21 + b22]


def _strassen_out(m, order=None):
    if order is None:
        return ((m[0] + m[3]) + (m[6] - m[4]), m[2] + m[4],
                m[1] + m[3], (m[0] - m[1]) + (m[2] + m[5]))

    def fold(ks, neg):
        ks = sorted(ks, key=order.index)
        if ks[0] == neg:
            ks[:2] = ks[1::-1]
        return functools.reduce(lambda a, k: a - m[k] if k == neg else a + m[k], ks[1:], m[ks[0]])

    return fold((0, 3, 4, 6), 4), m[2] + m[4], m[1] + m[3], fold((0, 1, 2, 5), 1)


SUMS = (0, 1, 4, 5, 6)


def _quads(a):
    m, n = a.shape[0] // 2, a.shape[1] // 2
    return a[:m, :n], a[:m, n:], a[m:, :n], a[m:, n:]


def _unsplit(c, n):
    top, bot = _cat(c[:2], 1), _cat(c[2:], 1)
    rows = top.shape[0] // n
    return _cat([v[b * rows:(b + 1) * rows] for b in range(n) for v in (top, bot)], 0)


def _hold(v, last, zero):
    if not last:
        return v
    z = jnp.tile(_as_u32(last[0]) & zero.astype(U32), (v.shape[0] // 8, pl.cdiv(v.shape[1], LANE)))
    return pltpu.bitcast(_as_u32(v) | z[:, :v.shape[1]], v.dtype)


def _lhs_operands(a, last, zero, extra):
    first = (0, 2, 0, 3, 0, 2, 1)
    for k in range(7):
        q = list(_quads(a))
        q[first[k]] = _hold(q[first[k]], last, zero)
        l = _strassen_lhs(*q)[k]
        out = []
        for grp in ((0, 1, 2, 3), (4, 5, 6)):
            q = list(_quads(l))
            if out:
                for b in sorted(set(first[i] for i in grp)):
                    q[b] = _hold(q[b], last, zero)
            v = _cat([_strassen_lhs(*q)[i] for i in grp], 1)
            out.append(_as_u32(v.astype(BF16)))
            last[:] = [functools.reduce(
                jnp.bitwise_or, [out[-1][:, c:c + LANE] for c in range(0, v.shape[1], LANE)])]
            for _ in range(extra):
                last[:] = [last[0] + last[0]]
        yield _cat(out, 1)


def _kernel(xt_hbm, c_hbm, wq_hbm, wuk_hbm, wuv_hbm, wot_hbm,
            bre_hbm, bim_hbm, cre_hbm, cim_hbm,
            lre_hbm, lim_hbm, ldt_hbm, dsk_hbm, gw_hbm,
            o_hbm,
            xt_ref, x_ref, lx_ref, c_ref, l_ref, wq_buf, wk_buf, wv_buf, wot_ref, lo_ref,
            b_ref, cre_ref, cim_ref, u_ref, out_ref, st_ref, co_ref, col_ref, smp_ref, vsc_ref,
            q_ref, ctx_ref, zero_ref, wsem, xsem, msem, vsem, osem,
            lre_ref, lim_ref, ldt_ref, dsk_ref, gw_ref,
            *, S, M, H, D):
    P = M
    FT = P // LANE
    PF = FT * LANE
    PP = PF + LANE
    NP = H // 2
    CH, DH, MH, TH = c_ref.shape[1] // 2, D // 2, M // 2, TP // 2
    TI = TH // 2
    assert P - PF == HALF and PP == 4 * LANE and DH == LANE and S // TP == NP and TP == 2 * TQ

    def w_copy(k, pair):
        src, dst = ((wq_hbm, wq_buf), (wuk_hbm, wk_buf), (wuv_hbm, wv_buf))[k]
        return pltpu.make_async_copy(src.bitcast(U32).at[:, pair, :], dst.at[pair], wsem.at[k, pair])

    def wo_copy(pair):
        heads = pl.ds(2 * pair, 2)
        return pltpu.make_async_copy(wot_hbm.bitcast(U32).at[heads], wot_ref.at[heads],
                                     wsem.at[3, pair])

    def c_copy(r):
        rows = pl.ds(pl.multiple_of(r * TH, TH), TH)
        return pltpu.make_async_copy(c_hbm.bitcast(U32).at[rows], c_ref.at[rows], wsem.at[4, r])

    def x_copy(t0, n, k):
        cols = pl.ds(t0, n)
        return pltpu.make_async_copy(xt_hbm.at[:, cols], xt_ref.at[:, cols], xsem.at[k])

    x_cps = [x_copy(0, TP, 0), x_copy(TP, TP, 1), x_copy(TU, TU, 2), x_copy(2 * TU, S - 2 * TU, 3)]
    bre32, bim32 = bre_hbm.bitcast(U32), bim_hbm.bitcast(U32)
    b_cps = [
        pltpu.make_async_copy(bre32, b_ref.at[pl.ds(0, P // 2), :], msem.at[0]),
        pltpu.make_async_copy(bim32.at[pl.ds(PF // 2, HALF // 2), :],
                              b_ref.at[pl.ds(P // 2, HALF // 2), :], msem.at[1]),
        pltpu.make_async_copy(bim32.at[pl.ds(0, PF // 2), :],
                              b_ref.at[pl.ds(PP // 2, PF // 2), :], msem.at[2]),
    ]
    cre_cp = pltpu.make_async_copy(cre_hbm.bitcast(U32), cre_ref, msem.at[3])
    cim_cp = pltpu.make_async_copy(cim_hbm.bitcast(U32), cim_ref, msem.at[4])
    smp_cps = [pltpu.make_async_copy(src.bitcast(U32).at[pl.ds(0, smp_ref.shape[1])],
                                     smp_ref.at[k], msem.at[5 + k])
               for k, src in enumerate((wuk_hbm, wuv_hbm, wq_hbm))]
    v_cps = [pltpu.make_async_copy(src, dst, vsem.at[k]) for k, (src, dst) in enumerate(
        ((lre_hbm, lre_ref), (lim_hbm, lim_ref), (ldt_hbm, ldt_ref),
         (dsk_hbm, dsk_ref), (gw_hbm, gw_ref)))]

    for cp in x_cps[:1] + v_cps + b_cps + x_cps[1:] + smp_cps:
        cp.start()
    for p in range(NP):
        w_copy(0, p).start()
        wo_copy(p).start()
        c_copy(p).start()
    for p in range(NP):
        w_copy(1, p).start()
        w_copy(2, p).start()
    cre_cp.start()
    cim_cp.start()

    zero_ref[0] = 0
    u_ref[pl.ds(0, 8), :] = jnp.zeros((8, u_ref.shape[1]), F32)
    st_ref[...] = jnp.zeros(st_ref.shape, F32)
    for cp in v_cps + x_cps[:1]:
        cp.wait()

    row = lambda r: r[...].astype(F32).reshape(1, P)
    lre, lim = row(lre_ref), row(lim_ref)
    dt = jnp.exp(row(ldt_ref)).astype(BF16).astype(F32)
    e = jnp.exp(dt * lre)
    ang = dt * lim
    ar = e * jnp.cos(ang)
    ai = e * jnp.sin(ang)
    sc = jnp.maximum(jnp.abs(lre), jnp.abs(lim))
    nre, nim = lre / sc, lim / sc
    den = (nre * nre + nim * nim) * sc
    gr = 2.0 * ((ar - 1.0) * nre + ai * nim) / den
    gi = 2.0 * (ai * nre - (ar - 1.0) * nim) / den

    def put(k, full, lo, hi):
        co_ref[k] = jnp.broadcast_to(_cat([full[:, :PF], lo[:, PF:], hi[:, PF:]], 1), (8, PP))

    put(0, gr, gr, -gr)
    put(1, -gi, -gi, -gi)
    pr, pi = ar, -ai
    for j in range(1, 5):
        put(2 * j, pr, pr, pr)
        put(2 * j + 1, -pi, -pi, pi)
        pr, pi = pr * pr - pi * pi, 2.0 * pr * pi

    zpad = jnp.zeros((1, PP - P), F32)
    for k, r in enumerate((dsk_ref, gw_ref)):
        col_ref[k] = jnp.broadcast_to(_cat([row(r), zpad], 1), (LANE, PP)).T[:M]

    zero1, last1 = zero_ref[0], []

    def transpose_x(t0, n):
        x_ref[pl.ds(t0 // 2, n // 2), :] = _as_u32(xt_ref[:, pl.ds(t0, n)].T)

    def x_operands(r):
        for n in range(TI // 16):
            x = _cat([x_ref[pl.ds(r * TH + g * TI // 2 + 8 * n, 8), :] for g in range(4)], 0)
            x = _as_bf16(_hold(x, last1, zero1)).astype(F32)
            x = _cat([x, jnp.zeros((x.shape[0], PP - M), F32)], 1)
            for k, v in enumerate(_lhs_operands(x, last1, zero1, 0)):
                lx_ref[k, pl.ds(r * TI // 2 + 8 * n, 8), :] = v

    def proj_u(r, lo=0, hi=2 * P, due=False, mark=False):
        x = x_ref[pl.ds(r * TH, TH), :]
        if due:
            x = _cat([_hold(x[:8], last1, zero1), x[8:]], 0)
        u = _dot_nt(_as_bf16(x), _as_bf16(b_ref[lo // 2:hi // 2, :]))
        u_ref[pl.ds(r * TP + 8, TP), lo:hi] = u
        if mark:
            last1[:] = [functools.reduce(jnp.bitwise_or, last1 + [_as_u32(u[:8, :LANE])])]

    transpose_x(0, TP)
    b_cps[0].wait()
    b_cps[1].wait()
    proj_u(0, 0, PP)
    b_cps[2].wait()
    x_cps[1].wait()
    proj_u(0, PP)
    transpose_x(TP, TP)
    x_cps[2].wait()
    proj_u(1, 0, 6 * LANE, mark=True)
    transpose_x(TU, TU)
    x_operands(0)
    proj_u(1, 6 * LANE, due=True)
    last1.clear()
    x_cps[3].wait()
    for cp in smp_cps:
        cp.wait()

    def exponent(k, e):
        mag = jnp.sum(jnp.abs(_unpack(smp_ref[k], jnp.uint32(16 - 16 * e))), axis=0)
        mag = jnp.sum(mag, axis=1, keepdims=True)
        return jnp.broadcast_to(pltpu.bitcast(mag, jnp.int32) >> 23, (NP, LANE))

    for n, (target, scaled) in enumerate((((0, 0), (1, 0)), ((0, 1), (1, 1)), ((2, 0), (2, 1)))):
        e0, e1 = exponent(*target), exponent(*scaled)
        d = jnp.where((e0 > 0) & (e1 > 0), jnp.clip(e0 - e1, -40, 40), 0)
        vsc_ref[0, n] = pltpu.bitcast((127 + d) << 23, F32)
        vsc_ref[1, n] = pltpu.bitcast((127 - d) << 23, F32)

    _run(U_SCHEDULE, dict(t=lambda r: transpose_x(r * TP, TU), x=x_operands,
                          u=lambda r: proj_u(r, mark=True),
                          v=lambda r: proj_u(r, 0, 6 * LANE, mark=True),
                          w=lambda r: proj_u(r, 6 * LANE, due=True)))

    def q_step(j, _):
        w_copy(0, j).wait()
        wo_copy(j).wait()
        c_copy(j).wait()
        zero = zero_ref[0]
        last, recent = [], []
        wq32 = _cat([wq_buf[j], jnp.zeros((PP - M, D), U32)], 0)
        rw = []
        for k in range(7):
            z = (zero << k).astype(U32) if k in Q_REMAT else jnp.uint32(0)
            w0 = pltpu.bitcast(wq32 << (z + 16), F32)
            w1 = pltpu.bitcast(wq32 & (z + jnp.uint32(0xFFFF0000)), F32)
            r0 = _strassen_rhs(*_quads(w0))[k]
            r1 = _strassen_rhs(*_quads(w1))[k] * vsc_ref[0, 2, pl.ds(j, 1), :]
            rw.append(_strassen_rhs(r0[:LANE], r1[:LANE], r0[LANE:], r1[LANE:]))
        qscale = _cat([jnp.ones((1, DH), F32), vsc_ref[1, 2, pl.ds(j, 1), :]], 1)
        qscale = qscale * ((D ** -0.5) * LOG2E)

        def c_operands(n):
            c = _cat([c_ref[pl.ds(pl.multiple_of(j * TH + g * (TI // 2) + 8 * n, 8), 8), :]
                      for g in range(4)], 0)
            c = _as_bf16(_hold(c, last, zero)).astype(F32)
            rows = pl.ds(pl.multiple_of(j * (TI // 2) + 8 * n, 8), 8)
            for k, v in enumerate(_lhs_operands(c, last, zero, C_EXTRA)):
                l_ref[k, rows, :] = v

        def wo_operands(e):
            z = _as_u32(_cat([v[:TI] for v in recent[-7:]], 0)) & zero.astype(U32)
            w = wot_ref[2 * j + e] | _cat([z[:MH], z[MH:]], 1)
            ls = _strassen_lhs(*_quads(_as_bf16(w).astype(F32)))
            lo_ref[2 * j + e] = _cat([ls[k] for k in SUMS], 1).astype(BF16)

        for r, n in Q_SCHEDULE:
            ms = [None] * 7
            for k in Q_ORDER:
                mi = [None] * 7
                for i in Q_INNER:
                    a = lx_ref[k, pl.ds(r * TI // 2, n * TI // 2), pl.ds(i * LANE, LANE)]
                    at = 7 * r + n * Q_ORDER.index(k) if i == Q_INNER[0] else -1
                    if at == C_DUE:
                        a = _cat([_hold(a[:8], last, zero), a[8:]], 0)
                    mi[i] = _dot(_as_bf16(a), rw[k][i].astype(BF16))
                    recent.append(mi[i])
                    if at in C_START:
                        last[:] = [_as_u32(mi[i][:8]) | last[0] if last else _as_u32(mi[i][:8])]
                        c_operands(C_START.index(at))
                    if at in WO_START:
                        wo_operands(WO_START.index(at))
                ms[k] = _unsplit(_strassen_out(mi), n)
            for k, v in enumerate(_strassen_out(ms)):
                q_ref[j, k, pl.ds(r * TH, n * TH), :] = (v * qscale).astype(BF16)
        return 0

    jax.lax.fori_loop(0, NP, q_step, 0)
    for p in range(NP):
        w_copy(1, p).wait()
        w_copy(2, p).wait()
    cre_cp.wait()
    cim_cp.wait()

    def head_step(h, _):
        pair = h >> 1
        zero = zero_ref[0]
        shift = (16 - 16 * (h & 1)).astype(U32)
        vscale, vinv = [vsc_ref[k, h & 1, pl.ds(pair, 1), :] for k in range(2)]
        rw = []
        for k in range(7):
            sh = shift + (zero << k).astype(U32)
            rk = _strassen_rhs(*_quads(_unpack(wk_buf[pair], sh)))[k]
            rv = _strassen_rhs(*_quads(_unpack(wv_buf[pair], sh)))[k] * vscale
            rw.append(_strassen_rhs(rk[:CH // 2], rv[:CH // 2], rk[CH // 2:], rv[CH // 2:]))
        causal = (jax.lax.broadcasted_iota(jnp.int32, (TQ, TQ), 1)
                  <= jax.lax.broadcasted_iota(jnp.int32, (TQ, TQ), 0))
        ks, rks, vs, rvs, ss, mxs = [], [], [], [], {}, {}

        def tie(a, b):
            return pltpu.bitcast(_as_u32(a) | (_as_u32(b) & zero.astype(U32)), F32)

        def proj_kv(r, n):
            ms = [None] * 7
            for k in KV_ORDER:
                mi = [None] * 7
                for i in KV_INNER:
                    a = l_ref[k, pl.ds(r * TI // 2, n * TI // 2), pl.ds(i * CH // 2, CH // 2)]
                    mi[i] = _dot(_as_bf16(a), rw[k][i].astype(BF16))
                ms[k] = _unsplit(_strassen_out(mi, KV_INNER if n == 1 else None), n)
                if k != KV_ORDER[-1]:
                    yield
            c = _strassen_out(ms, KV_ORDER if n == 1 else None)
            for b in range(n):
                c11, c12, c21, c22 = [v[b * TH:(b + 1) * TH, :DH] for v in c]
                ks.extend([_cat([c11, c12], 1), _cat([c21, c22], 1)])
                rks.append(_strassen_rhs(c11, c21, c12, c22))
                c11, c12, c21, c22 = [v[b * TH:(b + 1) * TH, DH:] for v in c]
                vs.extend([_cat([c11, c12], 1), _cat([c21, c22], 1)])
                rvs.append(_strassen_rhs(c11, c12, c21, c22))

        def scores(j):
            cols = pl.ds(pl.multiple_of((h & 1) * DH, DH), DH)
            qf = [q_ref[pair, k, j * TQ:(j + 1) * TQ, cols].astype(F32) for k in range(4)]
            q = _cat([_cat(qf[:2], 1), _cat(qf[2:], 1)], 0)
            lq = _strassen_lhs(*qf)
            s1, s2, done, mx = [], [], [], []
            for t in range(j):
                m = [None] * 7
                for k in QK_ORDER:
                    a = tie(lq[k], done[-2]) if k == 3 and t >= 2 else lq[k]
                    m[k] = _dot_nt(a.astype(BF16), rks[t][k].astype(BF16))
                c11, c12, c21, c22 = _strassen_out(m, tuple(range(7)))
                x1, x2 = jnp.maximum(c11, c12), jnp.maximum(c21, c22)
                if mx:
                    x1, x2 = jnp.maximum(x1, mx[0]), jnp.maximum(x2, mx[1])
                mx[:] = [x1, x2]
                done.append(_as_u32(x1) | _as_u32(x2))
                s1 += [c11, c12]
                s2 += [c21, c22]
            yield
            d = _dot_nt(q.astype(BF16), ks[2 * j].astype(BF16))
            ss[2 * j] = _cat(s1 + [d[:TQ]], 1)
            ss[2 * j + 1] = _cat(
                s2 + [d[TQ:], _dot_nt(q[TQ:].astype(BF16), ks[2 * j + 1].astype(BF16))], 1)
            if mx:
                mxs[2 * j], mxs[2 * j + 1] = mx

        def masked(i):
            lo = i * TQ
            s = ss.pop(i)
            sd = jnp.where(causal, s[:, lo:], -1e9 * LOG2E)
            s = sd if i == 0 else _cat([s[:, :lo], sd], 1)
            t = _cat([mxs[i], s[:, i // 2 * TP:]], 1) if i in mxs else s
            if LOOK[i // 2]:
                return s, functools.reduce(
                    jnp.maximum, [t[:, c:c + LANE] for c in range(0, t.shape[1], LANE)])
            return s, jnp.broadcast_to(jnp.max(t, axis=-1, keepdims=True), (TQ, LANE))

        def exp_rows(s, m, parts, look):
            ps = []
            for g in range(0, TQ, 8):
                mg = m[g:g + 8]
                if look:
                    if len(parts) >= look:
                        mg = tie(mg, parts[-look])
                    mg = jnp.broadcast_to(jnp.max(mg, axis=-1, keepdims=True), (8, LANE))
                if parts:
                    mg = tie(mg, parts[-1])
                pg = [jnp.exp2(s[g:g + 8, t * LANE:(t + 1) * LANE] - mg)
                      for t in range(s.shape[1] // LANE)]
                ps.append(_cat(pg, 1))
                parts.append(functools.reduce(lambda a, b: a + b, pg))
            return _cat(ps, 0), _cat(parts[-(TQ // 8):], 0)

        def context(j):
            (s1, m1), (s2, m2) = masked(2 * j), masked(2 * j + 1)
            parts = []
            p1, l1 = exp_rows(s1, m1, parts, LOOK[j])
            if j in EARLY_SUM:
                m2 = tie(m2, jnp.broadcast_to(jnp.sum(l1, axis=-1, keepdims=True), (TQ, LANE)))
            p2, l2 = exp_rows(s2, m2, parts, LOOK[j])
            l1 = _cat([tie(l1[:8], l1[TQ - 8:]), l1[8:]], 0)
            l1, l2 = [jnp.sum(l, axis=-1, keepdims=True) for l in (l1, l2)]
            lo = j * TP
            dot = lambda a, b: _dot(a.astype(BF16), b.astype(BF16))

            def recip(l):
                rl = pl.reciprocal(l, approx=True)
                return rl * (2.0 - l * rl)

            def diag():
                dg = dot(_cat([p1[:, lo:], p2[:, lo:lo + TQ]], 0), vs[2 * j])
                return dg[:TQ], dg[TQ:] + dot(p2[:, lo + TQ:], vs[2 * j + 1])

            r1, r2 = recip(l1), recip(l2)
            rho = l1 * r2
            r1, r2 = r1 * vinv, r2 * vinv
            if j == 0:
                c1, c2 = diag()
                c2 = c2 * _cat([r2, r2], 1)
            else:
                tiles = lambda p, o: _cat(
                    [p[:, (2 * t + o) * TQ:(2 * t + o + 1) * TQ] for t in range(j)], 1)
                a11, a12, a21, a22 = tiles(p1, 0), tiles(p1, 1), tiles(p2, 0), tiles(p2, 1)
                a22r = a22 * rho
                lp = [a11 + a22r, a21 + a22, a11, a22, a11 + a12, a21 * rho - a11, a12 - a22r]
                m = [None] * 7
                for n, k in enumerate(PV_ORDER):
                    if n == PV_DIAG[j]:
                        c1, c2 = diag()
                    if n == 6:
                        yield
                    m[k] = dot(lp[k], _cat([rvs[t][k] for t in range(j)], 0))
                c1 = c1 + _cat([(m[0] - m[4]) + (m[6] + m[3] * rho), m[2] + m[4]], 1)
                c2 = (c2 + _cat([m[1] + m[3], -m[1]], 1)) * _cat([r2, r2], 1)
                c2 = _cat([c2[:, :DH], c2[:, DH:] + ((m[0] + m[2]) + m[5]) * r1], 1)
            c1 = c1 * _cat([r1, r1], 1)
            ctx_ref[h, j * TQ:(j + 1) * TQ, :] = _cat(
                _strassen_rhs(c1[:, :DH], c2[:, :DH], c1[:, DH:], c2[:, DH:]), 1).astype(BF16)

        kvs = [proj_kv(r, 1) for r in range(NP)]
        qks = [scores(j) for j in range(NP)]
        pvs = [context(j) for j in range(NP)]
        _run(SCHEDULE, dict(d=lambda r: list(proj_kv(r, 2)), c=lambda r: list(kvs[r]),
                            x=lambda r: [next(kvs[r // 10]) for _ in range(r % 10)],
                            u=lambda j: next(qks[j]), t=lambda j: list(qks[j]),
                            b=lambda j: next(pvs[j]), p=lambda j: list(pvs[j])))
        return 0

    jax.lax.fori_loop(0, H, head_step, 0)

    pieces = ((0, 0, TP), (MH, 0, TQ), (MH, TQ, TQ))

    def o_copy(j, n):
        r0, c0, nc = pieces[n]
        return pltpu.make_async_copy(
            out_ref.at[j, pl.ds(r0, MH), pl.ds(c0, nc)],
            o_hbm.at[pl.ds(r0, MH), pl.ds(pl.multiple_of(j * TP + c0, TQ), nc)], osem.at[n, j])

    def o_step(jj, _):
        zero = zero_ref[0]
        js = (2 * jj, 2 * jj + 1)
        t0 = [pl.multiple_of(j * TP, TP) for j in js]
        last, state, ys, gates, m, recent = [], {}, [None, None], {}, [{}, {}], []
        rnd = lambda v: v.astype(BF16).astype(F32)

        def ssm_tile(u, t):
            rows = pl.ds(t0[u], TP + 8)
            cr, ci = pl.ds(t * LANE, LANE), pl.ds(PP + t * LANE, LANE)
            co = [co_ref[k, :, cr] for k in range(10)]
            u0 = u_ref[rows, cr]
            u1 = u_ref[rows, ci] if t < FT else pltpu.roll(u0, HALF, 1)
            mul = lambda k, x: (co[k] * x[0] + co[k + 1] * x[1], co[k] * x[1] - co[k + 1] * x[0])
            sub = jax.lax.broadcasted_iota(jnp.int32, (8, LANE), 0)
            s = state[t] if u else (st_ref[0, :, cr], st_ref[1, :, cr])
            prev, gs = [None] * 3, []
            for k in range(TP // 8 + 1):
                x0, x1 = _hold(u0[8 * k:8 * k + 8], last, zero), u1[8 * k:8 * k + 8]
                w = (co[0] * x0 + co[1] * x1, co[1] * x0 - co[0] * x1)
                for i in range(3):
                    cur = [pltpu.roll(v, 1 << i, 0) for v in w]
                    old = cur if k == 0 else prev[i]
                    d = mul(2 * i + 2, [jnp.where(sub < (1 << i), o, c) for o, c in zip(old, cur)])
                    w = [p + q for p, q in zip(d, w)]
                    prev[i] = cur
                if k > 0:
                    s = [p + q for p, q in zip(mul(8, s), w)]
                    gs.append(_cat(s, 1) if t < FT else s[0])
                    last[:] = [s[0]]
            state[t] = s
            if u:
                st_ref[0, :, cr] = s[0]
                st_ref[1, :, cr] = s[1]
            cols = cr if t < FT else pl.ds(PF, HALF)
            cc = _cat([cre_ref[:, cols], cim_ref[:, cols]], 1)
            g = _cat(gs, 0).astype(BF16)
            n = MH if t < FT else MH // 2
            y = _cat([_dot_nt(_as_bf16(cc[a:a + n]), g) for a in range(0, MH, n)], 0)
            ys[u] = y if ys[u] is None else y + ys[u]

        def gate(u):
            gcol = _as_u32(col_ref[1]) | (_as_u32(_cat(recent[-2:], 0)) & zero.astype(U32))
            gcol = _cat([pltpu.bitcast(gcol, F32)] * (TP // LANE), 1)
            xt = xt_ref[:, pl.ds(t0[u], TP)].astype(F32)
            z = jnp.sum(rnd(xt * gcol), axis=0, keepdims=True)
            gates[u] = rnd(1.0 / rnd(1.0 + rnd(jnp.exp(-rnd(z)))))

        def product(u, k):
            if k in SUMS:
                a = [lo_ref[n, :, pl.ds(SUMS.index(k) * DH, DH)] for n in range(H)]
            else:
                o = k - 2
                a = [_as_bf16(wot_ref[n, pl.ds(o * MH // 2, MH // 2), pl.ds(o * DH, DH)])
                     for n in range(H)]
            rows = pl.ds(pl.multiple_of(js[u] * TQ, TQ), TQ)
            b = [ctx_ref[n, rows, pl.ds(k * DH, DH)] for n in range(H)]
            m[u][k] = _dot_nt(_cat(a, 1), _cat(b, 1))
            recent.append(m[u][k])

        def emit(u, n, v):
            r0, c0, nc = pieces[n]
            g = gates[u][:, c0:c0 + nc]
            dcol = _cat([col_ref[0, r0:r0 + MH]] * (nc // LANE), 1)
            xt = xt_ref[pl.ds(r0, MH), pl.ds(pl.multiple_of(t0[u] + c0, TQ), nc)].astype(F32)
            b = ys[u][r0:r0 + MH, c0:c0 + nc] + rnd(xt * dcol)
            out_ref[js[u], pl.ds(r0, MH), pl.ds(c0, nc)] = g * v + rnd(1.0 - g) * b
            o_copy(js[u], n).start()

        _run(O_SCHEDULE, dict(a=lambda k: product(0, k), b=lambda k: product(1, k), g=gate,
                              m=lambda t: ssm_tile(0, t), n=lambda t: ssm_tile(1, t)))
        for u, p in enumerate(m):
            emit(u, 0, _cat([(p[0] + p[3]) + (p[6] - p[4]), p[2] + p[4]], 1))
            emit(u, 1, p[1] + p[3])
            emit(u, 2, ((p[0] + p[2]) - p[1]) + p[5])
        return 0

    jax.lax.fori_loop(0, NP // 2, o_step, 0)
    for j in range(NP):
        for n in range(3):
            o_copy(j, n).wait()


@jax.jit
def pallas_gated_mix__compressed_kv_cla__ssm_conv_s5__prompt_kernel(
    A_x: jax.Array,
    A_c_kv: jax.Array,
    A_w_q: jax.Array,
    A_w_uk: jax.Array,
    A_w_uv: jax.Array,
    A_w_o: jax.Array,
    B_x: jax.Array,
    B_Lambda_re: jax.Array,
    B_Lambda_im: jax.Array,
    B_B_re: jax.Array,
    B_B_im: jax.Array,
    B_C_re: jax.Array,
    B_C_im: jax.Array,
    B_log_dt: jax.Array,
    B_Dskip: jax.Array,
    gate_w: jax.Array,
):
    del B_x
    _, S, M = A_x.shape
    C = A_c_kv.shape[2]
    H, D = A_w_q.shape[1], A_w_q.shape[2]
    PP = (M + LANE - 1) // LANE * LANE

    hbm = pl.BlockSpec(memory_space=pl.ANY)
    out_t = pl.pallas_call(
        functools.partial(_kernel, S=S, M=M, H=H, D=D),
        in_specs=[hbm] * 15,
        out_specs=hbm,
        out_shape=jax.ShapeDtypeStruct((M, S), F32),
        scratch_shapes=[
            pltpu.VMEM((M, S), BF16),
            pltpu.VMEM((S // 2, M), U32),
            pltpu.VMEM((7, S // 8, 7 * PP // 4), U32),
            pltpu.VMEM((S // 2, C), U32),
            pltpu.VMEM((7, S // 8, 7 * C // 4), U32),
            pltpu.VMEM((H // 2, M, D), U32),
            pltpu.VMEM((H // 2, C, D), U32),
            pltpu.VMEM((H // 2, C, D), U32),
            pltpu.VMEM((H, M // 2, D), U32),
            pltpu.VMEM((H, M // 2, 5 * D // 2), BF16),
            pltpu.VMEM((M, M), U32),
            pltpu.VMEM((M // 2, M), U32),
            pltpu.VMEM((M // 2, M), U32),
            pltpu.VMEM((S + 32, 2 * M), F32),
            pltpu.VMEM((S // TP, M, TP), F32),
            pltpu.VMEM((2, 8, PP), F32),
            pltpu.VMEM((10, 8, PP), F32),
            pltpu.VMEM((2, M, LANE), F32),
            pltpu.VMEM((3, 8, H // 2, D), U32),
            pltpu.VMEM((2, 4, H // 2, LANE), F32),
            pltpu.VMEM((H // 2, 4, S // 2, D), BF16),
            pltpu.VMEM((H, S // 2, 7 * D // 2), BF16),
            pltpu.SMEM((1,), jnp.int32),
            pltpu.SemaphoreType.DMA((5, H // 2)),
            pltpu.SemaphoreType.DMA((4,)),
            pltpu.SemaphoreType.DMA((8,)),
            pltpu.SemaphoreType.DMA((5,)),
            pltpu.SemaphoreType.DMA((3, S // TP)),
        ] + [pltpu.VMEM((M,), BF16)] * 5,
        compiler_params=pltpu.CompilerParams(
            vmem_limit_bytes=124 * 1024 * 1024,
            disable_semaphore_checks=True,
            disable_bounds_checks=True,
        ),
    )(
        jnp.swapaxes(A_x, 1, 2).reshape(M, S), A_c_kv.reshape(S, C),
        A_w_q, A_w_uk, A_w_uv, jnp.swapaxes(A_w_o, 1, 2),
        B_B_re, B_B_im, B_C_re, B_C_im,
        B_Lambda_re, B_Lambda_im, B_log_dt, B_Dskip, gate_w,
    )
    return jnp.swapaxes(out_t.reshape(1, M, S), 1, 2)
```

```python
import functools

import jax
import jax.numpy as jnp
import jax.experimental.pallas as pl
import jax.experimental.pallas.tpu as pltpu

F32 = jnp.float32
BF16 = jnp.bfloat16
U32 = jnp.uint32

NT_DIMS = (((1,), (1,)), ((), ()))
LOG2E = 1.4426950408889634

LANE = 128
HALF = LANE // 2
TQ = 128
TP = 256
TU = 512

U_SCHEDULE = "t4 u2 x1 u3 x4 x2 u4 x5 t6 u5 x3 u6 x7 v7 x6 w7"
Q_SCHEDULE = ((0, 2), (2, 1), (3, 1), (4, 1), (5, 1), (6, 1), (7, 1))
Q_ORDER = (1, 6, 0, 3, 2, 5, 4)
Q_INNER = (1, 3, 5, 0, 2, 4, 6)
Q_REMAT = (0, 2, 3, 4, 5, 6)
C_START = (14, 20, 30, 38)
WO_START = (40, 52)
C_DUE = 53
C_EXTRA = 4
SCHEDULE = ("d0 x24 t0 t1 c2 p0 p1 t2 c3 u3 b2 t3 c4 u4 p2 b3 t4 c5 p3 p4 t5 c6 b5 t6 c7 t7 "
            "p5 b6 b7 p6 p7")
KV_ORDER = (1, 3, 2, 4, 0, 5, 6)
KV_INNER = (1, 3, 6, 0, 2, 4, 5)
QK_ORDER = (0, 1, 4, 3, 2, 6, 5)
PV_ORDER = (4, 3, 1, 5, 2, 0, 6)
PV_LAST = (4, 5, 2, 1, 3, 0, 6)
PV_DIAG = (0, 1, 0, 1, 3, 3, 3, 0)
EARLY_SUM = (2, 5, 7)
LOOK = (0, 0, 0, 0, 0, 0, 4, 0)
O_SCHEDULE = "a3 a4 a0 g0 m0 m3 a6 m1 a2 a1 a5 n3 b0 m2 b3 g1 b4 n2 n0 n1 b6 b2 b1 b5"


def _cat(xs, axis):
    return jnp.concatenate(xs, axis=axis)


def _dot(a, b):
    return jnp.dot(a, b, preferred_element_type=F32)


def _dot_nt(a, b):
    return jax.lax.dot_general(a, b, NT_DIMS, preferred_element_type=F32)


def _unpack(w32, shift):
    v = (w32 << shift) & jnp.uint32(0xFFFF0000)
    return pltpu.bitcast(v, F32)


def _as_bf16(w32):
    return pltpu.bitcast(w32, BF16)


def _as_u32(v):
    return pltpu.bitcast(v, U32)


def _run(schedule, ops):
    for op in schedule.split():
        ops[op[0]](int(op[1:]))


def _strassen_lhs(a11, a12, a21, a22):
    return [a11 + a22, a21 + a22, a11, a22, a11 + a12, a21 - a11, a12 - a22]


def _strassen_rhs(b11, b12, b21, b22):
    return [b11 + b22, b11, b12 - b22, b21 - b11, b22, b11 + b12, b21 + b22]


def _strassen_out(m, order=None):
    if order is None:
        return ((m[0] + m[3]) + (m[6] - m[4]), m[2] + m[4],
                m[1] + m[3], (m[0] - m[1]) + (m[2] + m[5]))

    def fold(ks, neg):
        ks = sorted(ks, key=order.index)
        if ks[0] == neg:
            ks[:2] = ks[1::-1]
        return functools.reduce(lambda a, k: a - m[k] if k == neg else a + m[k], ks[1:], m[ks[0]])

    return fold((0, 3, 4, 6), 4), m[2] + m[4], m[1] + m[3], fold((0, 1, 2, 5), 1)


SUMS = (0, 1, 4, 5, 6)


def _quads(a):
    m, n = a.shape[0] // 2, a.shape[1] // 2
    return a[:m, :n], a[:m, n:], a[m:, :n], a[m:, n:]


def _unsplit(c, n):
    top, bot = _cat(c[:2], 1), _cat(c[2:], 1)
    rows = top.shape[0] // n
    return _cat([v[b * rows:(b + 1) * rows] for b in range(n) for v in (top, bot)], 0)


def _hold(v, last, zero):
    if not last:
        return v
    z = jnp.tile(_as_u32(last[0]) & zero.astype(U32), (v.shape[0] // 8, pl.cdiv(v.shape[1], LANE)))
    return pltpu.bitcast(_as_u32(v) | z[:, :v.shape[1]], v.dtype)


def _lhs_operands(a, last, zero, extra):
    first = (0, 2, 0, 3, 0, 2, 1)
    for k in range(7):
        q = list(_quads(a))
        q[first[k]] = _hold(q[first[k]], last, zero)
        l = _strassen_lhs(*q)[k]
        out = []
        for grp in ((0, 1, 2, 3), (4, 5, 6)):
            q = list(_quads(l))
            if out:
                for b in sorted(set(first[i] for i in grp)):
                    q[b] = _hold(q[b], last, zero)
            v = _cat([_strassen_lhs(*q)[i] for i in grp], 1)
            out.append(_as_u32(v.astype(BF16)))
            last[:] = [functools.reduce(
                jnp.bitwise_or, [out[-1][:, c:c + LANE] for c in range(0, v.shape[1], LANE)])]
            for _ in range(extra):
                last[:] = [last[0] + last[0]]
        yield _cat(out, 1)


def _kernel(xt_hbm, c_hbm, wq_hbm, wuk_hbm, wuv_hbm, wot_hbm,
            bre_hbm, bim_hbm, cre_hbm, cim_hbm,
            lre_hbm, lim_hbm, ldt_hbm, dsk_hbm, gw_hbm,
            o_hbm,
            xt_ref, x_ref, lx_ref, c_ref, l_ref, wq_buf, wk_buf, wv_buf, wot_ref, lo_ref,
            b_ref, cre_ref, cim_ref, u_ref, out_ref, st_ref, co_ref, col_ref, smp_ref, vsc_ref,
            q_ref, ctx_ref, zero_ref, wsem, xsem, msem, vsem, osem,
            lre_ref, lim_ref, ldt_ref, dsk_ref, gw_ref,
            *, S, M, H, D):
    P = M
    FT = P // LANE
    PF = FT * LANE
    PP = PF + LANE
    NP = H // 2
    CH, DH, MH, TH = c_ref.shape[1] // 2, D // 2, M // 2, TP // 2
    TI = TH // 2
    assert P - PF == HALF and PP == 4 * LANE and DH == LANE and S // TP == NP and TP == 2 * TQ

    def w_copy(k, pair):
        src, dst = ((wq_hbm, wq_buf), (wuk_hbm, wk_buf), (wuv_hbm, wv_buf))[k]
        return pltpu.make_async_copy(src.bitcast(U32).at[:, pair, :], dst.at[pair], wsem.at[k, pair])

    def wo_copy(pair):
        heads = pl.ds(2 * pair, 2)
        return pltpu.make_async_copy(wot_hbm.bitcast(U32).at[heads], wot_ref.at[heads],
                                     wsem.at[3, pair])

    def c_copy(r):
        rows = pl.ds(pl.multiple_of(r * TH, TH), TH)
        return pltpu.make_async_copy(c_hbm.bitcast(U32).at[rows], c_ref.at[rows], wsem.at[4, r])

    def x_copy(t0, n, k):
        cols = pl.ds(t0, n)
        return pltpu.make_async_copy(xt_hbm.at[:, cols], xt_ref.at[:, cols], xsem.at[k])

    x_cps = [x_copy(0, TP, 0), x_copy(TP, TP, 1), x_copy(TU, TU, 2), x_copy(2 * TU, S - 2 * TU, 3)]
    bre32, bim32 = bre_hbm.bitcast(U32), bim_hbm.bitcast(U32)
    b_cps = [
        pltpu.make_async_copy(bre32, b_ref.at[pl.ds(0, P // 2), :], msem.at[0]),
        pltpu.make_async_copy(bim32.at[pl.ds(PF // 2, HALF // 2), :],
                              b_ref.at[pl.ds(P // 2, HALF // 2), :], msem.at[1]),
        pltpu.make_async_copy(bim32.at[pl.ds(0, PF // 2), :],
                              b_ref.at[pl.ds(PP // 2, PF // 2), :], msem.at[2]),
    ]
    cre_cp = pltpu.make_async_copy(cre_hbm.bitcast(U32), cre_ref, msem.at[3])
    cim_cp = pltpu.make_async_copy(cim_hbm.bitcast(U32), cim_ref, msem.at[4])
    smp_cps = [pltpu.make_async_copy(src.bitcast(U32).at[pl.ds(0, smp_ref.shape[1])],
                                     smp_ref.at[k], msem.at[5 + k])
               for k, src in enumerate((wuk_hbm, wuv_hbm, wq_hbm))]
    v_cps = [pltpu.make_async_copy(src, dst, vsem.at[k]) for k, (src, dst) in enumerate(
        ((lre_hbm, lre_ref), (lim_hbm, lim_ref), (ldt_hbm, ldt_ref),
         (dsk_hbm, dsk_ref), (gw_hbm, gw_ref)))]

    for cp in x_cps[:1] + v_cps + b_cps + x_cps[1:] + smp_cps:
        cp.start()
    for p in range(NP):
        w_copy(0, p).start()
        wo_copy(p).start()
        c_copy(p).start()
    for p in range(NP):
        w_copy(1, p).start()
        w_copy(2, p).start()
    cre_cp.start()
    cim_cp.start()

    zero_ref[0] = 0
    u_ref[pl.ds(0, 8), :] = jnp.zeros((8, u_ref.shape[1]), F32)
    st_ref[...] = jnp.zeros(st_ref.shape, F32)
    for cp in v_cps + x_cps[:1]:
        cp.wait()

    row = lambda r: r[...].astype(F32).reshape(1, P)
    lre, lim = row(lre_ref), row(lim_ref)
    dt = jnp.exp(row(ldt_ref)).astype(BF16).astype(F32)
    e = jnp.exp(dt * lre)
    ang = dt * lim
    ar = e * jnp.cos(ang)
    ai = e * jnp.sin(ang)
    sc = jnp.maximum(jnp.abs(lre), jnp.abs(lim))
    nre, nim = lre / sc, lim / sc
    den = (nre * nre + nim * nim) * sc
    gr = 2.0 * ((ar - 1.0) * nre + ai * nim) / den
    gi = 2.0 * (ai * nre - (ar - 1.0) * nim) / den

    def put(k, full, lo, hi):
        co_ref[k] = jnp.broadcast_to(_cat([full[:, :PF], lo[:, PF:], hi[:, PF:]], 1), (8, PP))

    put(0, gr, gr, -gr)
    put(1, -gi, -gi, -gi)
    pr, pi = ar, -ai
    for j in range(1, 5):
        put(2 * j, pr, pr, pr)
        put(2 * j + 1, -pi, -pi, pi)
        pr, pi = pr * pr - pi * pi, 2.0 * pr * pi

    zpad = jnp.zeros((1, PP - P), F32)
    for k, r in enumerate((dsk_ref, gw_ref)):
        col_ref[k] = jnp.broadcast_to(_cat([row(r), zpad], 1), (LANE, PP)).T[:M]

    zero1, last1 = zero_ref[0], []

    def transpose_x(t0, n):
        x_ref[pl.ds(t0 // 2, n // 2), :] = _as_u32(xt_ref[:, pl.ds(t0, n)].T)

    def x_operands(r):
        for n in range(TI // 16):
            x = _cat([x_ref[pl.ds(r * TH + g * TI // 2 + 8 * n, 8), :] for g in range(4)], 0)
            x = _as_bf16(_hold(x, last1, zero1)).astype(F32)
            x = _cat([x, jnp.zeros((x.shape[0], PP - M), F32)], 1)
            for k, v in enumerate(_lhs_operands(x, last1, zero1, 0)):
                lx_ref[k, pl.ds(r * TI // 2 + 8 * n, 8), :] = v

    def proj_u(r, lo=0, hi=2 * P, due=False, mark=False):
        x = x_ref[pl.ds(r * TH, TH), :]
        if due:
            x = _cat([_hold(x[:8], last1, zero1), x[8:]], 0)
        u = _dot_nt(_as_bf16(x), _as_bf16(b_ref[lo // 2:hi // 2, :]))
        u_ref[pl.ds(r * TP + 8, TP), lo:hi] = u
        if mark:
            last1[:] = [functools.reduce(jnp.bitwise_or, last1 + [_as_u32(u[:8, :LANE])])]

    transpose_x(0, TP)
    b_cps[0].wait()
    b_cps[1].wait()
    proj_u(0, 0, PP)
    b_cps[2].wait()
    x_cps[1].wait()
    proj_u(0, PP)
    transpose_x(TP, TP)
    x_cps[2].wait()
    proj_u(1, 0, 6 * LANE, mark=True)
    transpose_x(TU, TU)
    x_operands(0)
    proj_u(1, 6 * LANE, due=True)
    last1.clear()
    x_cps[3].wait()
    for cp in smp_cps:
        cp.wait()

    def exponent(k, e):
        mag = jnp.sum(jnp.abs(_unpack(smp_ref[k], jnp.uint32(16 - 16 * e))), axis=0)
        mag = jnp.sum(mag, axis=1, keepdims=True)
        return jnp.broadcast_to(pltpu.bitcast(mag, jnp.int32) >> 23, (NP, LANE))

    for n, (target, scaled) in enumerate((((0, 0), (1, 0)), ((0, 1), (1, 1)), ((2, 0), (2, 1)))):
        e0, e1 = exponent(*target), exponent(*scaled)
        d = jnp.where((e0 > 0) & (e1 > 0), jnp.clip(e0 - e1, -40, 40), 0)
        vsc_ref[0, n] = pltpu.bitcast((127 + d) << 23, F32)
        vsc_ref[1, n] = pltpu.bitcast((127 - d) << 23, F32)

    _run(U_SCHEDULE, dict(t=lambda r: transpose_x(r * TP, TU), x=x_operands,
                          u=lambda r: proj_u(r, mark=True),
                          v=lambda r: proj_u(r, 0, 6 * LANE, mark=True),
                          w=lambda r: proj_u(r, 6 * LANE, due=True)))

    def q_step(j, _):
        w_copy(0, j).wait()
        wo_copy(j).wait()
        c_copy(j).wait()
        zero = zero_ref[0]
        last, recent = [], []
        wq32 = _cat([wq_buf[j], jnp.zeros((PP - M, D), U32)], 0)
        rw = []
        for k in range(7):
            z = (zero << k).astype(U32) if k in Q_REMAT else jnp.uint32(0)
            w0 = pltpu.bitcast(wq32 << (z + 16), F32)
            w1 = pltpu.bitcast(wq32 & (z + jnp.uint32(0xFFFF0000)), F32)
            r0 = _strassen_rhs(*_quads(w0))[k]
            r1 = _strassen_rhs(*_quads(w1))[k] * vsc_ref[0, 2, pl.ds(j, 1), :]
            rw.append(_strassen_rhs(r0[:LANE], r1[:LANE], r0[LANE:], r1[LANE:]))
        qscale = _cat([jnp.ones((1, DH), F32), vsc_ref[1, 2, pl.ds(j, 1), :]], 1)
        qscale = qscale * ((D ** -0.5) * LOG2E)

        def c_operands(n):
            c = _cat([c_ref[pl.ds(pl.multiple_of(j * TH + g * (TI // 2) + 8 * n, 8), 8), :]
                      for g in range(4)], 0)
            c = _as_bf16(_hold(c, last, zero)).astype(F32)
            rows = pl.ds(pl.multiple_of(j * (TI // 2) + 8 * n, 8), 8)
            for k, v in enumerate(_lhs_operands(c, last, zero, C_EXTRA)):
                l_ref[k, rows, :] = v

        def wo_operands(e):
            z = _as_u32(_cat([v[:TI] for v in recent[-7:]], 0)) & zero.astype(U32)
            w = wot_ref[2 * j + e] | _cat([z[:MH], z[MH:]], 1)
            ls = _strassen_lhs(*_quads(_as_bf16(w).astype(F32)))
            lo_ref[2 * j + e] = _cat([ls[k] for k in SUMS], 1).astype(BF16)

        for r, n in Q_SCHEDULE:
            ms = [None] * 7
            for k in Q_ORDER:
                mi = [None] * 7
                for i in Q_INNER:
                    a = lx_ref[k, pl.ds(r * TI // 2, n * TI // 2), pl.ds(i * LANE, LANE)]
                    at = 7 * r + n * Q_ORDER.index(k) if i == Q_INNER[0] else -1
                    if at == C_DUE:
                        a = _cat([_hold(a[:8], last, zero), a[8:]], 0)
                    mi[i] = _dot(_as_bf16(a), rw[k][i].astype(BF16))
                    recent.append(mi[i])
                    if at in C_START:
                        last[:] = [_as_u32(mi[i][:8]) | last[0] if last else _as_u32(mi[i][:8])]
                        c_operands(C_START.index(at))
                    if at in WO_START:
                        wo_operands(WO_START.index(at))
                ms[k] = _unsplit(_strassen_out(mi), n)
            for k, v in enumerate(_strassen_out(ms)):
                q_ref[j, k, pl.ds(r * TH, n * TH), :] = (v * qscale).astype(BF16)
        return 0

    jax.lax.fori_loop(0, NP, q_step, 0)
    for p in range(NP):
        w_copy(1, p).wait()
        w_copy(2, p).wait()
    cre_cp.wait()
    cim_cp.wait()

    def head_step(h, _):
        pair = h >> 1
        zero = zero_ref[0]
        shift = (16 - 16 * (h & 1)).astype(U32)
        vscale, vinv = [vsc_ref[k, h & 1, pl.ds(pair, 1), :] for k in range(2)]
        rw = []
        for k in range(7):
            sh = shift + (zero << k).astype(U32) if k != 1 else shift
            rk = _strassen_rhs(*_quads(_unpack(wk_buf[pair], sh)))[k]
            rv = _strassen_rhs(*_quads(_unpack(wv_buf[pair], sh)))[k] * vscale
            rw.append(_strassen_rhs(rk[:CH // 2], rv[:CH // 2], rk[CH // 2:], rv[CH // 2:]))
        causal = (jax.lax.broadcasted_iota(jnp.int32, (TQ, TQ), 1)
                  <= jax.lax.broadcasted_iota(jnp.int32, (TQ, TQ), 0))
        ks, rks, vs, rvs, ss, mxs = [], [], [], [], {}, {}

        def tie(a, b):
            return pltpu.bitcast(_as_u32(a) | (_as_u32(b) & zero.astype(U32)), F32)

        def proj_kv(r, n):
            ms = [None] * 7
            for k in KV_ORDER:
                mi = [None] * 7
                for i in KV_INNER:
                    a = l_ref[k, pl.ds(r * TI // 2, n * TI // 2), pl.ds(i * CH // 2, CH // 2)]
                    mi[i] = _dot(_as_bf16(a), rw[k][i].astype(BF16))
                ms[k] = _unsplit(_strassen_out(mi, KV_INNER if n == 1 else None), n)
                if k != KV_ORDER[-1]:
                    yield
            c = _strassen_out(ms, KV_ORDER if n == 1 else None)
            for b in range(n):
                c11, c12, c21, c22 = [v[b * TH:(b + 1) * TH, :DH] for v in c]
                ks.extend([_cat([c11, c12], 1), _cat([c21, c22], 1)])
                rks.append(_strassen_rhs(c11, c21, c12, c22))
                c11, c12, c21, c22 = [v[b * TH:(b + 1) * TH, DH:] for v in c]
                vs.extend([_cat([c11, c12], 1), _cat([c21, c22], 1)])
                rvs.append(_strassen_rhs(c11, c12, c21, c22))

        def scores(j):
            cols = pl.ds(pl.multiple_of((h & 1) * DH, DH), DH)
            qf = [q_ref[pair, k, j * TQ:(j + 1) * TQ, cols].astype(F32) for k in range(4)]
            q = _cat([_cat(qf[:2], 1), _cat(qf[2:], 1)], 0)
            lq = _strassen_lhs(*qf)
            s1, s2, done, mx = [], [], [], []
            for t in range(j):
                m = [None] * 7
                for k in QK_ORDER:
                    a = tie(lq[k], done[-2]) if k == 3 and t >= 2 else lq[k]
                    m[k] = _dot_nt(a.astype(BF16), rks[t][k].astype(BF16))
                c11, c12, c21, c22 = _strassen_out(m, tuple(range(7)))
                x1, x2 = jnp.maximum(c11, c12), jnp.maximum(c21, c22)
                if mx:
                    x1, x2 = jnp.maximum(x1, mx[0]), jnp.maximum(x2, mx[1])
                mx[:] = [x1, x2]
                done.append(_as_u32(x1) | _as_u32(x2))
                s1 += [c11, c12]
                s2 += [c21, c22]
            yield
            d = _dot_nt(q.astype(BF16), ks[2 * j].astype(BF16))
            ss[2 * j] = _cat(s1 + [d[:TQ]], 1)
            ss[2 * j + 1] = _cat(
                s2 + [d[TQ:], _dot_nt(q[TQ:].astype(BF16), ks[2 * j + 1].astype(BF16))], 1)
            if mx:
                mxs[2 * j], mxs[2 * j + 1] = mx

        def masked(i):
            lo = i * TQ
            s = ss.pop(i)
            sd = jnp.where(causal, s[:, lo:], -1e9 * LOG2E)
            s = sd if i == 0 else _cat([s[:, :lo], sd], 1)
            t = _cat([mxs[i], s[:, i // 2 * TP:]], 1) if i in mxs else s
            if LOOK[i // 2]:
                return s, functools.reduce(
                    jnp.maximum, [t[:, c:c + LANE] for c in range(0, t.shape[1], LANE)])
            return s, jnp.broadcast_to(jnp.max(t, axis=-1, keepdims=True), (TQ, LANE))

        def exp_rows(s, m, parts, look):
            ps = []
            for g in range(0, TQ, 8):
                mg = m[g:g + 8]
                if look:
                    if len(parts) >= look:
                        mg = tie(mg, parts[-look])
                    mg = jnp.broadcast_to(jnp.max(mg, axis=-1, keepdims=True), (8, LANE))
                if parts:
                    mg = tie(mg, parts[-1])
                pg = [jnp.exp2(s[g:g + 8, t * LANE:(t + 1) * LANE] - mg)
                      for t in range(s.shape[1] // LANE)]
                ps.append(_cat(pg, 1))
                parts.append(functools.reduce(lambda a, b: a + b, pg))
            return _cat(ps, 0), _cat(parts[-(TQ // 8):], 0)

        def context(j):
            (s1, m1), (s2, m2) = masked(2 * j), masked(2 * j + 1)
            parts = []
            p1, l1 = exp_rows(s1, m1, parts, LOOK[j])
            if j in EARLY_SUM:
                m2 = tie(m2, jnp.broadcast_to(jnp.sum(l1, axis=-1, keepdims=True), (TQ, LANE)))
            p2, l2 = exp_rows(s2, m2, parts, LOOK[j])
            l1 = _cat([tie(l1[:8], l1[TQ - 8:]), l1[8:]], 0)
            l1, l2 = [jnp.sum(l, axis=-1, keepdims=True) for l in (l1, l2)]
            lo = j * TP
            dot = lambda a, b: _dot(a.astype(BF16), b.astype(BF16))

            def recip(l):
                rl = pl.reciprocal(l, approx=True)
                return rl * (2.0 - l * rl)

            def diag():
                dg = dot(_cat([p1[:, lo:], p2[:, lo:lo + TQ]], 0), vs[2 * j])
                return dg[:TQ], dg[TQ:] + dot(p2[:, lo + TQ:], vs[2 * j + 1])

            r1, r2 = recip(l1), recip(l2)
            rho = l1 * r2
            r1, r2 = r1 * vinv, r2 * vinv
            if j == 0:
                c1, c2 = diag()
                c2 = c2 * _cat([r2, r2], 1)
            else:
                tiles = lambda p, o: _cat(
                    [p[:, (2 * t + o) * TQ:(2 * t + o + 1) * TQ] for t in range(j)], 1)
                a11, a12, a21, a22 = tiles(p1, 0), tiles(p1, 1), tiles(p2, 0), tiles(p2, 1)
                a22r = a22 * rho
                lp = [a11 + a22r, a21 + a22, a11, a22, a11 + a12, a21 * rho - a11, a12 - a22r]
                m = [None] * 7
                for n, k in enumerate(PV_ORDER if j < NP - 1 else PV_LAST):
                    if n == PV_DIAG[j]:
                        c1, c2 = diag()
                    if n == 6:
                        yield
                    m[k] = dot(lp[k], _cat([rvs[t][k] for t in range(j)], 0))
                c1 = c1 + _cat([(m[0] - m[4]) + (m[6] + m[3] * rho), m[2] + m[4]], 1)
                c2 = (c2 + _cat([m[1] + m[3], -m[1]], 1)) * _cat([r2, r2], 1)
                c2 = _cat([c2[:, :DH], c2[:, DH:] + ((m[0] + m[2]) + m[5]) * r1], 1)
            c1 = c1 * _cat([r1, r1], 1)
            ctx_ref[h, j * TQ:(j + 1) * TQ, :] = _cat(
                _strassen_rhs(c1[:, :DH], c2[:, :DH], c1[:, DH:], c2[:, DH:]), 1).astype(BF16)

        kvs = [proj_kv(r, 1) for r in range(NP)]
        qks = [scores(j) for j in range(NP)]
        pvs = [context(j) for j in range(NP)]
        _run(SCHEDULE, dict(d=lambda r: list(proj_kv(r, 2)), c=lambda r: list(kvs[r]),
                            x=lambda r: [next(kvs[r // 10]) for _ in range(r % 10)],
                            u=lambda j: next(qks[j]), t=lambda j: list(qks[j]),
                            b=lambda j: next(pvs[j]), p=lambda j: list(pvs[j])))
        return 0

    jax.lax.fori_loop(0, H, head_step, 0)

    pieces = ((0, 0, TP), (MH, 0, TQ), (MH, TQ, TQ))

    def o_copy(j, n):
        r0, c0, nc = pieces[n]
        return pltpu.make_async_copy(
            out_ref.at[j, pl.ds(r0, MH), pl.ds(c0, nc)],
            o_hbm.at[pl.ds(r0, MH), pl.ds(pl.multiple_of(j * TP + c0, TQ), nc)], osem.at[n, j])

    def o_step(jj, _):
        zero = zero_ref[0]
        js = (2 * jj, 2 * jj + 1)
        t0 = [pl.multiple_of(j * TP, TP) for j in js]
        last, state, ys, gates, m, recent = [], {}, [None, None], {}, [{}, {}], []
        rnd = lambda v: v.astype(BF16).astype(F32)

        def ssm_tile(u, t):
            rows = pl.ds(t0[u], TP + 8)
            cr, ci = pl.ds(t * LANE, LANE), pl.ds(PP + t * LANE, LANE)
            co = [co_ref[k, :, cr] for k in range(10)]
            u0 = u_ref[rows, cr]
            u1 = u_ref[rows, ci] if t < FT else pltpu.roll(u0, HALF, 1)
            mul = lambda k, x: (co[k] * x[0] + co[k + 1] * x[1], co[k] * x[1] - co[k + 1] * x[0])
            sub = jax.lax.broadcasted_iota(jnp.int32, (8, LANE), 0)
            s = state[t] if u else (st_ref[0, :, cr], st_ref[1, :, cr])
            prev, gs = [None] * 3, []
            for k in range(TP // 8 + 1):
                x0, x1 = _hold(u0[8 * k:8 * k + 8], last, zero), u1[8 * k:8 * k + 8]
                w = (co[0] * x0 + co[1] * x1, co[1] * x0 - co[0] * x1)
                for i in range(3):
                    cur = [pltpu.roll(v, 1 << i, 0) for v in w]
                    old = cur if k == 0 else prev[i]
                    d = mul(2 * i + 2, [jnp.where(sub < (1 << i), o, c) for o, c in zip(old, cur)])
                    w = [p + q for p, q in zip(d, w)]
                    prev[i] = cur
                if k > 0:
                    s = [p + q for p, q in zip(mul(8, s), w)]
                    gs.append(_cat(s, 1) if t < FT else s[0])
                    last[:] = [s[0]]
            state[t] = s
            if u:
                st_ref[0, :, cr] = s[0]
                st_ref[1, :, cr] = s[1]
            cols = cr if t < FT else pl.ds(PF, HALF)
            cc = _cat([cre_ref[:, cols], cim_ref[:, cols]], 1)
            g = _cat(gs, 0).astype(BF16)
            n = MH if t < FT else MH // 2
            y = _cat([_dot_nt(_as_bf16(cc[a:a + n]), g) for a in range(0, MH, n)], 0)
            ys[u] = y if ys[u] is None else y + ys[u]

        def gate(u):
            gcol = _as_u32(col_ref[1]) | (_as_u32(_cat(recent[-2:], 0)) & zero.astype(U32))
            gcol = _cat([pltpu.bitcast(gcol, F32)] * (TP // LANE), 1)
            xt = xt_ref[:, pl.ds(t0[u], TP)].astype(F32)
            z = jnp.sum(rnd(xt * gcol), axis=0, keepdims=True)
            gates[u] = rnd(1.0 / rnd(1.0 + rnd(jnp.exp(-rnd(z)))))

        def product(u, k):
            if k in SUMS:
                a = [lo_ref[n, :, pl.ds(SUMS.index(k) * DH, DH)] for n in range(H)]
            else:
                o = k - 2
                a = [_as_bf16(wot_ref[n, pl.ds(o * MH // 2, MH // 2), pl.ds(o * DH, DH)])
                     for n in range(H)]
            rows = pl.ds(pl.multiple_of(js[u] * TQ, TQ), TQ)
            b = [ctx_ref[n, rows, pl.ds(k * DH, DH)] for n in range(H)]
            m[u][k] = _dot_nt(_cat(a, 1), _cat(b, 1))
            recent.append(m[u][k])

        def emit(u, n, v):
            r0, c0, nc = pieces[n]
            g = gates[u][:, c0:c0 + nc]
            dcol = _cat([col_ref[0, r0:r0 + MH]] * (nc // LANE), 1)
            xt = xt_ref[pl.ds(r0, MH), pl.ds(pl.multiple_of(t0[u] + c0, TQ), nc)].astype(F32)
            b = ys[u][r0:r0 + MH, c0:c0 + nc] + rnd(xt * dcol)
            out_ref[js[u], pl.ds(r0, MH), pl.ds(c0, nc)] = g * v + rnd(1.0 - g) * b
            o_copy(js[u], n).start()

        _run(O_SCHEDULE, dict(a=lambda k: product(0, k), b=lambda k: product(1, k), g=gate,
                              m=lambda t: ssm_tile(0, t), n=lambda t: ssm_tile(1, t)))
        for u, p in enumerate(m):
            emit(u, 0, _cat([(p[0] + p[3]) + (p[6] - p[4]), p[2] + p[4]], 1))
            emit(u, 1, p[1] + p[3])
            emit(u, 2, ((p[0] + p[2]) - p[1]) + p[5])
        return 0

    jax.lax.fori_loop(0, NP // 2, o_step, 0)
    for j in range(NP):
        for n in range(3):
            o_copy(j, n).wait()


@jax.jit
def pallas_gated_mix__compressed_kv_cla__ssm_conv_s5__prompt_kernel(
    A_x: jax.Array,
    A_c_kv: jax.Array,
    A_w_q: jax.Array,
    A_w_uk: jax.Array,
    A_w_uv: jax.Array,
    A_w_o: jax.Array,
    B_x: jax.Array,
    B_Lambda_re: jax.Array,
    B_Lambda_im: jax.Array,
    B_B_re: jax.Array,
    B_B_im: jax.Array,
    B_C_re: jax.Array,
    B_C_im: jax.Array,
    B_log_dt: jax.Array,
    B_Dskip: jax.Array,
    gate_w: jax.Array,
):
    del B_x
    _, S, M = A_x.shape
    C = A_c_kv.shape[2]
    H, D = A_w_q.shape[1], A_w_q.shape[2]
    PP = (M + LANE - 1) // LANE * LANE

    hbm = pl.BlockSpec(memory_space=pl.ANY)
    out_t = pl.pallas_call(
        functools.partial(_kernel, S=S, M=M, H=H, D=D),
        in_specs=[hbm] * 15,
        out_specs=hbm,
        out_shape=jax.ShapeDtypeStruct((M, S), F32),
        scratch_shapes=[
            pltpu.VMEM((M, S), BF16),
            pltpu.VMEM((S // 2, M), U32),
            pltpu.VMEM((7, S // 8, 7 * PP // 4), U32),
            pltpu.VMEM((S // 2, C), U32),
            pltpu.VMEM((7, S // 8, 7 * C // 4), U32),
            pltpu.VMEM((H // 2, M, D), U32),
            pltpu.VMEM((H // 2, C, D), U32),
            pltpu.VMEM((H // 2, C, D), U32),
            pltpu.VMEM((H, M // 2, D), U32),
            pltpu.VMEM((H, M // 2, 5 * D // 2), BF16),
            pltpu.VMEM((M, M), U32),
            pltpu.VMEM((M // 2, M), U32),
            pltpu.VMEM((M // 2, M), U32),
            pltpu.VMEM((S + 32, 2 * M), F32),
            pltpu.VMEM((S // TP, M, TP), F32),
            pltpu.VMEM((2, 8, PP), F32),
            pltpu.VMEM((10, 8, PP), F32),
            pltpu.VMEM((2, M, LANE), F32),
            pltpu.VMEM((3, 8, H // 2, D), U32),
            pltpu.VMEM((2, 4, H // 2, LANE), F32),
            pltpu.VMEM((H // 2, 4, S // 2, D), BF16),
            pltpu.VMEM((H, S // 2, 7 * D // 2), BF16),
            pltpu.SMEM((1,), jnp.int32),
            pltpu.SemaphoreType.DMA((5, H // 2)),
            pltpu.SemaphoreType.DMA((4,)),
            pltpu.SemaphoreType.DMA((8,)),
            pltpu.SemaphoreType.DMA((5,)),
            pltpu.SemaphoreType.DMA((3, S // TP)),
        ] + [pltpu.VMEM((M,), BF16)] * 5,
        compiler_params=pltpu.CompilerParams(
            vmem_limit_bytes=124 * 1024 * 1024,
            disable_semaphore_checks=True,
            disable_bounds_checks=True,
        ),
    )(
        jnp.swapaxes(A_x, 1, 2).reshape(M, S), A_c_kv.reshape(S, C),
        A_w_q, A_w_uk, A_w_uv, jnp.swapaxes(A_w_o, 1, 2),
        B_B_re, B_B_im, B_C_re, B_C_im,
        B_Lambda_re, B_Lambda_im, B_log_dt, B_Dskip, gate_w,
    )
    return jnp.swapaxes(out_t.reshape(1, M, S), 1, 2)
```

```python
import functools

import jax
import jax.numpy as jnp
import jax.experimental.pallas as pl
import jax.experimental.pallas.tpu as pltpu

F32 = jnp.float32
BF16 = jnp.bfloat16
U32 = jnp.uint32

NT_DIMS = (((1,), (1,)), ((), ()))
LOG2E = 1.4426950408889634

LANE = 128
HALF = LANE // 2
TQ = 128
TP = 256
TU = 512

U_SCHEDULE = "t4 u2 x1 u3 x4 x2 u4 x5 t6 u5 x3 u6 x7 v7 x6 w7"
Q_SCHEDULE = ((0, 2), (2, 1), (3, 1), (4, 1), (5, 1), (6, 1), (7, 1))
Q_ORDER = (1, 6, 0, 3, 2, 5, 4)
Q_INNER = (1, 3, 5, 0, 2, 4, 6)
Q_REMAT = (0, 2, 3, 4, 5, 6)
C_START = (14, 20, 30, 38)
WO_START = (40, 52)
C_DUE = 53
C_EXTRA = 4
SCHEDULE = ("d0 x24 t0 t1 c2 p0 p1 t2 c3 u3 x41 b2 t3 c4 p2 b3 t4 c5 u5 p3 p4 t5 c6 u6 b5 t6 c7 t7 "
            "p5 b6 b7 p6 p7")
KV_REMAT = (0, 2, 3, 5, 6)
KV_ORDER = {1: (1, 6, 5, 4, 2, 0, 3), 2: (1, 3, 2, 6, 0, 5, 4)}
KV_INNER = {1: (1, 3, 2, 0, 4, 6, 5), 2: (1, 3, 6, 0, 2, 4, 5)}
QK_ORDER = (0, 1, 2, 3, 4, 6, 5)
PV_ORDER = (1, 3, 4, 5, 2, 0, 6)
PV_LAST = (4, 3, 2, 0, 5, 6, 1)
PV_DIAG = (0, 3, 4, 5, 6, 4, 5, 5)
PV_SPLIT = (6, 6, 5, 6, 6, 4, 6, 5)
EARLY_SUM = (2, 4, 5)
LOOK = (0, 0, 0, 0, 0, 0, 4, 4)
O_SCHEDULE = "a3 a4 a0 g0 m0 m3 a6 m1 a2 a1 a5 n3 b0 m2 b3 g1 b4 n2 n0 n1 b6 b2 b1 b5"


def _cat(xs, axis):
    return jnp.concatenate(xs, axis=axis)


def _dot(a, b):
    return jnp.dot(a, b, preferred_element_type=F32)


def _dot_nt(a, b):
    return jax.lax.dot_general(a, b, NT_DIMS, preferred_element_type=F32)


def _unpack(w32, shift):
    v = (w32 << shift) & jnp.uint32(0xFFFF0000)
    return pltpu.bitcast(v, F32)


def _as_bf16(w32):
    return pltpu.bitcast(w32, BF16)


def _as_u32(v):
    return pltpu.bitcast(v, U32)


def _run(schedule, ops):
    for op in schedule.split():
        ops[op[0]](int(op[1:]))


def _strassen_lhs(a11, a12, a21, a22):
    return [a11 + a22, a21 + a22, a11, a22, a11 + a12, a21 - a11, a12 - a22]


def _strassen_rhs(b11, b12, b21, b22):
    return [b11 + b22, b11, b12 - b22, b21 - b11, b22, b11 + b12, b21 + b22]


def _strassen_out(m, order=None):
    if order is None:
        return ((m[0] + m[3]) + (m[6] - m[4]), m[2] + m[4],
                m[1] + m[3], (m[0] - m[1]) + (m[2] + m[5]))

    def fold(ks, neg):
        ks = sorted(ks, key=order.index)
        if ks[0] == neg:
            ks[:2] = ks[1::-1]
        return functools.reduce(lambda a, k: a - m[k] if k == neg else a + m[k], ks[1:], m[ks[0]])

    return fold((0, 3, 4, 6), 4), m[2] + m[4], m[1] + m[3], fold((0, 1, 2, 5), 1)


SUMS = (0, 1, 4, 5, 6)


def _quads(a):
    m, n = a.shape[0] // 2, a.shape[1] // 2
    return a[:m, :n], a[:m, n:], a[m:, :n], a[m:, n:]


def _unsplit(c, n):
    top, bot = _cat(c[:2], 1), _cat(c[2:], 1)
    rows = top.shape[0] // n
    return _cat([v[b * rows:(b + 1) * rows] for b in range(n) for v in (top, bot)], 0)


def _hold(v, last, zero):
    if not last:
        return v
    z = jnp.tile(_as_u32(last[0]) & zero.astype(U32), (v.shape[0] // 8, pl.cdiv(v.shape[1], LANE)))
    return pltpu.bitcast(_as_u32(v) | z[:, :v.shape[1]], v.dtype)


def _lhs_operands(a, last, zero, extra):
    first = (0, 2, 0, 3, 0, 2, 1)
    for k in range(7):
        q = list(_quads(a))
        q[first[k]] = _hold(q[first[k]], last, zero)
        l = _strassen_lhs(*q)[k]
        out = []
        for grp in ((0, 1, 2, 3), (4, 5, 6)):
            q = list(_quads(l))
            if out:
                for b in sorted(set(first[i] for i in grp)):
                    q[b] = _hold(q[b], last, zero)
            v = _cat([_strassen_lhs(*q)[i] for i in grp], 1)
            out.append(_as_u32(v.astype(BF16)))
            last[:] = [functools.reduce(
                jnp.bitwise_or, [out[-1][:, c:c + LANE] for c in range(0, v.shape[1], LANE)])]
            for _ in range(extra):
                last[:] = [last[0] + last[0]]
        yield _cat(out, 1)


def _kernel(xt_hbm, c_hbm, wq_hbm, wuk_hbm, wuv_hbm, wot_hbm,
            bre_hbm, bim_hbm, cre_hbm, cim_hbm,
            lre_hbm, lim_hbm, ldt_hbm, dsk_hbm, gw_hbm,
            o_hbm,
            xt_ref, x_ref, lx_ref, c_ref, l_ref, wq_buf, wk_buf, wv_buf, wot_ref, lo_ref,
            b_ref, cre_ref, cim_ref, u_ref, out_ref, st_ref, co_ref, col_ref, smp_ref, vsc_ref,
            q_ref, ctx_ref, zero_ref, wsem, xsem, msem, vsem, osem,
            lre_ref, lim_ref, ldt_ref, dsk_ref, gw_ref,
            *, S, M, H, D):
    P = M
    FT = P // LANE
    PF = FT * LANE
    PP = PF + LANE
    NP = H // 2
    CH, DH, MH, TH = c_ref.shape[1] // 2, D // 2, M // 2, TP // 2
    TI = TH // 2
    assert P - PF == HALF and PP == 4 * LANE and DH == LANE and S // TP == NP and TP == 2 * TQ

    def w_copy(k, pair):
        src, dst = ((wq_hbm, wq_buf), (wuk_hbm, wk_buf), (wuv_hbm, wv_buf))[k]
        return pltpu.make_async_copy(src.bitcast(U32).at[:, pair, :], dst.at[pair], wsem.at[k, pair])

    def wo_copy(pair):
        heads = pl.ds(2 * pair, 2)
        return pltpu.make_async_copy(wot_hbm.bitcast(U32).at[heads], wot_ref.at[heads],
                                     wsem.at[3, pair])

    def c_copy(r):
        rows = pl.ds(pl.multiple_of(r * TH, TH), TH)
        return pltpu.make_async_copy(c_hbm.bitcast(U32).at[rows], c_ref.at[rows], wsem.at[4, r])

    def x_copy(t0, n, k):
        cols = pl.ds(t0, n)
        return pltpu.make_async_copy(xt_hbm.at[:, cols], xt_ref.at[:, cols], xsem.at[k])

    x_cps = [x_copy(0, TP, 0), x_copy(TP, TP, 1), x_copy(TU, TU, 2), x_copy(2 * TU, S - 2 * TU, 3)]
    bre32, bim32 = bre_hbm.bitcast(U32), bim_hbm.bitcast(U32)
    b_cps = [
        pltpu.make_async_copy(bre32, b_ref.at[pl.ds(0, P // 2), :], msem.at[0]),
        pltpu.make_async_copy(bim32.at[pl.ds(PF // 2, HALF // 2), :],
                              b_ref.at[pl.ds(P // 2, HALF // 2), :], msem.at[1]),
        pltpu.make_async_copy(bim32.at[pl.ds(0, PF // 2), :],
                              b_ref.at[pl.ds(PP // 2, PF // 2), :], msem.at[2]),
    ]
    cre_cp = pltpu.make_async_copy(cre_hbm.bitcast(U32), cre_ref, msem.at[3])
    cim_cp = pltpu.make_async_copy(cim_hbm.bitcast(U32), cim_ref, msem.at[4])
    smp_cps = [pltpu.make_async_copy(src.bitcast(U32).at[pl.ds(0, smp_ref.shape[1])],
                                     smp_ref.at[k], msem.at[5 + k])
               for k, src in enumerate((wuk_hbm, wuv_hbm, wq_hbm))]
    v_cps = [pltpu.make_async_copy(src, dst, vsem.at[k]) for k, (src, dst) in enumerate(
        ((lre_hbm, lre_ref), (lim_hbm, lim_ref), (ldt_hbm, ldt_ref),
         (dsk_hbm, dsk_ref), (gw_hbm, gw_ref)))]

    for cp in x_cps[:1] + v_cps + b_cps + x_cps[1:] + smp_cps:
        cp.start()
    for p in range(NP):
        w_copy(0, p).start()
        wo_copy(p).start()
        c_copy(p).start()
    for p in range(NP):
        w_copy(1, p).start()
        w_copy(2, p).start()
    cre_cp.start()
    cim_cp.start()

    zero_ref[0] = 0
    u_ref[pl.ds(0, 8), :] = jnp.zeros((8, u_ref.shape[1]), F32)
    st_ref[...] = jnp.zeros(st_ref.shape, F32)
    for cp in v_cps + x_cps[:1]:
        cp.wait()

    row = lambda r: r[...].astype(F32).reshape(1, P)
    lre, lim = row(lre_ref), row(lim_ref)
    dt = jnp.exp(row(ldt_ref)).astype(BF16).astype(F32)
    e = jnp.exp(dt * lre)
    ang = dt * lim
    ar = e * jnp.cos(ang)
    ai = e * jnp.sin(ang)
    sc = jnp.maximum(jnp.abs(lre), jnp.abs(lim))
    nre, nim = lre / sc, lim / sc
    den = (nre * nre + nim * nim) * sc
    gr = 2.0 * ((ar - 1.0) * nre + ai * nim) / den
    gi = 2.0 * (ai * nre - (ar - 1.0) * nim) / den

    def put(k, full, lo, hi):
        co_ref[k] = jnp.broadcast_to(_cat([full[:, :PF], lo[:, PF:], hi[:, PF:]], 1), (8, PP))

    put(0, gr, gr, -gr)
    put(1, -gi, -gi, -gi)
    pr, pi = ar, -ai
    for j in range(1, 5):
        put(2 * j, pr, pr, pr)
        put(2 * j + 1, -pi, -pi, pi)
        pr, pi = pr * pr - pi * pi, 2.0 * pr * pi

    zpad = jnp.zeros((1, PP - P), F32)
    for k, r in enumerate((dsk_ref, gw_ref)):
        col_ref[k] = jnp.broadcast_to(_cat([row(r), zpad], 1), (LANE, PP)).T[:M]

    zero1, last1 = zero_ref[0], []

    def transpose_x(t0, n):
        x_ref[pl.ds(t0 // 2, n // 2), :] = _as_u32(xt_ref[:, pl.ds(t0, n)].T)

    def x_operands(r):
        for n in range(TI // 16):
            x = _cat([x_ref[pl.ds(r * TH + g * TI // 2 + 8 * n, 8), :] for g in range(4)], 0)
            x = _as_bf16(_hold(x, last1, zero1)).astype(F32)
            x = _cat([x, jnp.zeros((x.shape[0], PP - M), F32)], 1)
            for k, v in enumerate(_lhs_operands(x, last1, zero1, 0)):
                lx_ref[k, pl.ds(r * TI // 2 + 8 * n, 8), :] = v

    def proj_u(r, lo=0, hi=2 * P, due=False, mark=False):
        x = x_ref[pl.ds(r * TH, TH), :]
        if due:
            x = _cat([_hold(x[:8], last1, zero1), x[8:]], 0)
        u = _dot_nt(_as_bf16(x), _as_bf16(b_ref[lo // 2:hi // 2, :]))
        u_ref[pl.ds(r * TP + 8, TP), lo:hi] = u
        if mark:
            last1[:] = [functools.reduce(jnp.bitwise_or, last1 + [_as_u32(u[:8, :LANE])])]

    transpose_x(0, TP)
    b_cps[0].wait()
    b_cps[1].wait()
    proj_u(0, 0, PP)
    b_cps[2].wait()
    x_cps[1].wait()
    proj_u(0, PP)
    transpose_x(TP, TP)
    x_cps[2].wait()
    proj_u(1, 0, 6 * LANE, mark=True)
    transpose_x(TU, TU)
    x_operands(0)
    proj_u(1, 6 * LANE, due=True)
    last1.clear()
    x_cps[3].wait()
    for cp in smp_cps:
        cp.wait()

    def exponent(k, e):
        mag = jnp.sum(jnp.abs(_unpack(smp_ref[k], jnp.uint32(16 - 16 * e))), axis=0)
        mag = jnp.sum(mag, axis=1, keepdims=True)
        return jnp.broadcast_to(pltpu.bitcast(mag, jnp.int32) >> 23, (NP, LANE))

    for n, (target, scaled) in enumerate((((0, 0), (1, 0)), ((0, 1), (1, 1)), ((2, 0), (2, 1)))):
        e0, e1 = exponent(*target), exponent(*scaled)
        d = jnp.where((e0 > 0) & (e1 > 0), jnp.clip(e0 - e1, -40, 40), 0)
        vsc_ref[0, n] = pltpu.bitcast((127 + d) << 23, F32)
        vsc_ref[1, n] = pltpu.bitcast((127 - d) << 23, F32)

    _run(U_SCHEDULE, dict(t=lambda r: transpose_x(r * TP, TU), x=x_operands,
                          u=lambda r: proj_u(r, mark=True),
                          v=lambda r: proj_u(r, 0, 6 * LANE, mark=True),
                          w=lambda r: proj_u(r, 6 * LANE, due=True)))

    def q_step(j, _):
        w_copy(0, j).wait()
        wo_copy(j).wait()
        c_copy(j).wait()
        zero = zero_ref[0]
        last, recent = [], []
        wq32 = _cat([wq_buf[j], jnp.zeros((PP - M, D), U32)], 0)
        rw = []
        for k in range(7):
            z = (zero << k).astype(U32) if k in Q_REMAT else jnp.uint32(0)
            w0 = pltpu.bitcast(wq32 << (z + 16), F32)
            w1 = pltpu.bitcast(wq32 & (z + jnp.uint32(0xFFFF0000)), F32)
            r0 = _strassen_rhs(*_quads(w0))[k]
            r1 = _strassen_rhs(*_quads(w1))[k] * vsc_ref[0, 2, pl.ds(j, 1), :]
            rw.append(_strassen_rhs(r0[:LANE], r1[:LANE], r0[LANE:], r1[LANE:]))
        qscale = _cat([jnp.ones((1, DH), F32), vsc_ref[1, 2, pl.ds(j, 1), :]], 1)
        qscale = qscale * ((D ** -0.5) * LOG2E)

        def c_operands(n):
            c = _cat([c_ref[pl.ds(pl.multiple_of(j * TH + g * (TI // 2) + 8 * n, 8), 8), :]
                      for g in range(4)], 0)
            c = _as_bf16(_hold(c, last, zero)).astype(F32)
            rows = pl.ds(pl.multiple_of(j * (TI // 2) + 8 * n, 8), 8)
            for k, v in enumerate(_lhs_operands(c, last, zero, C_EXTRA)):
                l_ref[k, rows, :] = v

        def wo_operands(e):
            z = _as_u32(_cat([v[:TI] for v in recent[-7:]], 0)) & zero.astype(U32)
            w = wot_ref[2 * j + e] | _cat([z[:MH], z[MH:]], 1)
            ls = _strassen_lhs(*_quads(_as_bf16(w).astype(F32)))
            lo_ref[2 * j + e] = _cat([ls[k] for k in SUMS], 1).astype(BF16)

        for r, n in Q_SCHEDULE:
            ms = [None] * 7
            for k in Q_ORDER:
                mi = [None] * 7
                for i in Q_INNER:
                    a = lx_ref[k, pl.ds(r * TI // 2, n * TI // 2), pl.ds(i * LANE, LANE)]
                    at = 7 * r + n * Q_ORDER.index(k) if i == Q_INNER[0] else -1
                    if at == C_DUE:
                        a = _cat([_hold(a[:8], last, zero), a[8:]], 0)
                    mi[i] = _dot(_as_bf16(a), rw[k][i].astype(BF16))
                    recent.append(mi[i])
                    if at in C_START:
                        last[:] = [_as_u32(mi[i][:8]) | last[0] if last else _as_u32(mi[i][:8])]
                        c_operands(C_START.index(at))
                    if at in WO_START:
                        wo_operands(WO_START.index(at))
                ms[k] = _unsplit(_strassen_out(mi), n)
            for k, v in enumerate(_strassen_out(ms)):
                q_ref[j, k, pl.ds(r * TH, n * TH), :] = (v * qscale).astype(BF16)
        return 0

    jax.lax.fori_loop(0, NP, q_step, 0)
    for p in range(NP):
        w_copy(1, p).wait()
        w_copy(2, p).wait()
    cre_cp.wait()
    cim_cp.wait()

    def head_step(h, _):
        pair = h >> 1
        zero = zero_ref[0]
        shift = (16 - 16 * (h & 1)).astype(U32)
        vscale, vinv = [vsc_ref[k, h & 1, pl.ds(pair, 1), :] for k in range(2)]
        rw = []
        for k in range(7):
            sh = shift + (zero << k).astype(U32) if k in KV_REMAT else shift
            rk = _strassen_rhs(*_quads(_unpack(wk_buf[pair], sh)))[k]
            rv = _strassen_rhs(*_quads(_unpack(wv_buf[pair], sh)))[k] * vscale
            rw.append(_strassen_rhs(rk[:CH // 2], rv[:CH // 2], rk[CH // 2:], rv[CH // 2:]))
        causal = (jax.lax.broadcasted_iota(jnp.int32, (TQ, TQ), 1)
                  <= jax.lax.broadcasted_iota(jnp.int32, (TQ, TQ), 0))
        ks, rks, vs, rvs, ss, mxs = [], [], [], [], {}, {}

        def tie(a, b):
            return pltpu.bitcast(_as_u32(a) | (_as_u32(b) & zero.astype(U32)), F32)

        def proj_kv(r, n):
            ms = [None] * 7
            order, inner = KV_ORDER[n], KV_INNER[n]
            for k in order:
                mi = [None] * 7
                for i in inner:
                    a = l_ref[k, pl.ds(r * TI // 2, n * TI // 2), pl.ds(i * CH // 2, CH // 2)]
                    mi[i] = _dot(_as_bf16(a), rw[k][i].astype(BF16))
                ms[k] = _unsplit(_strassen_out(mi, inner if n == 1 else None), n)
                if k != order[-1]:
                    yield
            c = _strassen_out(ms, order if n == 1 else None)
            for b in range(n):
                c11, c12, c21, c22 = [v[b * TH:(b + 1) * TH, :DH] for v in c]
                ks.append(_cat([c11, c12], 1))
                rks.append(_strassen_rhs(c11, c21, c12, c22))
                c11, c12, c21, c22 = [v[b * TH:(b + 1) * TH, DH:] for v in c]
                vs.append(_cat([c11, c12], 1))
                rvs.append(_strassen_rhs(c11, c12, c21, c22))

        def scores(j):
            cols = pl.ds(pl.multiple_of((h & 1) * DH, DH), DH)
            qf = [q_ref[pair, k, j * TQ:(j + 1) * TQ, cols].astype(F32) for k in range(4)]
            lq = _strassen_lhs(*qf)
            s1, s2, done, mx = [], [], [], []
            for t in range(j):
                m = [None] * 7
                for k in QK_ORDER:
                    a = tie(lq[k], done[-2]) if k == 3 and t >= 2 else lq[k]
                    m[k] = _dot_nt(a.astype(BF16), rks[t][k].astype(BF16))
                c11, c12, c21, c22 = _strassen_out(m, tuple(range(7)))
                x1, x2 = jnp.maximum(c11, c12), jnp.maximum(c21, c22)
                if mx:
                    x1, x2 = jnp.maximum(x1, mx[0]), jnp.maximum(x2, mx[1])
                mx[:] = [x1, x2]
                done.append(_as_u32(x1) | _as_u32(x2))
                s1 += [c11, c12]
                s2 += [c21, c22]
            yield
            ss[2 * j] = _cat(s1 + [_dot_nt(_cat(qf[:2], 1).astype(BF16), ks[j].astype(BF16))], 1)
            lq = _strassen_lhs(*_quads(_cat(qf[2:], 1)))
            m = {k: _dot_nt(lq[k].astype(BF16), rks[j][k].astype(BF16)) for k in QK_ORDER}
            ss[2 * j + 1] = _cat(s2 + [_unsplit(_strassen_out(m), 1)], 1)
            if mx:
                mxs[2 * j], mxs[2 * j + 1] = mx

        def masked(i):
            lo = i * TQ
            s = ss.pop(i)
            sd = jnp.where(causal, s[:, lo:], -1e9 * LOG2E)
            s = sd if i == 0 else _cat([s[:, :lo], sd], 1)
            t = _cat([mxs[i], s[:, i // 2 * TP:]], 1) if i in mxs else s
            if LOOK[i // 2]:
                return s, functools.reduce(
                    jnp.maximum, [t[:, c:c + LANE] for c in range(0, t.shape[1], LANE)])
            return s, jnp.broadcast_to(jnp.max(t, axis=-1, keepdims=True), (TQ, LANE))

        def exp_rows(s, m, parts, look):
            ps = []
            for g in range(0, TQ, 8):
                mg = m[g:g + 8]
                if look:
                    if len(parts) >= look:
                        mg = tie(mg, parts[-look])
                    mg = jnp.broadcast_to(jnp.max(mg, axis=-1, keepdims=True), (8, LANE))
                if parts:
                    mg = tie(mg, parts[-1])
                pg = [jnp.exp2(s[g:g + 8, t * LANE:(t + 1) * LANE] - mg)
                      for t in range(s.shape[1] // LANE)]
                ps.append(_cat(pg, 1))
                parts.append(functools.reduce(lambda a, b: a + b, pg))
            return _cat(ps, 0), _cat(parts[-(TQ // 8):], 0)

        def context(j):
            (s1, m1), (s2, m2) = masked(2 * j), masked(2 * j + 1)
            parts = []
            p1, l1 = exp_rows(s1, m1, parts, LOOK[j])
            if j in EARLY_SUM:
                m2 = tie(m2, jnp.broadcast_to(jnp.sum(l1, axis=-1, keepdims=True), (TQ, LANE)))
            p2, l2 = exp_rows(s2, m2, parts, LOOK[j])
            l1 = _cat([tie(l1[:8], l1[TQ - 8:]), l1[8:]], 0)
            l1, l2 = [jnp.sum(l, axis=-1, keepdims=True) for l in (l1, l2)]
            lo = j * TP
            dot = lambda a, b: _dot(a.astype(BF16), b.astype(BF16))

            def recip(l):
                rl = pl.reciprocal(l, approx=True)
                return rl * (2.0 - l * rl)

            def p_operands(a11, a12, a21, a22, rho):
                a22r = a22 * rho
                return [a11 + a22r, a21 + a22, a11, a22, a11 + a12, a21 * rho - a11, a12 - a22r]

            def diag():
                c1 = dot(p1[:, lo:], vs[j])
                lp = p_operands(*_quads(p2[:, lo:]), sig)
                m = {k: dot(lp[k], rvs[j][k]) for k in (2, 4, 3, 1, 5, 0, 6)}
                return c1, _unsplit([(m[0] - m[4]) + (m[6] + m[3] * sig), m[2] + m[4], m[1] + m[3],
                                     ((m[0] + m[2]) + m[5]) * isig - m[1]], 1)

            r1, r2 = recip(l1), recip(l2)
            rho = l1 * r2
            sig, isig = l2[:TI] * r2[TI:], l2[TI:] * r2[:TI]
            r1, r2 = r1 * vinv, r2 * vinv
            if j == 0:
                c1, c2 = diag()
                c2 = c2 * _cat([r2, r2], 1)
            else:
                tiles = lambda p, o: _cat(
                    [p[:, (2 * t + o) * TQ:(2 * t + o + 1) * TQ] for t in range(j)], 1)
                lp = p_operands(tiles(p1, 0), tiles(p1, 1), tiles(p2, 0), tiles(p2, 1), rho)
                m = [None] * 7
                for n, k in enumerate(PV_ORDER if j < NP - 1 else PV_LAST):
                    if n == PV_DIAG[j]:
                        c1, c2 = diag()
                    if n == PV_SPLIT[j]:
                        yield
                    m[k] = dot(lp[k], _cat([rvs[t][k] for t in range(j)], 0))
                c1 = c1 + _cat([(m[0] - m[4]) + (m[6] + m[3] * rho), m[2] + m[4]], 1)
                c2 = (c2 + _cat([m[1] + m[3], -m[1]], 1)) * _cat([r2, r2], 1)
                c2 = _cat([c2[:, :DH], c2[:, DH:] + ((m[0] + m[2]) + m[5]) * r1], 1)
            c1 = c1 * _cat([r1, r1], 1)
            ctx_ref[h, j * TQ:(j + 1) * TQ, :] = _cat(
                _strassen_rhs(c1[:, :DH], c2[:, :DH], c1[:, DH:], c2[:, DH:]), 1).astype(BF16)

        kvs = [proj_kv(r, 1) for r in range(NP)]
        qks = [scores(j) for j in range(NP)]
        pvs = [context(j) for j in range(NP)]
        _run(SCHEDULE, dict(d=lambda r: list(proj_kv(r, 2)), c=lambda r: list(kvs[r]),
                            x=lambda r: [next(kvs[r // 10]) for _ in range(r % 10)],
                            u=lambda j: next(qks[j]), t=lambda j: list(qks[j]),
                            b=lambda j: next(pvs[j]), p=lambda j: list(pvs[j])))
        return 0

    jax.lax.fori_loop(0, H, head_step, 0)

    pieces = ((0, 0, TP), (MH, 0, TQ), (MH, TQ, TQ))

    def o_copy(j, n):
        r0, c0, nc = pieces[n]
        return pltpu.make_async_copy(
            out_ref.at[j, pl.ds(r0, MH), pl.ds(c0, nc)],
            o_hbm.at[pl.ds(r0, MH), pl.ds(pl.multiple_of(j * TP + c0, TQ), nc)], osem.at[n, j])

    def o_step(jj, _):
        zero = zero_ref[0]
        js = (2 * jj, 2 * jj + 1)
        t0 = [pl.multiple_of(j * TP, TP) for j in js]
        last, state, ys, gates, m, recent = [], {}, [None, None], {}, [{}, {}], []
        rnd = lambda v: v.astype(BF16).astype(F32)

        def ssm_tile(u, t):
            rows = pl.ds(t0[u], TP + 8)
            cr, ci = pl.ds(t * LANE, LANE), pl.ds(PP + t * LANE, LANE)
            co = [co_ref[k, :, cr] for k in range(10)]
            u0 = u_ref[rows, cr]
            u1 = u_ref[rows, ci] if t < FT else pltpu.roll(u0, HALF, 1)
            mul = lambda k, x: (co[k] * x[0] + co[k + 1] * x[1], co[k] * x[1] - co[k + 1] * x[0])
            sub = jax.lax.broadcasted_iota(jnp.int32, (8, LANE), 0)
            s = state[t] if u else (st_ref[0, :, cr], st_ref[1, :, cr])
            prev, gs = [None] * 3, []
            for k in range(TP // 8 + 1):
                x0, x1 = _hold(u0[8 * k:8 * k + 8], last, zero), u1[8 * k:8 * k + 8]
                w = (co[0] * x0 + co[1] * x1, co[1] * x0 - co[0] * x1)
                for i in range(3):
                    cur = [pltpu.roll(v, 1 << i, 0) for v in w]
                    old = cur if k == 0 else prev[i]
                    d = mul(2 * i + 2, [jnp.where(sub < (1 << i), o, c) for o, c in zip(old, cur)])
                    w = [p + q for p, q in zip(d, w)]
                    prev[i] = cur
                if k > 0:
                    s = [p + q for p, q in zip(mul(8, s), w)]
                    gs.append(_cat(s, 1) if t < FT else s[0])
                    last[:] = [s[0]]
            state[t] = s
            if u:
                st_ref[0, :, cr] = s[0]
                st_ref[1, :, cr] = s[1]
            cols = cr if t < FT else pl.ds(PF, HALF)
            cc = _cat([cre_ref[:, cols], cim_ref[:, cols]], 1)
            g = _cat(gs, 0).astype(BF16)
            n = MH if t < FT else MH // 2
            y = _cat([_dot_nt(_as_bf16(cc[a:a + n]), g) for a in range(0, MH, n)], 0)
            ys[u] = y if ys[u] is None else y + ys[u]

        def gate(u):
            gcol = _as_u32(col_ref[1]) | (_as_u32(_cat(recent[-2:], 0)) & zero.astype(U32))
            gcol = _cat([pltpu.bitcast(gcol, F32)] * (TP // LANE), 1)
            xt = xt_ref[:, pl.ds(t0[u], TP)].astype(F32)
            z = jnp.sum(rnd(xt * gcol), axis=0, keepdims=True)
            gates[u] = rnd(1.0 / rnd(1.0 + rnd(jnp.exp(-rnd(z)))))

        def product(u, k):
            if k in SUMS:
                a = [lo_ref[n, :, pl.ds(SUMS.index(k) * DH, DH)] for n in range(H)]
            else:
                o = k - 2
                a = [_as_bf16(wot_ref[n, pl.ds(o * MH // 2, MH // 2), pl.ds(o * DH, DH)])
                     for n in range(H)]
            rows = pl.ds(pl.multiple_of(js[u] * TQ, TQ), TQ)
            b = [ctx_ref[n, rows, pl.ds(k * DH, DH)] for n in range(H)]
            m[u][k] = _dot_nt(_cat(a, 1), _cat(b, 1))
            recent.append(m[u][k])

        def emit(u, n, v):
            r0, c0, nc = pieces[n]
            g = gates[u][:, c0:c0 + nc]
            dcol = _cat([col_ref[0, r0:r0 + MH]] * (nc // LANE), 1)
            xt = xt_ref[pl.ds(r0, MH), pl.ds(pl.multiple_of(t0[u] + c0, TQ), nc)].astype(F32)
            b = ys[u][r0:r0 + MH, c0:c0 + nc] + rnd(xt * dcol)
            out_ref[js[u], pl.ds(r0, MH), pl.ds(c0, nc)] = g * v + rnd(1.0 - g) * b
            o_copy(js[u], n).start()

        _run(O_SCHEDULE, dict(a=lambda k: product(0, k), b=lambda k: product(1, k), g=gate,
                              m=lambda t: ssm_tile(0, t), n=lambda t: ssm_tile(1, t)))
        for u, p in enumerate(m):
            emit(u, 0, _cat([(p[0] + p[3]) + (p[6] - p[4]), p[2] + p[4]], 1))
            emit(u, 1, p[1] + p[3])
            emit(u, 2, ((p[0] + p[2]) - p[1]) + p[5])
        return 0

    jax.lax.fori_loop(0, NP // 2, o_step, 0)
    for j in range(NP):
        for n in range(3):
            o_copy(j, n).wait()


@jax.jit
def pallas_gated_mix__compressed_kv_cla__ssm_conv_s5__prompt_kernel(
    A_x: jax.Array,
    A_c_kv: jax.Array,
    A_w_q: jax.Array,
    A_w_uk: jax.Array,
    A_w_uv: jax.Array,
    A_w_o: jax.Array,
    B_x: jax.Array,
    B_Lambda_re: jax.Array,
    B_Lambda_im: jax.Array,
    B_B_re: jax.Array,
    B_B_im: jax.Array,
    B_C_re: jax.Array,
    B_C_im: jax.Array,
    B_log_dt: jax.Array,
    B_Dskip: jax.Array,
    gate_w: jax.Array,
):
    del B_x
    _, S, M = A_x.shape
    C = A_c_kv.shape[2]
    H, D = A_w_q.shape[1], A_w_q.shape[2]
    PP = (M + LANE - 1) // LANE * LANE

    hbm = pl.BlockSpec(memory_space=pl.ANY)
    out_t = pl.pallas_call(
        functools.partial(_kernel, S=S, M=M, H=H, D=D),
        in_specs=[hbm] * 15,
        out_specs=hbm,
        out_shape=jax.ShapeDtypeStruct((M, S), F32),
        scratch_shapes=[
            pltpu.VMEM((M, S), BF16),
            pltpu.VMEM((S // 2, M), U32),
            pltpu.VMEM((7, S // 8, 7 * PP // 4), U32),
            pltpu.VMEM((S // 2, C), U32),
            pltpu.VMEM((7, S // 8, 7 * C // 4), U32),
            pltpu.VMEM((H // 2, M, D), U32),
            pltpu.VMEM((H // 2, C, D), U32),
            pltpu.VMEM((H // 2, C, D), U32),
            pltpu.VMEM((H, M // 2, D), U32),
            pltpu.VMEM((H, M // 2, 5 * D // 2), BF16),
            pltpu.VMEM((M, M), U32),
            pltpu.VMEM((M // 2, M), U32),
            pltpu.VMEM((M // 2, M), U32),
            pltpu.VMEM((S + 32, 2 * M), F32),
            pltpu.VMEM((S // TP, M, TP), F32),
            pltpu.VMEM((2, 8, PP), F32),
            pltpu.VMEM((10, 8, PP), F32),
            pltpu.VMEM((2, M, LANE), F32),
            pltpu.VMEM((3, 8, H // 2, D), U32),
            pltpu.VMEM((2, 4, H // 2, LANE), F32),
            pltpu.VMEM((H // 2, 4, S // 2, D), BF16),
            pltpu.VMEM((H, S // 2, 7 * D // 2), BF16),
            pltpu.SMEM((1,), jnp.int32),
            pltpu.SemaphoreType.DMA((5, H // 2)),
            pltpu.SemaphoreType.DMA((4,)),
            pltpu.SemaphoreType.DMA((8,)),
            pltpu.SemaphoreType.DMA((5,)),
            pltpu.SemaphoreType.DMA((3, S // TP)),
        ] + [pltpu.VMEM((M,), BF16)] * 5,
        compiler_params=pltpu.CompilerParams(
            vmem_limit_bytes=124 * 1024 * 1024,
            disable_semaphore_checks=True,
            disable_bounds_checks=True,
        ),
    )(
        jnp.swapaxes(A_x, 1, 2).reshape(M, S), A_c_kv.reshape(S, C),
        A_w_q, A_w_uk, A_w_uv, jnp.swapaxes(A_w_o, 1, 2),
        B_B_re, B_B_im, B_C_re, B_C_im,
        B_Lambda_re, B_Lambda_im, B_log_dt, B_Dskip, gate_w,
    )
    return jnp.swapaxes(out_t.reshape(1, M, S), 1, 2)
```

```python
import functools

import jax
import jax.numpy as jnp
import jax.experimental.pallas as pl
import jax.experimental.pallas.tpu as pltpu

F32 = jnp.float32
BF16 = jnp.bfloat16
U32 = jnp.uint32

NT_DIMS = (((1,), (1,)), ((), ()))
LOG2E = 1.4426950408889634

LANE = 128
HALF = LANE // 2
TQ = 128
TP = 256
TU = 512

U_SCHEDULE = "t4 u2 x1 u3 x4 x2 u4 x5 t6 u5 x3 u6 x7 v7 x6 w7"
Q_SCHEDULE = ((0, 2), (2, 1), (3, 1), (4, 1), (5, 1), (6, 1), (7, 1))
Q_ORDER = (1, 6, 0, 3, 2, 5, 4)
Q_INNER = (1, 3, 5, 0, 2, 4, 6)
Q_REMAT = (0, 2, 3, 4, 5, 6)
C_START = (14, 20, 30, 38)
WO_START = (40, 52)
C_DUE = 53
C_EXTRA = 4
SCHEDULE = ("d0 x24 t0 t1 c2 p0 p1 x31 t2 c3 u3 b2 t3 c4 p2 b3 t4 c5 u5 p3 p4 t5 c6 b5 t6 c7 t7 "
            "p5 b6 b7 p6 p7")
KV_REMAT = (0, 2, 3, 5, 6)
KV_ORDER = {1: (1, 3, 5, 4, 2, 0, 6), 2: (1, 6, 2, 3, 0, 5, 4)}
KV_INNER = {1: (3, 1, 2, 0, 4, 6, 5), 2: (1, 3, 6, 0, 2, 4, 5)}
QK_ORDER = (0, 1, 2, 3, 4, 6, 5)
PV_ORDER = (1, 3, 4, 5, 2, 0, 6)
PV_LAST = (4, 3, 2, 0, 5, 6, 1)
PV_DIAG = (0, 3, 4, 5, 6, 4, 5, 5)
PV_SPLIT = (6, 6, 5, 6, 6, 4, 6, 5)
EARLY_SUM = (2, 4, 5)
LOOK = (0, 0, 0, 0, 0, 0, 4, 4)
O_SCHEDULE = "a3 a4 a0 g0 m0 m3 a6 m1 a2 a1 a5 n3 b0 m2 b3 g1 b4 n2 n0 n1 b6 b2 b1 b5"


def _cat(xs, axis):
    return jnp.concatenate(xs, axis=axis)


def _dot(a, b):
    return jnp.dot(a, b, preferred_element_type=F32)


def _dot_nt(a, b):
    return jax.lax.dot_general(a, b, NT_DIMS, preferred_element_type=F32)


def _unpack(w32, shift):
    v = (w32 << shift) & jnp.uint32(0xFFFF0000)
    return pltpu.bitcast(v, F32)


def _as_bf16(w32):
    return pltpu.bitcast(w32, BF16)


def _as_u32(v):
    return v if v.dtype == U32 else pltpu.bitcast(v, U32)


def _run(schedule, ops):
    for op in schedule.split():
        ops[op[0]](int(op[1:]))


def _strassen_lhs(a11, a12, a21, a22):
    return [a11 + a22, a21 + a22, a11, a22, a11 + a12, a21 - a11, a12 - a22]


def _strassen_rhs(b11, b12, b21, b22):
    return [b11 + b22, b11, b12 - b22, b21 - b11, b22, b11 + b12, b21 + b22]


def _strassen_out(m, order=None):
    if order is None:
        return ((m[0] + m[3]) + (m[6] - m[4]), m[2] + m[4],
                m[1] + m[3], (m[0] - m[1]) + (m[2] + m[5]))

    def fold(ks, neg):
        ks = sorted(ks, key=order.index)
        if ks[0] == neg:
            ks[:2] = ks[1::-1]
        return functools.reduce(lambda a, k: a - m[k] if k == neg else a + m[k], ks[1:], m[ks[0]])

    return fold((0, 3, 4, 6), 4), m[2] + m[4], m[1] + m[3], fold((0, 1, 2, 5), 1)


SUMS = (0, 1, 4, 5, 6)


def _quads(a):
    m, n = a.shape[0] // 2, a.shape[1] // 2
    return a[:m, :n], a[:m, n:], a[m:, :n], a[m:, n:]


def _unsplit(c, n):
    top, bot = _cat(c[:2], 1), _cat(c[2:], 1)
    rows = top.shape[0] // n
    return _cat([v[b * rows:(b + 1) * rows] for b in range(n) for v in (top, bot)], 0)


def _hold(v, last, zero):
    if not last:
        return v
    z = _as_u32(last[0]) & zero
    if v.shape != z.shape:
        z = jnp.tile(z, (v.shape[0] // 8, pl.cdiv(v.shape[1], LANE)))[:, :v.shape[1]]
    z = _as_u32(v) | z
    return z if v.dtype == U32 else pltpu.bitcast(z, v.dtype)


def _lhs_operands(a, last, zero, extra):
    first = (0, 2, 0, 3, 0, 2, 1)
    for k in range(7):
        q = list(_quads(a))
        q[first[k]] = _hold(q[first[k]], last, zero)
        l = _strassen_lhs(*q)[k]
        out = []
        for grp in ((0, 1, 2, 3), (4, 5, 6)):
            q = list(_quads(l))
            if out:
                for b in sorted(set(first[i] for i in grp)):
                    q[b] = _hold(q[b], last, zero)
            v = _cat([_strassen_lhs(*q)[i] for i in grp], 1)
            out.append(_as_u32(v.astype(BF16)))
            last[:] = [functools.reduce(
                jnp.bitwise_or, [out[-1][:, c:c + LANE] for c in range(0, v.shape[1], LANE)])]
            for _ in range(extra):
                last[:] = [last[0] + last[0]]
        yield _cat(out, 1)


def _kernel(xt_hbm, c_hbm, wq_hbm, wuk_hbm, wuv_hbm, wot_hbm,
            bre_hbm, bim_hbm, cre_hbm, cim_hbm,
            lre_hbm, lim_hbm, ldt_hbm, dsk_hbm, gw_hbm,
            o_hbm,
            xt_ref, x_ref, lx_ref, c_ref, l_ref, wq_buf, wk_buf, wv_buf, wot_ref, lo_ref,
            b_ref, cre_ref, cim_ref, u_ref, out_ref, st_ref, co_ref, col_ref, smp_ref, vsc_ref,
            q_ref, ctx_ref, zero_ref, wsem, xsem, msem, vsem, osem,
            lre_ref, lim_ref, ldt_ref, dsk_ref, gw_ref,
            *, S, M, H, D):
    P = M
    FT = P // LANE
    PF = FT * LANE
    PP = PF + LANE
    NP = H // 2
    CH, DH, MH, TH = c_ref.shape[1] // 2, D // 2, M // 2, TP // 2
    TI = TH // 2
    assert P - PF == HALF and PP == 4 * LANE and DH == LANE and S // TP == NP and TP == 2 * TQ

    def w_copy(k, pair):
        src, dst = ((wq_hbm, wq_buf), (wuk_hbm, wk_buf), (wuv_hbm, wv_buf))[k]
        return pltpu.make_async_copy(src.bitcast(U32).at[:, pair, :], dst.at[pair], wsem.at[k, pair])

    def wo_copy(pair):
        heads = pl.ds(2 * pair, 2)
        return pltpu.make_async_copy(wot_hbm.bitcast(U32).at[heads], wot_ref.at[heads],
                                     wsem.at[3, pair])

    def c_copy(r):
        rows = pl.ds(pl.multiple_of(r * TH, TH), TH)
        return pltpu.make_async_copy(c_hbm.bitcast(U32).at[rows], c_ref.at[rows], wsem.at[4, r])

    def x_copy(t0, n, k):
        cols = pl.ds(t0, n)
        return pltpu.make_async_copy(xt_hbm.at[:, cols], xt_ref.at[:, cols], xsem.at[k])

    x_cps = [x_copy(0, TP, 0), x_copy(TP, TP, 1), x_copy(TU, TU, 2), x_copy(2 * TU, S - 2 * TU, 3)]
    bre32, bim32 = bre_hbm.bitcast(U32), bim_hbm.bitcast(U32)
    b_cps = [
        pltpu.make_async_copy(bre32, b_ref.at[pl.ds(0, P // 2), :], msem.at[0]),
        pltpu.make_async_copy(bim32.at[pl.ds(PF // 2, HALF // 2), :],
                              b_ref.at[pl.ds(P // 2, HALF // 2), :], msem.at[1]),
        pltpu.make_async_copy(bim32.at[pl.ds(0, PF // 2), :],
                              b_ref.at[pl.ds(PP // 2, PF // 2), :], msem.at[2]),
    ]
    cre_cp = pltpu.make_async_copy(cre_hbm.bitcast(U32), cre_ref, msem.at[3])
    cim_cp = pltpu.make_async_copy(cim_hbm.bitcast(U32), cim_ref, msem.at[4])
    smp_cps = [pltpu.make_async_copy(src.bitcast(U32).at[pl.ds(0, smp_ref.shape[1])],
                                     smp_ref.at[k], msem.at[5 + k])
               for k, src in enumerate((wuk_hbm, wuv_hbm, wq_hbm))]
    v_cps = [pltpu.make_async_copy(src, dst, vsem.at[k]) for k, (src, dst) in enumerate(
        ((lre_hbm, lre_ref), (lim_hbm, lim_ref), (ldt_hbm, ldt_ref),
         (dsk_hbm, dsk_ref), (gw_hbm, gw_ref)))]

    for cp in x_cps[:1] + v_cps + b_cps + x_cps[1:] + smp_cps:
        cp.start()
    for p in range(NP):
        w_copy(0, p).start()
        wo_copy(p).start()
        c_copy(p).start()
    for p in range(NP):
        w_copy(1, p).start()
        w_copy(2, p).start()
    cre_cp.start()
    cim_cp.start()

    zero_ref[0] = 0
    u_ref[pl.ds(0, 8), :] = jnp.zeros((8, u_ref.shape[1]), F32)
    st_ref[...] = jnp.zeros(st_ref.shape, F32)
    for cp in v_cps + x_cps[:1]:
        cp.wait()

    row = lambda r: r[...].astype(F32).reshape(1, P)
    lre, lim = row(lre_ref), row(lim_ref)
    dt = jnp.exp(row(ldt_ref)).astype(BF16).astype(F32)
    e = jnp.exp(dt * lre)
    ang = dt * lim
    ar = e * jnp.cos(ang)
    ai = e * jnp.sin(ang)
    sc = jnp.maximum(jnp.abs(lre), jnp.abs(lim))
    nre, nim = lre / sc, lim / sc
    den = (nre * nre + nim * nim) * sc
    gr = 2.0 * ((ar - 1.0) * nre + ai * nim) / den
    gi = 2.0 * (ai * nre - (ar - 1.0) * nim) / den

    def put(k, full, lo, hi):
        co_ref[k] = jnp.broadcast_to(_cat([full[:, :PF], lo[:, PF:], hi[:, PF:]], 1), (8, PP))

    put(0, gr, gr, -gr)
    put(1, -gi, -gi, -gi)
    pr, pi = ar, -ai
    for j in range(1, 5):
        put(2 * j, pr, pr, pr)
        put(2 * j + 1, -pi, -pi, pi)
        pr, pi = pr * pr - pi * pi, 2.0 * pr * pi

    zpad = jnp.zeros((1, PP - P), F32)
    for k, r in enumerate((dsk_ref, gw_ref)):
        col_ref[k] = jnp.broadcast_to(_cat([row(r), zpad], 1), (LANE, PP)).T[:M]

    zero1, last1 = zero_ref[0].astype(U32), []

    def transpose_x(t0, n):
        x_ref[pl.ds(t0 // 2, n // 2), :] = _as_u32(xt_ref[:, pl.ds(t0, n)].T)

    def x_operands(r):
        for n in range(TI // 16):
            x = _cat([x_ref[pl.ds(r * TH + g * TI // 2 + 8 * n, 8), :] for g in range(4)], 0)
            x = _as_bf16(_hold(x, last1, zero1)).astype(F32)
            x = _cat([x, jnp.zeros((x.shape[0], PP - M), F32)], 1)
            for k, v in enumerate(_lhs_operands(x, last1, zero1, 0)):
                lx_ref[k, pl.ds(r * TI // 2 + 8 * n, 8), :] = v

    def proj_u(r, lo=0, hi=2 * P, due=False, mark=False):
        x = x_ref[pl.ds(r * TH, TH), :]
        if due:
            x = _cat([_hold(x[:8], last1, zero1), x[8:]], 0)
        u = _dot_nt(_as_bf16(x), _as_bf16(b_ref[lo // 2:hi // 2, :]))
        u_ref[pl.ds(r * TP + 8, TP), lo:hi] = u
        if mark:
            last1[:] = [functools.reduce(jnp.bitwise_or, last1 + [_as_u32(u[:8, :LANE])])]

    transpose_x(0, TP)
    b_cps[0].wait()
    b_cps[1].wait()
    proj_u(0, 0, PP)
    b_cps[2].wait()
    x_cps[1].wait()
    proj_u(0, PP)
    transpose_x(TP, TP)
    x_cps[2].wait()
    proj_u(1, 0, 6 * LANE, mark=True)
    transpose_x(TU, TU)
    x_operands(0)
    proj_u(1, 6 * LANE, due=True)
    last1.clear()
    x_cps[3].wait()
    for cp in smp_cps:
        cp.wait()

    def exponent(k, e):
        mag = jnp.sum(jnp.abs(_unpack(smp_ref[k], jnp.uint32(16 - 16 * e))), axis=0)
        mag = jnp.sum(mag, axis=1, keepdims=True)
        return jnp.broadcast_to(pltpu.bitcast(mag, jnp.int32) >> 23, (NP, LANE))

    for n, (target, scaled) in enumerate((((0, 0), (1, 0)), ((0, 1), (1, 1)), ((2, 0), (2, 1)))):
        e0, e1 = exponent(*target), exponent(*scaled)
        d = jnp.where((e0 > 0) & (e1 > 0), jnp.clip(e0 - e1, -40, 40), 0)
        vsc_ref[0, n] = pltpu.bitcast((127 + d) << 23, F32)
        vsc_ref[1, n] = pltpu.bitcast((127 - d) << 23, F32)

    _run(U_SCHEDULE, dict(t=lambda r: transpose_x(r * TP, TU), x=x_operands,
                          u=lambda r: proj_u(r, mark=True),
                          v=lambda r: proj_u(r, 0, 6 * LANE, mark=True),
                          w=lambda r: proj_u(r, 6 * LANE, due=True)))

    def q_step(j, _):
        w_copy(0, j).wait()
        wo_copy(j).wait()
        c_copy(j).wait()
        zero = zero_ref[0].astype(U32)
        last, recent = [], []
        wq32 = _cat([wq_buf[j], jnp.zeros((PP - M, D), U32)], 0)
        rw = []
        for k in range(7):
            z = (zero << k) if k in Q_REMAT else jnp.uint32(0)
            w0 = pltpu.bitcast(wq32 << (z + 16), F32)
            w1 = pltpu.bitcast(wq32 & (z + jnp.uint32(0xFFFF0000)), F32)
            r0 = _strassen_rhs(*_quads(w0))[k]
            r1 = _strassen_rhs(*_quads(w1))[k] * vsc_ref[0, 2, pl.ds(j, 1), :]
            rw.append(_strassen_rhs(r0[:LANE], r1[:LANE], r0[LANE:], r1[LANE:]))
        qscale = _cat([jnp.ones((1, DH), F32), vsc_ref[1, 2, pl.ds(j, 1), :]], 1)
        qscale = qscale * ((D ** -0.5) * LOG2E)

        def c_operands(n):
            c = _cat([c_ref[pl.ds(pl.multiple_of(j * TH + g * (TI // 2) + 8 * n, 8), 8), :]
                      for g in range(4)], 0)
            c = _as_bf16(_hold(c, last, zero)).astype(F32)
            rows = pl.ds(pl.multiple_of(j * (TI // 2) + 8 * n, 8), 8)
            for k, v in enumerate(_lhs_operands(c, last, zero, C_EXTRA)):
                l_ref[k, rows, :] = v

        def wo_operands(e):
            z = _as_u32(_cat([v[:TI] for v in recent[-7:]], 0)) & zero
            w = wot_ref[2 * j + e] | _cat([z[:MH], z[MH:]], 1)
            ls = _strassen_lhs(*_quads(_as_bf16(w).astype(F32)))
            lo_ref[2 * j + e] = _cat([ls[k] for k in SUMS], 1).astype(BF16)

        for r, n in Q_SCHEDULE:
            ms = [None] * 7
            for k in Q_ORDER:
                mi = [None] * 7
                for i in Q_INNER:
                    a = lx_ref[k, pl.ds(r * TI // 2, n * TI // 2), pl.ds(i * LANE, LANE)]
                    at = 7 * r + n * Q_ORDER.index(k) if i == Q_INNER[0] else -1
                    if at == C_DUE:
                        a = _cat([_hold(a[:8], last, zero), a[8:]], 0)
                    mi[i] = _dot(_as_bf16(a), rw[k][i].astype(BF16))
                    recent.append(mi[i])
                    if at in C_START:
                        last[:] = [_as_u32(mi[i][:8]) | last[0] if last else _as_u32(mi[i][:8])]
                        c_operands(C_START.index(at))
                    if at in WO_START:
                        wo_operands(WO_START.index(at))
                ms[k] = _unsplit(_strassen_out(mi), n)
            for k, v in enumerate(_strassen_out(ms)):
                q_ref[j, k, pl.ds(r * TH, n * TH), :] = (v * qscale).astype(BF16)
        return 0

    jax.lax.fori_loop(0, NP, q_step, 0)
    for p in range(NP):
        w_copy(1, p).wait()
        w_copy(2, p).wait()
    cre_cp.wait()
    cim_cp.wait()

    def head_step(h, _):
        pair = h >> 1
        zero = zero_ref[0].astype(U32)
        shift = (16 - 16 * (h & 1)).astype(U32)
        vscale, vinv = [vsc_ref[k, h & 1, pl.ds(pair, 1), :] for k in range(2)]
        rw = []
        for k in range(7):
            sh = shift + (zero << k) if k in KV_REMAT else shift
            rk = _strassen_rhs(*_quads(_unpack(wk_buf[pair], sh)))[k]
            rv = _strassen_rhs(*_quads(_unpack(wv_buf[pair], sh)))[k] * vscale
            rw.append(_strassen_rhs(rk[:CH // 2], rv[:CH // 2], rk[CH // 2:], rv[CH // 2:]))
        causal = (jax.lax.broadcasted_iota(jnp.int32, (TQ, TQ), 1)
                  <= jax.lax.broadcasted_iota(jnp.int32, (TQ, TQ), 0))
        ks, rks, vs, rvs, ss, mxs = [], [], [], [], {}, {}

        def tie(a, b):
            return pltpu.bitcast(_as_u32(a) | (_as_u32(b) & zero), F32)

        def proj_kv(r, n):
            ms = [None] * 7
            order, inner = KV_ORDER[n], KV_INNER[n]
            for k in order:
                mi = [None] * 7
                for i in inner:
                    a = l_ref[k, pl.ds(r * TI // 2, n * TI // 2), pl.ds(i * CH // 2, CH // 2)]
                    mi[i] = _dot(_as_bf16(a), rw[k][i].astype(BF16))
                ms[k] = _unsplit(_strassen_out(mi, inner if n == 1 else None), n)
                if k != order[-1]:
                    yield
            c = _strassen_out(ms, order if n == 1 else None)
            for b in range(n):
                c11, c12, c21, c22 = [v[b * TH:(b + 1) * TH, :DH] for v in c]
                ks.append(_cat([c11, c12], 1))
                rks.append(_strassen_rhs(c11, c21, c12, c22))
                c11, c12, c21, c22 = [v[b * TH:(b + 1) * TH, DH:] for v in c]
                vs.append(_cat([c11, c12], 1))
                rvs.append(_strassen_rhs(c11, c12, c21, c22))

        def scores(j):
            cols = pl.ds(pl.multiple_of((h & 1) * DH, DH), DH)
            qf = [q_ref[pair, k, j * TQ:(j + 1) * TQ, cols].astype(F32) for k in range(4)]
            lq = _strassen_lhs(*qf)
            s1, s2, done, mx = [], [], [], []
            for t in range(j):
                m = [None] * 7
                for k in QK_ORDER:
                    a = tie(lq[k], done[-2]) if k == 3 and t >= 2 else lq[k]
                    m[k] = _dot_nt(a.astype(BF16), rks[t][k].astype(BF16))
                c11, c12, c21, c22 = _strassen_out(m, tuple(range(7)))
                x1, x2 = jnp.maximum(c11, c12), jnp.maximum(c21, c22)
                if mx:
                    x1, x2 = jnp.maximum(x1, mx[0]), jnp.maximum(x2, mx[1])
                mx[:] = [x1, x2]
                done.append(_as_u32(x1) | _as_u32(x2))
                s1 += [c11, c12]
                s2 += [c21, c22]
            yield
            ss[2 * j] = _cat(s1 + [_dot_nt(_cat(qf[:2], 1).astype(BF16), ks[j].astype(BF16))], 1)
            lq = _strassen_lhs(*_quads(_cat(qf[2:], 1)))
            m = {k: _dot_nt(lq[k].astype(BF16), rks[j][k].astype(BF16)) for k in QK_ORDER}
            ss[2 * j + 1] = _cat(s2 + [_unsplit(_strassen_out(m), 1)], 1)
            if mx:
                mxs[2 * j], mxs[2 * j + 1] = mx

        def masked(i):
            lo = i * TQ
            s = ss.pop(i)
            sd = jnp.where(causal, s[:, lo:], -1e9 * LOG2E)
            s = sd if i == 0 else _cat([s[:, :lo], sd], 1)
            t = _cat([mxs[i], s[:, i // 2 * TP:]], 1) if i in mxs else s
            if LOOK[i // 2]:
                return s, functools.reduce(
                    jnp.maximum, [t[:, c:c + LANE] for c in range(0, t.shape[1], LANE)])
            return s, jnp.broadcast_to(jnp.max(t, axis=-1, keepdims=True), (TQ, LANE))

        def exp_rows(s, m, parts, look):
            ps = []
            for g in range(0, TQ, 8):
                mg = m[g:g + 8]
                if look:
                    if len(parts) >= look:
                        mg = tie(mg, parts[-look])
                    mg = jnp.broadcast_to(jnp.max(mg, axis=-1, keepdims=True), (8, LANE))
                if parts:
                    mg = tie(mg, parts[-1])
                pg = [jnp.exp2(s[g:g + 8, t * LANE:(t + 1) * LANE] - mg)
                      for t in range(s.shape[1] // LANE)]
                ps.append(_cat(pg, 1))
                parts.append(functools.reduce(lambda a, b: a + b, pg))
            return _cat(ps, 0), _cat(parts[-(TQ // 8):], 0)

        def context(j):
            (s1, m1), (s2, m2) = masked(2 * j), masked(2 * j + 1)
            parts = []
            p1, l1 = exp_rows(s1, m1, parts, LOOK[j])
            if j in EARLY_SUM:
                m2 = tie(m2, jnp.broadcast_to(jnp.sum(l1, axis=-1, keepdims=True), (TQ, LANE)))
            p2, l2 = exp_rows(s2, m2, parts, LOOK[j])
            l1 = _cat([tie(l1[:8], l1[TQ - 8:]), l1[8:]], 0)
            l1, l2 = [jnp.sum(l, axis=-1, keepdims=True) for l in (l1, l2)]
            lo = j * TP
            dot = lambda a, b: _dot(a.astype(BF16), b.astype(BF16))

            def recip(l):
                rl = pl.reciprocal(l, approx=True)
                return rl * (2.0 - l * rl)

            def p_operands(a11, a12, a21, a22, rho):
                a22r = a22 * rho
                return [a11 + a22r, a21 + a22, a11, a22, a11 + a12, a21 * rho - a11, a12 - a22r]

            def diag():
                c1 = dot(p1[:, lo:], vs[j])
                lp = p_operands(*_quads(p2[:, lo:]), sig)
                m = {k: dot(lp[k], rvs[j][k]) for k in (2, 4, 3, 1, 5, 0, 6)}
                return c1, _unsplit([(m[0] - m[4]) + (m[6] + m[3] * sig), m[2] + m[4], m[1] + m[3],
                                     ((m[0] + m[2]) + m[5]) * isig - m[1]], 1)

            r1, r2 = recip(l1), recip(l2)
            rho = l1 * r2
            sig, isig = l2[:TI] * r2[TI:], l2[TI:] * r2[:TI]
            r1, r2 = r1 * vinv, r2 * vinv
            if j == 0:
                c1, c2 = diag()
                c2 = c2 * _cat([r2, r2], 1)
            else:
                tiles = lambda p, o: _cat(
                    [p[:, (2 * t + o) * TQ:(2 * t + o + 1) * TQ] for t in range(j)], 1)
                lp = p_operands(tiles(p1, 0), tiles(p1, 1), tiles(p2, 0), tiles(p2, 1), rho)
                m = [None] * 7
                for n, k in enumerate(PV_ORDER if j < NP - 1 else PV_LAST):
                    if n == PV_DIAG[j]:
                        c1, c2 = diag()
                    if n == PV_SPLIT[j]:
                        yield
                    m[k] = dot(lp[k], _cat([rvs[t][k] for t in range(j)], 0))
                c1 = c1 + _cat([(m[0] - m[4]) + (m[6] + m[3] * rho), m[2] + m[4]], 1)
                c2 = (c2 + _cat([m[1] + m[3], -m[1]], 1)) * _cat([r2, r2], 1)
                c2 = _cat([c2[:, :DH], c2[:, DH:] + ((m[0] + m[2]) + m[5]) * r1], 1)
            c1 = c1 * _cat([r1, r1], 1)
            ctx_ref[h, j * TQ:(j + 1) * TQ, :] = _cat(
                _strassen_rhs(c1[:, :DH], c2[:, :DH], c1[:, DH:], c2[:, DH:]), 1).astype(BF16)

        kvs = [proj_kv(r, 1) for r in range(NP)]
        qks = [scores(j) for j in range(NP)]
        pvs = [context(j) for j in range(NP)]
        _run(SCHEDULE, dict(d=lambda r: list(proj_kv(r, 2)), c=lambda r: list(kvs[r]),
                            x=lambda r: [next(kvs[r // 10]) for _ in range(r % 10)],
                            u=lambda j: next(qks[j]), t=lambda j: list(qks[j]),
                            b=lambda j: next(pvs[j]), p=lambda j: list(pvs[j])))
        return 0

    jax.lax.fori_loop(0, H, head_step, 0)

    pieces = ((0, 0, TP), (MH, 0, TQ), (MH, TQ, TQ))

    def o_copy(j, n):
        r0, c0, nc = pieces[n]
        return pltpu.make_async_copy(
            out_ref.at[j, pl.ds(r0, MH), pl.ds(c0, nc)],
            o_hbm.at[pl.ds(r0, MH), pl.ds(pl.multiple_of(j * TP + c0, TQ), nc)], osem.at[n, j])

    def o_step(jj, _):
        zero = zero_ref[0].astype(U32)
        js = (2 * jj, 2 * jj + 1)
        t0 = [pl.multiple_of(j * TP, TP) for j in js]
        last, state, ys, gates, m, recent = [], {}, [None, None], {}, [{}, {}], []
        rnd = lambda v: v.astype(BF16).astype(F32)
        top = [jax.lax.broadcasted_iota(jnp.int32, (8, LANE), 0) < (1 << i) for i in range(3)]

        def ssm_tile(u, t):
            rows = pl.ds(t0[u], TP + 8)
            cr, ci = pl.ds(t * LANE, LANE), pl.ds(PP + t * LANE, LANE)
            co = [co_ref[k, :, cr] for k in range(10)]
            u0 = u_ref[rows, cr]
            u1 = u_ref[rows, ci] if t < FT else pltpu.roll(u0, HALF, 1)
            mul = lambda k, x: (co[k] * x[0] + co[k + 1] * x[1], co[k] * x[1] - co[k + 1] * x[0])
            s = state[t] if u else (st_ref[0, :, cr], st_ref[1, :, cr])
            prev, gs = [None] * 3, []
            for k in range(TP // 8 + 1):
                x0, x1 = _hold(u0[8 * k:8 * k + 8], last, zero), u1[8 * k:8 * k + 8]
                w = (co[0] * x0 + co[1] * x1, co[1] * x0 - co[0] * x1)
                for i in range(3):
                    cur = [pltpu.roll(v, 1 << i, 0) for v in w]
                    old = cur if k == 0 else prev[i]
                    d = mul(2 * i + 2, [jax.lax.select(top[i], o, c) for o, c in zip(old, cur)])
                    w = [p + q for p, q in zip(d, w)]
                    prev[i] = cur
                if k > 0:
                    s = [p + q for p, q in zip(mul(8, s), w)]
                    gs.append(_cat(s, 1) if t < FT else s[0])
                    last[:] = [s[0]]
            state[t] = s
            if u:
                st_ref[0, :, cr] = s[0]
                st_ref[1, :, cr] = s[1]
            cols = cr if t < FT else pl.ds(PF, HALF)
            cc = _cat([cre_ref[:, cols], cim_ref[:, cols]], 1)
            g = _cat(gs, 0).astype(BF16)
            n = MH if t < FT else MH // 2
            y = _cat([_dot_nt(_as_bf16(cc[a:a + n]), g) for a in range(0, MH, n)], 0)
            ys[u] = y if ys[u] is None else y + ys[u]

        def gate(u):
            gcol = _as_u32(col_ref[1]) | (_as_u32(_cat(recent[-2:], 0)) & zero)
            gcol = _cat([pltpu.bitcast(gcol, F32)] * (TP // LANE), 1)
            xt = xt_ref[:, pl.ds(t0[u], TP)].astype(F32)
            z = jnp.sum(rnd(xt * gcol), axis=0, keepdims=True)
            gates[u] = rnd(1.0 / rnd(1.0 + rnd(jnp.exp(-rnd(z)))))

        def product(u, k):
            if k in SUMS:
                a = [lo_ref[n, :, pl.ds(SUMS.index(k) * DH, DH)] for n in range(H)]
            else:
                o = k - 2
                a = [_as_bf16(wot_ref[n, pl.ds(o * MH // 2, MH // 2), pl.ds(o * DH, DH)])
                     for n in range(H)]
            rows = pl.ds(pl.multiple_of(js[u] * TQ, TQ), TQ)
            b = [ctx_ref[n, rows, pl.ds(k * DH, DH)] for n in range(H)]
            m[u][k] = _dot_nt(_cat(a, 1), _cat(b, 1))
            recent.append(m[u][k])

        def emit(u, n, v):
            r0, c0, nc = pieces[n]
            g = gates[u][:, c0:c0 + nc]
            dcol = _cat([col_ref[0, r0:r0 + MH]] * (nc // LANE), 1)
            xt = xt_ref[pl.ds(r0, MH), pl.ds(pl.multiple_of(t0[u] + c0, TQ), nc)].astype(F32)
            b = ys[u][r0:r0 + MH, c0:c0 + nc] + rnd(xt * dcol)
            out_ref[js[u], pl.ds(r0, MH), pl.ds(c0, nc)] = g * v + rnd(1.0 - g) * b
            o_copy(js[u], n).start()

        _run(O_SCHEDULE, dict(a=lambda k: product(0, k), b=lambda k: product(1, k), g=gate,
                              m=lambda t: ssm_tile(0, t), n=lambda t: ssm_tile(1, t)))
        for u, p in enumerate(m):
            emit(u, 0, _cat([(p[0] + p[3]) + (p[6] - p[4]), p[2] + p[4]], 1))
            emit(u, 1, p[1] + p[3])
            emit(u, 2, ((p[0] + p[2]) - p[1]) + p[5])
        return 0

    jax.lax.fori_loop(0, NP // 2, o_step, 0)
    for j in range(NP):
        for n in range(3):
            o_copy(j, n).wait()


@jax.jit
def pallas_gated_mix__compressed_kv_cla__ssm_conv_s5__prompt_kernel(
    A_x: jax.Array,
    A_c_kv: jax.Array,
    A_w_q: jax.Array,
    A_w_uk: jax.Array,
    A_w_uv: jax.Array,
    A_w_o: jax.Array,
    B_x: jax.Array,
    B_Lambda_re: jax.Array,
    B_Lambda_im: jax.Array,
    B_B_re: jax.Array,
    B_B_im: jax.Array,
    B_C_re: jax.Array,
    B_C_im: jax.Array,
    B_log_dt: jax.Array,
    B_Dskip: jax.Array,
    gate_w: jax.Array,
):
    del B_x
    _, S, M = A_x.shape
    C = A_c_kv.shape[2]
    H, D = A_w_q.shape[1], A_w_q.shape[2]
    PP = (M + LANE - 1) // LANE * LANE

    hbm = pl.BlockSpec(memory_space=pl.ANY)
    out_t = pl.pallas_call(
        functools.partial(_kernel, S=S, M=M, H=H, D=D),
        in_specs=[hbm] * 15,
        out_specs=hbm,
        out_shape=jax.ShapeDtypeStruct((M, S), F32),
        scratch_shapes=[
            pltpu.VMEM((M, S), BF16),
            pltpu.VMEM((S // 2, M), U32),
            pltpu.VMEM((7, S // 8, 7 * PP // 4), U32),
            pltpu.VMEM((S // 2, C), U32),
            pltpu.VMEM((7, S // 8, 7 * C // 4), U32),
            pltpu.VMEM((H // 2, M, D), U32),
            pltpu.VMEM((H // 2, C, D), U32),
            pltpu.VMEM((H // 2, C, D), U32),
            pltpu.VMEM((H, M // 2, D), U32),
            pltpu.VMEM((H, M // 2, 5 * D // 2), BF16),
            pltpu.VMEM((M, M), U32),
            pltpu.VMEM((M // 2, M), U32),
            pltpu.VMEM((M // 2, M), U32),
            pltpu.VMEM((S + 32, 2 * M), F32),
            pltpu.VMEM((S // TP, M, TP), F32),
            pltpu.VMEM((2, 8, PP), F32),
            pltpu.VMEM((10, 8, PP), F32),
            pltpu.VMEM((2, M, LANE), F32),
            pltpu.VMEM((3, 8, H // 2, D), U32),
            pltpu.VMEM((2, 4, H // 2, LANE), F32),
            pltpu.VMEM((H // 2, 4, S // 2, D), BF16),
            pltpu.VMEM((H, S // 2, 7 * D // 2), BF16),
            pltpu.SMEM((1,), jnp.int32),
            pltpu.SemaphoreType.DMA((5, H // 2)),
            pltpu.SemaphoreType.DMA((4,)),
            pltpu.SemaphoreType.DMA((8,)),
            pltpu.SemaphoreType.DMA((5,)),
            pltpu.SemaphoreType.DMA((3, S // TP)),
        ] + [pltpu.VMEM((M,), BF16)] * 5,
        compiler_params=pltpu.CompilerParams(
            vmem_limit_bytes=124 * 1024 * 1024,
            disable_semaphore_checks=True,
            disable_bounds_checks=True,
        ),
    )(
        jnp.swapaxes(A_x, 1, 2).reshape(M, S), A_c_kv.reshape(S, C),
        A_w_q, A_w_uk, A_w_uv, jnp.swapaxes(A_w_o, 1, 2),
        B_B_re, B_B_im, B_C_re, B_C_im,
        B_Lambda_re, B_Lambda_im, B_log_dt, B_Dskip, gate_w,
    )
    return jnp.swapaxes(out_t.reshape(1, M, S), 1, 2)
```
